```python
import jax
import jax.numpy as jnp

def _softmax(x, axis=-1):
    return jax.nn.softmax(x, axis=axis)
def _gelu(x):
    return jax.nn.gelu(x, approximate=True)
def _silu(x):
    return jax.nn.silu(x)
def _sigmoid(x):
    return jax.nn.sigmoid(x)
def _layernorm(x, axis=-1, eps=1e-5):
    m = jnp.mean(x, axis=axis, keepdims=True)
    v = jnp.var(x, axis=axis, keepdims=True)
    return (x - m) / jnp.sqrt(v + eps)
def _scatter_add(tgt, idx, src, axis=0):
    return tgt.at[idx].add(src)
def _segment_sum(src, seg, n):
    return jax.ops.segment_sum(src, seg, n)
class _Rng:
    def __init__(self, key):
        self._k = key
    def _next(self):
        self._k, sub = jax.random.split(self._k)
        return sub
    def normal(self, shape):
        return jax.random.normal(self._next(), shape, dtype=jnp.bfloat16)
    def randint(self, lo, hi, shape):
        return jax.random.randint(self._next(), shape, lo, hi, dtype=jnp.int32)
    def uniform(self, shape, lo=0.0, hi=1.0):
        return jax.random.uniform(self._next(), shape, jnp.bfloat16, lo, hi)
    def permutation(self, n):
        return jax.random.permutation(self._next(), n)


kernel_name = 'concat_heads__ssm_conv_h3__compressed_kv_cla__prompt'

def setup_inputs():
    _rng = _Rng(jax.random.key(int.from_bytes(__import__("os").urandom(4), "little")))
    _w = (lambda a: (lambda t: t.astype(jnp.bfloat16) if jnp.issubdtype(t.dtype, jnp.floating) else t)(jnp.asarray(a)))
    def _A_setup():
        B, S, D = 1, 2048, 448
        ks = 4
        return {
            "q": _w((lambda *s: _rng.normal(s) * 0.05)(B, S, D)),
            "k": _w((lambda *s: _rng.normal(s) * 0.05)(B, S, D)),
            "v": _w((lambda *s: _rng.normal(s) * 0.05)(B, S, D)),
            "shift_k": _w((lambda *s: _rng.normal(s) * 0.05)(D, ks) * 0.5),
            "ssm_k": _w((lambda *s: _rng.normal(s) * 0.05)(D, S) * (1.0 / S ** 0.5)),
            "ssm_D": _w((lambda *s: _rng.normal(s) * 0.05)(D)),
        }
    _A_in = _A_setup()

    def _B_setup():
        B, H, Sq, Sk, D, M = 1, 16, 2048, 2048, 256, 448
        Dc = 4 * D
        return {
            "x": _w((lambda *s: _rng.normal(s) * 0.05)(B, Sq, M)),
            "c_kv": _w((lambda *s: _rng.normal(s) * 0.05)(B, Sk, Dc)),
            "w_q": _w((lambda *s: _rng.normal(s) * 0.05)(M, H, D) * (M ** -0.5)),
            "w_uk": _w((lambda *s: _rng.normal(s) * 0.05)(Dc, H, D) * (Dc ** -0.5)),
            "w_uv": _w((lambda *s: _rng.normal(s) * 0.05)(Dc, H, D) * (Dc ** -0.5)),
            "w_o": _w((lambda *s: _rng.normal(s) * 0.05)(H, D, M) * ((H * D) ** -0.5)),
        }
    _B_in = _B_setup()

    return {
        "A_q": _A_in["q"],
        "A_k": _A_in["k"],
        "A_v": _A_in["v"],
        "A_shift_k": _A_in["shift_k"],
        "A_ssm_k": _A_in["ssm_k"],
        "A_ssm_D": _A_in["ssm_D"],
        "B_x": _B_in["x"],
        "B_c_kv": _B_in["c_kv"],
        "B_w_q": _B_in["w_q"],
        "B_w_uk": _B_in["w_uk"],
        "B_w_uv": _B_in["w_uv"],
        "B_w_o": _B_in["w_o"],
    }

def reference(A_q, A_k, A_v, A_shift_k, A_ssm_k, A_ssm_D, B_x, B_c_kv, B_w_q, B_w_uk, B_w_uv, B_w_o):
    def _A_ref(q, k, v, shift_k, ssm_k, ssm_D):
        B, S, D = q.shape
        ks = shift_k.shape[-1]
        k_pad = jnp.pad(k, ((0, 0), (ks - 1, 0), (0, 0)))
        k_shift = jnp.zeros_like(k)
        for t in range(ks):
            k_shift = k_shift + k_pad[:, t:t + S, :] * shift_k[:, ks - 1 - t][None, None, :]
        kv = k_shift * v
        L = 2 * S
        kv_pad = jnp.pad(kv, ((0, 0), (0, S), (0, 0)))
        kf_pad = jnp.pad(ssm_k, ((0, 0), (0, S)))
        kv_f = (lambda x, axes=(-2,-1): jnp.fft.rfft2(x.astype(jnp.float32), axes=axes))(kv_pad[:, None, :, :], axes=(1, 2))
        kf_f = (lambda x, axes=(-2,-1): jnp.fft.rfft2(x.astype(jnp.float32), axes=axes))(kf_pad[:, None, :], axes=(1, 2))
        kf_f = (lambda x, *d: x.transpose(*d))(kf_f, 1, 2, 0)
        y_f = kv_f * kf_f[None, :, :, :]
        y = (lambda x, s, axes=(-2,-1): jnp.fft.irfft2(x, s=s, axes=axes).astype(jnp.bfloat16))(y_f, (1, L), axes=(1, 2))[:, 0, :S, :]
        y = y + kv * ssm_D[None, None, :]
        return q * y

    def _B_ref(x, c_kv, w_q, w_uk, w_uv, w_o):
        B, Sq, M = x.shape[0], x.shape[1], x.shape[2]
        Sk = c_kv.shape[1]
        H, D = w_q.shape[1], w_q.shape[2]
        q = jnp.einsum("bqm,mhd->bhqd", x, w_q)
        k = jnp.einsum("bkc,chd->bhkd", c_kv, w_uk)
        v = jnp.einsum("bkc,chd->bhkd", c_kv, w_uv)
        scores = jnp.einsum("bhqd,bhkd->bhqk", q, k) * (D ** -0.5)
        off = Sk - Sq
        qi = jnp.arange(Sq)[:, None]
        kj = jnp.arange(Sk)[None, :]
        cmask = kj <= (qi + off)
        scores = jnp.where(cmask[None, None], scores, -1e9)
        p = _softmax(scores, axis=-1)
        ctx = jnp.einsum("bhqk,bhkd->bhqd", p, v)
        return jnp.einsum("bhqd,hdm->bqm", ctx, w_o)

    a = _A_ref(A_q, A_k, A_v, A_shift_k, A_ssm_k, A_ssm_D)
    b = _B_ref(B_x, B_c_kv, B_w_q, B_w_uk, B_w_uv, B_w_o)
    return jnp.concatenate([a, b], axis=-1)
```

```python
import math

import jax
import jax.numpy as jnp
from jax import lax
import jax.experimental.pallas as pl
import jax.experimental.pallas.tpu as pltpu

F32 = jnp.float32
BF16 = jnp.bfloat16
U32 = jnp.uint32
I32 = jnp.int32

S = 2048
C = 448
H = 16
D = 256
DC = 1024
NB = S // 128
PITCH = 520
CPH = C // H
TQ = 512
NT = (((1,), (1,)), ((), ()))
LOG2E = math.log2(math.e)
QSCALE = (D ** -0.5) * LOG2E
NEG = -1e9 * LOG2E
HI_MASK = 0xFFFF0000


def _dot(a, b):
    return jnp.dot(a, b, preferred_element_type=F32)


def _dot_nt(a, b):
    return lax.dot_general(a, b, NT, preferred_element_type=F32)


def _head_cols(w_s, h, rows):
    out = []
    for b in range(2):
        x = w_s[b, pl.ds(h // 2, rows, stride=8), :]
        if isinstance(h, int):
            x = (x << 16) if h % 2 == 0 else (x & jnp.uint32(HI_MASK))
        else:
            sh = ((1 - h % 2) * 16).astype(U32)
            x = (x << sh) & jnp.uint32(HI_MASK)
        out.append(pltpu.bitcast(x, F32))
    return out


def _kernel(qa_hbm, ka_hbm, va_hbm, sk_ref, hk_hbm, d_ref, x_hbm, c_hbm, wq_hbm, wk_hbm, wv_hbm, wo_hbm,
            o_hbm,
            c_s, wk_s, wv_s, qa_s, qc_s, aw_s, g_s, y_s, wot_s, sems):
    def cp(src, dst, i):
        return pltpu.make_async_copy(src, dst, sems.at[i])

    wq32 = wq_hbm.bitcast(U32)
    wk32 = wk_hbm.bitcast(U32)
    wv32 = wv_hbm.bitcast(U32)
    g3 = ([cp(c_hbm.at[:, pl.ds(128 * b, 128)], c_s.at[b], 8 + b) for b in range(8)]
          + [cp(wk32.at[:, pl.ds(128 * b, 128)], wk_s.at[b], 16 + b) for b in range(2)]
          + [cp(wv32.at[:, pl.ds(128 * b, 128)], wv_s.at[b], 18 + b) for b in range(2)]
          )
    g4 = [cp(qa_hbm, qa_s, 21)] + [cp(wo_hbm.at[:, pl.ds(128 * b, 128)], wot_s.at[b], 6 + b) for b in range(2)]

    def phase0(x_s, wq_s, ka_s, va_s, hk_s, wd_s):
        g1 = [cp(wq32.at[:, pl.ds(128 * b, 128)], wq_s.at[b], b) for b in range(2)] + [cp(x_hbm, x_s, 2)]
        g2 = [cp(ka_hbm, ka_s, 3), cp(va_hbm, va_s, 4), cp(hk_hbm, hk_s, 5)]
        for c_ in g1:
            c_.start()
        for c_ in g1:
            c_.wait()
        for c_ in g2:
            c_.start()

        def qproj(h):
            wt = jnp.concatenate(
                [jnp.concatenate([t, jnp.zeros((512 - C, 128), F32)], axis=0).T[:, :C].astype(BF16)
                 for t in _head_cols(wq_s, h, C)], axis=0)
            qt = (_dot(wt, x_s[...]) * QSCALE).astype(BF16)
            for t in range(NB):
                qc_s[h, t] = qt[:, 128 * t:128 * (t + 1)]

        qproj(0)
        qproj(1)
        for c_ in g2:
            c_.wait()
        for c_ in g3 + g4:
            c_.start()

        def column(row):
            row = jnp.concatenate([row.astype(F32), jnp.zeros((1, 512 - C), F32)], axis=1)
            return jnp.broadcast_to(row, (128, 512)).T

        taps = [column(sk_ref[j:j + 1, :]) for j in range(4)]
        dcol = column(d_ref[...].reshape(1, C))

        def shifted(cur, prev, n, lane):
            r = pltpu.roll(pltpu.bitcast(cur, U32), n, 1)
            x = jnp.where(lane >= n, r, 0 if prev is None else prev)
            return pltpu.bitcast(x, BF16).astype(F32), r

        def prep_u(b):
            w = 128 if b < 3 else C - 384
            rows = slice(128 * b, 128 * b + w)
            lane = lax.broadcasted_iota(I32, (w // 2, 128), 1)
            prev = jnp.zeros((w, 128), F32)
            pr = [None] * 4
            for sg in range(NB):
                cols = slice(128 * sg, 128 * (sg + 1))
                kb = ka_s[rows, cols]
                ks = [kb.astype(F32)]
                for n in range(1, 4):
                    x, pr[n] = shifted(kb, pr[n], n, lane)
                    ks.append(x)
                ksh = ((ks[3] * taps[3][rows] + ks[2] * taps[2][rows])
                       + (ks[1] * taps[1][rows] + ks[0] * taps[0][rows]))
                kv = ksh * va_s[rows, cols].astype(F32)
                wrd = pltpu.pack_elementwise([prev, kv], packed_dtype=BF16).astype(U32)
                if w < 128:
                    wrd = jnp.concatenate([wrd, jnp.zeros((128 - w, 128), U32)], axis=0)
                wd_s[b, cols, :] = wrd.T
                prev = kv

        def windows(b):
            for p in range(8):
                for j in range(8):
                    parts = []
                    for sg in range(2 * j - 6, 2 * j + 2):
                        if sg < 0:
                            parts.append(jnp.zeros((16, 128), U32))
                        else:
                            parts.append(wd_s[b, 128 * sg + 16 * p:128 * sg + 16 * p + 16, :])
                    plane = 32 * (j // 4) + 8 * (p // 2) + 4 * (p % 2) + j % 4
                    r0 = plane * PITCH + 128 * b
                    aw_s[r0:r0 + 128, :] = jnp.concatenate(parts, axis=0).T

        def prep_g(cb):
            rows = slice(64 * cb, 64 * (cb + 1))
            lane = lax.broadcasted_iota(I32, (64, 128), 1)
            prev = jnp.zeros((64, 128), F32)
            for a in range(NB):
                hf = hk_s[rows, 128 * a:128 * (a + 1)].astype(F32)
                if a == 0:
                    hf = jnp.where(lane == 0, hf + dcol[rows], hf)
                r = pltpu.roll(hf, 1, 1)
                hs = jnp.where(lane >= 1, r, prev)
                prev = r
                g_s[a, rows, :] = pltpu.pack_elementwise([hf, hs], packed_dtype=BF16).astype(U32)

        for b in range(4):
            prep_u(b)
            windows(b)
        for cb in range(C // 64):
            prep_g(cb)
        for h in range(2, H):
            qproj(h)

    pl.run_scoped(
        phase0,
        pltpu.VMEM((C, S), BF16), pltpu.VMEM((2, C * 8, 128), U32), pltpu.VMEM((C, S), BF16),
        pltpu.VMEM((C, S), BF16), pltpu.VMEM((C, S), BF16), pltpu.VMEM((4, S, 128), U32))

    for c_ in g3:
        c_.wait()

    def phase1(k_s, vt_s):
        def head(h, carry):
            lane8 = lax.broadcasted_iota(I32, (8, 128), 1)
            sub8 = lax.broadcasted_iota(I32, (8, 128), 0)
            lane16 = lax.broadcasted_iota(I32, (16, 128), 1)
            sub16 = lax.broadcasted_iota(I32, (16, 128), 0)
            tri = (lax.broadcasted_iota(I32, (128, 128), 0) <= lax.broadcasted_iota(I32, (128, 128), 1))
            m_b = lane8 < 128 - 2 * sub8

            def chan(c):
                gs = [jnp.broadcast_to(g_s[a, pl.ds(c, 1), :], (8, 128)) for a in range(NB)]
                zero = jnp.zeros((8, 128), U32)
                bt = [pltpu.roll(jnp.where(m_b, gs[a], gs[a - 1] if a > 0 else zero), 0, 1,
                                 stride=2, stride_axis=0) for a in range(NB)]
                b1 = pltpu.bitcast(jnp.concatenate(bt[7::-1], axis=0), BF16)
                b2 = pltpu.bitcast(jnp.concatenate(bt[15:7:-1], axis=0), BF16)
                am = pltpu.bitcast(aw_s[pl.ds(c, 64, stride=PITCH), :], BF16)
                z1 = _dot(am, b1)
                z2 = _dot(am[:64], b2)
                zlo = z1[:64]
                zhi = z1[64:] + z2
                acc = car = None
                for p in range(8):
                    z = jnp.concatenate([zlo[8 * p:8 * p + 8], zhi[8 * p:8 * p + 8]], axis=0)
                    if p == 0:
                        acc = z
                    else:
                        z = pltpu.roll(z, 16 * p, 1)
                        cz = jnp.where(lane16 < 16 * p, z, 0.0)
                        acc = acc + z
                        car = cz if car is None else car + cz
                y = (acc - car) + jnp.where(sub16 > 0, pltpu.roll(car, 1, 0), 0.0)
                y_s[pl.ds(c, NB, stride=PITCH), :] = y

            chans = [h * CPH + i for i in range(CPH)]

            def some_chans(n):
                for _ in range(min(n, len(chans))):
                    chan(chans.pop(0))

            wk = jnp.concatenate([t.astype(BF16) for t in _head_cols(wk_s, h, DC)], axis=1)
            wvt = jnp.concatenate([t.T.astype(BF16) for t in _head_cols(wv_s, h, DC)], axis=0)

            def c_rows(r0, r1):
                return jnp.concatenate([c_s[b, r0:r1, :] for b in range(8)], axis=1)

            def kproj(r0, r1):
                k = _dot(c_rows(r0, r1), wk).astype(BF16)
                k_s[0, r0:r1, :] = k[:, :128]
                k_s[1, r0:r1, :] = k[:, 128:]

            def vproj(r0, r1):
                vt = _dot_nt(wvt, c_rows(r0, r1)).astype(BF16)
                for t in range(r0 // 128, r1 // 128):
                    vt_s[t] = vt[:, 128 * t - r0:128 * (t + 1) - r0]

            def k_rows(r0, r1):
                return jnp.concatenate([k_s[0, r0:r1, :], k_s[1, r0:r1, :]], axis=1)

            def q_cols(r0, r1):
                return jnp.concatenate([qc_s[h, t] for t in range(r0 // 128, r1 // 128)], axis=1)

            st = {}

            def qk(t):
                q0 = t * TQ
                if q0 > 0:
                    s_rect = _dot(k_rows(0, q0), q_cols(q0, q0 + TQ))
                ps = []
                for u in range(TQ // 128):
                    qs = q0 + u * 128
                    sd = _dot(k_rows(q0, qs + 128), q_cols(qs, qs + 128))
                    parts = []
                    if q0 > 0:
                        parts.append(s_rect[:, u * 128:(u + 1) * 128])
                    if u > 0:
                        parts.append(sd[:u * 128, :])
                    parts.append(jnp.where(tri, sd[u * 128:, :], NEG))
                    s = jnp.concatenate(parts, axis=0) if len(parts) > 1 else parts[0]
                    m = jnp.max(s, axis=0, keepdims=True)
                    p = jnp.exp2(s - m)
                    l = jnp.sum(p, axis=0, keepdims=True)
                    ps.append((p.astype(BF16), 1.0 / l))
                st[t] = ps

            def pv(t):
                for u, (p, rl) in enumerate(st.pop(t)):
                    qs = t * TQ + u * 128
                    vt = jnp.concatenate([vt_s[i] for i in range(qs // 128 + 1)], axis=1)
                    qc_s[h, qs // 128] = (_dot(vt, p) * rl).astype(BF16)

            nt = S // TQ
            tiles = list(range(nt))[::-1]
            for i in range(4):
                kproj(512 * i, 512 * (i + 1))
                some_chans(4 if i < 3 else 2)
            qk(tiles[0])
            for i in range(4):
                vproj(512 * i, 512 * (i + 1))
                some_chans(4 if i < 3 else 2)
            assert not chans
            for i in range(nt):
                if i + 1 < nt:
                    qk(tiles[i + 1])
                pv(tiles[i])
            return carry

        lax.fori_loop(0, H, head, 0)

    pl.run_scoped(phase1, pltpu.VMEM((2, S, 128), BF16), pltpu.VMEM((NB, D, 128), BF16))

    def phase2(out_s):
        for c_ in g4:
            c_.wait()
        wot = jnp.concatenate([wot_s[b, C * h:C * (h + 1), :] for h in range(H) for b in range(2)], axis=1)
        outs = []
        CH = 4
        for ck in range(NB // CH):
            tiles = range(ck * CH, (ck + 1) * CH)
            ctx = jnp.concatenate(
                [jnp.concatenate([qc_s[h, t] for h in range(H)], axis=0) for t in tiles], axis=1)
            ot = _dot(wot, ctx)
            for t in tiles:
                rows = slice(128 * t, 128 * (t + 1))
                za = y_s[t * PITCH:t * PITCH + C, :] * qa_s[:, rows].astype(F32)
                z = jnp.concatenate([za, ot[:, 128 * (t - ck * CH):128 * (t - ck * CH + 1)]], axis=0)
                for b in range(7):
                    out_s[rows, 128 * b:128 * (b + 1)] = z[128 * b:128 * (b + 1)].T.astype(BF16)
            rows = pl.ds(128 * CH * ck, 128 * CH)
            oc = cp(out_s.at[rows], o_hbm.at[rows], 22 + ck)
            oc.start()
            outs.append(oc)
        for oc in outs:
            oc.wait()

    pl.run_scoped(phase2, pltpu.VMEM((S, 2 * C), BF16))


@jax.jit
def pallas_concat_heads__ssm_conv_h3__compressed_kv_cla__prompt_kernel(
    A_q: jax.Array,
    A_k: jax.Array,
    A_v: jax.Array,
    A_shift_k: jax.Array,
    A_ssm_k: jax.Array,
    A_ssm_D: jax.Array,
    B_x: jax.Array,
    B_c_kv: jax.Array,
    B_w_q: jax.Array,
    B_w_uk: jax.Array,
    B_w_uv: jax.Array,
    B_w_o: jax.Array,
):
    hbm = pl.BlockSpec(memory_space=pltpu.HBM)
    vmem = pl.BlockSpec(memory_space=pltpu.VMEM)
    out = pl.pallas_call(
        _kernel,
        in_specs=[hbm, hbm, hbm, vmem, hbm, vmem, hbm, hbm, hbm, hbm, hbm, hbm],
        out_specs=hbm,
        out_shape=jax.ShapeDtypeStruct((S, 2 * C), BF16),
        scratch_shapes=[
            pltpu.VMEM((8, S, 128), BF16),
            pltpu.VMEM((2, DC * 8, 128), U32),
            pltpu.VMEM((2, DC * 8, 128), U32),
            pltpu.VMEM((C, S), BF16),
            pltpu.VMEM((H, NB, D, 128), BF16),
            pltpu.VMEM((64 * PITCH, 128), U32),
            pltpu.VMEM((NB, C, 128), U32),
            pltpu.VMEM((NB * PITCH, 128), F32),
            pltpu.VMEM((2, H * C, 128), BF16),
            pltpu.SemaphoreType.DMA((26,)),
        ],
        compiler_params=pltpu.CompilerParams(vmem_limit_bytes=120 * 2 ** 20),
    )(
        A_q[0].T, A_k[0].T, A_v[0].T, A_shift_k.T, A_ssm_k, A_ssm_D, B_x[0].T, B_c_kv[0],
        B_w_q.reshape(C * H, D), B_w_uk.reshape(DC * H, D), B_w_uv.reshape(DC * H, D),
        jnp.swapaxes(B_w_o, 1, 2).reshape(H * C, D),
    )
    return out.reshape(1, S, 2 * C)
```

```python
import math

import jax
import jax.numpy as jnp
from jax import lax
import jax.experimental.pallas as pl
import jax.experimental.pallas.tpu as pltpu

F32 = jnp.float32
BF16 = jnp.bfloat16
U32 = jnp.uint32
I32 = jnp.int32

S = 2048
C = 448
H = 16
D = 256
DC = 1024
NB = S // 128
PITCH = 520
CPH = C // H
TQ = 512
NT = (((1,), (1,)), ((), ()))
LOG2E = math.log2(math.e)
QSCALE = (D ** -0.5) * LOG2E
NEG = -1e9 * LOG2E
HI_MASK = 0xFFFF0000


def _dot(a, b):
    return jnp.dot(a, b, preferred_element_type=F32)


def _dot_nt(a, b):
    return lax.dot_general(a, b, NT, preferred_element_type=F32)


def _head_cols(w_s, h, rows, halves=(0, 1)):
    out = []
    for b in halves:
        x = w_s[b, pl.ds(h // 2, rows, stride=8), :]
        if isinstance(h, int):
            x = (x << 16) if h % 2 == 0 else (x & jnp.uint32(HI_MASK))
        else:
            sh = ((1 - h % 2) * 16).astype(U32)
            x = (x << sh) & jnp.uint32(HI_MASK)
        out.append(pltpu.bitcast(x, F32))
    return out


def _kernel(qa_hbm, ka_hbm, va_hbm, sk_hbm, hk_hbm, d_hbm, x_hbm, c_hbm, wq_hbm, wk_hbm, wv_hbm, wo_hbm,
            o_hbm,
            c_s, wk_s, wv_s, qa_s, qc_s, aw_s, g_s, y_s, wot_s, sems):
    def cp(src, dst, i):
        return pltpu.make_async_copy(src, dst, sems.at[i])

    wq32 = wq_hbm.bitcast(U32)
    wk32 = wk_hbm.bitcast(U32)
    wv32 = wv_hbm.bitcast(U32)
    g3 = ([cp(c_hbm.at[:, pl.ds(128 * b, 128)], c_s.at[b], 8 + b) for b in range(8)]
          + [cp(wk32.at[:, pl.ds(128 * b, 128)], wk_s.at[b], 16 + b) for b in range(2)]
          + [cp(wv32.at[:, pl.ds(128 * b, 128)], wv_s.at[b], 18 + b) for b in range(2)])
    g4 = [cp(qa_hbm, qa_s, 21)] + [cp(wo_hbm.at[:, pl.ds(128 * b, 128)], wot_s.at[b], 6 + b) for b in range(2)]

    def phase0(x_s, wq_s, ka_s, va_s, hk_s, wd_s, sk_ref, d_ref):
        XC = 512
        cq = [cp(wq32.at[:, pl.ds(128 * b, 128)], wq_s.at[b], b) for b in range(2)]
        cx = [cp(x_hbm.at[:, pl.ds(XC * i, XC)], x_s.at[:, pl.ds(XC * i, XC)], 26 + i) for i in range(S // XC)]
        g2 = [cq[1], cp(sk_hbm, sk_ref, 2), cp(d_hbm, d_ref, 20),
              cp(ka_hbm, ka_s, 3), cp(va_hbm, va_s, 4), cp(hk_hbm, hk_s, 5)]
        for c_ in [cq[0]] + cx + g2 + g3 + g4:
            c_.start()

        def wq_t(h, b):
            t = _head_cols(wq_s, h, C, (b,))[0]
            return jnp.concatenate([t, jnp.zeros((512 - C, 128), F32)], axis=0).T[:, :C].astype(BF16)

        def qproj(wt, h, b, c0, c1):
            qt = (_dot(wt, x_s[:, c0:c1]) * QSCALE).astype(BF16)
            for t in range(c0 // 128, c1 // 128):
                qc_s[h, t, 128 * b:128 * (b + 1), :] = qt[:, 128 * t - c0:128 * (t + 1) - c0]

        cq[0].wait()
        first = [wq_t(h, 0) for h in range(2)]
        for i in range(S // XC):
            cx[i].wait()
            for h in range(2):
                qproj(first[h], h, 0, XC * i, XC * (i + 1))
        for h in range(2, 10):
            qproj(wq_t(h, 0), h, 0, 0, S)
        for c_ in g2:
            c_.wait()

        def column(row):
            row = jnp.concatenate([row.astype(F32), jnp.zeros((1, 512 - C), F32)], axis=1)
            return jnp.broadcast_to(row, (128, 512)).T

        taps = [column(sk_ref[j:j + 1, :]) for j in range(4)]
        dcol = column(d_ref[...].reshape(1, C))

        def shifted(cur, prev, n, lane):
            r = pltpu.roll(pltpu.bitcast(cur, U32), n, 1)
            x = jnp.where(lane >= n, r, 0 if prev is None else prev)
            return pltpu.bitcast(x, BF16).astype(F32), r

        def prep_u(b):
            w = 128 if b < 3 else C - 384
            rows = slice(128 * b, 128 * b + w)
            lane = lax.broadcasted_iota(I32, (w // 2, 128), 1)
            prev = jnp.zeros((w, 128), F32)
            pr = [None] * 4
            for sg in range(NB):
                cols = slice(128 * sg, 128 * (sg + 1))
                kb = ka_s[rows, cols]
                ks = [kb.astype(F32)]
                for n in range(1, 4):
                    x, pr[n] = shifted(kb, pr[n], n, lane)
                    ks.append(x)
                ksh = ((ks[3] * taps[3][rows] + ks[2] * taps[2][rows])
                       + (ks[1] * taps[1][rows] + ks[0] * taps[0][rows]))
                kv = ksh * va_s[rows, cols].astype(F32)
                wrd = pltpu.pack_elementwise([prev, kv], packed_dtype=BF16).astype(U32)
                if w < 128:
                    wrd = jnp.concatenate([wrd, jnp.zeros((128 - w, 128), U32)], axis=0)
                wd_s[b, cols, :] = wrd.T
                prev = kv

        def windows(b):
            for p in range(8):
                for j in range(8):
                    parts = []
                    for sg in range(2 * j - 6, 2 * j + 2):
                        if sg < 0:
                            parts.append(jnp.zeros((16, 128), U32))
                        else:
                            parts.append(wd_s[b, 128 * sg + 16 * p:128 * sg + 16 * p + 16, :])
                    plane = 32 * (j // 4) + 8 * (p // 2) + 4 * (p % 2) + j % 4
                    r0 = plane * PITCH + 128 * b
                    aw_s[r0:r0 + 128, :] = jnp.concatenate(parts, axis=0).T

        def prep_g(cb):
            rows = slice(64 * cb, 64 * (cb + 1))
            lane = lax.broadcasted_iota(I32, (64, 128), 1)
            prev = jnp.zeros((64, 128), F32)
            for a in range(NB):
                hf = hk_s[rows, 128 * a:128 * (a + 1)].astype(F32)
                if a == 0:
                    hf = jnp.where(lane == 0, hf + dcol[rows], hf)
                r = pltpu.roll(hf, 1, 1)
                hs = jnp.where(lane >= 1, r, prev)
                prev = r
                g_s[a, rows, :] = pltpu.pack_elementwise([hf, hs], packed_dtype=BF16).astype(U32)

        for b in range(4):
            prep_u(b)
            windows(b)
        for cb in range(C // 64):
            prep_g(cb)
        for h in range(10, H):
            qproj(wq_t(h, 0), h, 0, 0, S)
        for h in range(H):
            qproj(wq_t(h, 1), h, 1, 0, S)

    pl.run_scoped(
        phase0,
        pltpu.VMEM((C, S), BF16), pltpu.VMEM((2, C * 8, 128), U32), pltpu.VMEM((C, S), BF16),
        pltpu.VMEM((C, S), BF16), pltpu.VMEM((C, S), BF16), pltpu.VMEM((4, S, 128), U32),
        pltpu.VMEM((4, C), BF16), pltpu.VMEM((C,), BF16))

    for c_ in g3:
        c_.wait()

    def phase1(k_s, vt_s, wkx_s, wvx_s, *s_s):
        def extract_wk(h):
            for b, t in enumerate(_head_cols(wk_s, h, DC)):
                wkx_s[b] = t.astype(BF16)

        def extract_wv(h):
            for b, t in enumerate(_head_cols(wv_s, h, DC)):
                for i in range(DC // 128):
                    wvx_s[i, 128 * b:128 * (b + 1), :] = t[128 * i:128 * (i + 1)].T.astype(BF16)

        extract_wk(0)
        extract_wv(0)

        def head(h, carry):
            lane8 = lax.broadcasted_iota(I32, (8, 128), 1)
            sub8 = lax.broadcasted_iota(I32, (8, 128), 0)
            lane16 = lax.broadcasted_iota(I32, (16, 128), 1)
            sub16 = lax.broadcasted_iota(I32, (16, 128), 0)
            tri = (lax.broadcasted_iota(I32, (128, 128), 0) <= lax.broadcasted_iota(I32, (128, 128), 1))
            m_b = lane8 < 128 - 2 * sub8
            zero = h // H

            def chan_mm(c):
                gs = [jnp.broadcast_to(g_s[a, pl.ds(c, 1), :], (8, 128)) for a in range(NB)]
                bt = [pltpu.roll(jnp.where(m_b, gs[a], gs[a - 1] if a > 0 else jnp.uint32(0)), 0, 1,
                                 stride=2, stride_axis=0) for a in range(NB)]
                b1 = pltpu.bitcast(jnp.concatenate(bt[7::-1], axis=0), BF16)
                b2 = pltpu.bitcast(jnp.concatenate(bt[15:7:-1], axis=0), BF16)
                am = pltpu.bitcast(aw_s[pl.ds(c, 64, stride=PITCH), :], BF16)
                z1 = _dot(am, b1)
                z2 = _dot(am[:64], b2)
                return c, z1[:64], z1[64:] + z2

            def chan_post(c, zlo, zhi):
                acc = car = None
                for p in range(8):
                    z = jnp.concatenate([zlo[8 * p:8 * p + 8], zhi[8 * p:8 * p + 8]], axis=0)
                    if p == 0:
                        acc = z
                    else:
                        z = pltpu.roll(z, 16 * p, 1)
                        cz = jnp.where(lane16 < 16 * p, z, 0.0)
                        acc = acc + z
                        car = cz if car is None else car + cz
                y = (acc - car) + jnp.where(sub16 > 0, pltpu.roll(car, 1, 0), 0.0)
                y_s[pl.ds(c, NB, stride=PITCH), :] = y

            chans = [h * CPH + i for i in range(CPH)]
            pend = []

            def some_chans(n):
                old = list(pend)
                pend.clear()
                for _ in range(min(n, len(chans))):
                    pend.append(chan_mm(chans.pop(0)))
                for args in old:
                    chan_post(*args)

            wk = jnp.concatenate([wkx_s[0], wkx_s[1]], axis=1)
            h_next = jnp.minimum(h + 1, H - 1)

            def c_rows(r0, r1):
                return jnp.concatenate([c_s[b, r0:r1, :] for b in range(8)], axis=1)

            def kproj(r0, r1):
                k = _dot(c_rows(r0, r1), wk).astype(BF16)
                k_s[0, r0:r1, :] = k[:, :128]
                k_s[1, r0:r1, :] = k[:, 128:]

            def vproj(wvt, r0, r1):
                vt = _dot_nt(wvt, c_rows(r0, r1)).astype(BF16)
                for t in range(r0 // 128, r1 // 128):
                    vt_s[t] = vt[:, 128 * t - r0:128 * (t + 1) - r0]

            def k_rows(r0, r1):
                return jnp.concatenate([k_s[0, r0:r1, :], k_s[1, r0:r1, :]], axis=1)

            def q_cols(r0, r1):
                return jnp.concatenate([qc_s[h, t] for t in range(r0 // 128, r1 // 128)], axis=1)

            st = {}

            def qk(t):
                q0 = t * TQ
                if q0 > 0:
                    s_rect = _dot(k_rows(0, q0), q_cols(q0, q0 + TQ))
                ps = []
                for u in range(TQ // 128):
                    qs = q0 + u * 128
                    sd = _dot(k_rows(q0, qs + 128), q_cols(qs, qs + 128))
                    parts = []
                    if q0 > 0:
                        parts.append(s_rect[:, u * 128:(u + 1) * 128])
                    if u > 0:
                        parts.append(sd[:u * 128, :])
                    parts.append(jnp.where(tri, sd[u * 128:, :], NEG))
                    s = jnp.concatenate(parts, axis=0) if len(parts) > 1 else parts[0]
                    s_s[t % 2][u, 0:qs + 128, :] = s
                    ps.append(jnp.max(s, axis=0, keepdims=True))
                st[t] = ps

            def pv(t):
                for u, m in enumerate(st.pop(t)):
                    qs = t * TQ + u * 128
                    p = jnp.exp2(s_s[t % 2][u + zero, 0:qs + 128, :] - m)
                    rl = 1.0 / jnp.sum(p, axis=0, keepdims=True)
                    vt = jnp.concatenate([vt_s[i] for i in range(qs // 128 + 1)], axis=1)
                    qc_s[h, qs // 128] = (_dot(vt, p.astype(BF16)) * rl).astype(BF16)

            nt = S // TQ
            tiles = list(range(nt))[::-1]
            PC = 256
            for i in range(S // PC):
                kproj(PC * i, PC * (i + 1))
                some_chans(2 if i < 6 else 1)
            wvt = jnp.concatenate([wvx_s[i] for i in range(DC // 128)], axis=1)
            qk(tiles[0])
            extract_wk(h_next)
            for i in range(S // PC):
                vproj(wvt, PC * i, PC * (i + 1))
                some_chans(2 if i < 6 else 1)
            assert not chans
            for i in range(nt):
                if i + 1 < nt:
                    qk(tiles[i + 1])
                some_chans(0)
                if i == 0:
                    extract_wv(h_next)
                pv(tiles[i])
            return carry

        lax.fori_loop(0, H, head, 0)

    pl.run_scoped(phase1, pltpu.VMEM((2, S, 128), BF16), pltpu.VMEM((NB, D, 128), BF16),
                  pltpu.VMEM((2, DC, 128), BF16), pltpu.VMEM((DC // 128, D, 128), BF16),
                  pltpu.VMEM((TQ // 128, S, 128), F32), pltpu.VMEM((TQ // 128, S, 128), F32))

    def phase2(out_s):
        for c_ in g4:
            c_.wait()
        wot = jnp.concatenate([wot_s[b, C * h:C * (h + 1), :] for h in range(H) for b in range(2)], axis=1)
        outs = []
        CH = 4
        for ck in range(NB // CH):
            tiles = range(ck * CH, (ck + 1) * CH)
            ctx = jnp.concatenate(
                [jnp.concatenate([qc_s[h, t] for h in range(H)], axis=0) for t in tiles], axis=1)
            ot = _dot(wot, ctx)
            for t in tiles:
                rows = slice(128 * t, 128 * (t + 1))
                za = y_s[t * PITCH:t * PITCH + C, :] * qa_s[:, rows].astype(F32)
                z = jnp.concatenate([za, ot[:, 128 * (t - ck * CH):128 * (t - ck * CH + 1)]], axis=0)
                for b in range(7):
                    out_s[rows, 128 * b:128 * (b + 1)] = z[128 * b:128 * (b + 1)].T.astype(BF16)
            rows = pl.ds(128 * CH * ck, 128 * CH)
            oc = cp(out_s.at[rows], o_hbm.at[rows], 22 + ck)
            oc.start()
            outs.append(oc)
        for oc in outs:
            oc.wait()

    pl.run_scoped(phase2, pltpu.VMEM((S, 2 * C), BF16))


@jax.jit
def pallas_concat_heads__ssm_conv_h3__compressed_kv_cla__prompt_kernel(
    A_q: jax.Array,
    A_k: jax.Array,
    A_v: jax.Array,
    A_shift_k: jax.Array,
    A_ssm_k: jax.Array,
    A_ssm_D: jax.Array,
    B_x: jax.Array,
    B_c_kv: jax.Array,
    B_w_q: jax.Array,
    B_w_uk: jax.Array,
    B_w_uv: jax.Array,
    B_w_o: jax.Array,
):
    hbm = pl.BlockSpec(memory_space=pltpu.HBM)
    out = pl.pallas_call(
        _kernel,
        in_specs=[hbm] * 12,
        out_specs=hbm,
        out_shape=jax.ShapeDtypeStruct((S, 2 * C), BF16),
        scratch_shapes=[
            pltpu.VMEM((8, S, 128), BF16),
            pltpu.VMEM((2, DC * 8, 128), U32),
            pltpu.VMEM((2, DC * 8, 128), U32),
            pltpu.VMEM((C, S), BF16),
            pltpu.VMEM((H, NB, D, 128), BF16),
            pltpu.VMEM((64 * PITCH, 128), U32),
            pltpu.VMEM((NB, C, 128), U32),
            pltpu.VMEM((NB * PITCH, 128), F32),
            pltpu.VMEM((2, H * C, 128), BF16),
            pltpu.SemaphoreType.DMA((30,)),
        ],
        compiler_params=pltpu.CompilerParams(vmem_limit_bytes=120 * 2 ** 20),
    )(
        A_q[0].T, A_k[0].T, A_v[0].T, A_shift_k.T, A_ssm_k, A_ssm_D, B_x[0].T, B_c_kv[0],
        B_w_q.reshape(C * H, D), B_w_uk.reshape(DC * H, D), B_w_uv.reshape(DC * H, D),
        jnp.swapaxes(B_w_o, 1, 2).reshape(H * C, D),
    )
    return out.reshape(1, S, 2 * C)
```

```python
import math

import jax
import jax.numpy as jnp
from jax import lax
import jax.experimental.pallas as pl
import jax.experimental.pallas.tpu as pltpu

F32 = jnp.float32
BF16 = jnp.bfloat16
U32 = jnp.uint32
I32 = jnp.int32

S = 2048
C = 448
H = 16
D = 256
DC = 1024
NB = S // 128
NP = NB // 2
CH = C // 2
PITCH = 520
CPH = C // H
TQ = 512
NT = (((1,), (1,)), ((), ()))
LOG2E = math.log2(math.e)
QSCALE = (D ** -0.5) * LOG2E
NEG = -1e9 * LOG2E
HI_MASK = 0xFFFF0000


def _dot(a, b):
    return jnp.dot(a, b, preferred_element_type=F32)


def _dot_nt(a, b):
    return lax.dot_general(a, b, NT, preferred_element_type=F32)


def _lo(x):
    return pltpu.bitcast(x << 16, F32)


def _hi(x):
    return pltpu.bitcast(x & jnp.uint32(HI_MASK), F32)


def _head_cols(w_s, h, rows):
    out = []
    for b in range(2):
        x = w_s[b, pl.ds(h // 2, rows, stride=8), :]
        if isinstance(h, int):
            out.append(_lo(x) if h % 2 == 0 else _hi(x))
        else:
            out.append(_hi(x << ((1 - h % 2) * 16).astype(U32)))
    return out


def _lhs_terms(a11, a12, a21, a22):
    return [a11 + a22, a21 + a22, a11, a22, a11 + a12, a21 - a11, a12 - a22]


def _rhs_terms(b11, b12, b21, b22):
    return [b11 + b22, b11, b12 - b22, b21 - b11, b22, b11 + b12, b21 + b22]


_LHS_SUMS = (0, 1, 4, 5, 6)


def _strassen(prod, emit, order=(0, 1, 3, 2, 4, 5, 6)):
    uses = {(0, 0): {0: 1, 3: 1, 4: -1, 6: 1}, (0, 1): {2: 1, 4: 1},
            (1, 0): {1: 1, 3: 1}, (1, 1): {0: 1, 1: -1, 2: 1, 5: 1}}
    acc = {}
    neg = {}
    for i in order:
        m = prod(i)
        for key, terms in uses.items():
            if i not in terms:
                continue
            sign = terms.pop(i)
            if key not in acc:
                acc[key] = m
                neg[key] = sign < 0
            elif neg[key]:
                acc[key] = m - acc[key]
                neg[key] = False
            else:
                acc[key] = acc[key] + m if sign > 0 else acc[key] - m
            if not terms:
                emit(key[0], key[1], acc.pop(key))


def _kernel(qa_hbm, ka_hbm, va_hbm, sk_hbm, hk_hbm, d_hbm, x_hbm, c_hbm, wq_hbm, wk_hbm, wv_hbm, wo_hbm,
            o_hbm,
            c_s, cs_s, wk_s, wv_s, qa_s, qc_s, aw_s, g_s, y_s, wot_s, sems):
    def cp(src, dst, i):
        return pltpu.make_async_copy(src, dst, sems.at[i])

    wq32 = wq_hbm.bitcast(U32)
    wk32 = wk_hbm.bitcast(U32)
    wv32 = wv_hbm.bitcast(U32)
    gc = [cp(c_hbm.at[:, pl.ds(128 * b, 128)], c_s.at[b], 8 + b) for b in range(8)]
    g3 = ([cp(wk32.at[:, pl.ds(128 * b, 128)], wk_s.at[b], 16 + b) for b in range(2)]
          + [cp(wv32.at[:, pl.ds(128 * b, 128)], wv_s.at[b], 18 + b) for b in range(2)])
    g4 = [cp(qa_hbm, qa_s, 21)] + [cp(wo_hbm.at[:, pl.ds(128 * b, 128)], wot_s.at[b], 6 + b) for b in range(2)]

    def phase0(x_s, xs_s, wq_s, ka_s, va_s, hk_s, wd_s, sk_ref, d_ref):
        XC = 512
        cq = [cp(wq32.at[:, pl.ds(128 * b, 128)], wq_s.at[b], b) for b in range(2)]
        cx = [cp(x_hbm.at[:, pl.ds(XC * i, XC)], x_s.at[:, pl.ds(XC * i, XC)], 22 + i) for i in range(S // XC)]
        g2 = [cq[1], cp(sk_hbm, sk_ref, 2), cp(d_hbm, d_ref, 20),
              cp(ka_hbm, ka_s, 3), cp(va_hbm, va_s, 4), cp(hk_hbm, hk_s, 5)]
        for c_ in [cq[0]] + cx + g2 + gc + g3 + g4:
            c_.start()

        def pad_rows(t):
            return jnp.concatenate([t, jnp.zeros((256 - CH, 128), t.dtype)], axis=0)

        def wq_terms(j, b):
            x = wq_s[b, pl.ds(j, C, stride=8), :]
            lo, hi = _lo(x), _hi(x)
            blocks = [pad_rows(t).T for t in (lo[:CH], hi[:CH], lo[CH:], hi[CH:])]
            return [t.astype(BF16) for t in _rhs_terms(*blocks)]

        def x_terms(jp):
            top = slice(256 * jp, 256 * jp + 128)
            bot = slice(256 * jp + 128, 256 * jp + 256)
            blocks = [x_s[:CH, top], x_s[CH:, top], x_s[:CH, bot], x_s[CH:, bot]]
            for i, t in enumerate(_lhs_terms(*[t.astype(F32) for t in blocks])):
                xs_s[i, jp] = pad_rows(t.astype(BF16))

        def qproj(wt, j, b, p0, p1):
            def prod(i):
                return _dot(wt[i], jnp.concatenate([xs_s[i, jp] for jp in range(p0, p1)], axis=1))

            def emit(r, c, val):
                val = (val * QSCALE).astype(BF16)
                for jp in range(p0, p1):
                    qc_s[2 * j + c, 2 * jp + r, 128 * b:128 * (b + 1), :] = (
                        val[:, 128 * (jp - p0):128 * (jp - p0 + 1)])

            _strassen(prod, emit)

        def qproj_all(j, b):
            wt = wq_terms(j, b)
            for p0 in range(0, NP, 2):
                qproj(wt, j, b, p0, p0 + 2)

        cq[0].wait()
        first = wq_terms(0, 0)
        for i in range(S // XC):
            cx[i].wait()
            x_terms(2 * i)
            x_terms(2 * i + 1)
            qproj(first, 0, 0, 2 * i, 2 * i + 2)
        for j in range(1, 5):
            qproj_all(j, 0)
        for c_ in g2:
            c_.wait()

        def column(row):
            row = jnp.concatenate([row.astype(F32), jnp.zeros((1, 512 - C), F32)], axis=1)
            return jnp.broadcast_to(row, (128, 512)).T

        taps = [column(sk_ref[j:j + 1, :]) for j in range(4)]
        dcol = column(d_ref[...].reshape(1, C))

        def shifted(cur, prev, n, lane):
            r = pltpu.roll(pltpu.bitcast(cur, U32), n, 1)
            x = jnp.where(lane >= n, r, 0 if prev is None else prev)
            return pltpu.bitcast(x, BF16).astype(F32), r

        def prep_u(b):
            w = 128 if b < 3 else C - 384
            rows = slice(128 * b, 128 * b + w)
            lane = lax.broadcasted_iota(I32, (w // 2, 128), 1)
            prev = jnp.zeros((w, 128), F32)
            pr = [None] * 4
            for sg in range(NB):
                cols = slice(128 * sg, 128 * (sg + 1))
                kb = ka_s[rows, cols]
                ks = [kb.astype(F32)]
                for n in range(1, 4):
                    x, pr[n] = shifted(kb, pr[n], n, lane)
                    ks.append(x)
                ksh = ((ks[3] * taps[3][rows] + ks[2] * taps[2][rows])
                       + (ks[1] * taps[1][rows] + ks[0] * taps[0][rows]))
                kv = ksh * va_s[rows, cols].astype(F32)
                wrd = pltpu.pack_elementwise([prev, kv], packed_dtype=BF16).astype(U32)
                if w < 128:
                    wrd = jnp.concatenate([wrd, jnp.zeros((128 - w, 128), U32)], axis=0)
                wd_s[b, cols, :] = wrd.T
                prev = kv

        def windows(b):
            for p in range(8):
                for j in range(8):
                    parts = []
                    for sg in range(2 * j - 6, 2 * j + 2):
                        if sg < 0:
                            parts.append(jnp.zeros((16, 128), U32))
                        else:
                            parts.append(wd_s[b, 128 * sg + 16 * p:128 * sg + 16 * p + 16, :])
                    plane = 32 * (j // 4) + 8 * (p // 2) + 4 * (p % 2) + j % 4
                    r0 = plane * PITCH + 128 * b
                    aw_s[r0:r0 + 128, :] = jnp.concatenate(parts, axis=0).T

        def prep_g(cb):
            rows = slice(64 * cb, 64 * (cb + 1))
            lane = lax.broadcasted_iota(I32, (64, 128), 1)
            prev = jnp.zeros((64, 128), F32)
            for a in range(NB):
                hf = hk_s[rows, 128 * a:128 * (a + 1)].astype(F32)
                if a == 0:
                    hf = jnp.where(lane == 0, hf + dcol[rows], hf)
                r = pltpu.roll(hf, 1, 1)
                hs = jnp.where(lane >= 1, r, prev)
                prev = r
                g_s[a, rows, :] = pltpu.pack_elementwise([hf, hs], packed_dtype=BF16).astype(U32)

        def c_terms(jp):
            top = slice(256 * jp, 256 * jp + 128)
            bot = slice(256 * jp + 128, 256 * jp + 256)
            for cb in range(4):
                blocks = [c_s[cb, top, :], c_s[4 + cb, top, :], c_s[cb, bot, :], c_s[4 + cb, bot, :]]
                terms = _lhs_terms(*[t.astype(F32) for t in blocks])
                for n, i in enumerate(_LHS_SUMS):
                    cs_s[n, cb, 128 * jp:128 * (jp + 1), :] = terms[i].astype(BF16)

        for b in range(4):
            prep_u(b)
            windows(b)
        for cb in range(C // 64):
            prep_g(cb)
        for j in range(5, H // 2):
            qproj_all(j, 0)
        for j in range(H // 2 - 2):
            qproj_all(j, 1)
        for c_ in gc:
            c_.wait()
        for jp in range(NP):
            c_terms(jp)
        for j in range(H // 2 - 2, H // 2):
            qproj_all(j, 1)

    pl.run_scoped(
        phase0,
        pltpu.VMEM((C, S), BF16), pltpu.VMEM((7, NP, 256, 128), BF16), pltpu.VMEM((2, C * 8, 128), U32),
        pltpu.VMEM((C, S), BF16), pltpu.VMEM((C, S), BF16), pltpu.VMEM((C, S), BF16),
        pltpu.VMEM((4, S, 128), U32), pltpu.VMEM((4, C), BF16), pltpu.VMEM((C,), BF16))

    for c_ in g3:
        c_.wait()

    def phase1(k_s, vt_s, wkx_s, wvx_s, *s_s):
        KH = DC // 2

        def extract_wk(h):
            b0, b1 = _head_cols(wk_s, h, DC)
            for i, t in enumerate(_rhs_terms(b0[:KH], b1[:KH], b0[KH:], b1[KH:])):
                wkx_s[i] = t.astype(BF16)

        def extract_wv(h):
            b0, b1 = _head_cols(wv_s, h, DC)
            for cb in range(4):
                lo = slice(128 * cb, 128 * (cb + 1))
                hi = slice(KH + 128 * cb, KH + 128 * (cb + 1))
                for i, t in enumerate(_rhs_terms(b0[lo].T, b1[lo].T, b0[hi].T, b1[hi].T)):
                    wvx_s[i, cb] = t.astype(BF16)

        extract_wk(0)
        extract_wv(0)

        def head(h, carry):
            lane8 = lax.broadcasted_iota(I32, (8, 128), 1)
            sub8 = lax.broadcasted_iota(I32, (8, 128), 0)
            lane16 = lax.broadcasted_iota(I32, (16, 128), 1)
            sub16 = lax.broadcasted_iota(I32, (16, 128), 0)
            tri = (lax.broadcasted_iota(I32, (128, 128), 0) <= lax.broadcasted_iota(I32, (128, 128), 1))
            m_b = lane8 < 128 - 2 * sub8
            zero = h // H
            h_next = jnp.minimum(h + 1, H - 1)

            def chan_mm(c):
                gs = [jnp.broadcast_to(g_s[a, pl.ds(c, 1), :], (8, 128)) for a in range(NB)]
                bt = [pltpu.roll(jnp.where(m_b, gs[a], gs[a - 1] if a > 0 else jnp.uint32(0)), 0, 1,
                                 stride=2, stride_axis=0) for a in range(NB)]
                b1 = pltpu.bitcast(jnp.concatenate(bt[7::-1], axis=0), BF16)
                b2 = pltpu.bitcast(jnp.concatenate(bt[15:7:-1], axis=0), BF16)
                am = pltpu.bitcast(aw_s[pl.ds(c, 64, stride=PITCH), :], BF16)
                z1 = _dot(am, b1)
                z2 = _dot(am[:64], b2)
                return c, z1[:64], z1[64:] + z2

            def chan_post(c, zlo, zhi):
                acc = car = None
                for p in range(8):
                    z = jnp.concatenate([zlo[8 * p:8 * p + 8], zhi[8 * p:8 * p + 8]], axis=0)
                    if p == 0:
                        acc = z
                    else:
                        z = pltpu.roll(z, 16 * p, 1)
                        cz = jnp.where(lane16 < 16 * p, z, 0.0)
                        acc = acc + z
                        car = cz if car is None else car + cz
                y = (acc - car) + jnp.where(sub16 > 0, pltpu.roll(car, 1, 0), 0.0)
                y_s[pl.ds(c, NB, stride=PITCH), :] = y

            chans = [h * CPH + i for i in range(CPH)]
            pend = []

            def some_chans(n):
                old = list(pend)
                pend.clear()
                for _ in range(min(n, len(chans))):
                    pend.append(chan_mm(chans.pop(0)))
                for args in old:
                    chan_post(*args)

            def c_term(i, jp):
                if i == 2:
                    blocks = [c_s[cb, 256 * jp:256 * jp + 128, :] for cb in range(4)]
                elif i == 3:
                    blocks = [c_s[4 + cb, 256 * jp + 128:256 * jp + 256, :] for cb in range(4)]
                else:
                    n = _LHS_SUMS.index(i)
                    blocks = [cs_s[n, cb, 128 * jp:128 * (jp + 1), :] for cb in range(4)]
                return jnp.concatenate(blocks, axis=1)

            def kproj(jp):
                def emit(r, c, val):
                    k_s[c, 256 * jp + 128 * r:256 * jp + 128 * (r + 1), :] = val.astype(BF16)

                _strassen(lambda i: _dot(c_term(i, jp), wkx_s[i]), emit)

            def vproj(jp):
                def prod(i):
                    return _dot_nt(jnp.concatenate([wvx_s[i, cb] for cb in range(4)], axis=1), c_term(i, jp))

                def emit(r, c, val):
                    vt_s[2 * jp + r, 128 * c:128 * (c + 1), :] = val.astype(BF16)

                _strassen(prod, emit)

            def k_rows(r0, r1):
                return jnp.concatenate([k_s[0, r0:r1, :], k_s[1, r0:r1, :]], axis=1)

            def q_cols(r0, r1):
                return jnp.concatenate([qc_s[h, t] for t in range(r0 // 128, r1 // 128)], axis=1)

            st = {}

            def qk(t):
                q0 = t * TQ
                if q0 > 0:
                    s_rect = _dot(k_rows(0, q0), q_cols(q0, q0 + TQ))
                ms = []
                for u in range(TQ // 128):
                    qs = q0 + u * 128
                    sd = _dot(k_rows(q0, qs + 128), q_cols(qs, qs + 128))
                    parts = []
                    if q0 > 0:
                        parts.append(s_rect[:, u * 128:(u + 1) * 128])
                    if u > 0:
                        parts.append(sd[:u * 128, :])
                    parts.append(jnp.where(tri, sd[u * 128:, :], NEG))
                    s = jnp.concatenate(parts, axis=0) if len(parts) > 1 else parts[0]
                    s_s[t % 2][u, 0:qs + 128, :] = s
                    ms.append(jnp.max(s, axis=0, keepdims=True))
                st[t] = ms

            def pv(t):
                for u, m in enumerate(st.pop(t)):
                    qs = t * TQ + u * 128
                    p = jnp.exp2(s_s[t % 2][u + zero, 0:qs + 128, :] - m)
                    rl = 1.0 / jnp.sum(p, axis=0, keepdims=True)
                    vt = jnp.concatenate([vt_s[i] for i in range(qs // 128 + 1)], axis=1)
                    qc_s[h, qs // 128] = (_dot(vt, p.astype(BF16)) * rl).astype(BF16)

            nt = S // TQ
            tiles = list(range(nt))[::-1]
            for jp in range(NP):
                kproj(jp)
                some_chans(2 if jp < 6 else 1)
            qk(tiles[0])
            extract_wk(h_next)
            for jp in range(NP):
                vproj(jp)
                some_chans(2 if jp < 6 else 1)
            assert not chans
            for i in range(nt):
                if i + 1 < nt:
                    qk(tiles[i + 1])
                some_chans(0)
                if i == 0:
                    extract_wv(h_next)
                pv(tiles[i])
            return carry

        lax.fori_loop(0, H, head, 0)

    pl.run_scoped(phase1, pltpu.VMEM((2, S, 128), BF16), pltpu.VMEM((NB, D, 128), BF16),
                  pltpu.VMEM((7, DC // 2, 128), BF16), pltpu.VMEM((7, 4, 128, 128), BF16),
                  pltpu.VMEM((TQ // 128, S, 128), F32), pltpu.VMEM((TQ // 128, S, 128), F32))

    def phase2(out_s):
        for c_ in g4:
            c_.wait()
        HH = H // 2

        def wo_block(rh, kh):
            return jnp.concatenate(
                [wot_s[b, C * h + CH * rh:C * h + CH * (rh + 1), :]
                 for h in range(HH * kh, HH * (kh + 1)) for b in range(2)], axis=1)

        raw = [wo_block(0, 0), wo_block(1, 0), wo_block(0, 1), wo_block(1, 1)]
        wt = [t.astype(BF16) for t in _rhs_terms(*[t.astype(F32) for t in raw])]
        wt[1], wt[4] = raw[0], raw[3]
        outs = []
        for jp in range(NP):
            def ctx_block(r, kh):
                return jnp.concatenate([qc_s[h, 2 * jp + r] for h in range(HH * kh, HH * (kh + 1))], axis=0)

            craw = [ctx_block(0, 0), ctx_block(0, 1), ctx_block(1, 0), ctx_block(1, 1)]
            ct = [t.astype(BF16) for t in _lhs_terms(*[t.astype(F32) for t in craw])]
            ct[2], ct[3] = craw[0], craw[3]
            res = {}
            _strassen(lambda i: _dot(wt[i], ct[i]), lambda r, c, val: res.__setitem__((r, c), val),
                      order=(1, 4, 3, 2, 0, 5, 6))
            for r in range(2):
                t = 2 * jp + r
                rows = slice(128 * t, 128 * (t + 1))
                za = y_s[t * PITCH:t * PITCH + C, :] * qa_s[:, rows].astype(F32)
                z = jnp.concatenate([za, res[(r, 0)], res[(r, 1)]], axis=0)
                for b in range(7):
                    out_s[rows, 128 * b:128 * (b + 1)] = z[128 * b:128 * (b + 1)].T.astype(BF16)
            rows = pl.ds(256 * jp, 256)
            oc = cp(out_s.at[rows], o_hbm.at[rows], 26 + jp)
            oc.start()
            outs.append(oc)
        for oc in outs:
            oc.wait()

    pl.run_scoped(phase2, pltpu.VMEM((S, 2 * C), BF16))


@jax.jit
def pallas_concat_heads__ssm_conv_h3__compressed_kv_cla__prompt_kernel(
    A_q: jax.Array,
    A_k: jax.Array,
    A_v: jax.Array,
    A_shift_k: jax.Array,
    A_ssm_k: jax.Array,
    A_ssm_D: jax.Array,
    B_x: jax.Array,
    B_c_kv: jax.Array,
    B_w_q: jax.Array,
    B_w_uk: jax.Array,
    B_w_uv: jax.Array,
    B_w_o: jax.Array,
):
    hbm = pl.BlockSpec(memory_space=pltpu.HBM)
    out = pl.pallas_call(
        _kernel,
        in_specs=[hbm] * 12,
        out_specs=hbm,
        out_shape=jax.ShapeDtypeStruct((S, 2 * C), BF16),
        scratch_shapes=[
            pltpu.VMEM((8, S, 128), BF16),
            pltpu.VMEM((5, 4, S // 2, 128), BF16),
            pltpu.VMEM((2, DC * 8, 128), U32),
            pltpu.VMEM((2, DC * 8, 128), U32),
            pltpu.VMEM((C, S), BF16),
            pltpu.VMEM((H, NB, D, 128), BF16),
            pltpu.VMEM((64 * PITCH, 128), U32),
            pltpu.VMEM((NB, C, 128), U32),
            pltpu.VMEM((NB * PITCH, 128), F32),
            pltpu.VMEM((2, H * C, 128), BF16),
            pltpu.SemaphoreType.DMA((34,)),
        ],
        compiler_params=pltpu.CompilerParams(vmem_limit_bytes=120 * 2 ** 20),
    )(
        A_q[0].T, A_k[0].T, A_v[0].T, A_shift_k.T, A_ssm_k, A_ssm_D, B_x[0].T, B_c_kv[0],
        B_w_q.reshape(C * H, D), B_w_uk.reshape(DC * H, D), B_w_uv.reshape(DC * H, D),
        jnp.swapaxes(B_w_o, 1, 2).reshape(H * C, D),
    )
    return out.reshape(1, S, 2 * C)
```

```python
import math

import jax
import jax.numpy as jnp
from jax import lax
import jax.experimental.pallas as pl
import jax.experimental.pallas.tpu as pltpu

F32 = jnp.float32
BF16 = jnp.bfloat16
U32 = jnp.uint32
I32 = jnp.int32

S = 2048
C = 448
H = 16
D = 256
DC = 1024
NB = S // 128
NP = NB // 2
CH = C // 2
PITCH = 520
CPH = C // H
TQ = 512
NT = (((1,), (1,)), ((), ()))
LOG2E = math.log2(math.e)
QSCALE = (D ** -0.5) * LOG2E
NEG = -1e9 * LOG2E
HI_MASK = 0xFFFF0000
CFG = dict(gback=8,nf=1,costs=(2,2,1),slack=8,cg=3,sched='K0 C2 K1 C2 Q0 K2 C2 xw0 K3 C2 E00 E01 E02 E03 Q1 K4 C2 xw1 K5 C2 E10 E11 Q2 E12 E13 K6 C2 xw2 K7 C2 E20 Q3 xw3 V0 C2 E21 V1 C2 E22 P0 V2 C2 E23 V3 C2 E30 P1 V4 C2 E31 V5 C2 E32 P20 xk0 P21 P22 xk1 P23 V6 E33 V7 P30 xk2 P31 P32 xk3 P33')


def _dot(a, b):
    return jnp.dot(a, b, preferred_element_type=F32)


def _dot_nt(a, b):
    return lax.dot_general(a, b, NT, preferred_element_type=F32)


def _lo(x):
    return pltpu.bitcast(x << 16, F32)


def _hi(x):
    return pltpu.bitcast(x & jnp.uint32(HI_MASK), F32)


def _head_cols(w_s, h, rows):
    out = []
    for b in range(2):
        x = w_s[b, pl.ds(h // 2, rows, stride=8), :]
        if isinstance(h, int):
            out.append(_lo(x) if h % 2 == 0 else _hi(x))
        else:
            out.append(_hi(x << ((1 - h % 2) * 16).astype(U32)))
    return out


def _lhs_terms(a11, a12, a21, a22):
    return [a11 + a22, a21 + a22, a11, a22, a11 + a12, a21 - a11, a12 - a22]


def _rhs_terms(b11, b12, b21, b22):
    return [b11 + b22, b11, b12 - b22, b21 - b11, b22, b11 + b12, b21 + b22]


_LHS_SUMS = (0, 1, 4, 5, 6)


def _strassen(prod, emit, order=(0, 1, 3, 2, 4, 5, 6)):
    uses = {(0, 0): {0: 1, 3: 1, 4: -1, 6: 1}, (0, 1): {2: 1, 4: 1},
            (1, 0): {1: 1, 3: 1}, (1, 1): {0: 1, 1: -1, 2: 1, 5: 1}}
    acc = {}
    neg = {}
    for i in order:
        m = prod(i)
        for key, terms in uses.items():
            if i not in terms:
                continue
            sign = terms.pop(i)
            if key not in acc:
                acc[key] = m
                neg[key] = sign < 0
            elif neg[key]:
                acc[key] = m - acc[key]
                neg[key] = False
            else:
                acc[key] = acc[key] + m if sign > 0 else acc[key] - m
            if not terms:
                emit(key[0], key[1], acc.pop(key))


def _mult(i, n):
    return i if isinstance(i, int) else pl.multiple_of(i, n)


def _never(zero):
    return lax.broadcasted_iota(I32, (8, 128), 1) < zero


def _after(x, tok, never):
    if tok is None:
        return x
    return jnp.where(never, pltpu.bitcast(tok, x.dtype), x)


def _tied(lhs, due, never):
    if not due:
        return lhs
    t = None
    for d in due:
        d = pltpu.bitcast(jnp.broadcast_to(d, (8, 128)), U32)
        t = d if t is None else t ^ d
    due.clear()
    x = pltpu.bitcast(_after(pltpu.bitcast(lhs[:16, :128], U32), t, never), BF16)
    if lhs.shape[1] > 128:
        x = jnp.concatenate([x, lhs[:16, 128:]], axis=1)
    return jnp.concatenate([x, lhs[16:]], axis=0) if lhs.shape[0] > 16 else x


def _digest(vals):
    acc = None
    words = [v if v.dtype == U32 else pltpu.bitcast(v, U32) for v in vals]
    for r in range(words[0].shape[0] // 8):
        for w in words:
            w = w[8 * r:8 * (r + 1)]
            acc = w if acc is None else acc ^ w
    return acc


def _kernel(qa_hbm, ka_hbm, va_hbm, sk_hbm, hk_hbm, d_hbm, x_hbm, c_hbm, wq_hbm, wk_hbm, wv_hbm, wo_hbm,
            o_hbm,
            c_s, cs_s, wk_s, wv_s, qa_s, qc_s, aw_s, g_s, y_s, wot_s, wd_s, hk_s, dc_s, sems):
    def cp(src, dst, i):
        return pltpu.make_async_copy(src, dst, sems.at[i])

    wq32 = wq_hbm.bitcast(U32)
    wk32 = wk_hbm.bitcast(U32)
    wv32 = wv_hbm.bitcast(U32)
    gc = [cp(c_hbm.at[:, pl.ds(128 * b, 128)], c_s.at[b], 8 + b) for b in range(8)]
    g3 = ([cp(wk32.at[:, pl.ds(128 * b, 128)], wk_s.at[b], 16 + b) for b in range(2)]
          + [cp(wv32.at[:, pl.ds(128 * b, 128)], wv_s.at[b], 18 + b) for b in range(2)])
    g4 = [cp(qa_hbm, qa_s, 21)] + [cp(wo_hbm.at[:, pl.ds(128 * b, 128)], wot_s.at[b], 6 + b) for b in range(2)]

    def delayed(ref, rows, sg, n, gate=None):
        cur = pltpu.bitcast(ref[rows, 128 * sg:128 * (sg + 1)], U32)
        lane = lax.broadcasted_iota(I32, (8, 128), 1)
        if gate is not None:
            lane = gate(lane)
        lane = jnp.concatenate([lane] * (cur.shape[0] // 8), axis=0)
        prev = pltpu.bitcast(ref[rows, 128 * (sg - 1):128 * sg], U32) if sg > 0 else jnp.uint32(0)
        x = pltpu.roll(jnp.where(lane < 128 - n, cur, prev), n, 1)
        return pltpu.bitcast(x, BF16).astype(F32)

    def gated_t(x, gate):
        if gate is not None:
            x = jnp.concatenate([gate(x[:8]), x[8:]], axis=0)
        return x.T

    def windows(b, q, e, js, gate=None):
        out = []
        for j in js:
            parts = []
            for sg in range(2 * j - 6, 2 * j + 2):
                if sg < 0:
                    parts.append(jnp.zeros((16, 128), U32))
                else:
                    parts.append(wd_s[b, pl.ds(_mult(128 * sg + 32 * q + 16 * e, 16), 16), :])
            plane = 32 * (j // 4) + 8 * q + 4 * e + j % 4
            win = gated_t(jnp.concatenate(parts, axis=0), gate)
            aw_s[pl.ds(_mult(plane * PITCH + 128 * b, 8), 128), :] = win
            out.append(win[120:])
        return out

    def prep_g(r0, n, gate=None):
        rows = pl.ds(_mult(r0, 16), n)
        lane = lax.broadcasted_iota(I32, (n, 128), 1)
        for a in range(NB):
            hf = hk_s[rows, 128 * a:128 * (a + 1)].astype(F32)
            hs = delayed(hk_s, rows, a, 1, gate)
            if a == 0:
                hf = jnp.where(lane == 0, hf + dc_s[rows, :], hf)
                hs = jnp.where(lane == 1, hs + dc_s[rows, :], hs)
            wrd = pltpu.pack_elementwise([hf, hs], packed_dtype=BF16).astype(U32)
            g_s[a, rows, :] = wrd
            yield _digest([wrd])

    def phase0(x_s, xs_s, wq_s, ka_s, va_s, wc_s, sk_ref, d_ref):
        XC = 512
        cq = [cp(wq32.at[:, pl.ds(128 * b, 128)], wq_s.at[b], b) for b in range(2)]
        cx = [cp(x_hbm.at[:, pl.ds(XC * i, XC)], x_s.at[:, pl.ds(XC * i, XC)], 22 + i) for i in range(S // XC)]
        g2 = [cp(sk_hbm, sk_ref, 2), cp(d_hbm, d_ref, 20),
              cp(ka_hbm, ka_s, 3), cp(va_hbm, va_s, 4), cp(hk_hbm, hk_s, 5)]
        order = CFG.get('order', 'A')
        if order == 'A':
            ga, gb = g2, [cq[1]] + gc
        else:
            ga, gb = gc, g2 + [cq[1]]
        for c_ in [cx[0], cq[0]] + cx[1:] + ga + gb + g3 + g4:
            c_.start()
        never = _never(pl.semaphore_read(sems.at[34]))
        due = []
        toks = []

        def pad_rows(t):
            return jnp.concatenate([t, jnp.zeros((256 - CH, 128), t.dtype)], axis=0)

        def wq_terms(j, b, gate):
            x = wq_s[b, pl.ds(j, C, stride=8), :]
            g16 = jnp.concatenate([_after(jnp.full((8, 128), 16, U32), gate, never)] * (C // 8), axis=0)
            gm = jnp.concatenate([_after(jnp.full((8, 128), HI_MASK, U32), gate, never)] * (C // 8), axis=0)
            lo, hi = pltpu.bitcast(x << g16, F32), pltpu.bitcast(x & gm, F32)
            blocks = [pad_rows(t).T for t in (lo[:CH], hi[:CH], lo[CH:], hi[CH:])]
            return [t.astype(BF16) for t in _rhs_terms(*blocks)]

        def x_terms(jp):
            top = slice(256 * jp, 256 * jp + 128)
            bot = slice(256 * jp + 128, 256 * jp + 256)
            blocks = [x_s[:CH, top], x_s[CH:, top], x_s[:CH, bot], x_s[CH:, bot]]
            for i, t in enumerate(_lhs_terms(*[t.astype(F32) for t in blocks])):
                xs_s[i, jp] = pad_rows(t.astype(BF16))

        def qproj(g, jp, waits):
            j, b = groups[g]
            for c_ in waits:
                c_.wait()
            if False:
                x_terms(jp)
                x_terms(jp + 1)

            def prod(i):
                pump()
                m = _dot(_tied(wts[g][i], due, never), xs_s[i, jp])
                toks.append(m[:8])
                return m

            def emit(r, c, val):
                qc_s[2 * j + c, 2 * jp + r, 128 * b:128 * (b + 1), :] = (val * QSCALE).astype(BF16)

            _strassen(prod, emit)

        def column(row):
            row = jnp.concatenate([row.astype(F32), jnp.zeros((1, 512 - C), F32)], axis=1)
            return jnp.broadcast_to(row, (128, 512)).T

        consts = {}

        def make_consts():
            consts['taps'] = [column(sk_ref[j:j + 1, :]) for j in range(4)]
            dc_s[...] = column(d_ref[...].reshape(1, C))

        def gate(x):
            back = CFG.get('gback', 6)
            return _after(x, toks[-back], never) if back else x

        def prep_u(r0, n):
            rows = slice(r0, r0 + n)
            tp = [t[rows] for t in consts['taps']]
            prev = jnp.zeros((n, 128), F32)
            for sg in range(NB):
                cols = slice(128 * sg, 128 * (sg + 1))
                ksh = ((delayed(ka_s, rows, sg, 3, gate) * tp[3] + delayed(ka_s, rows, sg, 2, gate) * tp[2])
                       + (delayed(ka_s, rows, sg, 1, gate) * tp[1] + ka_s[rows, cols].astype(F32) * tp[0]))
                kv = ksh * va_s[rows, cols].astype(F32)
                wrd = pltpu.pack_elementwise([prev, kv], packed_dtype=BF16).astype(U32)
                wc_s[sg, rows, :] = wrd
                prev = kv
                yield _digest([wrd])

        def words_t(b):
            for sg in range(NB):
                if b < 3:
                    wrd = wc_s[sg, 128 * b:128 * (b + 1), :]
                else:
                    wrd = jnp.concatenate([wc_s[sg, 384:C, :], jnp.zeros((512 - C, 128), U32)], axis=0)
                wrd = gated_t(wrd, gate)
                wd_s[b, 128 * sg:128 * (sg + 1), :] = wrd
                yield wrd[120:]

        def all_windows(b):
            for p in range(8):
                for j in range(8):
                    yield windows(b, p // 2, p % 2, [j], gate)[0]

        def c_terms():
            RG = CFG.get('rg', 32)
            for jp in range(NP):
                for cb in range(4):
                    for r in range(0, 128, RG):
                        top = slice(256 * jp + r, 256 * jp + r + RG)
                        bot = slice(256 * jp + 128 + r, 256 * jp + 128 + r + RG)
                        blocks = [c_s[cb, top, :], c_s[4 + cb, top, :], c_s[cb, bot, :], c_s[4 + cb, bot, :]]
                        terms = _lhs_terms(*[t.astype(F32) for t in blocks])
                        terms = [terms[i].astype(BF16) for i in _LHS_SUMS]
                        for n, t in enumerate(terms):
                            cs_s[n, cb, 128 * jp + r:128 * jp + r + RG, :] = t
                        yield _digest(terms)

        UG = CFG.get('ug', 32)

        def a_stream():
            make_consts()
            cu, ct, cg = CFG.get('costs', (3, 2, 1))
            gs = [prep_g(r0, 32, gate) for r0 in range(0, C, 32)]
            for b in range(4):
                for r0 in range(128 * b, min(C, 128 * (b + 1)), UG):
                    for v in prep_u(r0, UG):
                        yield cu * UG // 32, v
                for v in words_t(b):
                    yield ct, v
                for v in all_windows(b):
                    yield ct, v
                if CFG.get('gpos', 'end') == 'blk' or b == 3:
                    for g_ in (gs[4 * b:4 * b + 4] if CFG.get('gpos', 'end') == 'blk' else gs):
                        for v in g_:
                            yield cg, v

        cu, ct, cg = CFG.get('costs', (3, 2, 1))
        a_total = cu * 14 * NB + ct * 4 * (NB + 64) + cg * 14 * NB
        streams = []
        nprod = [0]
        later = {}
        LAG = CFG.get('lag', 0)

        def pump():
            for st_ in streams:
                gen, n, p0, p1, done = st_
                want = min(n, max(0, (nprod[0] - p0 + 1) * n // (p1 - p0)))
                while st_[4] < want:
                    cost, v = next(gen)
                    later.setdefault(nprod[0] + LAG, []).append(v)
                    st_[4] += cost
            due.extend(later.pop(nprod[0], []))
            nprod[0] += 1

        groups = [(j, 0) for j in range(H // 2)] + [(j, 1) for j in range(H // 2)]
        NF = CFG.get('nf', 3)
        units = [(g, jp) for c in range(0, NP, 2) for g in range(NF) for jp in (c, c + 1)]
        units += [(g, jp) for g in range(NF, len(groups)) for jp in range(NP)]
        NU = len(units)
        wts = {}
        lead = CFG.get('lead', 4)
        ua = CFG.get('ua', 32)
        ub = 8 * NP - lead
        waits = {2 * NF: [cx[1]], 4 * NF: [cx[2]], 6 * NF: [cx[3]], ua: ga, ub: gb}
        sl = CFG.get('slack', 4)
        PA, PB, PE = 7 * ua + sl, 7 * ub + sl, 7 * NU - 2 - LAG
        c_stream = ((1, v) for v in c_terms())
        nc = NP * 4 * 128 // CFG.get('rg', 32)
        if order == 'A':
            streams.append([a_stream(), a_total, PA, PE, 0])
            streams.append([c_stream, nc, PB, PE, 0])
        else:
            streams.append([c_stream, nc, PA, CFG.get('cend', PB), 0])
            streams.append([a_stream(), a_total, PB, PE, 0])

        if not CFG.get('p0', 1):
            for c_ in cq + cx + g2 + gc:
                c_.wait()
            return
        cx[0].wait()
        x_terms(0)
        x_terms(1)
        cq[0].wait()
        first_use = {}
        for u, (g, jp) in enumerate(units):
            first_use.setdefault(g, u)
        for u, (g, jp) in enumerate(units):
            for c_ in waits.get(u, []):
                c_.wait()
                if any(c_ is o for o in cx):
                    x_terms(jp)
                    x_terms(jp + 1)
            for g_, fu in first_use.items():
                if g_ not in wts and fu - (lead if g_ >= NF else 1) <= u:
                    back = CFG.get('wback', 8)
                    wts[g_] = wq_terms(*groups[g_], toks[-back] if len(toks) >= back else None)
            qproj(g, jp, [])
        assert all(st_[4] == st_[1] for st_ in streams) and not later, streams

    pl.run_scoped(
        phase0,
        pltpu.VMEM((C, S), BF16), pltpu.VMEM((7, NP, 256, 128), BF16), pltpu.VMEM((2, C * 8, 128), U32),
        pltpu.VMEM((C, S), BF16), pltpu.VMEM((C, S), BF16), pltpu.VMEM((NB, C, 128), U32), pltpu.VMEM((4, C), BF16), pltpu.VMEM((C,), BF16))

    for c_ in g3:
        c_.wait()

    def phase1(k_s, vt_s, wkx_s, wvx_s, *s_s):
        KH = DC // 2

        def w_blocks(w_s, h, cb, gate):
            out = []
            for kh in range(2):
                for b in range(2):
                    x = w_s[b, pl.ds(8 * (KH * kh + 128 * cb) + h // 2, 128, stride=8), :]
                    if isinstance(h, int):
                        out.append(_lo(x) if h % 2 == 0 else _hi(x))
                    else:
                        out.append(_hi(x << jnp.concatenate([gate] * 16, axis=0)))
            return out

        digest = _digest

        def extract_wk(h, cb, gate=None):
            terms = [t.astype(BF16) for t in _rhs_terms(*w_blocks(wk_s, h, cb, gate))]
            for i, t in enumerate(terms):
                wkx_s[i, 128 * cb:128 * (cb + 1), :] = t
            return digest(terms)

        def extract_wv(h, cb, gate=None):
            terms = [t.astype(BF16) for t in _rhs_terms(*[t.T for t in w_blocks(wv_s, h, cb, gate)])]
            for i, t in enumerate(terms):
                wvx_s[i, cb] = t
            return digest(terms)

        for cb in range(4):
            extract_wk(0, cb)
            if 'xw' not in CFG.get('sched', ''):
                extract_wv(0, cb)

        def head(h, carry):
            lane8 = lax.broadcasted_iota(I32, (8, 128), 1)
            sub8 = lax.broadcasted_iota(I32, (8, 128), 0)
            lane16 = lax.broadcasted_iota(I32, (16, 128), 1)
            sub16 = lax.broadcasted_iota(I32, (16, 128), 0)
            tri = (lax.broadcasted_iota(I32, (128, 128), 0) <= lax.broadcasted_iota(I32, (128, 128), 1))
            zero = h // H
            h_next = jnp.minimum(h + 1, H - 1)
            toks = []
            due = []

            never = _never(zero)

            def after(x, tok):
                return _after(x, tok, never)

            def tied(lhs):
                return _tied(lhs, due, never)

            def tok(back):
                return toks[-back] if (back and len(toks) >= back) else None

            def chan_mm(c, gate):
                m_b = lane8 < after(128 - 2 * sub8, gate)
                gs = [jnp.broadcast_to(g_s[a, pl.ds(c, 1), :], (8, 128)) for a in range(NB)]
                bt = [pltpu.roll(jnp.where(m_b, gs[a], gs[a - 1] if a > 0 else jnp.uint32(0)), 0, 1,
                                 stride=2, stride_axis=0) for a in range(NB)]
                b1 = pltpu.bitcast(jnp.concatenate(bt[7::-1], axis=0), BF16)
                b2 = pltpu.bitcast(jnp.concatenate(bt[15:7:-1], axis=0), BF16)
                am = pltpu.bitcast(aw_s[pl.ds(c, 64, stride=PITCH), :], BF16)
                z1 = _dot(tied(am), b1)
                z2 = _dot(am[:64], b2)
                return c, z1[:64], z1[64:] + z2

            def chan_post(c, zlo, zhi):
                acc = car = None
                for p in range(8):
                    z = jnp.concatenate([zlo[8 * p:8 * p + 8], zhi[8 * p:8 * p + 8]], axis=0)
                    if p == 0:
                        acc = z
                    else:
                        z = pltpu.roll(z, 16 * p, 1)
                        cz = jnp.where(lane16 < 16 * p, z, 0.0)
                        acc = acc + z
                        car = cz if car is None else car + cz
                y = (acc - car) + jnp.where(sub16 > 0, pltpu.roll(car, 1, 0), 0.0)
                y_s[pl.ds(c, NB, stride=PITCH), :] = y
                if CFG.get('pd', 0):
                    due.append(y[:8])
                    due.append(y[8:])

            chans = [h * CPH + i for i in range(CPH)]

            def c_term(i, jp):
                if i == 2:
                    blocks = [c_s[cb, 256 * jp:256 * jp + 128, :] for cb in range(4)]
                elif i == 3:
                    blocks = [c_s[4 + cb, 256 * jp + 128:256 * jp + 256, :] for cb in range(4)]
                else:
                    n = _LHS_SUMS.index(i)
                    blocks = [cs_s[n, cb, 128 * jp:128 * (jp + 1), :] for cb in range(4)]
                return jnp.concatenate(blocks, axis=1)

            def kproj(jp):
                def emit(r, c, val):
                    if (r, c) == (1, 0):
                        toks.append(val[:8])
                    k_s[c, 256 * jp + 128 * r:256 * jp + 128 * (r + 1), :] = val.astype(BF16)

                _strassen(lambda i: _dot(tied(c_term(i, jp)), wkx_s[i]), emit)

            def vproj(jp):
                def prod(i):
                    return _dot_nt(tied(jnp.concatenate([wvx_s[i, cb] for cb in range(4)], axis=1)), c_term(i, jp))

                def emit(r, c, val):
                    if (r, c) == (1, 0):
                        toks.append(val[:8])
                    vt_s[2 * jp + r, 128 * c:128 * (c + 1), :] = val.astype(BF16)

                _strassen(prod, emit)

            def k_rows(r0, r1):
                return jnp.concatenate([k_s[0, r0:r1, :], k_s[1, r0:r1, :]], axis=1)

            def q_cols(r0, r1):
                return jnp.concatenate([qc_s[h, t] for t in range(r0 // 128, r1 // 128)], axis=1)

            mx, pr = {}, {}

            def qk(t):
                q0 = t * TQ
                if q0 > 0:
                    s_rect = _dot(tied(k_rows(0, q0)), q_cols(q0, q0 + TQ))
                    toks.append(s_rect[:8, :128])
                for u in range(TQ // 128):
                    qs = q0 + u * 128
                    sd = _dot(tied(k_rows(q0, qs + 128)), q_cols(qs, qs + 128))
                    parts = []
                    if q0 > 0:
                        parts.append(s_rect[:, u * 128:(u + 1) * 128])
                    if u > 0:
                        parts.append(sd[:u * 128, :])
                    parts.append(jnp.where(tri, sd[u * 128:, :], NEG))
                    s = jnp.concatenate(parts, axis=0) if len(parts) > 1 else parts[0]
                    s_s[t % 2][u, 0:qs + 128, :] = s
                    mx[(t, u)] = jnp.max(s, axis=0, keepdims=True)
                toks.append(sd[:8])

            def softmax(t, u, deadline):
                qs = t * TQ + u * 128
                p = jnp.exp2(s_s[t % 2][u + zero, 0:qs + 128, :] - mx.pop((t, u)))
                rl = 1.0 / jnp.sum(p, axis=0, keepdims=True)
                pr[(t, u)] = (p.astype(BF16), rl)
                if deadline:
                    due.append(rl)

            def pv(t, u):
                if (t, u) not in pr:
                    softmax(t, u, False)
                p, rl = pr.pop((t, u))
                qs = t * TQ + u * 128
                vt = jnp.concatenate([vt_s[i] for i in range(qs // 128 + 1)], axis=1)
                ctx = _dot(tied(vt), p)
                toks.append(ctx[:8])
                qc_s[h, qs // 128] = (ctx * rl).astype(BF16)

            def shift_of(hh, gate):
                return after(jnp.full((8, 128), (1 - hh % 2) * 16, I32).astype(U32), gate)

            CG, XG = CFG.get('cg', 0), CFG.get('xg', 0)
            pend = []
            for st_ in CFG['sched'].split():
                kind, arg = st_[0], st_[1:]
                if st_[:2] in ('xk', 'xv', 'xw'):
                    hh = h if st_[1] == 'w' else h_next
                    for cb in ([int(st_[2:])] if st_[2:] else range(4)):
                        due.append((extract_wk if st_[1] == 'k' else extract_wv)(hh, cb, shift_of(hh, tok(XG))))
                    continue
                if st_[0] in 'Ww':
                    e, j0, n = int(st_[1]), int(st_[2]), int(st_[3])
                    r = windows(jnp.minimum(1 + h // 4, 3), h % 4, e, range(j0, j0 + n), lambda x, t=tok(CFG.get('wg', 0)): after(x, t))
                    if st_[0] == 'W':
                        due.extend(r)
                    continue
                if st_ == 'dk':
                    due.append(pltpu.bitcast(wkx_s[zero, 0:16, :], F32))
                    continue
                if kind == 'E':
                    softmax(int(arg[0]), int(arg[1]), True)
                    continue
                old = list(pend)
                pend.clear()
                if kind == 'C':
                    for _ in range(int(arg)):
                        pend.append(chan_mm(chans.pop(0), tok(CG)))
                elif kind == 'K':
                    kproj(int(arg))
                elif kind == 'V':
                    vproj(int(arg))
                elif kind == 'Q':
                    qk(int(arg))
                elif kind == 'P':
                    for u in ([int(arg[1])] if len(arg) > 1 else range(TQ // 128)):
                        pv(int(arg[0]), u)
                for args in old:
                    chan_post(*args)
            assert not chans and not pend and (not due or CFG.get('pd')) and not pr and not mx
            return carry + zero

        if CFG.get('p1', 1):
            return lax.fori_loop(0, H, head, 0)
        else:
            def keep(h, carry):
                r = pl.multiple_of(h * 16, 16)
                t = (qc_s[h, h, 0:16, :].astype(F32) + cs_s[h % 5, h % 4, pl.ds(r, 16), :].astype(F32)
                     + pltpu.bitcast(aw_s[pl.ds(r, 16), :] + g_s[h, pl.ds(r, 16), :], F32)
                     + wkx_s[h % 7, pl.ds(r, 16), :].astype(F32) + wvx_s[h % 7, h % 4, 0:16, :].astype(F32))
                y_s[pl.ds(r, 16), :] = t
                return carry + h // H
            return lax.fori_loop(0, H, keep, 0)

    zero_end = pl.run_scoped(phase1, pltpu.VMEM((2, S, 128), BF16), pltpu.VMEM((NB, D, 128), BF16),
                  pltpu.VMEM((7, DC // 2, 128), BF16), pltpu.VMEM((7, 4, 128, 128), BF16),
                  pltpu.VMEM((TQ // 128, S, 128), F32), pltpu.VMEM((TQ // 128, S, 128), F32))

    def phase2(out_s):
        for c_ in g4:
            c_.wait()
        HH = H // 2

        def wo_block(rh, kh):
            return jnp.concatenate(
                [wot_s[b, C * h + CH * rh:C * h + CH * (rh + 1), :]
                 for h in range(HH * kh, HH * (kh + 1)) for b in range(2)], axis=1)

        raw = [wo_block(0, 0), wo_block(1, 0), wo_block(0, 1), wo_block(1, 1)]
        wt = [t.astype(BF16) for t in _rhs_terms(*[t.astype(F32) for t in raw])]
        wt[1], wt[4] = raw[0], raw[3]
        outs = []
        due, late = [], []
        DL = CFG.get('dl', 3)
        never = _never(zero_end)

        def put(t, b, z, opaque=False):
            o = z.T.astype(BF16)
            r0 = pl.multiple_of(zero_end * 16 + 128 * t, 16) if opaque else 128 * t
            out_s[pl.ds(r0, 128), 128 * b:128 * (b + 1)] = o
            late.append(pltpu.bitcast(o[112:], U32))

        for jp in range(NP if CFG.get('p2', 1) else 0):
            def ctx_block(r, kh):
                return jnp.concatenate([qc_s[h, 2 * jp + r] for h in range(HH * kh, HH * (kh + 1))], axis=0)

            craw = [ctx_block(0, 0), ctx_block(0, 1), ctx_block(1, 0), ctx_block(1, 1)]
            ct = [t.astype(BF16) for t in _lhs_terms(*[t.astype(F32) for t in craw])]
            ct[2], ct[3] = craw[0], craw[3]
            za = {}
            prev_late = list(late)
            late.clear()
            for r in range(2):
                t = 2 * jp + r
                za[r] = y_s[t * PITCH:t * PITCH + C, :] * qa_s[:, 128 * t:128 * (t + 1)].astype(F32)
                for b in range(3):
                    put(t, b, za[r][128 * b:128 * (b + 1)], opaque=(r == 0 and b == 0 and jp > 0))
            a_late = list(late)
            late.clear()
            res = {}
            count = [0]

            def prod(i):
                if count[0] == DL:
                    due.extend(prev_late)
                if count[0] == 6:
                    due.extend(a_late)
                count[0] += 1
                return _dot(_tied(wt[i], due, never), ct[i])

            _strassen(prod, lambda r, c, val: res.__setitem__((r, c), val), order=(1, 4, 3, 2, 0, 5, 6))
            for r in (1, 0):
                z = jnp.concatenate([za[r][384:], res[(r, 0)], res[(r, 1)]], axis=0)
                for b in (3, 2, 1, 0):
                    put(2 * jp + r, 3 + b, z[128 * b:128 * (b + 1)])
            rows = pl.ds(256 * jp, 256)
            oc = cp(out_s.at[rows], o_hbm.at[rows], 26 + jp)
            oc.start()
            outs.append(oc)
        if not CFG.get('p2', 1):
            def keep(h, carry):
                r = pl.multiple_of(h * 16, 16)
                out_s[pl.ds(r, 16), 0:128] = y_s[pl.ds(r, 16), :].astype(BF16) + qc_s[h, h, 0:16, :]
                return carry
            lax.fori_loop(0, H, keep, 0)
            oc = cp(out_s.at[pl.ds(0, 256)], o_hbm.at[pl.ds(0, 256)], 26)
            oc.start()
            outs.append(oc)
        for oc in outs:
            oc.wait()

    pl.run_scoped(phase2, pltpu.VMEM((S, 2 * C), BF16))


@jax.jit
def pallas_concat_heads__ssm_conv_h3__compressed_kv_cla__prompt_kernel(
    A_q: jax.Array,
    A_k: jax.Array,
    A_v: jax.Array,
    A_shift_k: jax.Array,
    A_ssm_k: jax.Array,
    A_ssm_D: jax.Array,
    B_x: jax.Array,
    B_c_kv: jax.Array,
    B_w_q: jax.Array,
    B_w_uk: jax.Array,
    B_w_uv: jax.Array,
    B_w_o: jax.Array,
):
    hbm = pl.BlockSpec(memory_space=pltpu.HBM)
    out = pl.pallas_call(
        _kernel,
        in_specs=[hbm] * 12,
        out_specs=hbm,
        out_shape=jax.ShapeDtypeStruct((S, 2 * C), BF16),
        scratch_shapes=[
            pltpu.VMEM((8, S, 128), BF16),
            pltpu.VMEM((5, 4, S // 2, 128), BF16),
            pltpu.VMEM((2, DC * 8, 128), U32),
            pltpu.VMEM((2, DC * 8, 128), U32),
            pltpu.VMEM((C, S), BF16),
            pltpu.VMEM((H, NB, D, 128), BF16),
            pltpu.VMEM((64 * PITCH, 128), U32),
            pltpu.VMEM((NB, C, 128), U32),
            pltpu.VMEM((NB * PITCH, 128), F32),
            pltpu.VMEM((2, H * C, 128), BF16),
            pltpu.VMEM((4, S, 128), U32),
            pltpu.VMEM((C, S), BF16),
            pltpu.VMEM((512, 128), F32),
            pltpu.SemaphoreType.DMA((35,)),
        ],
        compiler_params=pltpu.CompilerParams(vmem_limit_bytes=120 * 2 ** 20),
    )(
        A_q[0].T, A_k[0].T, A_v[0].T, A_shift_k.T, A_ssm_k, A_ssm_D, B_x[0].T, B_c_kv[0],
        B_w_q.reshape(C * H, D), B_w_uk.reshape(DC * H, D), B_w_uv.reshape(DC * H, D),
        jnp.swapaxes(B_w_o, 1, 2).reshape(H * C, D),
    )
    return out.reshape(1, S, 2 * C)
```

```python
import math

import jax
import jax.numpy as jnp
from jax import lax
import jax.experimental.pallas as pl
import jax.experimental.pallas.tpu as pltpu

F32 = jnp.float32
BF16 = jnp.bfloat16
U32 = jnp.uint32
I32 = jnp.int32

S = 2048
C = 448
H = 16
D = 256
DC = 1024
NB = S // 128
NP = NB // 2
CH = C // 2
PITCH = 520
CPH = C // H
TQ = 512
NT = (((1,), (1,)), ((), ()))
LOG2E = math.log2(math.e)
QSCALE = (D ** -0.5) * LOG2E
NEG = -1e9 * LOG2E
HI_MASK = 0xFFFF0000
CFG = dict(gback=8,nf=1,costs=(2,2,1),slack=8,cg=3,sched='K0 C2 K1 C2 Q0 K2 C2 xw0 K3 C2 E00 E01 E02 E03 Q1 K4 C2 xw1 K5 C2 E10 E11 Q2 E12 E13 K6 C2 xw2 K7 C2 E20 Q3 xw3 V0 C2 E21 V1 C2 E22 P0 V2 C2 E23 V3 C2 E30 P1 V4 C2 E31 V5 C2 E32 P20 xk0 P21 P22 xk1 P23 V6 E33 V7 P30 xk2 P31 P32 xk3 P33')


def _wait(copies, name):
    if CFG.get('scopes'):
        with jax.named_scope(name):
            for c_ in copies:
                c_.wait()
    else:
        for c_ in copies:
            c_.wait()


def _dot(a, b):
    return jnp.dot(a, b, preferred_element_type=F32)


def _dot_nt(a, b):
    return lax.dot_general(a, b, NT, preferred_element_type=F32)


def _lo(x):
    return pltpu.bitcast(x << 16, F32)


def _hi(x):
    return pltpu.bitcast(x & jnp.uint32(HI_MASK), F32)


def _head_cols(w_s, h, rows):
    out = []
    for b in range(2):
        x = w_s[b, pl.ds(h // 2, rows, stride=8), :]
        if isinstance(h, int):
            out.append(_lo(x) if h % 2 == 0 else _hi(x))
        else:
            out.append(_hi(x << ((1 - h % 2) * 16).astype(U32)))
    return out


def _lhs_terms(a11, a12, a21, a22):
    return [a11 + a22, a21 + a22, a11, a22, a11 + a12, a21 - a11, a12 - a22]


def _rhs_terms(b11, b12, b21, b22):
    return [b11 + b22, b11, b12 - b22, b21 - b11, b22, b11 + b12, b21 + b22]


_LHS_SUMS = (0, 1, 4, 5, 6)


def _strassen(prod, emit, order=(0, 1, 3, 2, 4, 5, 6)):
    uses = {(0, 0): {0: 1, 3: 1, 4: -1, 6: 1}, (0, 1): {2: 1, 4: 1},
            (1, 0): {1: 1, 3: 1}, (1, 1): {0: 1, 1: -1, 2: 1, 5: 1}}
    acc = {}
    neg = {}
    for i in order:
        m = prod(i)
        for key, terms in uses.items():
            if i not in terms:
                continue
            sign = terms.pop(i)
            if key not in acc:
                acc[key] = m
                neg[key] = sign < 0
            elif neg[key]:
                acc[key] = m - acc[key]
                neg[key] = False
            else:
                acc[key] = acc[key] + m if sign > 0 else acc[key] - m
            if not terms:
                emit(key[0], key[1], acc.pop(key))


def _mult(i, n):
    return i if isinstance(i, int) else pl.multiple_of(i, n)


def _never(zero):
    return lax.broadcasted_iota(I32, (8, 128), 1) < zero


def _after(x, tok, never):
    if tok is None:
        return x
    return jnp.where(never, pltpu.bitcast(tok, x.dtype), x)


def _tied(lhs, due, never):
    if not due:
        return lhs
    t = None
    for d in due:
        d = pltpu.bitcast(jnp.broadcast_to(d, (8, 128)), U32)
        t = d if t is None else t ^ d
    due.clear()
    x = pltpu.bitcast(_after(pltpu.bitcast(lhs[:16, :128], U32), t, never), BF16)
    if lhs.shape[1] > 128:
        x = jnp.concatenate([x, lhs[:16, 128:]], axis=1)
    return jnp.concatenate([x, lhs[16:]], axis=0) if lhs.shape[0] > 16 else x


def _digest(vals):
    acc = None
    words = [v if v.dtype == U32 else pltpu.bitcast(v, U32) for v in vals]
    for r in range(words[0].shape[0] // 8):
        for w in words:
            w = w[8 * r:8 * (r + 1)]
            acc = w if acc is None else acc ^ w
    return acc


def _kernel(qa_hbm, ka_hbm, va_hbm, sk_hbm, hk_hbm, d_hbm, x_hbm, c_hbm, wq_hbm, wk_hbm, wv_hbm, wo_hbm,
            o_hbm,
            c_s, cs_s, wk_s, wv_s, qa_s, qc_s, aw_s, g_s, y_s, wot_s, wd_s, hk_s, dc_s, sems):
    def cp(src, dst, i):
        return pltpu.make_async_copy(src, dst, sems.at[i])

    wq32 = wq_hbm.bitcast(U32)
    wk32 = wk_hbm.bitcast(U32)
    wv32 = wv_hbm.bitcast(U32)
    gc = [cp(c_hbm.at[:, pl.ds(128 * b, 128)], c_s.at[b], 8 + b) for b in range(8)]
    g3 = [cp(wk32.at[:, 0], wk_s.at[0], 16), cp(wv32.at[:, 0], wv_s.at[0], 17)]
    g3b = [cp(wk32.at[:, 1], wk_s.at[1], 18), cp(wv32.at[:, 1], wv_s.at[1], 19)]
    g4 = [cp(qa_hbm, qa_s, 21)] + [cp(wo_hbm.at[:, pl.ds(128 * b, 128)], wot_s.at[b], 6 + b) for b in range(2)]

    def delayed(ref, rows, sg, n, gate=None):
        cur = pltpu.bitcast(ref[rows, 128 * sg:128 * (sg + 1)], U32)
        lane = lax.broadcasted_iota(I32, (8, 128), 1)
        if gate is not None:
            lane = gate(lane)
        lane = jnp.concatenate([lane] * (cur.shape[0] // 8), axis=0)
        prev = pltpu.bitcast(ref[rows, 128 * (sg - 1):128 * sg], U32) if sg > 0 else jnp.uint32(0)
        x = pltpu.roll(jnp.where(lane < 128 - n, cur, prev), n, 1)
        return pltpu.bitcast(x, BF16).astype(F32)

    def gated_t(x, gate):
        if gate is not None:
            x = jnp.concatenate([gate(x[:8]), x[8:]], axis=0)
        return x.T

    def windows(b, q, e, js, gate=None):
        out = []
        for j in js:
            parts = []
            for sg in range(2 * j - 6, 2 * j + 2):
                if sg < 0:
                    parts.append(jnp.zeros((16, 128), U32))
                else:
                    parts.append(wd_s[b, pl.ds(_mult(128 * sg + 32 * q + 16 * e, 16), 16), :])
            plane = 32 * (j // 4) + 8 * q + 4 * e + j % 4
            win = gated_t(jnp.concatenate(parts, axis=0), gate)
            aw_s[pl.ds(_mult(plane * PITCH + 128 * b, 8), 128), :] = win
            out.append(win[120:])
        return out

    def prep_g(r0, n, gate=None):
        rows = pl.ds(_mult(r0, 16), n)
        lane = lax.broadcasted_iota(I32, (n, 128), 1)
        for a in range(NB):
            hf = hk_s[rows, 128 * a:128 * (a + 1)].astype(F32)
            hs = delayed(hk_s, rows, a, 1, gate)
            if a == 0:
                hf = jnp.where(lane == 0, hf + dc_s[rows, :], hf)
                hs = jnp.where(lane == 1, hs + dc_s[rows, :], hs)
            wrd = pltpu.pack_elementwise([hf, hs], packed_dtype=BF16).astype(U32)
            g_s[a, rows, :] = wrd
            yield _digest([wrd])

    def phase0(x_s, xs_s, wq_s, ka_s, va_s, wc_s, sk_ref, d_ref):
        XC = 512
        cq = [cp(wq32.at[:, g], wq_s.at[g], g) for g in range(2)]
        cx = [cp(x_hbm.at[:, pl.ds(XC * i, XC)], x_s.at[:, pl.ds(XC * i, XC)], 22 + i) for i in range(S // XC)]
        g2 = [cp(sk_hbm, sk_ref, 2), cp(d_hbm, d_ref, 20),
              cp(ka_hbm, ka_s, 3), cp(va_hbm, va_s, 4), cp(hk_hbm, hk_s, 5)]
        order = CFG.get('order', 'A')
        if order == 'A':
            ga, gb = g2, [cq[1]] + gc
        else:
            ga, gb = gc, g2 + [cq[1]]
        for c_ in [cx[0], cq[0]] + cx[1:] + ga + gb + g3 + g3b + g4:
            c_.start()
        never = _never(pl.semaphore_read(sems.at[34]))
        due = []
        toks = []

        def pad_rows(t):
            return jnp.concatenate([t, jnp.zeros((256 - CH, 128), t.dtype)], axis=0)

        def wq_terms(j, b, gate):
            x = wq_s.reshape(2, C * 8, 128)[j // 4, pl.ds(4 * b + j % 4, C, stride=8), :]
            g16 = jnp.concatenate([_after(jnp.full((8, 128), 16, U32), gate, never)] * (C // 8), axis=0)
            gm = jnp.concatenate([_after(jnp.full((8, 128), HI_MASK, U32), gate, never)] * (C // 8), axis=0)
            lo, hi = pltpu.bitcast(x << g16, F32), pltpu.bitcast(x & gm, F32)
            blocks = [pad_rows(t).T for t in (lo[:CH], hi[:CH], lo[CH:], hi[CH:])]
            return [t.astype(BF16) for t in _rhs_terms(*blocks)]

        def x_terms(jp):
            top = slice(256 * jp, 256 * jp + 128)
            bot = slice(256 * jp + 128, 256 * jp + 256)
            blocks = [x_s[:CH, top], x_s[CH:, top], x_s[:CH, bot], x_s[CH:, bot]]
            for i, t in enumerate(_lhs_terms(*[t.astype(F32) for t in blocks])):
                xs_s[i, jp] = pad_rows(t.astype(BF16))

        def qproj(g, jp, waits):
            j, b = groups[g]
            for c_ in waits:
                c_.wait()
            if False:
                x_terms(jp)
                x_terms(jp + 1)

            def prod(i):
                pump()
                m = _dot(_tied(wts[g][i], due, never), xs_s[i, jp])
                toks.append(m[:8])
                return m

            def emit(r, c, val):
                qc_s[2 * j + c, 2 * jp + r, 128 * b:128 * (b + 1), :] = (val * QSCALE).astype(BF16)

            _strassen(prod, emit)

        def column(row):
            row = jnp.concatenate([row.astype(F32), jnp.zeros((1, 512 - C), F32)], axis=1)
            return jnp.broadcast_to(row, (128, 512)).T

        consts = {}

        def make_consts():
            consts['taps'] = [column(sk_ref[j:j + 1, :]) for j in range(4)]
            dc_s[...] = column(d_ref[...].reshape(1, C))

        def gate(x):
            back = CFG.get('gback', 6)
            return _after(x, toks[-back], never) if back else x

        def prep_u(r0, n):
            rows = slice(r0, r0 + n)
            tp = [t[rows] for t in consts['taps']]
            prev = jnp.zeros((n, 128), F32)
            for sg in range(NB):
                cols = slice(128 * sg, 128 * (sg + 1))
                ksh = ((delayed(ka_s, rows, sg, 3, gate) * tp[3] + delayed(ka_s, rows, sg, 2, gate) * tp[2])
                       + (delayed(ka_s, rows, sg, 1, gate) * tp[1] + ka_s[rows, cols].astype(F32) * tp[0]))
                kv = ksh * va_s[rows, cols].astype(F32)
                wrd = pltpu.pack_elementwise([prev, kv], packed_dtype=BF16).astype(U32)
                wc_s[sg, rows, :] = wrd
                prev = kv
                yield _digest([wrd])

        def words_t(b):
            for sg in range(NB):
                if b < 3:
                    wrd = wc_s[sg, 128 * b:128 * (b + 1), :]
                else:
                    wrd = jnp.concatenate([wc_s[sg, 384:C, :], jnp.zeros((512 - C, 128), U32)], axis=0)
                wrd = gated_t(wrd, gate)
                wd_s[b, 128 * sg:128 * (sg + 1), :] = wrd
                yield wrd[120:]

        def all_windows(b):
            for p in range(8):
                for j in range(8):
                    yield windows(b, p // 2, p % 2, [j], gate)[0]

        def c_terms():
            RG = CFG.get('rg', 32)
            for jp in range(NP):
                for cb in range(4):
                    for r in range(0, 128, RG):
                        top = slice(256 * jp + r, 256 * jp + r + RG)
                        bot = slice(256 * jp + 128 + r, 256 * jp + 128 + r + RG)
                        blocks = [c_s[cb, top, :], c_s[4 + cb, top, :], c_s[cb, bot, :], c_s[4 + cb, bot, :]]
                        terms = _lhs_terms(*[t.astype(F32) for t in blocks])
                        terms = [terms[i].astype(BF16) for i in _LHS_SUMS]
                        for n, t in enumerate(terms):
                            cs_s[n, cb, 128 * jp + r:128 * jp + r + RG, :] = t
                        yield _digest(terms)

        UG = CFG.get('ug', 32)

        def a_stream():
            make_consts()
            cu, ct, cg = CFG.get('costs', (3, 2, 1))
            gs = [prep_g(r0, 32, gate) for r0 in range(0, C, 32)]
            for b in range(4):
                for r0 in range(128 * b, min(C, 128 * (b + 1)), UG):
                    for v in prep_u(r0, UG):
                        yield cu * UG // 32, v
                for v in words_t(b):
                    yield ct, v
                for v in all_windows(b):
                    yield ct, v
                if CFG.get('gpos', 'end') == 'blk' or b == 3:
                    for g_ in (gs[4 * b:4 * b + 4] if CFG.get('gpos', 'end') == 'blk' else gs):
                        for v in g_:
                            yield cg, v

        cu, ct, cg = CFG.get('costs', (3, 2, 1))
        a_total = cu * 14 * NB + ct * 4 * (NB + 64) + cg * 14 * NB
        streams = []
        nprod = [0]
        later = {}
        LAG = CFG.get('lag', 0)

        def pump():
            for st_ in streams:
                gen, n, p0, p1, done = st_
                want = min(n, max(0, (nprod[0] - p0 + 1) * n // (p1 - p0)))
                while st_[4] < want:
                    cost, v = next(gen)
                    later.setdefault(nprod[0] + LAG, []).append(v)
                    st_[4] += cost
            due.extend(later.pop(nprod[0], []))
            nprod[0] += 1

        groups = [(j, b) for j in range(H // 2) for b in range(2)]
        NF = CFG.get('nf', 3)
        units = [(g, jp) for c in range(0, NP, 2) for g in range(NF) for jp in (c, c + 1)]
        units += [(g, jp) for g in range(NF, len(groups)) for jp in range(NP)]
        NU = len(units)
        wts = {}
        lead = CFG.get('lead', 4)
        ua = CFG.get('ua', 32)
        ub = 8 * NP - lead
        waits = {2 * NF: [cx[1]], 4 * NF: [cx[2]], 6 * NF: [cx[3]], ua: ga, ub: gb}
        sl = CFG.get('slack', 4)
        PA, PB, PE = 7 * ua + sl, 7 * ub + sl, 7 * NU - 2 - LAG
        c_stream = ((1, v) for v in c_terms())
        nc = NP * 4 * 128 // CFG.get('rg', 32)
        if order == 'A':
            streams.append([a_stream(), a_total, PA, PE, 0])
            streams.append([c_stream, nc, PB, PE, 0])
        else:
            streams.append([c_stream, nc, PA, CFG.get('cend', PB), 0])
            streams.append([a_stream(), a_total, PB, PE, 0])

        if not CFG.get('p0', 1):
            for c_ in cq + cx + g2 + gc:
                c_.wait()
            return
        _wait([cx[0]], 'wx0')
        x_terms(0)
        x_terms(1)
        _wait([cq[0]], 'wq0')
        first_use = {}
        for u, (g, jp) in enumerate(units):
            first_use.setdefault(g, u)
        for u, (g, jp) in enumerate(units):
            if u in waits:
                _wait(waits[u], 'wu%d' % u)
                if any(waits[u][0] is o for o in cx):
                    x_terms(jp)
                    x_terms(jp + 1)
            for g_, fu in first_use.items():
                if g_ not in wts and fu - (lead if g_ >= NF else 1) <= u:
                    back = CFG.get('wback', 8)
                    wts[g_] = wq_terms(*groups[g_], toks[-back] if len(toks) >= back else None)
            qproj(g, jp, [])
        assert all(st_[4] == st_[1] for st_ in streams) and not later, streams

    pl.run_scoped(
        phase0,
        pltpu.VMEM((C, S), BF16), pltpu.VMEM((7, NP, 256, 128), BF16), pltpu.VMEM((2, C, 8, 128), U32),
        pltpu.VMEM((C, S), BF16), pltpu.VMEM((C, S), BF16), pltpu.VMEM((NB, C, 128), U32), pltpu.VMEM((4, C), BF16), pltpu.VMEM((C,), BF16))

    _wait(g3, 'wg3')

    def phase1(k_s, vt_s, wkx_s, wvx_s, *s_s):
        KH = DC // 2

        def w_blocks(w_s, h, cb, gate):
            out = []
            for kh in range(2):
                for b in range(2):
                    r0 = 8 * (KH * kh + 128 * cb) + 4 * b + (h // 2) % 4
                    x = w_s.reshape(2, DC * 8, 128)[h // 8, pl.ds(r0, 128, stride=8), :]
                    if isinstance(h, int):
                        out.append(_lo(x) if h % 2 == 0 else _hi(x))
                    else:
                        out.append(_hi(x << jnp.concatenate([gate] * 16, axis=0)))
            return out

        digest = _digest

        def extract_wk(h, cb, gate=None):
            terms = [t.astype(BF16) for t in _rhs_terms(*w_blocks(wk_s, h, cb, gate))]
            for i, t in enumerate(terms):
                wkx_s[i, 128 * cb:128 * (cb + 1), :] = t
            return digest(terms)

        def extract_wv(h, cb, gate=None):
            terms = [t.astype(BF16) for t in _rhs_terms(*[t.T for t in w_blocks(wv_s, h, cb, gate)])]
            for i, t in enumerate(terms):
                wvx_s[i, cb] = t
            return digest(terms)

        for cb in range(4):
            extract_wk(0, cb)
            if 'xw' not in CFG.get('sched', ''):
                extract_wv(0, cb)

        def head(h, carry):
            @pl.when(h == 1)
            def _():
                _wait(g3b, 'wg3b')

            lane8 = lax.broadcasted_iota(I32, (8, 128), 1)
            sub8 = lax.broadcasted_iota(I32, (8, 128), 0)
            lane16 = lax.broadcasted_iota(I32, (16, 128), 1)
            sub16 = lax.broadcasted_iota(I32, (16, 128), 0)
            tri = (lax.broadcasted_iota(I32, (128, 128), 0) <= lax.broadcasted_iota(I32, (128, 128), 1))
            zero = h // H
            h_next = jnp.minimum(h + 1, H - 1)
            toks = []
            due = []

            never = _never(zero)

            def after(x, tok):
                return _after(x, tok, never)

            def tied(lhs):
                return _tied(lhs, due, never)

            def tok(back):
                return toks[-back] if (back and len(toks) >= back) else None

            def chan_mm(c, gate):
                m_b = lane8 < after(128 - 2 * sub8, gate)
                gs = [jnp.broadcast_to(g_s[a, pl.ds(c, 1), :], (8, 128)) for a in range(NB)]
                bt = [pltpu.roll(jnp.where(m_b, gs[a], gs[a - 1] if a > 0 else jnp.uint32(0)), 0, 1,
                                 stride=2, stride_axis=0) for a in range(NB)]
                b1 = pltpu.bitcast(jnp.concatenate(bt[7::-1], axis=0), BF16)
                b2 = pltpu.bitcast(jnp.concatenate(bt[15:7:-1], axis=0), BF16)
                am = pltpu.bitcast(aw_s[pl.ds(c, 64, stride=PITCH), :], BF16)
                z1 = _dot(tied(am), b1)
                z2 = _dot(am[:64], b2)
                return c, z1[:64], z1[64:] + z2

            def chan_post(c, zlo, zhi):
                acc = car = None
                for p in range(8):
                    z = jnp.concatenate([zlo[8 * p:8 * p + 8], zhi[8 * p:8 * p + 8]], axis=0)
                    if p == 0:
                        acc = z
                    else:
                        z = pltpu.roll(z, 16 * p, 1)
                        cz = jnp.where(lane16 < 16 * p, z, 0.0)
                        acc = acc + z
                        car = cz if car is None else car + cz
                y = (acc - car) + jnp.where(sub16 > 0, pltpu.roll(car, 1, 0), 0.0)
                y_s[pl.ds(c, NB, stride=PITCH), :] = y
                if CFG.get('pd', 0):
                    due.append(y[:8])
                    due.append(y[8:])

            chans = [h * CPH + i for i in range(CPH)]

            def c_term(i, jp):
                if i == 2:
                    blocks = [c_s[cb, 256 * jp:256 * jp + 128, :] for cb in range(4)]
                elif i == 3:
                    blocks = [c_s[4 + cb, 256 * jp + 128:256 * jp + 256, :] for cb in range(4)]
                else:
                    n = _LHS_SUMS.index(i)
                    blocks = [cs_s[n, cb, 128 * jp:128 * (jp + 1), :] for cb in range(4)]
                return jnp.concatenate(blocks, axis=1)

            def kproj(jp):
                def emit(r, c, val):
                    if (r, c) == (1, 0):
                        toks.append(val[:8])
                    k_s[c, 256 * jp + 128 * r:256 * jp + 128 * (r + 1), :] = val.astype(BF16)

                _strassen(lambda i: _dot(tied(c_term(i, jp)), wkx_s[i]), emit)

            def vproj(jp):
                def prod(i):
                    return _dot_nt(tied(jnp.concatenate([wvx_s[i, cb] for cb in range(4)], axis=1)), c_term(i, jp))

                def emit(r, c, val):
                    if (r, c) == (1, 0):
                        toks.append(val[:8])
                    vt_s[2 * jp + r, 128 * c:128 * (c + 1), :] = val.astype(BF16)

                _strassen(prod, emit)

            def k_rows(r0, r1):
                return jnp.concatenate([k_s[0, r0:r1, :], k_s[1, r0:r1, :]], axis=1)

            def q_cols(r0, r1):
                return jnp.concatenate([qc_s[h, t] for t in range(r0 // 128, r1 // 128)], axis=1)

            mx, pr = {}, {}

            def qk(t):
                q0 = t * TQ
                if q0 > 0:
                    s_rect = _dot(tied(k_rows(0, q0)), q_cols(q0, q0 + TQ))
                    toks.append(s_rect[:8, :128])
                for u in range(TQ // 128):
                    qs = q0 + u * 128
                    sd = _dot(tied(k_rows(q0, qs + 128)), q_cols(qs, qs + 128))
                    parts = []
                    if q0 > 0:
                        parts.append(s_rect[:, u * 128:(u + 1) * 128])
                    if u > 0:
                        parts.append(sd[:u * 128, :])
                    parts.append(jnp.where(tri, sd[u * 128:, :], NEG))
                    s = jnp.concatenate(parts, axis=0) if len(parts) > 1 else parts[0]
                    s_s[t % 2][u, 0:qs + 128, :] = s
                    mx[(t, u)] = jnp.max(s, axis=0, keepdims=True)
                toks.append(sd[:8])

            def softmax(t, u, deadline):
                qs = t * TQ + u * 128
                p = jnp.exp2(s_s[t % 2][u + zero, 0:qs + 128, :] - mx.pop((t, u)))
                rl = 1.0 / jnp.sum(p, axis=0, keepdims=True)
                pr[(t, u)] = (p.astype(BF16), rl)
                if deadline:
                    due.append(rl)

            def pv(t, u):
                if (t, u) not in pr:
                    softmax(t, u, False)
                p, rl = pr.pop((t, u))
                qs = t * TQ + u * 128
                vt = jnp.concatenate([vt_s[i] for i in range(qs // 128 + 1)], axis=1)
                ctx = _dot(tied(vt), p)
                toks.append(ctx[:8])
                qc_s[h, qs // 128] = (ctx * rl).astype(BF16)

            def shift_of(hh, gate):
                return after(jnp.full((8, 128), (1 - hh % 2) * 16, I32).astype(U32), gate)

            CG, XG = CFG.get('cg', 0), CFG.get('xg', 0)
            pend = []
            for st_ in CFG['sched'].split():
                kind, arg = st_[0], st_[1:]
                if st_[:2] in ('xk', 'xv', 'xw'):
                    hh = h if st_[1] == 'w' else h_next
                    for cb in ([int(st_[2:])] if st_[2:] else range(4)):
                        due.append((extract_wk if st_[1] == 'k' else extract_wv)(hh, cb, shift_of(hh, tok(XG))))
                    continue
                if st_[0] in 'Ww':
                    e, j0, n = int(st_[1]), int(st_[2]), int(st_[3])
                    r = windows(jnp.minimum(1 + h // 4, 3), h % 4, e, range(j0, j0 + n), lambda x, t=tok(CFG.get('wg', 0)): after(x, t))
                    if st_[0] == 'W':
                        due.extend(r)
                    continue
                if st_ == 'dk':
                    due.append(pltpu.bitcast(wkx_s[zero, 0:16, :], F32))
                    continue
                if kind == 'E':
                    softmax(int(arg[0]), int(arg[1]), True)
                    continue
                old = list(pend)
                pend.clear()
                if kind == 'C':
                    for _ in range(int(arg)):
                        pend.append(chan_mm(chans.pop(0), tok(CG)))
                elif kind == 'K':
                    kproj(int(arg))
                elif kind == 'V':
                    vproj(int(arg))
                elif kind == 'Q':
                    qk(int(arg))
                elif kind == 'P':
                    for u in ([int(arg[1])] if len(arg) > 1 else range(TQ // 128)):
                        pv(int(arg[0]), u)
                for args in old:
                    chan_post(*args)
            assert not chans and not pend and (not due or CFG.get('pd')) and not pr and not mx
            return carry + zero

        if CFG.get('p1', 1):
            return lax.fori_loop(0, H, head, 0)
        else:
            _wait(g3b, 'wg3b')

            def keep(h, carry):
                r = pl.multiple_of(h * 16, 16)
                t = (qc_s[h, h, 0:16, :].astype(F32) + cs_s[h % 5, h % 4, pl.ds(r, 16), :].astype(F32)
                     + pltpu.bitcast(aw_s[pl.ds(r, 16), :] + g_s[h, pl.ds(r, 16), :], F32)
                     + wkx_s[h % 7, pl.ds(r, 16), :].astype(F32) + wvx_s[h % 7, h % 4, 0:16, :].astype(F32))
                y_s[pl.ds(r, 16), :] = t
                return carry + h // H
            return lax.fori_loop(0, H, keep, 0)

    zero_end = pl.run_scoped(phase1, pltpu.VMEM((2, S, 128), BF16), pltpu.VMEM((NB, D, 128), BF16),
                  pltpu.VMEM((7, DC // 2, 128), BF16), pltpu.VMEM((7, 4, 128, 128), BF16),
                  pltpu.VMEM((TQ // 128, S, 128), F32), pltpu.VMEM((TQ // 128, S, 128), F32))

    def phase2(out_s):
        _wait(g4, 'wg4')
        HH = H // 2

        def wo_block(rh, kh):
            return jnp.concatenate(
                [wot_s[b, C * h + CH * rh:C * h + CH * (rh + 1), :]
                 for h in range(HH * kh, HH * (kh + 1)) for b in range(2)], axis=1)

        raw = [wo_block(0, 0), wo_block(1, 0), wo_block(0, 1), wo_block(1, 1)]
        wt = [t.astype(BF16) for t in _rhs_terms(*[t.astype(F32) for t in raw])]
        wt[1], wt[4] = raw[0], raw[3]
        outs = []
        due, late = [], []
        DL = CFG.get('dl', 3)
        never = _never(zero_end)

        def put(t, b, z, opaque=False):
            o = z.T.astype(BF16)
            r0 = pl.multiple_of(zero_end * 16 + 128 * t, 16) if opaque else 128 * t
            out_s[pl.ds(r0, 128), 128 * b:128 * (b + 1)] = o
            late.append(pltpu.bitcast(o[112:], U32))

        for jp in range(NP if CFG.get('p2', 1) else 0):
            def ctx_block(r, kh):
                return jnp.concatenate([qc_s[h, 2 * jp + r] for h in range(HH * kh, HH * (kh + 1))], axis=0)

            craw = [ctx_block(0, 0), ctx_block(0, 1), ctx_block(1, 0), ctx_block(1, 1)]
            ct = [t.astype(BF16) for t in _lhs_terms(*[t.astype(F32) for t in craw])]
            ct[2], ct[3] = craw[0], craw[3]
            za = {}
            prev_late = list(late)
            late.clear()
            for r in range(2):
                t = 2 * jp + r
                za[r] = y_s[t * PITCH:t * PITCH + C, :] * qa_s[:, 128 * t:128 * (t + 1)].astype(F32)
                for b in range(3):
                    put(t, b, za[r][128 * b:128 * (b + 1)], opaque=(r == 0 and b == 0 and jp > 0))
            a_late = list(late)
            late.clear()
            res = {}
            count = [0]

            def prod(i):
                if count[0] == DL:
                    due.extend(prev_late)
                if count[0] == 6:
                    due.extend(a_late)
                count[0] += 1
                return _dot(_tied(wt[i], due, never), ct[i])

            _strassen(prod, lambda r, c, val: res.__setitem__((r, c), val), order=(1, 4, 3, 2, 0, 5, 6))
            for r in (1, 0):
                z = jnp.concatenate([za[r][384:], res[(r, 0)], res[(r, 1)]], axis=0)
                for b in (3, 2, 1, 0):
                    put(2 * jp + r, 3 + b, z[128 * b:128 * (b + 1)])
            rows = pl.ds(256 * jp, 256)
            oc = cp(out_s.at[rows], o_hbm.at[rows], 26 + jp)
            oc.start()
            outs.append(oc)
        if not CFG.get('p2', 1):
            def keep(h, carry):
                r = pl.multiple_of(h * 16, 16)
                out_s[pl.ds(r, 16), 0:128] = y_s[pl.ds(r, 16), :].astype(BF16) + qc_s[h, h, 0:16, :]
                return carry
            lax.fori_loop(0, H, keep, 0)
            oc = cp(out_s.at[pl.ds(0, 256)], o_hbm.at[pl.ds(0, 256)], 26)
            oc.start()
            outs.append(oc)
        _wait(outs, 'wout')

    pl.run_scoped(phase2, pltpu.VMEM((S, 2 * C), BF16))


def _tiles(w):
    rows = w.shape[0]
    return w.reshape(rows, 2, 8, 2, 128).transpose(0, 1, 3, 2, 4).reshape(rows, 2, 16, 128)


@jax.jit
def pallas_concat_heads__ssm_conv_h3__compressed_kv_cla__prompt_kernel(
    A_q: jax.Array,
    A_k: jax.Array,
    A_v: jax.Array,
    A_shift_k: jax.Array,
    A_ssm_k: jax.Array,
    A_ssm_D: jax.Array,
    B_x: jax.Array,
    B_c_kv: jax.Array,
    B_w_q: jax.Array,
    B_w_uk: jax.Array,
    B_w_uv: jax.Array,
    B_w_o: jax.Array,
):
    hbm = pl.BlockSpec(memory_space=pltpu.HBM)
    out = pl.pallas_call(
        _kernel,
        in_specs=[hbm] * 12,
        out_specs=hbm,
        out_shape=jax.ShapeDtypeStruct((S, 2 * C), BF16),
        scratch_shapes=[
            pltpu.VMEM((8, S, 128), BF16),
            pltpu.VMEM((5, 4, S // 2, 128), BF16),
            pltpu.VMEM((2, DC, 8, 128), U32),
            pltpu.VMEM((2, DC, 8, 128), U32),
            pltpu.VMEM((C, S), BF16),
            pltpu.VMEM((H, NB, D, 128), BF16),
            pltpu.VMEM((64 * PITCH, 128), U32),
            pltpu.VMEM((NB, C, 128), U32),
            pltpu.VMEM((NB * PITCH, 128), F32),
            pltpu.VMEM((2, H * C, 128), BF16),
            pltpu.VMEM((4, S, 128), U32),
            pltpu.VMEM((C, S), BF16),
            pltpu.VMEM((512, 128), F32),
            pltpu.SemaphoreType.DMA((35,)),
        ],
        compiler_params=pltpu.CompilerParams(vmem_limit_bytes=120 * 2 ** 20),
    )(
        A_q[0].T, A_k[0].T, A_v[0].T, A_shift_k.T, A_ssm_k, A_ssm_D, B_x[0].T, B_c_kv[0],
        _tiles(B_w_q), _tiles(B_w_uk), _tiles(B_w_uv),
        jnp.swapaxes(B_w_o, 1, 2).reshape(H * C, D),
    )
    return out.reshape(1, S, 2 * C)
```

```python
import math

import jax
import jax.numpy as jnp
from jax import lax
import jax.experimental.pallas as pl
import jax.experimental.pallas.tpu as pltpu

F32 = jnp.float32
BF16 = jnp.bfloat16
U32 = jnp.uint32
I32 = jnp.int32

S = 2048
C = 448
H = 16
D = 256
DC = 1024
NB = S // 128
NP = NB // 2
CH = C // 2
PITCH = 520
CPH = C // H
TQ = 512
NT = (((1,), (1,)), ((), ()))
LOG2E = math.log2(math.e)
QSCALE = (D ** -0.5) * LOG2E
NEG = -1e9 * LOG2E
HI_MASK = 0xFFFF0000
CFG = dict(clob=0,gback=8,nf=5,defer=0,ux=8,costs=(2,2,1),slack=8,cg=3,sched='K0 C2 K1 C2 Q0 K2 C2 xw0 K3 C2 E00 E01 E02 E03 Q1 K4 C2 xw1 K5 C2 E10 E11 Q2 E12 E13 K6 C2 xw2 K7 C2 E20 Q3 xw3 V0 C2 E21 V1 C2 E22 P0 V2 C2 E23 V3 C2 E30 P1 V4 C2 E31 V5 C2 E32 P20 xk0 P21 P22 xk1 P23 V6 E33 V7 P30 xk2 P31 P32 xk3 P33')


def _wait(copies, name):
    if CFG.get('scopes'):
        with jax.named_scope(name):
            for c_ in copies:
                c_.wait()
    else:
        for c_ in copies:
            c_.wait()


def _dot(a, b):
    return jnp.dot(a, b, preferred_element_type=F32)


def _dot_nt(a, b):
    return lax.dot_general(a, b, NT, preferred_element_type=F32)


def _lo(x):
    return pltpu.bitcast(x << 16, F32)


def _hi(x):
    return pltpu.bitcast(x & jnp.uint32(HI_MASK), F32)


def _head_cols(w_s, h, rows):
    out = []
    for b in range(2):
        x = w_s[b, pl.ds(h // 2, rows, stride=8), :]
        if isinstance(h, int):
            out.append(_lo(x) if h % 2 == 0 else _hi(x))
        else:
            out.append(_hi(x << ((1 - h % 2) * 16).astype(U32)))
    return out


def _lhs_terms(a11, a12, a21, a22):
    return [a11 + a22, a21 + a22, a11, a22, a11 + a12, a21 - a11, a12 - a22]


def _rhs_terms(b11, b12, b21, b22):
    return [b11 + b22, b11, b12 - b22, b21 - b11, b22, b11 + b12, b21 + b22]


_LHS_SUMS = (0, 1, 4, 5, 6)


def _strassen(prod, emit, order=(0, 1, 3, 2, 4, 5, 6)):
    uses = {(0, 0): {0: 1, 3: 1, 4: -1, 6: 1}, (0, 1): {2: 1, 4: 1},
            (1, 0): {1: 1, 3: 1}, (1, 1): {0: 1, 1: -1, 2: 1, 5: 1}}
    acc = {}
    neg = {}
    for i in order:
        m = prod(i)
        for key, terms in uses.items():
            if i not in terms:
                continue
            sign = terms.pop(i)
            if key not in acc:
                acc[key] = m
                neg[key] = sign < 0
            elif neg[key]:
                acc[key] = m - acc[key]
                neg[key] = False
            else:
                acc[key] = acc[key] + m if sign > 0 else acc[key] - m
            if not terms:
                emit(key[0], key[1], acc.pop(key))


def _mult(i, n):
    return i if isinstance(i, int) else pl.multiple_of(i, n)


def _never(zero):
    return lax.broadcasted_iota(I32, (8, 128), 1) < zero


def _after(x, tok, never):
    if tok is None:
        return x
    return jnp.where(never, pltpu.bitcast(tok, x.dtype), x)


def _tied(lhs, due, never):
    if not due:
        return lhs
    t = None
    for d in due:
        d = pltpu.bitcast(jnp.broadcast_to(d, (8, 128)), U32)
        t = d if t is None else t ^ d
    due.clear()
    x = pltpu.bitcast(_after(pltpu.bitcast(lhs[:16, :128], U32), t, never), BF16)
    if lhs.shape[1] > 128:
        x = jnp.concatenate([x, lhs[:16, 128:]], axis=1)
    return jnp.concatenate([x, lhs[16:]], axis=0) if lhs.shape[0] > 16 else x


def _digest(vals):
    acc = None
    words = [v if v.dtype == U32 else pltpu.bitcast(v, U32) for v in vals]
    for r in range(words[0].shape[0] // 8):
        for w in words:
            w = w[8 * r:8 * (r + 1)]
            acc = w if acc is None else acc ^ w
    return acc


def _kernel(qa_hbm, ka_hbm, va_hbm, sk_hbm, hk_hbm, d_hbm, x_hbm, c_hbm, wq_hbm, wk_hbm, wv_hbm, wo_hbm,
            o_hbm,
            c_s, cs_s, wk_s, wv_s, qa_s, qc_s, aw_s, g_s, y_s, wot_s, wd_s, hk_s, dc_s, k_s, vt_s, wkx_s, wvx_s, sa_s, sb_s, x_s, xs_s, wq_s, ka_s, va_s, wc_s, out_s, sk_ref, d_ref, sems):
    def cp(src, dst, i):
        return pltpu.make_async_copy(src, dst, sems.at[i])

    wq32 = wq_hbm.bitcast(U32)
    wk32 = wk_hbm.bitcast(U32)
    wv32 = wv_hbm.bitcast(U32)
    gc = [cp(c_hbm.at[:, pl.ds(128 * b, 128)], c_s.at[b], 8 + b) for b in range(8)]
    g3 = [cp(wk32.at[:, 0], wk_s.at[0], 16), cp(wv32.at[:, 0], wv_s.at[0], 17)]
    g3b = [cp(wk32.at[:, 1], wk_s.at[1], 18), cp(wv32.at[:, 1], wv_s.at[1], 19)]
    g4 = [cp(qa_hbm, qa_s, 21)] + [cp(wo_hbm.at[:, pl.ds(128 * b, 128)], wot_s.at[b], 6 + b) for b in range(2)]

    def delayed(ref, rows, sg, n, gate=None):
        cur = pltpu.bitcast(ref[rows, 128 * sg:128 * (sg + 1)], U32)
        lane = lax.broadcasted_iota(I32, (8, 128), 1)
        if gate is not None:
            lane = gate(lane)
        lane = jnp.concatenate([lane] * (cur.shape[0] // 8), axis=0)
        prev = pltpu.bitcast(ref[rows, 128 * (sg - 1):128 * sg], U32) if sg > 0 else jnp.uint32(0)
        x = pltpu.roll(jnp.where(lane < 128 - n, cur, prev), n, 1)
        return pltpu.bitcast(x, BF16).astype(F32)

    def gated_t(x, gate):
        if gate is not None:
            x = jnp.concatenate([gate(x[:8]), x[8:]], axis=0)
        return x.T

    def windows(b, q, e, js, gate=None):
        out = []
        for j in js:
            parts = []
            for sg in range(2 * j - 6, 2 * j + 2):
                if sg < 0:
                    parts.append(jnp.zeros((16, 128), U32))
                else:
                    parts.append(wd_s[b, pl.ds(_mult(128 * sg + 32 * q + 16 * e, 16), 16), :])
            plane = 32 * (j // 4) + 8 * q + 4 * e + j % 4
            win = gated_t(jnp.concatenate(parts, axis=0), gate)
            aw_s[pl.ds(_mult(plane * PITCH + 128 * b, 8), 128), :] = win
            out.append(win[120:])
        return out

    def prep_g(r0, n, gate=None):
        rows = pl.ds(_mult(r0, 16), n)
        lane = lax.broadcasted_iota(I32, (n, 128), 1)
        for a in range(NB):
            hf = hk_s[rows, 128 * a:128 * (a + 1)].astype(F32)
            hs = delayed(hk_s, rows, a, 1, gate)
            if a == 0:
                hf = jnp.where(lane == 0, hf + dc_s[rows, :], hf)
                hs = jnp.where(lane == 1, hs + dc_s[rows, :], hs)
            wrd = pltpu.pack_elementwise([hf, hs], packed_dtype=BF16).astype(U32)
            g_s[a, rows, :] = wrd
            yield _digest([wrd])

    def phase0(x_s, xs_s, wq_s, ka_s, va_s, wc_s, sk_ref, d_ref):
        XC = 512
        cq = [cp(wq32.at[:, g], wq_s.at[g], g) for g in range(2)]
        cx = [cp(x_hbm.at[:, pl.ds(XC * i, XC)], x_s.at[:, pl.ds(XC * i, XC)], 22 + i) for i in range(S // XC)]
        g2 = [cp(sk_hbm, sk_ref, 2), cp(d_hbm, d_ref, 20),
              cp(ka_hbm, ka_s, 3), cp(va_hbm, va_s, 4), cp(hk_hbm, hk_s, 5)]
        order = CFG.get('order', 'A')
        if order == 'A':
            ga, gb = g2, [cq[1]] + gc
        else:
            ga, gb = gc, g2 + [cq[1]]
        rest = cx[1:] + ga + gb + g3 + g3b + g4
        for c_ in [cx[0], cq[0]] + ([] if CFG.get('defer') else rest):
            c_.start()
        zero = pl.semaphore_read(sems.at[34])
        never = _never(zero)
        due = []
        toks = []

        def pad_rows(t):
            return jnp.concatenate([t, jnp.zeros((256 - CH, 128), t.dtype)], axis=0)

        def wq_terms(j, b, gate):
            x = wq_s.reshape(2, C * 8, 128)[j // 4, pl.ds(4 * b + j % 4, C, stride=8), :]
            g16 = jnp.concatenate([_after(jnp.full((8, 128), 16, U32), gate, never)] * (C // 8), axis=0)
            gm = jnp.concatenate([_after(jnp.full((8, 128), HI_MASK, U32), gate, never)] * (C // 8), axis=0)
            lo, hi = pltpu.bitcast(x << g16, F32), pltpu.bitcast(x & gm, F32)
            blocks = [pad_rows(t).T for t in (lo[:CH], hi[:CH], lo[CH:], hi[CH:])]
            return [t.astype(BF16) for t in _rhs_terms(*blocks)]

        def x_terms(jp):
            top = slice(256 * jp, 256 * jp + 128)
            bot = slice(256 * jp + 128, 256 * jp + 256)
            for i in range(7):
                xs_s[i, jp, CH:, :] = jnp.zeros((256 - CH, 128), BF16)
            for r in range(0, CH, 32):
                lo, hi = slice(r, r + 32), slice(CH + r, CH + r + 32)
                blocks = [x_s[lo, top], x_s[hi, top], x_s[lo, bot], x_s[hi, bot]]
                terms = [t.astype(BF16) for t in _lhs_terms(*[t.astype(F32) for t in blocks])]
                terms[2], terms[3] = blocks[0], blocks[3]
                for i, t in enumerate(terms):
                    xs_s[i, jp, lo, :] = t
                yield 1, _digest(terms)

        def qproj(g, jp, waits):
            j, b = groups[g]
            for c_ in waits:
                c_.wait()
            if False:
                x_terms(jp)
                x_terms(jp + 1)

            def prod(i):
                pump()
                m = _dot(_tied(wts[g][i], due, never), xs_s[i, jp])
                toks.append(m[:8])
                return m

            def emit(r, c, val):
                qc_s[2 * j + c, 2 * jp + r, 128 * b:128 * (b + 1), :] = (val * QSCALE).astype(BF16)

            _strassen(prod, emit)

        def column(row):
            row = jnp.concatenate([row.astype(F32), jnp.zeros((1, 512 - C), F32)], axis=1)
            return jnp.broadcast_to(row, (128, 512)).T

        consts = {}

        def make_consts():
            consts['taps'] = [column(sk_ref[j:j + 1, :]) for j in range(4)]
            dc_s[...] = column(d_ref[...].reshape(1, C))

        def gate(x):
            back = CFG.get('gback', 6)
            return _after(x, toks[-back], never) if back else x

        def prep_u(r0, n):
            rows = slice(r0, r0 + n)
            tp = [t[rows] for t in consts['taps']]
            prev = jnp.zeros((n, 128), F32)
            for sg in range(NB):
                cols = slice(128 * sg, 128 * (sg + 1))
                ksh = ((delayed(ka_s, rows, sg, 3, gate) * tp[3] + delayed(ka_s, rows, sg, 2, gate) * tp[2])
                       + (delayed(ka_s, rows, sg, 1, gate) * tp[1] + ka_s[rows, cols].astype(F32) * tp[0]))
                kv = ksh * va_s[rows, cols].astype(F32)
                wrd = pltpu.pack_elementwise([prev, kv], packed_dtype=BF16).astype(U32)
                wc_s[sg, rows, :] = wrd
                prev = kv
                yield _digest([wrd])

        def words_t(b):
            for sg in range(NB):
                if b < 3:
                    wrd = wc_s[sg, 128 * b:128 * (b + 1), :]
                else:
                    wrd = jnp.concatenate([wc_s[sg, 384:C, :], jnp.zeros((512 - C, 128), U32)], axis=0)
                wrd = gated_t(wrd, gate)
                wd_s[b, 128 * sg:128 * (sg + 1), :] = wrd
                yield wrd[120:]

        def all_windows(b):
            for p in range(8):
                for j in range(8):
                    yield windows(b, p // 2, p % 2, [j], gate)[0]

        def c_terms():
            RG = CFG.get('rg', 32)
            for jp in range(NP):
                for cb in range(4):
                    for r in range(0, 128, RG):
                        top = slice(256 * jp + r, 256 * jp + r + RG)
                        bot = slice(256 * jp + 128 + r, 256 * jp + 128 + r + RG)
                        blocks = [c_s[cb, top, :], c_s[4 + cb, top, :], c_s[cb, bot, :], c_s[4 + cb, bot, :]]
                        terms = _lhs_terms(*[t.astype(F32) for t in blocks])
                        terms = [terms[i].astype(BF16) for i in _LHS_SUMS]
                        for n, t in enumerate(terms):
                            cs_s[n, cb, 128 * jp + r:128 * jp + r + RG, :] = t
                        yield _digest(terms)

        UG = CFG.get('ug', 32)

        def a_stream():
            make_consts()
            cu, ct, cg = CFG.get('costs', (3, 2, 1))
            gs = [prep_g(r0, 32, gate) for r0 in range(0, C, 32)]
            for b in range(4):
                for r0 in range(128 * b, min(C, 128 * (b + 1)), UG):
                    for v in prep_u(r0, UG):
                        yield cu * UG // 32, v
                for v in words_t(b):
                    yield ct, v
                for v in all_windows(b):
                    yield ct, v
                if CFG.get('gpos', 'end') == 'blk' or b == 3:
                    for g_ in (gs[4 * b:4 * b + 4] if CFG.get('gpos', 'end') == 'blk' else gs):
                        for v in g_:
                            yield cg, v

        cu, ct, cg = CFG.get('costs', (3, 2, 1))
        a_total = cu * 14 * NB + ct * 4 * (NB + 64) + cg * 14 * NB
        streams = []
        nprod = [0]
        later = {}
        LAG = CFG.get('lag', 0)

        def pump():
            for st_ in streams:
                gen, n, p0, p1, done = st_
                want = min(n, max(0, (nprod[0] - p0 + 1) * n // (p1 - p0)))
                while st_[4] < want:
                    cost, v = next(gen)
                    later.setdefault(nprod[0] + LAG, []).append(v)
                    st_[4] += cost
            due.extend(later.pop(nprod[0], []))
            nprod[0] += 1

        groups = [(j, b) for j in range(H // 2) for b in range(2)]
        NF = CFG.get('nf', 3)
        units = [(g, jp) for c in range(0, NP, 2) for g in range(NF) for jp in (c, c + 1)]
        units += [(g, jp) for g in range(NF, len(groups)) for jp in range(NP)]
        NU = len(units)
        wts = {}
        lead = CFG.get('lead', 4)
        ua = CFG.get('ua', 32)
        ub = 8 * NP - lead
        ux = CFG.get('ux', 5)
        waits = {ux: cx[1:], ua: ga, ub: gb}
        xe = [7 * ux + 2] + [7 * NF * 2 * c - 1 for c in (1, 2, 3)]
        for c in range(3):
            streams.append([(v for jp in (2 * c + 2, 2 * c + 3) for v in x_terms(jp)), 14, xe[c], xe[c + 1], 0])
        sl = CFG.get('slack', 4)
        PA, PB, PE = 7 * ua + sl, 7 * ub + sl, 7 * NU - 2 - LAG
        c_stream = ((1, v) for v in c_terms())
        nc = NP * 4 * 128 // CFG.get('rg', 32)
        if order == 'A':
            streams.append([a_stream(), a_total, PA, PE, 0])
            streams.append([c_stream, nc, PB, PE, 0])
        else:
            streams.append([c_stream, nc, PA, CFG.get('cend', PB), 0])
            streams.append([a_stream(), a_total, PB, PE, 0])

        if not CFG.get('p0', 1):
            for c_ in cq + cx + g2 + gc:
                c_.wait()
            return
        _wait([cx[0]], 'wx0')
        list(x_terms(0))
        list(x_terms(1))
        _wait([cq[0]], 'wq0')
        if CFG.get('defer'):
            @pl.when(zero == 0)
            def _():
                for c_ in rest:
                    c_.start()

        first_use = {}
        for u, (g, jp) in enumerate(units):
            first_use.setdefault(g, u)
        for u, (g, jp) in enumerate(units):
            if u in waits:
                _wait(waits[u], 'wu%d' % u)
            for g_, fu in first_use.items():
                if g_ not in wts and fu - (lead if g_ >= NF else 1) <= u:
                    back = CFG.get('wback', 8)
                    wts[g_] = wq_terms(*groups[g_], toks[-back] if len(toks) >= back else None)
            qproj(g, jp, [])
        assert all(st_[4] == st_[1] for st_ in streams) and not later, streams

    phase0(x_s, xs_s, wq_s, ka_s, va_s, wc_s, sk_ref, d_ref)

    _wait(g3, 'wg3')

    def phase1(k_s, vt_s, wkx_s, wvx_s, *s_s):
        KH = DC // 2

        def w_blocks(w_s, h, cb, gate):
            out = []
            for kh in range(2):
                for b in range(2):
                    r0 = 8 * (KH * kh + 128 * cb) + 4 * b + (h // 2) % 4
                    x = w_s.reshape(2, DC * 8, 128)[h // 8, pl.ds(r0, 128, stride=8), :]
                    if isinstance(h, int):
                        out.append(_lo(x) if h % 2 == 0 else _hi(x))
                    elif isinstance(gate, int):
                        out.append(_lo(x) if gate == 0 else _hi(x))
                    else:
                        out.append(_hi(x << jnp.concatenate([gate] * 16, axis=0)))
            return out

        digest = _digest

        def extract_wk(h, cb, gate=None):
            terms = [t.astype(BF16) for t in _rhs_terms(*w_blocks(wk_s, h, cb, gate))]
            for i, t in enumerate(terms):
                wkx_s[i, 128 * cb:128 * (cb + 1), :] = t
            return digest(terms)

        def extract_wv(h, cb, gate=None):
            terms = [t.astype(BF16) for t in _rhs_terms(*[t.T for t in w_blocks(wv_s, h, cb, gate)])]
            for i, t in enumerate(terms):
                wvx_s[i, cb] = t
            return digest(terms)

        for cb in range(4):
            extract_wk(0, cb)
            if 'xw' not in CFG.get('sched', ''):
                extract_wv(0, cb)

        UN = CFG.get('unroll', 1)

        def heads(it, carry):
            @pl.when(it == 1)
            def _():
                _wait(g3b, 'wg3b')

            zero = it // H
            toks = []
            due = []
            for r in range(UN):
                head(it * UN + r, None if UN % 2 else r % 2, zero, toks, due)
            return carry + zero

        def head(h, par, zero, toks, due):
            lane8 = lax.broadcasted_iota(I32, (8, 128), 1)
            sub8 = lax.broadcasted_iota(I32, (8, 128), 0)
            lane16 = lax.broadcasted_iota(I32, (16, 128), 1)
            sub16 = lax.broadcasted_iota(I32, (16, 128), 0)
            tri = (lax.broadcasted_iota(I32, (128, 128), 0) <= lax.broadcasted_iota(I32, (128, 128), 1))
            h_next = h + 1 if isinstance(h, int) else jnp.minimum(h + 1, H - 1)
            never = _never(zero)

            def after(x, tok):
                return _after(x, tok, never)

            def tied(lhs):
                return _tied(lhs, due, never)

            def tok(back):
                return toks[-back] if (back and len(toks) >= back) else None

            def chan_mm(c, gate):
                m_b = lane8 < after(128 - 2 * sub8, gate)
                gs = [jnp.broadcast_to(g_s[a, pl.ds(c, 1), :], (8, 128)) for a in range(NB)]
                bt = [pltpu.roll(jnp.where(m_b, gs[a], gs[a - 1] if a > 0 else jnp.uint32(0)), 0, 1,
                                 stride=2, stride_axis=0) for a in range(NB)]
                b1 = pltpu.bitcast(jnp.concatenate(bt[7::-1], axis=0), BF16)
                b2 = pltpu.bitcast(jnp.concatenate(bt[15:7:-1], axis=0), BF16)
                am = pltpu.bitcast(aw_s[pl.ds(c, 64, stride=PITCH), :], BF16)
                z1 = _dot(tied(am), b1)
                z2 = _dot(am[:64], b2)
                return c, z1[:64], z1[64:] + z2

            def chan_post(c, zlo, zhi):
                acc = car = None
                for p in range(8):
                    z = jnp.concatenate([zlo[8 * p:8 * p + 8], zhi[8 * p:8 * p + 8]], axis=0)
                    if p == 0:
                        acc = z
                    else:
                        z = pltpu.roll(z, 16 * p, 1)
                        cz = jnp.where(lane16 < 16 * p, z, 0.0)
                        acc = acc + z
                        car = cz if car is None else car + cz
                y = (acc - car) + jnp.where(sub16 > 0, pltpu.roll(car, 1, 0), 0.0)
                y_s[pl.ds(c, NB, stride=PITCH), :] = y
                if CFG.get('pd', 0):
                    due.append(y[:8])
                    due.append(y[8:])

            chans = [h * CPH + i for i in range(CPH)]

            def c_term(i, jp):
                if i == 2:
                    blocks = [c_s[cb, 256 * jp:256 * jp + 128, :] for cb in range(4)]
                elif i == 3:
                    blocks = [c_s[4 + cb, 256 * jp + 128:256 * jp + 256, :] for cb in range(4)]
                else:
                    n = _LHS_SUMS.index(i)
                    blocks = [cs_s[n, cb, 128 * jp:128 * (jp + 1), :] for cb in range(4)]
                return jnp.concatenate(blocks, axis=1)

            def kproj(jp):
                def emit(r, c, val):
                    if (r, c) == (1, 0):
                        toks.append(val[:8])
                    k_s[c, 256 * jp + 128 * r:256 * jp + 128 * (r + 1), :] = val.astype(BF16)

                _strassen(lambda i: _dot(tied(c_term(i, jp)), wkx_s[i]), emit)

            def vproj(jp):
                def prod(i):
                    return _dot_nt(tied(jnp.concatenate([wvx_s[i, cb] for cb in range(4)], axis=1)), c_term(i, jp))

                def emit(r, c, val):
                    if (r, c) == (1, 0):
                        toks.append(val[:8])
                    vt_s[2 * jp + r, 128 * c:128 * (c + 1), :] = val.astype(BF16)

                _strassen(prod, emit)

            def k_rows(r0, r1):
                return jnp.concatenate([k_s[0, r0:r1, :], k_s[1, r0:r1, :]], axis=1)

            def q_cols(r0, r1):
                return jnp.concatenate([qc_s[h, t] for t in range(r0 // 128, r1 // 128)], axis=1)

            mx, pr = {}, {}

            def qk(t):
                q0 = t * TQ
                if q0 > 0:
                    s_rect = _dot(tied(k_rows(0, q0)), q_cols(q0, q0 + TQ))
                    toks.append(s_rect[:8, :128])
                for u in range(TQ // 128):
                    qs = q0 + u * 128
                    sd = _dot(tied(k_rows(q0, qs + 128)), q_cols(qs, qs + 128))
                    parts = []
                    if q0 > 0:
                        parts.append(s_rect[:, u * 128:(u + 1) * 128])
                    if u > 0:
                        parts.append(sd[:u * 128, :])
                    parts.append(jnp.where(tri, sd[u * 128:, :], NEG))
                    s = jnp.concatenate(parts, axis=0) if len(parts) > 1 else parts[0]
                    s_s[t % 2][u, 0:qs + 128, :] = s
                    mx[(t, u)] = jnp.max(s, axis=0, keepdims=True)
                toks.append(sd[:8])
                if CFG.get('clob', 1):
                    s_s[t % 2][zero, S:S + 8, :] = sd[:8]

            def softmax(t, u, deadline):
                qs = t * TQ + u * 128
                p = jnp.exp2(s_s[t % 2][u if CFG.get('clob', 1) else u + zero, 0:qs + 128, :] - mx.pop((t, u)))
                rl = 1.0 / jnp.sum(p, axis=0, keepdims=True)
                pr[(t, u)] = (p.astype(BF16), rl)
                if deadline:
                    due.append(rl)

            def pv(t, u):
                if (t, u) not in pr:
                    softmax(t, u, False)
                p, rl = pr.pop((t, u))
                qs = t * TQ + u * 128
                vt = jnp.concatenate([vt_s[i] for i in range(qs // 128 + 1)], axis=1)
                ctx = _dot(tied(vt), p)
                toks.append(ctx[:8])
                qc_s[h, qs // 128] = (ctx * rl).astype(BF16)

            def shift_of(hh, gate):
                return after(jnp.full((8, 128), (1 - hh % 2) * 16, I32).astype(U32), gate)

            CG, XG = CFG.get('cg', 0), CFG.get('xg', 0)
            pend = []
            def run_step(st_):
                kind, arg = st_[0], st_[1:]
                if st_[:2] in ('xk', 'xv', 'xw'):
                    hh = h if st_[1] == 'w' else h_next
                    if isinstance(hh, int) and hh == H:
                        return
                    for cb in ([int(st_[2:])] if st_[2:] else range(4)):
                        due.append((extract_wk if st_[1] == 'k' else extract_wv)(
                            hh, cb, shift_of(hh, tok(XG)) if par is None else (par + (st_[1] != 'w')) % 2))
                    return
                if st_[0] in 'Ww':
                    e, j0, n = int(st_[1]), int(st_[2]), int(st_[3])
                    r = windows(jnp.minimum(1 + h // 4, 3), h % 4, e, range(j0, j0 + n), lambda x, t=tok(CFG.get('wg', 0)): after(x, t))
                    if st_[0] == 'W':
                        due.extend(r)
                    return
                if st_ == 'dk':
                    due.append(pltpu.bitcast(wkx_s[zero, 0:16, :], F32))
                    return
                if kind == 'E':
                    softmax(int(arg[0]), int(arg[1]), True)
                    return
                old = list(pend)
                pend.clear()
                if kind == 'C':
                    for _ in range(int(arg)):
                        pend.append(chan_mm(chans.pop(0), tok(CG)))
                elif kind == 'K':
                    kproj(int(arg))
                elif kind == 'V':
                    vproj(int(arg))
                elif kind == 'Q':
                    qk(int(arg))
                elif kind == 'P':
                    for u in ([int(arg[1])] if len(arg) > 1 else range(TQ // 128)):
                        pv(int(arg[0]), u)
                for args in old:
                    chan_post(*args)

            for seg in [g for g in CFG['sched'].split('|') if g.strip()]:
                if CFG.get('scopes') and '|' in CFG['sched']:
                    with jax.named_scope('s_' + seg.split()[0]):
                        for st_ in seg.split():
                            run_step(st_)
                else:
                    for st_ in seg.split():
                        run_step(st_)
            assert CFG.get('noassert') or not chans and not pend and (not due or CFG.get('pd')) and not pr and not mx

        if CFG.get('flat'):
            zero = pl.semaphore_read(sems.at[34])
            FB = CFG['flat']
            for h0 in range(0, CFG.get('nheads', H), FB):
                if h0 == FB:
                    _wait(g3b, 'wg3b')

                @pl.when(zero == 0)
                def _():
                    toks, due = [], []
                    for h in range(h0, h0 + FB):
                        head(h, h % 2, zero, toks, due)
            return zero
        if CFG.get('p1', 1):
            return lax.fori_loop(0, H // UN, heads, 0)
        else:
            _wait(g3b, 'wg3b')

            def keep(h, carry):
                r = pl.multiple_of(h * 16, 16)
                t = (qc_s[h, h, 0:16, :].astype(F32) + cs_s[h % 5, h % 4, pl.ds(r, 16), :].astype(F32)
                     + pltpu.bitcast(aw_s[pl.ds(r, 16), :] + g_s[h, pl.ds(r, 16), :], F32)
                     + wkx_s[h % 7, pl.ds(r, 16), :].astype(F32) + wvx_s[h % 7, h % 4, 0:16, :].astype(F32))
                y_s[pl.ds(r, 16), :] = t
                return carry + h // H
            return lax.fori_loop(0, H, keep, 0)

    zero_end = phase1(k_s, vt_s, wkx_s, wvx_s, sa_s, sb_s)

    def phase2(out_s):
        _wait(g4, 'wg4')
        HH = H // 2

        def wo_block(rh, kh):
            return jnp.concatenate(
                [wot_s[b, C * h + CH * rh:C * h + CH * (rh + 1), :]
                 for h in range(HH * kh, HH * (kh + 1)) for b in range(2)], axis=1)

        raw = [wo_block(0, 0), wo_block(1, 0), wo_block(0, 1), wo_block(1, 1)]
        wt = [t.astype(BF16) for t in _rhs_terms(*[t.astype(F32) for t in raw])]
        wt[1], wt[4] = raw[0], raw[3]
        outs = []
        due, late = [], []
        DL = CFG.get('dl', 3)
        never = _never(zero_end)

        def put(t, b, z, opaque=False):
            o = z.T.astype(BF16)
            r0 = pl.multiple_of(zero_end * 16 + 128 * t, 16) if opaque else 128 * t
            out_s[pl.ds(r0, 128), 128 * b:128 * (b + 1)] = o
            late.append(pltpu.bitcast(o[112:], U32))

        for jp in range(CFG.get('np2', NP) if CFG.get('p2', 1) else 0):
            def ctx_block(r, kh):
                return jnp.concatenate([qc_s[h, 2 * jp + r] for h in range(HH * kh, HH * (kh + 1))], axis=0)

            craw = [ctx_block(0, 0), ctx_block(0, 1), ctx_block(1, 0), ctx_block(1, 1)]
            ct = [t.astype(BF16) for t in _lhs_terms(*[t.astype(F32) for t in craw])]
            ct[2], ct[3] = craw[0], craw[3]
            za = {}
            prev_late = list(late)
            late.clear()
            for r in range(2):
                t = 2 * jp + r
                za[r] = y_s[t * PITCH:t * PITCH + C, :] * qa_s[:, 128 * t:128 * (t + 1)].astype(F32)
                for b in range(3):
                    put(t, b, za[r][128 * b:128 * (b + 1)], opaque=(r == 0 and b == 0 and jp > 0))
            a_late = list(late)
            late.clear()
            res = {}
            count = [0]

            def prod(i):
                if count[0] == DL:
                    due.extend(prev_late)
                if count[0] == 6:
                    due.extend(a_late)
                count[0] += 1
                return _dot(_tied(wt[i], due, never), ct[i])

            _strassen(prod, lambda r, c, val: res.__setitem__((r, c), val), order=(1, 4, 3, 2, 0, 5, 6))
            for r in (1, 0):
                z = jnp.concatenate([za[r][384:], res[(r, 0)], res[(r, 1)]], axis=0)
                for b in (3, 2, 1, 0):
                    put(2 * jp + r, 3 + b, z[128 * b:128 * (b + 1)])
            rows = pl.ds(256 * jp, 256)
            oc = cp(out_s.at[rows], o_hbm.at[rows], 26 + jp)
            oc.start()
            outs.append(oc)
        if not CFG.get('p2', 1):
            def keep(h, carry):
                r = pl.multiple_of(h * 16, 16)
                out_s[pl.ds(r, 16), 0:128] = y_s[pl.ds(r, 16), :].astype(BF16) + qc_s[h, h, 0:16, :]
                return carry
            lax.fori_loop(0, H, keep, 0)
            oc = cp(out_s.at[pl.ds(0, 256)], o_hbm.at[pl.ds(0, 256)], 26)
            oc.start()
            outs.append(oc)
        _wait(outs, 'wout')

    phase2(out_s)


def _tiles(w):
    rows = w.shape[0]
    return w.reshape(rows, 2, 8, 2, 128).transpose(0, 1, 3, 2, 4).reshape(rows, 2, 16, 128)


@jax.jit
def pallas_concat_heads__ssm_conv_h3__compressed_kv_cla__prompt_kernel(
    A_q: jax.Array,
    A_k: jax.Array,
    A_v: jax.Array,
    A_shift_k: jax.Array,
    A_ssm_k: jax.Array,
    A_ssm_D: jax.Array,
    B_x: jax.Array,
    B_c_kv: jax.Array,
    B_w_q: jax.Array,
    B_w_uk: jax.Array,
    B_w_uv: jax.Array,
    B_w_o: jax.Array,
):
    hbm = pl.BlockSpec(memory_space=pltpu.HBM)
    out = pl.pallas_call(
        _kernel,
        in_specs=[hbm] * 12,
        out_specs=hbm,
        out_shape=jax.ShapeDtypeStruct((S, 2 * C), BF16),
        scratch_shapes=[
            pltpu.VMEM((8, S, 128), BF16),
            pltpu.VMEM((5, 4, S // 2, 128), BF16),
            pltpu.VMEM((2, DC, 8, 128), U32),
            pltpu.VMEM((2, DC, 8, 128), U32),
            pltpu.VMEM((C, S), BF16),
            pltpu.VMEM((H, NB, D, 128), BF16),
            pltpu.VMEM((64 * PITCH, 128), U32),
            pltpu.VMEM((NB, C, 128), U32),
            pltpu.VMEM((NB * PITCH, 128), F32),
            pltpu.VMEM((2, H * C, 128), BF16),
            pltpu.VMEM((4, S, 128), U32),
            pltpu.VMEM((C, S), BF16),
            pltpu.VMEM((512, 128), F32),
            pltpu.VMEM((2, S, 128), BF16),
            pltpu.VMEM((NB, D, 128), BF16),
            pltpu.VMEM((7, DC // 2, 128), BF16),
            pltpu.VMEM((7, 4, 128, 128), BF16),
            pltpu.VMEM((TQ // 128, S + 8, 128), F32),
            pltpu.VMEM((TQ // 128, S + 8, 128), F32),
            pltpu.VMEM((C, S), BF16),
            pltpu.VMEM((7, NP, 256, 128), BF16),
            pltpu.VMEM((2, C, 8, 128), U32),
            pltpu.VMEM((C, S), BF16),
            pltpu.VMEM((C, S), BF16),
            pltpu.VMEM((NB, C, 128), U32),
            pltpu.VMEM((S, 2 * C), BF16),
            pltpu.VMEM((4, C), BF16),
            pltpu.VMEM((C,), BF16),
            pltpu.SemaphoreType.DMA((35,)),
        ],
        compiler_params=pltpu.CompilerParams(vmem_limit_bytes=124 * 2 ** 20),
    )(
        A_q[0].T, A_k[0].T, A_v[0].T, A_shift_k.T, A_ssm_k, A_ssm_D, B_x[0].T, B_c_kv[0],
        _tiles(B_w_q), _tiles(B_w_uk), _tiles(B_w_uv),
        jnp.swapaxes(B_w_o, 1, 2).reshape(H * C, D),
    )
    return out.reshape(1, S, 2 * C)
```

```python
import math

import jax
import jax.numpy as jnp
from jax import lax
import jax.experimental.pallas as pl
import jax.experimental.pallas.tpu as pltpu

F32 = jnp.float32
BF16 = jnp.bfloat16
U32 = jnp.uint32
I32 = jnp.int32

S = 2048
C = 448
H = 16
D = 256
DC = 1024
NB = S // 128
NP = NB // 2
CH = C // 2
PITCH = 520
CPH = C // H
TQ = 512
NT = (((1,), (1,)), ((), ()))
LOG2E = math.log2(math.e)
QSCALE = (D ** -0.5) * LOG2E
NEG = -1e9 * LOG2E
HI_MASK = 0xFFFF0000
CFG = dict(clob=0,gback=8,costs=(2,2,1),slack=8,cg=3,rl=1,ph=2,wn=0,xb=0,xp=(2200,8190),nf=4,ux=6,sched='M001 C2 M034 C2 M06 M101 C2 Q0 M134 C2 M16 M201 C2 E00 E01 E02 E03 Q1 M234 C2 M26 M301 C2 E10 E11 Q2 M334 C2 E12 M36 E13 M02 C2 Q3 M05 C2 E20 M12 C2 E21 M15 C2 E22 M22 C2 E23 M25 C2 E30 M32 M35 E31 P0 P1 P2 P3')


def _wait(copies, name):
    if CFG.get('scopes'):
        with jax.named_scope(name):
            for c_ in copies:
                c_.wait()
    else:
        for c_ in copies:
            c_.wait()


def _dot(a, b):
    return jnp.dot(a, b, preferred_element_type=F32)


def _dot_nt(a, b):
    return lax.dot_general(a, b, NT, preferred_element_type=F32)


def _lo(x):
    return pltpu.bitcast(x << 16, F32)


def _hi(x):
    return pltpu.bitcast(x & jnp.uint32(HI_MASK), F32)


def _head_cols(w_s, h, rows):
    out = []
    for b in range(2):
        x = w_s[b, pl.ds(h // 2, rows, stride=8), :]
        if isinstance(h, int):
            out.append(_lo(x) if h % 2 == 0 else _hi(x))
        else:
            out.append(_hi(x << ((1 - h % 2) * 16).astype(U32)))
    return out


def _lhs_terms(a11, a12, a21, a22):
    return [a11 + a22, a21 + a22, a11, a22, a11 + a12, a21 - a11, a12 - a22]


def _rhs_terms(b11, b12, b21, b22):
    return [b11 + b22, b11, b12 - b22, b21 - b11, b22, b11 + b12, b21 + b22]


_LHS_SUMS = (0, 1, 4, 5, 6)


def _strassen_steps(prod, emit):
    uses = {(0, 0): {0: 1, 3: 1, 4: -1, 6: 1}, (0, 1): {2: 1, 4: 1},
            (1, 0): {1: 1, 3: 1}, (1, 1): {0: 1, 1: -1, 2: 1, 5: 1}}
    acc = {}
    neg = {}

    def step(i):
        m = prod(i)
        for key, terms in uses.items():
            if i not in terms:
                continue
            sign = terms.pop(i)
            if key not in acc:
                acc[key] = m
                neg[key] = sign < 0
            elif neg[key]:
                assert sign > 0
                acc[key] = m - acc[key]
                neg[key] = False
            else:
                acc[key] = acc[key] + m if sign > 0 else acc[key] - m
            if not terms:
                emit(key[0], key[1], acc.pop(key))

    return step


def _strassen(prod, emit, order=(0, 1, 3, 2, 4, 5, 6)):
    step = _strassen_steps(prod, emit)
    for i in order:
        step(i)


def _terms2(terms, blk):
    outer = {(r, k): terms(blk[0][0][r][k], blk[0][1][r][k], blk[1][0][r][k], blk[1][1][r][k])
             for r in range(2) for k in range(2)}
    for o in range(7):
        for i, t in enumerate(terms(outer[0, 0][o], outer[0, 1][o], outer[1, 0][o], outer[1, 1][o])):
            yield o, i, t


def _mult(i, n):
    return i if isinstance(i, int) else pl.multiple_of(i, n)


def _never(zero):
    return lax.broadcasted_iota(I32, (8, 128), 1) < zero


def _after(x, tok, never):
    if tok is None:
        return x
    return jnp.where(never, pltpu.bitcast(tok, x.dtype), x)


def _tied(lhs, due, never):
    if not due:
        return lhs
    t = None
    for d in due:
        d = pltpu.bitcast(jnp.broadcast_to(d, (8, 128)), U32)
        t = d if t is None else t ^ d
    due.clear()
    x = pltpu.bitcast(_after(pltpu.bitcast(lhs[:16, :128], U32), t, never), BF16)
    if lhs.shape[1] > 128:
        x = jnp.concatenate([x, lhs[:16, 128:]], axis=1)
    return jnp.concatenate([x, lhs[16:]], axis=0) if lhs.shape[0] > 16 else x


def _digest(vals):
    acc = None
    words = [v if v.dtype == U32 else pltpu.bitcast(v, U32) for v in vals]
    for r in range(words[0].shape[0] // 8):
        for w in words:
            w = w[8 * r:8 * (r + 1)]
            acc = w if acc is None else acc ^ w
    return acc


def _kernel(qa_hbm, ka_hbm, va_hbm, sk_hbm, hk_hbm, d_hbm, x_hbm, c_hbm, wq_hbm, wk_hbm, wv_hbm, wo_hbm,
            o_hbm,
            c_s, cs_s, wp_s, qc_s, aw_s, g_s, y_s, hk_s, dc_s, k_s, vt_s, wx_s, wn_s, sa_s, sb_s, x_s, xs_s, ka_s, va_s, sk_ref, d_ref, sems):
    def cp(src, dst, i):
        return pltpu.make_async_copy(src, dst, sems.at[i])

    wq32 = wq_hbm.bitcast(U32)
    wk32 = wk_hbm.bitcast(U32)
    wv32 = wv_hbm.bitcast(U32)
    gc = [cp(c_hbm.at[:, pl.ds(128 * b, 128)], c_s.at[b], 8 + b) for b in range(8)]

    def word_row(pair, b):
        return 8 * (pair // 4) + 4 * b + pair % 4

    def kv_copies(pair):
        return [cp(w.at[:, word_row(pair, b), :], wp_s.at[pair % 2, 2 * n + b], 16 + pair % 2)
                for n, w in enumerate((wk32, wv32)) for b in range(2)]

    g3 = kv_copies(0)
    g3b = kv_copies(1)
    g4 = [cp(qa_hbm, x_s, 21)] + [cp(wo_hbm.at[:, pl.ds(128 * b, 128)], xs_s.at[pl.ds(H * C * b, H * C)], 6 + b)
                                  for b in range(2)]

    def delayed(ref, rows, sg, n, gate=None):
        cur = pltpu.bitcast(ref[rows, 128 * sg:128 * (sg + 1)], U32)
        lane = lax.broadcasted_iota(I32, (8, 128), 1)
        if gate is not None:
            lane = gate(lane)
        lane = jnp.concatenate([lane] * (cur.shape[0] // 8), axis=0)
        prev = pltpu.bitcast(ref[rows, 128 * (sg - 1):128 * sg], U32) if sg > 0 else jnp.uint32(0)
        x = pltpu.roll(jnp.where(lane < 128 - n, cur, prev), n, 1)
        return pltpu.bitcast(x, BF16).astype(F32)

    def gated_t(x, gate):
        if gate is not None:
            x = jnp.concatenate([gate(x[:8]), x[8:]], axis=0)
        return x.T

    def windows(b, q, e, js, gate=None):
        out = []
        for j in js:
            parts = []
            for sg in range(2 * j - 6, 2 * j + 2):
                if sg < 0:
                    parts.append(jnp.zeros((16, 128), U32))
                else:
                    parts.append(pltpu.bitcast(sa_s[b, pl.ds(_mult(128 * sg + 32 * q + 16 * e, 16), 16), :], U32))
            plane = 32 * (j // 4) + 8 * q + 4 * e + j % 4
            win = gated_t(jnp.concatenate(parts, axis=0), gate)
            aw_s[pl.ds(_mult(plane * PITCH + 128 * b, 8), 128), :] = win
            out.append(win[120:])
        return out

    def prep_g(r0, n, gate=None):
        rows = pl.ds(_mult(r0, 16), n)
        lane = lax.broadcasted_iota(I32, (n, 128), 1)
        for a in range(NB):
            hf = hk_s[rows, 128 * a:128 * (a + 1)].astype(F32)
            hs = delayed(hk_s, rows, a, 1, gate)
            if a == 0:
                hf = jnp.where(lane == 0, hf + dc_s[rows, :], hf)
                hs = jnp.where(lane == 1, hs + dc_s[rows, :], hs)
            wrd = pltpu.pack_elementwise([hf, hs], packed_dtype=BF16).astype(U32)
            g_s[a, rows, :] = wrd
            yield _digest([wrd])

    def phase0():
        XC = 512
        NF = CFG.get('nf', 4)
        cq = [cp(wq32.at[:, word_row(g // 2, g % 2), :], y_s.at[pl.ds(C * g, C)], 0 if g < NF else 1 if g < 8 else 18)
              for g in range(H)]
        cx = [cp(x_hbm.at[:, pl.ds(XC * i, XC)], x_s.at[:, pl.ds(XC * i, XC)], 22 + i) for i in range(S // XC)]
        g2 = [cp(sk_hbm, sk_ref, 2), cp(d_hbm, d_ref, 20),
              cp(ka_hbm, ka_s, 3), cp(va_hbm, va_s, 4), cp(hk_hbm, hk_s, 5)]
        order = CFG.get('order', 'A')
        if order == 'A':
            ga, gb = g2, cq[8:] + gc
        else:
            ga, gb = gc, g2 + cq[8:]
        rest = cx[1:] + cq[NF:8] + ga + gb + g3 + g3b
        for c_ in [cx[0]] + cq[:NF] + rest:
            c_.start()
        zero = pl.semaphore_read(sems.at[34])
        never = _never(zero)
        due = []
        toks = []

        def pad_rows(t):
            return jnp.concatenate([t, jnp.zeros((256 - CH, 128), t.dtype)], axis=0)

        def wq_terms(j, b, gate):
            x = y_s[C * (2 * j + b):C * (2 * j + b + 1), :]
            g16 = jnp.concatenate([_after(jnp.full((8, 128), 16, U32), gate, never)] * (C // 8), axis=0)
            gm = jnp.concatenate([_after(jnp.full((8, 128), HI_MASK, U32), gate, never)] * (C // 8), axis=0)
            lo, hi = pltpu.bitcast(x << g16, F32), pltpu.bitcast(x & gm, F32)
            blocks = [pad_rows(t).T for t in (lo[:CH], hi[:CH], lo[CH:], hi[CH:])]
            return [t.astype(BF16) for t in _rhs_terms(*blocks)]

        def x_terms(jp):
            top = slice(256 * jp, 256 * jp + 128)
            bot = slice(256 * jp + 128, 256 * jp + 256)
            for i in range(7):
                xs_s[256 * (NP * i + jp) + CH:256 * (NP * i + jp + 1), :] = jnp.zeros((256 - CH, 128), BF16)
            for r in range(0, CH, 32):
                lo, hi = slice(r, r + 32), slice(CH + r, CH + r + 32)
                blocks = [x_s[lo, top], x_s[hi, top], x_s[lo, bot], x_s[hi, bot]]
                terms = [t.astype(BF16) for t in _lhs_terms(*[t.astype(F32) for t in blocks])]
                terms[2], terms[3] = blocks[0], blocks[3]
                for i, t in enumerate(terms):
                    xs_s[256 * (NP * i + jp) + r:256 * (NP * i + jp) + r + 32, :] = t
                yield 1, _digest(terms)

        def qproj(g, jp, waits):
            j, b = groups[g]
            for c_ in waits:
                c_.wait()
            if False:
                x_terms(jp)
                x_terms(jp + 1)

            def prod(i):
                pump()
                m = _dot(_tied(wts[g][i], due, never), xs_s[256 * (NP * i + jp):256 * (NP * i + jp + 1), :])
                toks.append(m[:8])
                return m

            def emit(r, c, val):
                qc_s[2 * j + c, 2 * jp + r, 128 * b:128 * (b + 1), :] = (val * QSCALE).astype(BF16)

            _strassen(prod, emit)

        def column(row):
            row = jnp.concatenate([row.astype(F32), jnp.zeros((1, 512 - C), F32)], axis=1)
            return jnp.broadcast_to(row, (128, 512)).T

        consts = {}

        def make_consts():
            consts['taps'] = [column(sk_ref[j:j + 1, :]) for j in range(4)]
            dc_s[...] = column(d_ref[...].reshape(1, C))

        def gate(x):
            back = CFG.get('gback', 6)
            return _after(x, toks[-back], never) if back else x

        def prep_u(r0, n):
            rows = slice(r0, r0 + n)
            tp = [t[rows] for t in consts['taps']]
            prev = jnp.zeros((n, 128), F32)
            for sg in range(NB):
                cols = slice(128 * sg, 128 * (sg + 1))
                ksh = ((delayed(ka_s, rows, sg, 3, gate) * tp[3] + delayed(ka_s, rows, sg, 2, gate) * tp[2])
                       + (delayed(ka_s, rows, sg, 1, gate) * tp[1] + ka_s[rows, cols].astype(F32) * tp[0]))
                kv = ksh * va_s[rows, cols].astype(F32)
                wrd = pltpu.pack_elementwise([prev, kv], packed_dtype=BF16).astype(U32)
                sb_s[sg // 4, C * (sg % 4) + r0:C * (sg % 4) + r0 + n, :] = pltpu.bitcast(wrd, F32)
                prev = kv
                yield _digest([wrd])

        def words_t(b):
            for sg in range(NB):
                r0 = C * (sg % 4) + 128 * b
                if b < 3:
                    wrd = sb_s[sg // 4, r0:r0 + 128, :]
                else:
                    wrd = jnp.concatenate([sb_s[sg // 4, r0:r0 + C - 384, :], jnp.zeros((512 - C, 128), F32)], axis=0)
                wrd = gated_t(pltpu.bitcast(wrd, U32), gate)
                sa_s[b, 128 * sg:128 * (sg + 1), :] = pltpu.bitcast(wrd, F32)
                yield wrd[120:]

        def all_windows(b):
            for p in range(8):
                for j in range(8):
                    yield windows(b, p // 2, p % 2, [j], gate)[0]

        def c_terms():
            for ck in range(4):
                for half in range(2):
                    for r0 in range(0, 128, 16):
                        blk = [[[[c_s[4 * K + 2 * k + half,
                                      512 * ck + 256 * R + 128 * r + r0:512 * ck + 256 * R + 128 * r + r0 + 16,
                                      :].astype(F32)
                                  for k in range(2)] for r in range(2)] for K in range(2)] for R in range(2)]
                        acc = None
                        for o, i, t in _terms2(_lhs_terms, blk):
                            t = t.astype(BF16)
                            cs_s[ck, 7 * o + i, half, r0:r0 + 16, :] = t
                            acc = _digest([t]) if acc is None else acc ^ _digest([t])
                            if i == 6:
                                yield acc
                                acc = None

        UG = CFG.get('ug', 32)

        def a_stream():
            make_consts()
            cu, ct, cg = CFG.get('costs', (3, 2, 1))
            gs = [prep_g(r0, 32, gate) for r0 in range(0, C, 32)]
            for b in range(4):
                for r0 in range(128 * b, min(C, 128 * (b + 1)), UG):
                    for v in prep_u(r0, UG):
                        yield cu * UG // 32, v
                for v in words_t(b):
                    yield ct, v
                for v in all_windows(b):
                    yield ct, v
                if CFG.get('gpos', 'end') == 'blk' or b == 3:
                    for g_ in (gs[4 * b:4 * b + 4] if CFG.get('gpos', 'end') == 'blk' else gs):
                        for v in g_:
                            yield cg, v

        cu, ct, cg = CFG.get('costs', (3, 2, 1))
        a_total = cu * 14 * NB + ct * 4 * (NB + 64) + cg * 14 * NB
        streams = []
        nprod = [0]
        later = {}
        LAG = CFG.get('lag', 0)

        def pump():
            for st_ in streams:
                gen, n, p0, p1, done = st_
                want = min(n, max(0, (nprod[0] - p0 + 1) * n // (p1 - p0)))
                while st_[4] < want:
                    cost, v = next(gen)
                    later.setdefault(nprod[0] + LAG, []).append(v)
                    st_[4] += cost
            due.extend(later.pop(nprod[0], []))
            nprod[0] += 1

        groups = [(j, b) for j in range(H // 2) for b in range(2)]
        units = [(g, jp) for c in range(0, NP, 2) for g in range(NF) for jp in (c, c + 1)]
        units += [(g, jp) for g in range(NF, len(groups)) for jp in range(NP)]
        NU = len(units)
        wts = {}
        lead = CFG.get('lead', 4)
        ua = CFG.get('ua', 32)
        ub = 8 * NP - lead
        ux = CFG.get('ux', 5)
        waits = {ux: cx[1:] + cq[NF:8], ua: ga, ub: gb}
        xe = [7 * ux + 2] + [7 * NF * 2 * c - 1 for c in (1, 2, 3)]
        for c in range(3):
            streams.append([(v for jp in (2 * c + 2, 2 * c + 3) for v in x_terms(jp)), 14, xe[c], xe[c + 1], 0])
        sl = CFG.get('slack', 4)
        PA, PB, PE = 7 * ua + sl, 7 * ub + sl, 7 * NU - 2 - LAG
        c_stream = ((1, v) for v in c_terms())
        nc = 4 * 2 * 8 * 7
        if order == 'A':
            streams.append([a_stream(), a_total, PA, PE, 0])
            streams.append([c_stream, nc, PB, PE, 0])
        else:
            streams.append([c_stream, nc, PA, CFG.get('cend', PB), 0])
            streams.append([a_stream(), a_total, PB, PE, 0])

        if not CFG.get('p0', 1):
            for c_ in cq + cx + g2 + gc:
                c_.wait()
            return
        _wait([cx[0]], 'wx0')
        list(x_terms(0))
        list(x_terms(1))
        _wait(cq[:NF], 'wq0')
        first_use = {}
        for u, (g, jp) in enumerate(units):
            first_use.setdefault(g, u)
        for u, (g, jp) in enumerate(units):
            if u in waits:
                _wait(waits[u], 'wu%d' % u)
            for g_, fu in first_use.items():
                if g_ not in wts and fu - (lead if g_ >= NF else 1) <= u:
                    back = CFG.get('wback', 8)
                    wts[g_] = wq_terms(*groups[g_], toks[-back] if len(toks) >= back else None)
            qproj(g, jp, [])
        assert all(st_[4] == st_[1] for st_ in streams) and not later, streams

    phase0()

    _wait(g3, 'wg3')

    def phase1(k_s, vt_s, wx_s, wn_s, *s_s):
        def extract(h, r0, shift, dst, zero=None):
            def block(n, kq, b, z):
                x = wp_s[(h // 2) % 2 + z, 2 * n + b, 256 * kq + r0:256 * kq + r0 + 16, :]
                if isinstance(h, int):
                    return _lo(x) if h % 2 == 0 else _hi(x)
                return _hi(x << jnp.concatenate([shift] * 2, axis=0))

            def blocks(z):
                return [[[[block(N, 2 * K + k, n, z) for n in range(2)] for k in range(2)]
                         for N in range(2)] for K in range(2)]

            if zero is None:
                terms = list(_terms2(_rhs_terms, blocks(0)))
            acc = None
            for o in range(7):
                if zero is not None:
                    terms = list(_terms2(_rhs_terms, blocks(zero * (o + 1))))
                for _, i, t in terms[7 * o:7 * (o + 1)]:
                    t = t.astype(BF16)
                    dst[7 * o + i, r0:r0 + 16, :] = t
                    acc = _digest([t]) if acc is None else acc ^ _digest([t])
                yield acc
                acc = None

        for r0 in range(0, 256, 16):
            list(extract(0, r0, None, wx_s))

        UN = CFG.get('unroll', 1)

        def heads(it, carry):
            @pl.when(it == 1)
            def _():
                for c_ in g4:
                    c_.start()

            @pl.when(jnp.logical_and(it % 2 == 1, it < H - 1))
            def _():
                _wait(kv_copies((it + 1) // 2), 'wkv')

            @pl.when(jnp.logical_and(it % 2 == 1, it < H - 3))
            def _():
                for c_ in kv_copies((it + 3) // 2):
                    c_.start()

            zero = it // H
            toks = []
            due = []
            for r in range(UN):
                head(it * UN + r, None if UN % 2 else r % 2, zero, toks, due)
            return carry + zero

        def head(h, par, zero, toks, due):
            lane8 = lax.broadcasted_iota(I32, (8, 128), 1)
            sub8 = lax.broadcasted_iota(I32, (8, 128), 0)
            lane16 = lax.broadcasted_iota(I32, (16, 128), 1)
            sub16 = lax.broadcasted_iota(I32, (16, 128), 0)
            tri = (lax.broadcasted_iota(I32, (128, 128), 0) <= lax.broadcasted_iota(I32, (128, 128), 1))
            h_next = h + 1 if isinstance(h, int) else jnp.minimum(h + 1, H - 1)
            never = _never(zero)

            def after(x, tok):
                return _after(x, tok, never)

            def tied(lhs):
                return _tied(lhs, due, never)

            def tok(back):
                return toks[-back] if (back and len(toks) >= back) else None

            def chan_mm(c, gate):
                m_b = lane8 < after(128 - 2 * sub8, gate)
                gs = [jnp.broadcast_to(g_s[a, pl.ds(c, 1), :], (8, 128)) for a in range(NB)]
                bt = [pltpu.roll(jnp.where(m_b, gs[a], gs[a - 1] if a > 0 else jnp.uint32(0)), 0, 1,
                                 stride=2, stride_axis=0) for a in range(NB)]
                b1 = pltpu.bitcast(jnp.concatenate(bt[7::-1], axis=0), BF16)
                b2 = pltpu.bitcast(jnp.concatenate(bt[15:7:-1], axis=0), BF16)
                am = pltpu.bitcast(aw_s[pl.ds(c, 64, stride=PITCH), :], BF16)
                z1 = _dot(tied(am), b1)
                z2 = _dot(am[:64], b2)
                return c, z1[:64], z1[64:] + z2

            def chan_post(c, zlo, zhi):
                acc = car = None
                for p in range(8):
                    z = jnp.concatenate([zlo[8 * p:8 * p + 8], zhi[8 * p:8 * p + 8]], axis=0)
                    if p == 0:
                        acc = z
                    else:
                        z = pltpu.roll(z, 16 * p, 1)
                        cz = jnp.where(lane16 < 16 * p, z, 0.0)
                        acc = acc + z
                        car = cz if car is None else car + cz
                y = (acc - car) + jnp.where(sub16 > 0, pltpu.roll(car, 1, 0), 0.0)
                y_s[pl.ds(c, NB, stride=PITCH), :] = pltpu.bitcast(y, U32)
                if CFG.get('pd', 0):
                    due.append(y[:8])
                    due.append(y[8:])

            chans = [h * CPH + i for i in range(CPH)]

            fine = []
            state = [0, 0, 0, 0]

            def x_stream():
                for r0 in range(0, 256, 16):
                    back = CFG.get('xb', 8)
                    gate = fine[-back] if back and len(fine) >= back else None
                    yield from extract(h_next, r0, shift_of(h_next, gate), wn_s if CFG.get('wn', 1) else wx_s,
                                       zero if CFG.get('rl') else None)

            xgen = x_stream()

            def pump():
                if 'xs' in CFG:
                    p0, p1 = CFG['xs']
                    want = min(112, max(0, (state[0] - p0 + 1) * 112 // (p1 - p0)))
                    while state[1] < want:
                        due.append(next(xgen))
                        state[1] += 1
                state[0] += 1

            def qpump(cycles):
                if 'xq' in CFG:
                    c0, c1 = CFG['xq']
                    want = min(112, max(0, (state[2] - c0) * 112 // (c1 - c0)))
                    while state[1] < want:
                        due.append(next(xgen))
                        state[1] += 1
                state[2] += cycles

            def ppump(cycles):
                if 'xp' in CFG:
                    c0, c1 = CFG['xp']
                    want = min(112, max(0, (state[3] - c0) * 112 // (c1 - c0)))
                    while state[1] < want:
                        due.append(next(xgen))
                        state[1] += 1
                state[3] += cycles

            def shift_of(hh, gate):
                return after(jnp.full((8, 128), (1 - hh % 2) * 16, I32).astype(U32), gate)

            def kv_chunk(ck):
                def prod(o):
                    out = {}

                    def inner(i):
                        pump()
                        lhs = jnp.concatenate([cs_s[ck, 7 * o + i, 0], cs_s[ck, 7 * o + i, 1]], axis=1)
                        m = _dot(tied(lhs), wx_s[7 * o + i])
                        fine.append(m[:8])
                        if i == CFG.get('ti', 3):
                            toks.append(m[:8])
                        return m

                    _strassen(inner, lambda r, n, val: out.__setitem__((r, n), val))
                    return jnp.concatenate(
                        [jnp.concatenate([out[r, 0], out[r, 1]], axis=1) for r in range(2)], axis=0)

                def emit(R, N, val):
                    if N == 0:
                        rows = slice(512 * ck + 256 * R, 512 * ck + 256 * (R + 1))
                        val = val.astype(BF16)
                        k_s[0, rows, :] = val[:, :128]
                        k_s[1, rows, :] = val[:, 128:]
                    else:
                        for r in range(2):
                            for n in range(2):
                                vt_s[4 * ck + 2 * R + r, 128 * n:128 * (n + 1), :] = (
                                    val[128 * r:128 * (r + 1), 128 * n:128 * (n + 1)].T.astype(BF16))

                return _strassen_steps(prod, emit)

            kv = [kv_chunk(ck) for ck in range(4)]

            def k_rows(r0, r1):
                return jnp.concatenate([k_s[0, r0:r1, :], k_s[1, r0:r1, :]], axis=1)

            def q_cols(r0, r1):
                return jnp.concatenate([qc_s[h, t] for t in range(r0 // 128, r1 // 128)], axis=1)

            mx, pr = {}, {}

            def qk(t):
                q0 = t * TQ
                if q0 > 0:
                    QR = CFG.get('qr', 2048)
                    rect = []
                    for r0 in range(0, q0, QR):
                        qpump(min(QR, q0 - r0) * 2)
                        rect.append(_dot(tied(k_rows(r0, min(q0, r0 + QR))), q_cols(q0, q0 + TQ)))
                        fine.append(rect[-1][:8, :128])
                    s_rect = jnp.concatenate(rect, axis=0) if len(rect) > 1 else rect[0]
                    toks.append(s_rect[:8, :128])
                for u in range(TQ // 128):
                    qs = q0 + u * 128
                    qpump(64 * (u + 1))
                    sd = _dot(tied(k_rows(q0, qs + 128)), q_cols(qs, qs + 128))
                    fine.append(sd[:8])
                    parts = []
                    if q0 > 0:
                        parts.append(s_rect[:, u * 128:(u + 1) * 128])
                    if u > 0:
                        parts.append(sd[:u * 128, :])
                    parts.append(jnp.where(tri, sd[u * 128:, :], NEG))
                    s = jnp.concatenate(parts, axis=0) if len(parts) > 1 else parts[0]
                    s_s[t % 2][u, 0:qs + 128, :] = s
                    mx[(t, u)] = jnp.max(s, axis=0, keepdims=True)
                toks.append(sd[:8])
                if CFG.get('clob', 1):
                    s_s[t % 2][zero, S:S + 8, :] = sd[:8]

            def softmax(t, u, deadline):
                qs = t * TQ + u * 128
                p = jnp.exp2(s_s[t % 2][u if CFG.get('clob', 1) else u + zero, 0:qs + 128, :] - mx.pop((t, u)))
                rl = 1.0 / jnp.sum(p, axis=0, keepdims=True)
                pr[(t, u)] = (p.astype(BF16), rl)
                if deadline:
                    due.append(rl)

            def pv(t, u):
                if (t, u) not in pr:
                    softmax(t, u, False)
                p, rl = pr.pop((t, u))
                qs = t * TQ + u * 128
                vt = jnp.concatenate([vt_s[i] for i in range(qs // 128 + 1)], axis=1)
                PH = D // CFG.get('ph', 1)
                for d0 in range(0, D, PH):
                    ppump((qs + 128) * PH // 512)
                    ctx = _dot(tied(vt[d0:d0 + PH]), p)
                    fine.append(ctx[:8])
                    qc_s[h, qs // 128, d0:d0 + PH, :] = (ctx * rl).astype(BF16)
                toks.append(ctx[:8])

            CG, XG = CFG.get('cg', 0), CFG.get('xg', 0)
            pend = []
            def run_step(st_):
                kind, arg = st_[0], st_[1:]
                if kind == 'x' and st_ != 'xr':
                    p0, n = int(arg[0], 16), int(arg[1], 16)
                    for p in range(p0, p0 + n):
                        due.extend(extract(h_next, 16 * p, shift_of(h_next, tok(XG)),
                                           wn_s if CFG.get('wn', 1) else wx_s))
                    return
                if st_ == 'xr':
                    due.extend(xgen)
                    return
                if kind == 'y':
                    for o in arg:
                        vals = [wn_s[7 * int(o) + i] for i in range(7)]
                        for i, v in enumerate(vals):
                            wx_s[7 * int(o) + i] = v
                        if CFG.get('yd', 1):
                            due.append(_digest(vals))
                    return
                if kind == 'E':
                    softmax(int(arg[0]), int(arg[1]), True)
                    return
                old = list(pend)
                pend.clear()
                if kind == 'C':
                    for _ in range(int(arg)):
                        pend.append(chan_mm(chans.pop(0), tok(CG)))
                elif kind == 'M':
                    for o in arg[1:]:
                        kv[int(arg[0])](int(o))
                elif kind == 'Q':
                    qk(int(arg))
                elif kind == 'P':
                    for u in ([int(arg[1])] if len(arg) > 1 else range(TQ // 128)):
                        pv(int(arg[0]), u)
                for args in old:
                    chan_post(*args)

            for seg in [g for g in CFG['sched'].split('|') if g.strip()]:
                if CFG.get('scopes') and '|' in CFG['sched']:
                    with jax.named_scope('s_' + seg.split()[0]):
                        for st_ in seg.split():
                            run_step(st_)
                else:
                    for st_ in seg.split():
                        run_step(st_)
            assert next(xgen, None) is None or CFG.get('noassert')
            assert CFG.get('noassert') or not chans and not pend and (not due or CFG.get('pd')) and not pr and not mx

        if CFG.get('p1', 1):
            return lax.fori_loop(0, H // UN, heads, 0)
        else:
            _wait(g3b, 'wg3b')
            for c_ in g4:
                c_.start()

            def keep(h, carry):
                r = pl.multiple_of(h * 16, 16)
                t = (qc_s[h, h, 0:16, :].astype(F32) + cs_s[h % 4, h, h % 2, 0:16, :].astype(F32)
                     + pltpu.bitcast(aw_s[pl.ds(r, 16), :] + g_s[h, pl.ds(r, 16), :], F32)
                     + wx_s[h, pl.ds(r, 16), :].astype(F32))
                y_s[pl.ds(r, 16), :] = pltpu.bitcast(t, U32)
                return carry + h // H
            return lax.fori_loop(0, H, keep, 0)

    zero_end = phase1(k_s, vt_s, wx_s, wn_s, sa_s, sb_s)

    def phase2():
        _wait(g4, 'wg4')
        HH = H // 2

        def wo_block(rh, kh):
            return jnp.concatenate(
                [xs_s[C * (H * b + h) + CH * rh:C * (H * b + h) + CH * (rh + 1), :]
                 for h in range(HH * kh, HH * (kh + 1)) for b in range(2)], axis=1)

        raw = [wo_block(0, 0), wo_block(1, 0), wo_block(0, 1), wo_block(1, 1)]
        wt = [t.astype(BF16) for t in _rhs_terms(*[t.astype(F32) for t in raw])]
        wt[1], wt[4] = raw[0], raw[3]
        outs = []
        due, late = [], []
        DL = CFG.get('dl', 3)
        never = _never(zero_end)

        def put(t, b, z, opaque=False):
            o = z.T.astype(BF16)
            r0 = pl.multiple_of(zero_end * 16 + 128 * t, 16) if opaque else 128 * t
            c_s[b, pl.ds(r0, 128), :] = o
            late.append(pltpu.bitcast(o[112:], U32))

        for jp in range(CFG.get('np2', NP) if CFG.get('p2', 1) else 0):
            def ctx_block(r, kh):
                return jnp.concatenate([qc_s[h, 2 * jp + r] for h in range(HH * kh, HH * (kh + 1))], axis=0)

            craw = [ctx_block(0, 0), ctx_block(0, 1), ctx_block(1, 0), ctx_block(1, 1)]
            ct = [t.astype(BF16) for t in _lhs_terms(*[t.astype(F32) for t in craw])]
            ct[2], ct[3] = craw[0], craw[3]
            za = {}
            prev_late = list(late)
            late.clear()
            for r in range(2):
                t = 2 * jp + r
                za[r] = (pltpu.bitcast(y_s[t * PITCH:t * PITCH + C, :], F32)
                         * x_s[:, 128 * t:128 * (t + 1)].astype(F32))
                for b in range(3):
                    put(t, b, za[r][128 * b:128 * (b + 1)], opaque=(r == 0 and b == 0 and jp > 0))
            a_late = list(late)
            late.clear()
            res = {}
            count = [0]

            def prod(i):
                if count[0] == DL:
                    due.extend(prev_late)
                if count[0] == 6:
                    due.extend(a_late)
                count[0] += 1
                return _dot(_tied(wt[i], due, never), ct[i])

            _strassen(prod, lambda r, c, val: res.__setitem__((r, c), val), order=(1, 4, 3, 2, 0, 5, 6))
            for r in (1, 0):
                z = jnp.concatenate([za[r][384:], res[(r, 0)], res[(r, 1)]], axis=0)
                for b in (3, 2, 1, 0):
                    put(2 * jp + r, 3 + b, z[128 * b:128 * (b + 1)])
            rows = pl.ds(256 * jp, 256)
            for b in range(7):
                oc = cp(c_s.at[b, rows], o_hbm.at[rows, pl.ds(128 * b, 128)], 26 + jp)
                oc.start()
                outs.append(oc)
        if not CFG.get('p2', 1):
            def keep(h, carry):
                r = pl.multiple_of(h * 16, 16)
                c_s[0, pl.ds(r, 16), :] = pltpu.bitcast(y_s[pl.ds(r, 16), :], F32).astype(BF16) + qc_s[h, h, 0:16, :]
                return carry
            lax.fori_loop(0, H, keep, 0)
            oc = cp(c_s.at[0, pl.ds(0, 256)], o_hbm.at[pl.ds(0, 256), pl.ds(0, 128)], 26)
            oc.start()
            outs.append(oc)
        _wait(outs, 'wout')

    phase2()


def _tiles(w):
    rows = w.shape[0]
    return w.reshape(rows, 2, 8, 2, 128).transpose(0, 1, 3, 2, 4).reshape(rows, 32, 128)


@jax.jit
def pallas_concat_heads__ssm_conv_h3__compressed_kv_cla__prompt_kernel(
    A_q: jax.Array,
    A_k: jax.Array,
    A_v: jax.Array,
    A_shift_k: jax.Array,
    A_ssm_k: jax.Array,
    A_ssm_D: jax.Array,
    B_x: jax.Array,
    B_c_kv: jax.Array,
    B_w_q: jax.Array,
    B_w_uk: jax.Array,
    B_w_uv: jax.Array,
    B_w_o: jax.Array,
):
    hbm = pl.BlockSpec(memory_space=pltpu.HBM)
    out = pl.pallas_call(
        _kernel,
        in_specs=[hbm] * 12,
        out_specs=hbm,
        out_shape=jax.ShapeDtypeStruct((S, 2 * C), BF16),
        scratch_shapes=[
            pltpu.VMEM((8, S, 128), BF16),
            pltpu.VMEM((4, 49, 2, 128, 128), BF16),
            pltpu.VMEM((2, 4, DC, 128), U32),
            pltpu.VMEM((H, NB, D, 128), BF16),
            pltpu.VMEM((64 * PITCH, 128), U32),
            pltpu.VMEM((NB, C, 128), U32),
            pltpu.VMEM((NB * PITCH, 128), U32),
            pltpu.VMEM((C, S), BF16),
            pltpu.VMEM((512, 128), F32),
            pltpu.VMEM((2, S, 128), BF16),
            pltpu.VMEM((NB, D, 128), BF16),
            pltpu.VMEM((49, DC // 4, 128), BF16),
            pltpu.VMEM((49, DC // 4, 128), BF16),
            pltpu.VMEM((TQ // 128, S + 8, 128), F32),
            pltpu.VMEM((TQ // 128, S + 8, 128), F32),
            pltpu.VMEM((C, S), BF16),
            pltpu.VMEM((7 * NP * 256, 128), BF16),
            pltpu.VMEM((C, S), BF16),
            pltpu.VMEM((C, S), BF16),
            pltpu.VMEM((4, C), BF16),
            pltpu.VMEM((C,), BF16),
            pltpu.SemaphoreType.DMA((35,)),
        ],
        compiler_params=pltpu.CompilerParams(vmem_limit_bytes=127 * 2 ** 20),
    )(
        A_q[0].T, A_k[0].T, A_v[0].T, A_shift_k.T, A_ssm_k, A_ssm_D, B_x[0].T, B_c_kv[0],
        _tiles(B_w_q), _tiles(B_w_uk), _tiles(B_w_uv),
        jnp.swapaxes(B_w_o, 1, 2).reshape(H * C, D),
    )
    return out.reshape(1, S, 2 * C)
```

```python
import math

import jax
import jax.numpy as jnp
from jax import lax
import jax.experimental.pallas as pl
import jax.experimental.pallas.tpu as pltpu

F32 = jnp.float32
BF16 = jnp.bfloat16
U32 = jnp.uint32
I32 = jnp.int32

S = 2048
C = 448
H = 16
D = 256
DC = 1024
NB = S // 128
NP = NB // 2
CH = C // 2
PITCH = 520
CPH = C // H
TQ = 512
NT = (((1,), (1,)), ((), ()))
LOG2E = math.log2(math.e)
QSCALE = (D ** -0.5) * LOG2E
NEG = -1e9 * LOG2E
HI_MASK = 0xFFFF0000
CFG = dict(nf=8,n0=3,ux=13,crl=1,gback=8,costs=(2,2,1),slack=8,clob=0,cg=3,ph=2,late=(),x2=('P',0,1),x1=('P',2200,8190),sched='M001 C2 M034 C2 M06 M101 C2 Q0 M134 C2 M16 M201 C2 E00 E01 E02 E03 Q1 M234 C2 M26 M301 C2 E10 E11 Q2 M334 C2 E12 M36 E13 M02 C2 Q3 M05 C2 E20 M12 C2 E21 M15 C2 E22 M22 C2 E23 M25 C2 E30 M32 M35 E31 P0 P1 P2 P3')


def _wait(copies, name):
    if CFG.get('scopes'):
        with jax.named_scope(name):
            for c_ in copies:
                c_.wait()
    else:
        for c_ in copies:
            c_.wait()


def _dot(a, b):
    return jnp.dot(a, b, preferred_element_type=F32)


def _dot_nt(a, b):
    return lax.dot_general(a, b, NT, preferred_element_type=F32)


def _lo(x):
    return pltpu.bitcast(x << 16, F32)


def _hi(x):
    return pltpu.bitcast(x & jnp.uint32(HI_MASK), F32)


def _head_cols(w_s, h, rows):
    out = []
    for b in range(2):
        x = w_s[b, pl.ds(h // 2, rows, stride=8), :]
        if isinstance(h, int):
            out.append(_lo(x) if h % 2 == 0 else _hi(x))
        else:
            out.append(_hi(x << ((1 - h % 2) * 16).astype(U32)))
    return out


def _lhs_terms(a11, a12, a21, a22):
    return [a11 + a22, a21 + a22, a11, a22, a11 + a12, a21 - a11, a12 - a22]


def _rhs_terms(b11, b12, b21, b22):
    return [b11 + b22, b11, b12 - b22, b21 - b11, b22, b11 + b12, b21 + b22]


_LHS_SUMS = (0, 1, 4, 5, 6)


def _strassen_steps(prod, emit):
    uses = {(0, 0): {0: 1, 3: 1, 4: -1, 6: 1}, (0, 1): {2: 1, 4: 1},
            (1, 0): {1: 1, 3: 1}, (1, 1): {0: 1, 1: -1, 2: 1, 5: 1}}
    acc = {}
    neg = {}

    def step(i):
        m = prod(i)
        for key, terms in uses.items():
            if i not in terms:
                continue
            sign = terms.pop(i)
            if key not in acc:
                acc[key] = m
                neg[key] = sign < 0
            elif neg[key]:
                assert sign > 0
                acc[key] = m - acc[key]
                neg[key] = False
            else:
                acc[key] = acc[key] + m if sign > 0 else acc[key] - m
            if not terms:
                emit(key[0], key[1], acc.pop(key))

    return step


def _strassen(prod, emit, order=(0, 1, 3, 2, 4, 5, 6)):
    step = _strassen_steps(prod, emit)
    for i in order:
        step(i)


def _terms2(terms, blk):
    outer = {(r, k): terms(blk[0][0][r][k], blk[0][1][r][k], blk[1][0][r][k], blk[1][1][r][k])
             for r in range(2) for k in range(2)}
    for o in range(7):
        for i, t in enumerate(terms(outer[0, 0][o], outer[0, 1][o], outer[1, 0][o], outer[1, 1][o])):
            yield o, i, t


def _mult(i, n):
    return i if isinstance(i, int) else pl.multiple_of(i, n)


def _never(zero):
    return lax.broadcasted_iota(I32, (8, 128), 1) < zero


def _after(x, tok, never):
    if tok is None:
        return x
    return jnp.where(never, pltpu.bitcast(tok, x.dtype), x)


def _tied(lhs, due, never):
    if not due:
        return lhs
    t = None
    for d in due:
        d = pltpu.bitcast(jnp.broadcast_to(d, (8, 128)), U32)
        t = d if t is None else t ^ d
    due.clear()
    x = pltpu.bitcast(_after(pltpu.bitcast(lhs[:16, :128], U32), t, never), BF16)
    if lhs.shape[1] > 128:
        x = jnp.concatenate([x, lhs[:16, 128:]], axis=1)
    return jnp.concatenate([x, lhs[16:]], axis=0) if lhs.shape[0] > 16 else x


def _digest(vals):
    acc = None
    words = [v if v.dtype == U32 else pltpu.bitcast(v, U32) for v in vals]
    for r in range(words[0].shape[0] // 8):
        for w in words:
            w = w[8 * r:8 * (r + 1)]
            acc = w if acc is None else acc ^ w
    return acc


class _Packed:
    def __init__(self, ref):
        self.ref = ref

    def _index(self, idx):
        idx = idx if isinstance(idx, tuple) else (idx,)
        axis = len(self.ref.shape) - 2
        if len(idx) <= axis:
            return idx + (slice(None),) * (axis + 2 - len(idx))
        r = idx[axis]
        if isinstance(r, slice):
            r = slice(None if r.start is None else r.start // 2, None if r.stop is None else r.stop // 2)
        else:
            r = pl.ds(_mult(r.start // 2, 8), r.size // 2)
        return idx[:axis] + (r,) + idx[axis + 1:]

    def __getitem__(self, idx):
        return pltpu.bitcast(self.ref[self._index(idx)], BF16)

    def __setitem__(self, idx, val):
        self.ref[self._index(idx)] = pltpu.bitcast(val, U32)


def _kernel(qa_hbm, ka_hbm, va_hbm, sk_hbm, hk_hbm, d_hbm, x_hbm, c_hbm, wq_hbm, wk_hbm, wv_hbm, wo_hbm,
            o_hbm,
            c_s, cs_s, wp_s, qc_s, aw_s, g_s, y_s, hk_s, dc_s, k_s, vt_s, wx_s, sa_s, sb_s, x_s, xs_s, ka_s, va_s, sk_ref, d_ref, sems):
    def cp(src, dst, i):
        return pltpu.make_async_copy(src, dst, sems.at[i])

    c_w, xs_w, x_w, ka_w, va_w, hk_w = c_s, xs_s, x_s, ka_s, va_s, hk_s
    c_s, cs_s, qc_s, k_s, vt_s, wx_s, xs_s, x_s, ka_s, va_s, hk_s = (
        _Packed(r) for r in (c_s, cs_s, qc_s, k_s, vt_s, wx_s, xs_s, x_s, ka_s, va_s, hk_s))
    qa_hbm, ka_hbm, va_hbm, hk_hbm, x_hbm, c_hbm, wo_hbm, o_hbm = (
        r.bitcast(U32) for r in (qa_hbm, ka_hbm, va_hbm, hk_hbm, x_hbm, c_hbm, wo_hbm, o_hbm))
    wq32 = wq_hbm.bitcast(U32)
    wk32 = wk_hbm.bitcast(U32)
    wv32 = wv_hbm.bitcast(U32)
    gc = [cp(c_hbm.at[:, pl.ds(128 * b, 128)], c_w.at[b], 8 + b) for b in range(8)]

    def word_row(pair, b):
        return 8 * (pair // 4) + 4 * b + pair % 4

    def kv_copies(pair):
        return [cp(w.at[:, word_row(pair, b), :], wp_s.at[pair % 2, 2 * n + b], 16 + pair % 2)
                for n, w in enumerate((wk32, wv32)) for b in range(2)]

    g3 = kv_copies(0)
    g3b = kv_copies(1)
    g4 = [cp(qa_hbm, x_w, 21)] + [cp(wo_hbm.at[:, pl.ds(128 * b, 128)], xs_w.at[pl.ds(H * CH * b, H * CH)], 6 + b)
                                  for b in range(2)]

    def delayed(ref, rows, sg, n, gate=None):
        cur = pltpu.bitcast(ref[rows, 128 * sg:128 * (sg + 1)], U32)
        lane = lax.broadcasted_iota(I32, (8, 128), 1)
        if gate is not None:
            lane = gate(lane)
        lane = jnp.concatenate([lane] * (cur.shape[0] // 8), axis=0)
        prev = pltpu.bitcast(ref[rows, 128 * (sg - 1):128 * sg], U32) if sg > 0 else jnp.uint32(0)
        x = pltpu.roll(jnp.where(lane < 128 - n, cur, prev), n, 1)
        return pltpu.bitcast(x, BF16).astype(F32)

    def gated_t(x, gate):
        if gate is not None:
            x = jnp.concatenate([gate(x[:8]), x[8:]], axis=0)
        return x.T

    def windows(b, q, e, js, gate=None):
        out = []
        for j in js:
            parts = []
            for sg in range(2 * j - 6, 2 * j + 2):
                if sg < 0:
                    parts.append(jnp.zeros((16, 128), U32))
                else:
                    parts.append(pltpu.bitcast(sa_s[b, pl.ds(_mult(128 * sg + 32 * q + 16 * e, 16), 16), :], U32))
            plane = 32 * (j // 4) + 8 * q + 4 * e + j % 4
            win = gated_t(jnp.concatenate(parts, axis=0), gate)
            aw_s[pl.ds(_mult(plane * PITCH + 128 * b, 8), 128), :] = win
            out.append(win[120:])
        return out

    def prep_g(r0, n, gate=None):
        rows = pl.ds(_mult(r0, 16), n)
        lane = lax.broadcasted_iota(I32, (n, 128), 1)
        for a in range(NB):
            hf = hk_s[rows, 128 * a:128 * (a + 1)].astype(F32)
            hs = delayed(hk_s, rows, a, 1, gate)
            if a == 0:
                hf = jnp.where(lane == 0, hf + dc_s[rows, :], hf)
                hs = jnp.where(lane == 1, hs + dc_s[rows, :], hs)
            wrd = pltpu.pack_elementwise([hf, hs], packed_dtype=BF16).astype(U32)
            g_s[a, rows, :] = wrd
            yield _digest([wrd])

    def phase0():
        XC = 512
        NF = CFG.get('nf', 4)
        N0 = CFG.get('n0', NF)
        cq = [cp(wq32.at[:, word_row(g // 2, g % 2), :], y_s.at[pl.ds(C * g, C)],
                 0 if g < N0 else 19 if g < NF else 1 if g < 8 else 18)
              for g in range(H)]
        cx = [cp(x_hbm.at[:, pl.ds(XC * i, XC)], x_w.at[:, pl.ds(XC * i, XC)], 22 + i) for i in range(S // XC)]
        g2 = [cp(sk_hbm, sk_ref, 2), cp(d_hbm, d_ref, 20),
              cp(ka_hbm, ka_w, 3), cp(va_hbm, va_w, 4), cp(hk_hbm, hk_w, 5)]
        order = CFG.get('order', 'A')
        if order == 'A':
            ga, gb = g2, cq[8:] + gc
        else:
            ga, gb = gc, g2 + cq[8:]
        rest = cx[1:] + cq[NF:8] + ga + gb + g3 + g3b
        for c_ in [cx[0]] + cq[:NF] + rest:
            c_.start()
        zero = pl.semaphore_read(sems.at[34])
        never = _never(zero)
        due = []
        toks = []

        def pad_rows(t):
            return jnp.concatenate([t, jnp.zeros((256 - CH, 128), t.dtype)], axis=0)

        def wq_terms(j, b, gate):
            x = y_s[C * (2 * j + b):C * (2 * j + b + 1), :]
            g16 = jnp.concatenate([_after(jnp.full((8, 128), 16, U32), gate, never)] * (C // 8), axis=0)
            gm = jnp.concatenate([_after(jnp.full((8, 128), HI_MASK, U32), gate, never)] * (C // 8), axis=0)
            lo, hi = pltpu.bitcast(x << g16, F32), pltpu.bitcast(x & gm, F32)
            blocks = [pad_rows(t).T for t in (lo[:CH], hi[:CH], lo[CH:], hi[CH:])]
            return [t.astype(BF16) for t in _rhs_terms(*blocks)]

        def x_terms(jp):
            top = slice(256 * jp, 256 * jp + 128)
            bot = slice(256 * jp + 128, 256 * jp + 256)
            for i in range(7):
                xs_s[256 * (NP * i + jp) + CH:256 * (NP * i + jp + 1), :] = jnp.zeros((256 - CH, 128), BF16)
            for r in range(0, CH, 32):
                lo, hi = slice(r, r + 32), slice(CH + r, CH + r + 32)
                blocks = [x_s[lo, top], x_s[hi, top], x_s[lo, bot], x_s[hi, bot]]
                terms = [t.astype(BF16) for t in _lhs_terms(*[t.astype(F32) for t in blocks])]
                terms[2], terms[3] = blocks[0], blocks[3]
                for i, t in enumerate(terms):
                    xs_s[256 * (NP * i + jp) + r:256 * (NP * i + jp) + r + 32, :] = t
                yield 1, _digest(terms)

        def qproj(g, jp, waits):
            j, b = groups[g]
            for c_ in waits:
                c_.wait()
            if False:
                x_terms(jp)
                x_terms(jp + 1)

            def prod(i):
                pump()
                m = _dot(_tied(wts[g][i], due, never), xs_s[256 * (NP * i + jp):256 * (NP * i + jp + 1), :])
                toks.append(m[:8])
                return m

            def emit(r, c, val):
                qc_s[2 * j + c, 2 * jp + r, 128 * b:128 * (b + 1), :] = (val * QSCALE).astype(BF16)

            _strassen(prod, emit)

        def column(row):
            row = jnp.concatenate([row.astype(F32), jnp.zeros((1, 512 - C), F32)], axis=1)
            return jnp.broadcast_to(row, (128, 512)).T

        consts = {}

        def make_consts():
            consts['taps'] = [column(sk_ref[j:j + 1, :]) for j in range(4)]
            dc_s[...] = column(d_ref[...].reshape(1, C))

        def gate(x):
            back = CFG.get('gback', 6)
            return _after(x, toks[-back], never) if back else x

        def prep_u(r0, n):
            rows = slice(r0, r0 + n)
            tp = [t[rows] for t in consts['taps']]
            prev = jnp.zeros((n, 128), F32)
            for sg in range(NB):
                cols = slice(128 * sg, 128 * (sg + 1))
                ksh = ((delayed(ka_s, rows, sg, 3, gate) * tp[3] + delayed(ka_s, rows, sg, 2, gate) * tp[2])
                       + (delayed(ka_s, rows, sg, 1, gate) * tp[1] + ka_s[rows, cols].astype(F32) * tp[0]))
                kv = ksh * va_s[rows, cols].astype(F32)
                wrd = pltpu.pack_elementwise([prev, kv], packed_dtype=BF16).astype(U32)
                sb_s[sg // 4, C * (sg % 4) + r0:C * (sg % 4) + r0 + n, :] = pltpu.bitcast(wrd, F32)
                prev = kv
                yield _digest([wrd])

        def words_t(b):
            for sg in range(NB):
                r0 = C * (sg % 4) + 128 * b
                if b < 3:
                    wrd = sb_s[sg // 4, r0:r0 + 128, :]
                else:
                    wrd = jnp.concatenate([sb_s[sg // 4, r0:r0 + C - 384, :], jnp.zeros((512 - C, 128), F32)], axis=0)
                wrd = gated_t(pltpu.bitcast(wrd, U32), gate)
                sa_s[b, 128 * sg:128 * (sg + 1), :] = pltpu.bitcast(wrd, F32)
                yield wrd[120:]

        def all_windows(b):
            for p in range(8):
                for j in range(8):
                    yield windows(b, p // 2, p % 2, [j], gate)[0]

        def c_terms():
            for ck in range(4):
                for half in range(2):
                    for r0 in range(0, 128, 16):
                        def blocks(z):
                            return [[[[c_s[4 * K + 2 * k + half + z,
                                           512 * ck + 256 * R + 128 * r + r0:512 * ck + 256 * R + 128 * r + r0 + 16,
                                           :].astype(F32)
                                       for k in range(2)] for r in range(2)] for K in range(2)] for R in range(2)]

                        if CFG.get('crl'):
                            terms = [x for o in range(7)
                                     for x in list(_terms2(_lhs_terms, blocks(zero * (o + 1))))[7 * o:7 * (o + 1)]]
                        else:
                            terms = _terms2(_lhs_terms, blocks(0))
                        acc = None
                        for o, i, t in terms:
                            t = t.astype(BF16)
                            cs_s[ck, 7 * o + i, half, r0:r0 + 16, :] = t
                            acc = _digest([t]) if acc is None else acc ^ _digest([t])
                            if i == 6:
                                yield acc
                                acc = None

        UG = CFG.get('ug', 32)

        def a_stream():
            make_consts()
            cu, ct, cg = CFG.get('costs', (3, 2, 1))
            gs = [prep_g(r0, 32, gate) for r0 in range(0, C, 32)]
            for b in range(4):
                for r0 in range(128 * b, min(C, 128 * (b + 1)), UG):
                    for v in prep_u(r0, UG):
                        yield cu * UG // 32, v
                for v in words_t(b):
                    yield ct, v
                for v in all_windows(b):
                    yield ct, v
                if CFG.get('gpos', 'end') == 'blk' or b == 3:
                    for g_ in (gs[4 * b:4 * b + 4] if CFG.get('gpos', 'end') == 'blk' else gs):
                        for v in g_:
                            yield cg, v

        cu, ct, cg = CFG.get('costs', (3, 2, 1))
        a_total = cu * 14 * NB + ct * 4 * (NB + 64) + cg * 14 * NB
        streams = []
        nprod = [0]
        later = {}
        LAG = CFG.get('lag', 0)

        def pump():
            for st_ in streams:
                gen, n, p0, p1, done = st_
                want = min(n, max(0, (nprod[0] - p0 + 1) * n // (p1 - p0)))
                while st_[4] < want:
                    cost, v = next(gen)
                    later.setdefault(nprod[0] + LAG, []).append(v)
                    st_[4] += cost
            due.extend(later.pop(nprod[0], []))
            nprod[0] += 1

        groups = [(j, b) for j in range(H // 2) for b in range(2)]
        units = [(g, jp) for c in range(0, NP, 2) for g in range(NF) for jp in (c, c + 1)]
        units += [(g, jp) for g in range(NF, len(groups)) for jp in range(NP)]
        NU = len(units)
        wts = {}
        lead = CFG.get('lead', 4)
        ua = CFG.get('ua', 32)
        ub = 8 * NP - lead
        ux = CFG.get('ux', 5)
        waits = {ux: cx[1:] + cq[NF:8], ua: ga, ub: gb}
        if N0 < NF:
            waits[2 * N0 - 1] = cq[N0:NF]
        xe = [7 * ux + 2] + [7 * NF * 2 * c - 1 for c in (1, 2, 3)]
        for c in range(3):
            streams.append([(v for jp in (2 * c + 2, 2 * c + 3) for v in x_terms(jp)), 14, xe[c], xe[c + 1], 0])
        sl = CFG.get('slack', 4)
        PA, PB, PE = 7 * ua + sl, 7 * ub + sl, 7 * NU - 2 - LAG
        c_stream = ((1, v) for v in c_terms())
        nc = 4 * 2 * 8 * 7
        if order == 'A':
            streams.append([a_stream(), a_total, PA, PE, 0])
            streams.append([c_stream, nc, PB, PE, 0])
        else:
            streams.append([c_stream, nc, PA, CFG.get('cend', PB), 0])
            streams.append([a_stream(), a_total, PB, PE, 0])

        if not CFG.get('p0', 1):
            for c_ in cq + cx + g2 + gc:
                c_.wait()
            return
        _wait([cx[0]], 'wx0')
        list(x_terms(0))
        list(x_terms(1))
        _wait(cq[:N0], 'wq0')
        first_use = {}
        for u, (g, jp) in enumerate(units):
            first_use.setdefault(g, u)
        for u, (g, jp) in enumerate(units):
            if u in waits:
                _wait(waits[u], 'wu%d' % u)
            for g_, fu in first_use.items():
                if g_ not in wts and fu - (lead if g_ >= NF else 1) <= u:
                    back = CFG.get('wback', 8)
                    wts[g_] = wq_terms(*groups[g_], toks[-back] if len(toks) >= back else None)
            qproj(g, jp, [])
        assert all(st_[4] == st_[1] for st_ in streams) and not later, streams

    phase0()

    _wait(g3, 'wg3')

    def phase1(k_s, vt_s, wx_s, *s_s):
        def extract(h, r0, o, shift, z):
            def block(n, kq, b):
                x = wp_s[(h // 2) % 2 + z, 2 * n + b, 256 * kq + r0:256 * kq + r0 + 16, :]
                if isinstance(h, int):
                    return _lo(x) if h % 2 == 0 else _hi(x)
                return _hi(x << jnp.concatenate([shift] * 2, axis=0))

            blk = [[[[block(N, 2 * K + k, n) for n in range(2)] for k in range(2)]
                    for N in range(2)] for K in range(2)]
            terms = [t.astype(BF16) for _, _, t in list(_terms2(_rhs_terms, blk))[7 * o:7 * (o + 1)]]
            for i, t in enumerate(terms):
                wx_s[7 * o + i, r0:r0 + 16, :] = t
            return _digest(terms)

        LATE = CFG.get('late', (2, 5))
        EARLY = tuple(o for o in (0, 1, 3, 4, 6, 2, 5) if o not in LATE)
        for r0 in range(0, 256, 16):
            for o in EARLY:
                extract(0, r0, o, None, 0)

        UN = CFG.get('unroll', 1)

        def heads(it, carry):
            @pl.when(it == 1)
            def _():
                for c_ in g4:
                    c_.start()

            @pl.when(jnp.logical_and(it % 2 == 1, it < H - 1))
            def _():
                _wait(kv_copies((it + 1) // 2), 'wkv')

            @pl.when(jnp.logical_and(jnp.logical_and(it % 2 == 0, it > 0), it < H - 2))
            def _():
                for c_ in kv_copies(it // 2 + 1):
                    c_.start()

            zero = it // H
            toks = []
            due = []
            for r in range(UN):
                head(it * UN + r, None if UN % 2 else r % 2, zero, toks, due)
            return carry + zero

        def head(h, par, zero, toks, due):
            lane8 = lax.broadcasted_iota(I32, (8, 128), 1)
            sub8 = lax.broadcasted_iota(I32, (8, 128), 0)
            lane16 = lax.broadcasted_iota(I32, (16, 128), 1)
            sub16 = lax.broadcasted_iota(I32, (16, 128), 0)
            tri = (lax.broadcasted_iota(I32, (128, 128), 0) <= lax.broadcasted_iota(I32, (128, 128), 1))
            h_next = h + 1 if isinstance(h, int) else jnp.minimum(h + 1, H - 1)
            never = _never(zero)

            def after(x, tok):
                return _after(x, tok, never)

            def tied(lhs):
                return _tied(lhs, due, never)

            def tok(back):
                return toks[-back] if (back and len(toks) >= back) else None

            def chan_mm(c, gate):
                m_b = lane8 < after(128 - 2 * sub8, gate)
                gs = [jnp.broadcast_to(g_s[a, pl.ds(c, 1), :], (8, 128)) for a in range(NB)]
                bt = [pltpu.roll(jnp.where(m_b, gs[a], gs[a - 1] if a > 0 else jnp.uint32(0)), 0, 1,
                                 stride=2, stride_axis=0) for a in range(NB)]
                b1 = pltpu.bitcast(jnp.concatenate(bt[7::-1], axis=0), BF16)
                b2 = pltpu.bitcast(jnp.concatenate(bt[15:7:-1], axis=0), BF16)
                am = pltpu.bitcast(aw_s[pl.ds(c, 64, stride=PITCH), :], BF16)
                tick('C', 48)
                z1 = _dot(tied(am), b1)
                z2 = _dot(am[:64], b2)
                return c, z1[:64], z1[64:] + z2

            def chan_post(c, zlo, zhi):
                acc = car = None
                for p in range(8):
                    z = jnp.concatenate([zlo[8 * p:8 * p + 8], zhi[8 * p:8 * p + 8]], axis=0)
                    if p == 0:
                        acc = z
                    else:
                        z = pltpu.roll(z, 16 * p, 1)
                        cz = jnp.where(lane16 < 16 * p, z, 0.0)
                        acc = acc + z
                        car = cz if car is None else car + cz
                y = (acc - car) + jnp.where(sub16 > 0, pltpu.roll(car, 1, 0), 0.0)
                later(CFG.get('ly', 0), [y])
                if CFG.get('ylate'):
                    ys.append((c, y))
                else:
                    y_s[pl.ds(c, NB, stride=PITCH), :] = pltpu.bitcast(y, U32)
                if CFG.get('pd', 0):
                    due.append(y[:8])
                    due.append(y[8:])

            chans = [h * CPH + i for i in range(CPH)]
            ys, cs = [], []

            def x_stream(hh, outers):
                n = 16 * len(outers)
                for r0 in range(0, 256, 16):
                    for o in outers:
                        n -= 1
                        free = n < CFG.get('xfree', 0) and hh is h_next
                        d = extract(hh, r0, o, shift_of(hh, tok(CFG.get('xfb', 1)) if free else None), zero * (o + 1))
                        yield None if free else d

            streams = [[x_stream(h_next, EARLY), 16 * len(EARLY), 0, 0] + list(CFG['x1']),
                       [x_stream(h, LATE), 16 * len(LATE), 0, 0] + list(CFG['x2'])]

            clock, queue = [0], []

            def later(lag, vals):
                if lag:
                    queue.append((clock[0] + lag, _digest(vals)))

            def tick(kind, cycles):
                due.extend(v for t, v in queue if t <= clock[0])
                queue[:] = [q for q in queue if q[0] > clock[0]]
                clock[0] += cycles
                for st_ in streams:
                    gen, n, done, clk, kinds, c0, c1 = st_
                    if kind in kinds:
                        want = min(n, max(0, (clk - c0) * n // (c1 - c0)))
                        while st_[2] < want:
                            d = next(gen)
                            if d is not None:
                                due.append(d)
                            st_[2] += 1
                        st_[3] += cycles

            def shift_of(hh, gate):
                return after(jnp.full((8, 128), (1 - hh % 2) * 16, I32).astype(U32), gate)

            def kv_chunk(ck):
                def prod(o):
                    out = {}

                    def inner(i):
                        tick('M', 64)
                        lhs = jnp.concatenate([cs_s[ck, 7 * o + i, 0], cs_s[ck, 7 * o + i, 1]], axis=1)
                        m = _dot(tied(lhs), wx_s[7 * o + i])
                        if i == CFG.get('ti', 3):
                            toks.append(m[:8])
                        return m

                    _strassen(inner, lambda r, n, val: out.__setitem__((r, n), val))
                    return jnp.concatenate(
                        [jnp.concatenate([out[r, 0], out[r, 1]], axis=1) for r in range(2)], axis=0)

                def emit(R, N, val):
                    if N == 0:
                        rows = slice(512 * ck + 256 * R, 512 * ck + 256 * (R + 1))
                        val = val.astype(BF16)
                        k_s[0, rows, :] = val[:, :128]
                        k_s[1, rows, :] = val[:, 128:]
                    else:
                        for r in range(2):
                            for n in range(2):
                                v = val[128 * r:128 * (r + 1), 128 * n:128 * (n + 1)].T.astype(BF16)
                                vt_s[4 * ck + 2 * R + r, 128 * n:128 * (n + 1), :] = v
                                later(CFG.get('lv', 0), [v[112:]])

                return _strassen_steps(prod, emit)

            kv = [kv_chunk(ck) for ck in range(4)]

            def k_rows(r0, r1):
                return jnp.concatenate([k_s[0, r0:r1, :], k_s[1, r0:r1, :]], axis=1)

            def q_cols(r0, r1):
                return jnp.concatenate([qc_s[h, t] for t in range(r0 // 128, r1 // 128)], axis=1)

            mx, pr = {}, {}

            def qk(t):
                q0 = t * TQ
                if q0 > 0:
                    QR = CFG.get('qr', 2048)
                    rect = []
                    for r0 in range(0, q0, QR):
                        for e in CFG.get('qe', {}).get((t, r0 // QR), '').split():
                            softmax(int(e[0]), int(e[1]), True)
                        tick('Q', min(QR, q0 - r0) * 2)
                        rect.append(_dot(tied(k_rows(r0, min(q0, r0 + QR))), q_cols(q0, q0 + TQ)))
                    s_rect = jnp.concatenate(rect, axis=0) if len(rect) > 1 else rect[0]
                    toks.append(s_rect[:8, :128])
                for u in range(TQ // 128):
                    qs = q0 + u * 128
                    if u == 0:
                        for e in CFG.get('qe', {}).get((t, 'd'), '').split():
                            softmax(int(e[0]), int(e[1]), True)
                    tick('Q', 64 * (u + 1))
                    sd = _dot(tied(k_rows(q0, qs + 128)), q_cols(qs, qs + 128))
                    parts = []
                    if q0 > 0:
                        parts.append(s_rect[:, u * 128:(u + 1) * 128])
                    if u > 0:
                        parts.append(sd[:u * 128, :])
                    parts.append(jnp.where(tri, sd[u * 128:, :], NEG))
                    s = jnp.concatenate(parts, axis=0) if len(parts) > 1 else parts[0]
                    s_s[t % 2][u, 0:qs + 128, :] = s
                    mx[(t, u)] = jnp.max(s, axis=0, keepdims=True)
                toks.append(sd[:8])
                if CFG.get('clob', 1):
                    s_s[t % 2][zero, S:S + 8, :] = sd[:8]

            def softmax(t, u, deadline):
                qs = t * TQ + u * 128
                p = jnp.exp2(s_s[t % 2][u if CFG.get('clob', 1) else u + zero, 0:qs + 128, :] - mx.pop((t, u)))
                NA = CFG.get('na', 0)
                if NA:
                    accs = [None] * NA
                    for r in range(p.shape[0] // 8):
                        v = p[8 * r:8 * (r + 1)]
                        accs[r % NA] = v if accs[r % NA] is None else accs[r % NA] + v
                    while len(accs) > 1:
                        accs = [a + b for a, b in zip(accs[::2], accs[1::2])]
                    part = accs[0]
                    rl = 1.0 / jnp.sum(part, axis=0, keepdims=True)
                else:
                    rl = part = 1.0 / jnp.sum(p, axis=0, keepdims=True)
                pb = p.astype(BF16)
                pr[(t, u)] = (pb, rl)
                if deadline:
                    due.append(part)
                    if CFG.get('pk'):
                        due.append(_digest([pb]))

            def pv(t, u):
                if (t, u) not in pr:
                    softmax(t, u, False)
                p, rl = pr.pop((t, u))
                qs = t * TQ + u * 128
                vt = jnp.concatenate([vt_s[i] for i in range(qs // 128 + 1)], axis=1)
                PH = D // CFG.get('ph', 1)
                for d0 in range(0, D, PH):
                    tick('P', (qs + 128) * PH // 512)
                    ctx = _dot(tied(vt[d0:d0 + PH]), p)
                    v = (ctx * rl).astype(BF16)
                    later(CFG.get('lc', 0), [v])
                    if CFG.get('clate'):
                        cs.append((qs // 128, d0, PH, v))
                    else:
                        qc_s[h, qs // 128, d0:d0 + PH, :] = v
                toks.append(ctx[:8])

            CG, XG = CFG.get('cg', 0), CFG.get('xg', 0)
            pend = []
            def run_step(st_):
                kind, arg = st_[0], st_[1:]
                if kind == 'E':
                    softmax(int(arg[0]), int(arg[1]), True)
                    return
                old = list(pend)
                pend.clear()
                if kind == 'C':
                    for _ in range(int(arg)):
                        pend.append(chan_mm(chans.pop(0), tok(CG)))
                elif kind == 'M':
                    for o in arg[1:]:
                        kv[int(arg[0])](int(o))
                elif kind == 'Q':
                    qk(int(arg))
                elif kind == 'P':
                    for u in ([int(arg[1])] if len(arg) > 1 else range(TQ // 128)):
                        pv(int(arg[0]), u)
                for args in old:
                    chan_post(*args)

            for seg in [g for g in CFG['sched'].split('|') if g.strip()]:
                if CFG.get('scopes') and '|' in CFG['sched']:
                    with jax.named_scope('s_' + seg.split()[0]):
                        for st_ in seg.split():
                            run_step(st_)
                else:
                    for st_ in seg.split():
                        run_step(st_)
            for c, y in ys:
                y_s[pl.ds(c, NB, stride=PITCH), :] = pltpu.bitcast(y, U32)
            for t, d0, n, v in cs:
                qc_s[h, t, d0:d0 + n, :] = v
            assert all(st_[1] == st_[2] for st_ in streams), [st_[1:] for st_ in streams]
            assert CFG.get('noassert') or not chans and not pend and (not due or CFG.get('pd')) and not pr and not mx

        if CFG.get('p1', 1):
            return lax.fori_loop(0, H // UN, heads, 0)
        else:
            _wait(g3b, 'wg3b')
            for c_ in g4:
                c_.start()

            def keep(h, carry):
                r = pl.multiple_of(h * 16, 16)
                t = (qc_s[h, h, 0:16, :].astype(F32) + cs_s[h % 4, h, h % 2, 0:16, :].astype(F32)
                     + pltpu.bitcast(aw_s[pl.ds(r, 16), :] + g_s[h, pl.ds(r, 16), :], F32)
                     + wx_s[h, pl.ds(r, 16), :].astype(F32))
                y_s[pl.ds(r, 16), :] = pltpu.bitcast(t, U32)
                return carry + h // H
            return lax.fori_loop(0, H, keep, 0)

    zero_end = phase1(k_s, vt_s, wx_s, sa_s, sb_s)

    def phase2():
        _wait(g4, 'wg4')
        HH = H // 2

        def wo_block(rh, kh):
            return jnp.concatenate(
                [xs_s[C * (H * b + h) + CH * rh:C * (H * b + h) + CH * (rh + 1), :]
                 for h in range(HH * kh, HH * (kh + 1)) for b in range(2)], axis=1)

        raw = [wo_block(0, 0), wo_block(1, 0), wo_block(0, 1), wo_block(1, 1)]
        wt = [t.astype(BF16) for t in _rhs_terms(*[t.astype(F32) for t in raw])]
        wt[1], wt[4] = raw[0], raw[3]
        outs = []
        due, late = [], []
        DL = CFG.get('dl', 3)
        never = _never(zero_end)

        def put(t, b, z, opaque=False):
            o = z.T.astype(BF16)
            r0 = pl.multiple_of(zero_end * 16 + 128 * t, 16) if opaque else 128 * t
            c_s[b, pl.ds(r0, 128), :] = o
            late.append(pltpu.bitcast(o[112:], U32))

        for jp in range(CFG.get('np2', NP) if CFG.get('p2', 1) else 0):
            def ctx_block(r, kh):
                return jnp.concatenate([qc_s[h, 2 * jp + r] for h in range(HH * kh, HH * (kh + 1))], axis=0)

            craw = [ctx_block(0, 0), ctx_block(0, 1), ctx_block(1, 0), ctx_block(1, 1)]
            ct = [t.astype(BF16) for t in _lhs_terms(*[t.astype(F32) for t in craw])]
            ct[2], ct[3] = craw[0], craw[3]
            za = {}
            prev_late = list(late)
            late.clear()
            for r in range(2):
                t = 2 * jp + r
                za[r] = (pltpu.bitcast(y_s[t * PITCH:t * PITCH + C, :], F32)
                         * x_s[:, 128 * t:128 * (t + 1)].astype(F32))
                for b in range(3):
                    put(t, b, za[r][128 * b:128 * (b + 1)], opaque=(r == 0 and b == 0 and jp > 0))
            a_late = list(late)
            late.clear()
            res = {}
            count = [0]

            def prod(i):
                if count[0] == DL:
                    due.extend(prev_late)
                if count[0] == 6:
                    due.extend(a_late)
                count[0] += 1
                return _dot(_tied(wt[i], due, never), ct[i])

            _strassen(prod, lambda r, c, val: res.__setitem__((r, c), val), order=(1, 4, 3, 2, 0, 5, 6))
            for r in (1, 0):
                z = jnp.concatenate([za[r][384:], res[(r, 0)], res[(r, 1)]], axis=0)
                for b in (3, 2, 1, 0):
                    put(2 * jp + r, 3 + b, z[128 * b:128 * (b + 1)])
            rows = pl.ds(128 * jp, 128)
            for b in range(7):
                oc = cp(c_w.at[b, rows], o_hbm.at[rows, pl.ds(128 * b, 128)], 26 + jp)
                oc.start()
                outs.append(oc)
        if not CFG.get('p2', 1):
            def keep(h, carry):
                r = pl.multiple_of(h * 16, 16)
                c_s[0, pl.ds(r, 16), :] = pltpu.bitcast(y_s[pl.ds(r, 16), :], F32).astype(BF16) + qc_s[h, h, 0:16, :]
                return carry
            lax.fori_loop(0, H, keep, 0)
            oc = cp(c_w.at[0, pl.ds(0, 128)], o_hbm.at[pl.ds(0, 128), pl.ds(0, 128)], 26)
            oc.start()
            outs.append(oc)
        _wait(outs, 'wout')

    phase2()


def _tiles(w):
    rows = w.shape[0]
    return w.reshape(rows, 2, 8, 2, 128).transpose(0, 1, 3, 2, 4).reshape(rows, 32, 128)


@jax.jit
def pallas_concat_heads__ssm_conv_h3__compressed_kv_cla__prompt_kernel(
    A_q: jax.Array,
    A_k: jax.Array,
    A_v: jax.Array,
    A_shift_k: jax.Array,
    A_ssm_k: jax.Array,
    A_ssm_D: jax.Array,
    B_x: jax.Array,
    B_c_kv: jax.Array,
    B_w_q: jax.Array,
    B_w_uk: jax.Array,
    B_w_uv: jax.Array,
    B_w_o: jax.Array,
):
    hbm = pl.BlockSpec(memory_space=pltpu.HBM)
    out = pl.pallas_call(
        _kernel,
        in_specs=[hbm] * 12,
        out_specs=hbm,
        out_shape=jax.ShapeDtypeStruct((S, 2 * C), BF16),
        scratch_shapes=[
            pltpu.VMEM((8, S // 2, 128), U32),
            pltpu.VMEM((4, 49, 2, 64, 128), U32),
            pltpu.VMEM((2, 4, DC, 128), U32),
            pltpu.VMEM((H, NB, D // 2, 128), U32),
            pltpu.VMEM((64 * PITCH, 128), U32),
            pltpu.VMEM((NB, C, 128), U32),
            pltpu.VMEM((NB * PITCH, 128), U32),
            pltpu.VMEM((CH, S), U32),
            pltpu.VMEM((512, 128), F32),
            pltpu.VMEM((2, S // 2, 128), U32),
            pltpu.VMEM((NB, D // 2, 128), U32),
            pltpu.VMEM((49, DC // 8, 128), U32),
            pltpu.VMEM((TQ // 128, S + 8, 128), F32),
            pltpu.VMEM((TQ // 128, S + 8, 128), F32),
            pltpu.VMEM((CH, S), U32),
            pltpu.VMEM((7 * NP * 128, 128), U32),
            pltpu.VMEM((CH, S), U32),
            pltpu.VMEM((CH, S), U32),
            pltpu.VMEM((4, C), BF16),
            pltpu.VMEM((C,), BF16),
            pltpu.SemaphoreType.DMA((35,)),
        ],
        compiler_params=pltpu.CompilerParams(vmem_limit_bytes=127 * 2 ** 20),
    )(
        A_q[0].T, A_k[0].T, A_v[0].T, A_shift_k.T, A_ssm_k, A_ssm_D, B_x[0].T, B_c_kv[0],
        _tiles(B_w_q), _tiles(B_w_uk), _tiles(B_w_uv),
        jnp.swapaxes(B_w_o, 1, 2).reshape(H * C, D),
    )
    return out.reshape(1, S, 2 * C)
```

```python
import math

import jax
import jax.numpy as jnp
from jax import lax
import jax.experimental.pallas as pl
import jax.experimental.pallas.tpu as pltpu

F32 = jnp.float32
BF16 = jnp.bfloat16
U32 = jnp.uint32
I32 = jnp.int32

S = 2048
C = 448
H = 16
D = 256
DC = 1024
NB = S // 128
NP = NB // 2
CH = C // 2
PITCH = 520
CPH = C // H
TQ = 512
NT = (((1,), (1,)), ((), ()))
LOG2E = math.log2(math.e)
QSCALE = (D ** -0.5) * LOG2E
NEG = -1e9 * LOG2E
HI_MASK = 0xFFFF0000
CFG = dict(nf=8,n0=3,ux=13,crl=1,gback=8,costs=(2,2,1),slack=8,clob=0,cg=3,ph=2,late=(),x2=('P',0,1),x1=('P',2200,8190),sched='M001 C2 M034 C2 M06 M101 C2 Q0 M134 C2 M16 M201 C2 E00 E01 E02 E03 Q1 M234 C2 M26 M301 C2 E10 E11 Q2 M334 C2 E12 M36 E13 M02 C2 Q3 M05 C2 E20 M12 C2 E21 M15 C2 E22 M22 C2 E23 M25 C2 E30 M32 M35 E31 P0 P1 P2 P3')


def _wait(copies, name):
    if CFG.get('scopes'):
        with jax.named_scope(name):
            for c_ in copies:
                c_.wait()
    else:
        for c_ in copies:
            c_.wait()


def _dot(a, b):
    return jnp.dot(a, b, preferred_element_type=F32)


def _dot_nt(a, b):
    return lax.dot_general(a, b, NT, preferred_element_type=F32)


def _lo(x):
    return pltpu.bitcast(x << 16, F32)


def _hi(x):
    return pltpu.bitcast(x & jnp.uint32(HI_MASK), F32)


def _pack(even, odd):
    return pltpu.pack_elementwise([even, odd], packed_dtype=BF16).astype(U32)


def _split(words):
    return jnp.concatenate([_lo(words), _hi(words)], axis=0)


def _join(x):
    n = x.shape[0] // 2
    return _pack(x[:n], x[n:])


def _head_cols(w_s, h, rows):
    out = []
    for b in range(2):
        x = w_s[b, pl.ds(h // 2, rows, stride=8), :]
        if isinstance(h, int):
            out.append(_lo(x) if h % 2 == 0 else _hi(x))
        else:
            out.append(_hi(x << ((1 - h % 2) * 16).astype(U32)))
    return out


def _lhs_terms(a11, a12, a21, a22):
    return [a11 + a22, a21 + a22, a11, a22, a11 + a12, a21 - a11, a12 - a22]


def _rhs_terms(b11, b12, b21, b22):
    return [b11 + b22, b11, b12 - b22, b21 - b11, b22, b11 + b12, b21 + b22]


_LHS_SUMS = (0, 1, 4, 5, 6)


def _strassen_steps(prod, emit):
    uses = {(0, 0): {0: 1, 3: 1, 4: -1, 6: 1}, (0, 1): {2: 1, 4: 1},
            (1, 0): {1: 1, 3: 1}, (1, 1): {0: 1, 1: -1, 2: 1, 5: 1}}
    acc = {}
    neg = {}

    def step(i):
        m = prod(i)
        for key, terms in uses.items():
            if i not in terms:
                continue
            sign = terms.pop(i)
            if key not in acc:
                acc[key] = m
                neg[key] = sign < 0
            elif neg[key]:
                assert sign > 0
                acc[key] = m - acc[key]
                neg[key] = False
            else:
                acc[key] = acc[key] + m if sign > 0 else acc[key] - m
            if not terms:
                emit(key[0], key[1], acc.pop(key))

    return step


def _strassen(prod, emit, order=(0, 1, 3, 2, 4, 5, 6)):
    step = _strassen_steps(prod, emit)
    for i in order:
        step(i)


def _terms2(terms, blk):
    outer = {(r, k): terms(blk[0][0][r][k], blk[0][1][r][k], blk[1][0][r][k], blk[1][1][r][k])
             for r in range(2) for k in range(2)}
    for o in range(7):
        for i, t in enumerate(terms(outer[0, 0][o], outer[0, 1][o], outer[1, 0][o], outer[1, 1][o])):
            yield o, i, t


def _mult(i, n):
    return i if isinstance(i, int) else pl.multiple_of(i, n)


def _never(zero):
    return lax.broadcasted_iota(I32, (8, 128), 1) < zero


def _after(x, tok, never):
    if tok is None:
        return x
    return jnp.where(never, pltpu.bitcast(tok, x.dtype), x)


def _tied(lhs, due, never):
    if not due:
        return lhs
    t = None
    for d in due:
        d = pltpu.bitcast(jnp.broadcast_to(d, (8, 128)), U32)
        t = d if t is None else t ^ d
    due.clear()
    x = pltpu.bitcast(_after(pltpu.bitcast(lhs[:16, :128], U32), t, never), BF16)
    if lhs.shape[1] > 128:
        x = jnp.concatenate([x, lhs[:16, 128:]], axis=1)
    return jnp.concatenate([x, lhs[16:]], axis=0) if lhs.shape[0] > 16 else x


def _digest(vals):
    acc = None
    words = [v if v.dtype == U32 else pltpu.bitcast(v, U32) for v in vals]
    for r in range(words[0].shape[0] // 8):
        for w in words:
            w = w[8 * r:8 * (r + 1)]
            acc = w if acc is None else acc ^ w
    return acc


class _Packed:
    def __init__(self, ref):
        self.ref = ref

    def _index(self, idx):
        idx = idx if isinstance(idx, tuple) else (idx,)
        axis = len(self.ref.shape) - 2
        if len(idx) <= axis:
            return idx + (slice(None),) * (axis + 2 - len(idx))
        r = idx[axis]
        if isinstance(r, slice):
            r = slice(None if r.start is None else r.start // 2, None if r.stop is None else r.stop // 2)
        else:
            r = pl.ds(_mult(r.start // 2, 8), r.size // 2)
        return idx[:axis] + (r,) + idx[axis + 1:]

    def __getitem__(self, idx):
        return pltpu.bitcast(self.ref[self._index(idx)], BF16)

    def __setitem__(self, idx, val):
        self.ref[self._index(idx)] = pltpu.bitcast(val, U32)


def _kernel(qa_hbm, ka_hbm, va_hbm, sk_hbm, hk_hbm, d_hbm, x_hbm, c_hbm, wq_hbm, wk_hbm, wv_hbm, wo_hbm,
            o_hbm,
            c_s, cs_s, wp_s, qc_s, aw_s, g_s, y_s, hk_s, dc_s, k_s, vt_s, wx_s, sa_s, sb_s, x_s, xs_s, ka_s, va_s, wt_s, sk_ref, d_ref, sems):
    def cp(src, dst, i):
        return pltpu.make_async_copy(src, dst, sems.at[i])

    c_w, xs_w, x_w, ka_w, va_w, hk_w, cs_w, wx_w, qc_w = c_s, xs_s, x_s, ka_s, va_s, hk_s, cs_s, wx_s, qc_s
    c_s, cs_s, qc_s, k_s, vt_s, wx_s, xs_s, x_s, ka_s, va_s, hk_s = (
        _Packed(r) for r in (c_s, cs_s, qc_s, k_s, vt_s, wx_s, xs_s, x_s, ka_s, va_s, hk_s))
    qa_hbm, ka_hbm, va_hbm, hk_hbm, x_hbm, c_hbm, wo_hbm, o_hbm = (
        r.bitcast(U32) for r in (qa_hbm, ka_hbm, va_hbm, hk_hbm, x_hbm, c_hbm, wo_hbm, o_hbm))
    wq32 = wq_hbm.bitcast(U32)
    wk32 = wk_hbm.bitcast(U32)
    wv32 = wv_hbm.bitcast(U32)
    gc = [cp(c_hbm.at[:, pl.ds(128 * b, 128)], c_w.at[b], 8 + b) for b in range(8)]

    def word_row(pair, b):
        return 8 * (pair // 4) + 4 * b + pair % 4

    def kv_copies(pair):
        return [cp(w.at[:, word_row(pair, b), :], wp_s.at[pair % 2, 2 * n + b], 16 + pair % 2)
                for n, w in enumerate((wk32, wv32)) for b in range(2)]

    g3 = kv_copies(0)
    g3b = kv_copies(1)
    g4 = [cp(qa_hbm, x_w, 21)] + [cp(wo_hbm.at[:, pl.ds(128 * b, 128)], xs_w.at[pl.ds(H * CH * b, H * CH)], 6 + b)
                                  for b in range(2)]

    def delayed(ref, rows, sg, n, gate=None):
        cur = pltpu.bitcast(ref[rows, 128 * sg:128 * (sg + 1)], U32)
        lane = lax.broadcasted_iota(I32, (8, 128), 1)
        if gate is not None:
            lane = gate(lane)
        lane = jnp.concatenate([lane] * (cur.shape[0] // 8), axis=0)
        prev = pltpu.bitcast(ref[rows, 128 * (sg - 1):128 * sg], U32) if sg > 0 else jnp.uint32(0)
        x = pltpu.roll(jnp.where(lane < 128 - n, cur, prev), n, 1)
        return pltpu.bitcast(x, BF16).astype(F32)

    def gated_t(x, gate):
        if gate is not None:
            x = jnp.concatenate([gate(x[:8]), x[8:]], axis=0)
        return x.T

    def windows(b, q, e, js, gate=None):
        out = []
        for j in js:
            parts = []
            for sg in range(2 * j - 6, 2 * j + 2):
                if sg < 0:
                    parts.append(jnp.zeros((16, 128), U32))
                else:
                    parts.append(pltpu.bitcast(sa_s[b, pl.ds(_mult(128 * sg + 32 * q + 16 * e, 16), 16), :], U32))
            plane = 32 * (j // 4) + 8 * q + 4 * e + j % 4
            win = gated_t(jnp.concatenate(parts, axis=0), gate)
            aw_s[pl.ds(_mult(plane * PITCH + 128 * b, 8), 128), :] = win
            out.append(win[120:])
        return out

    def prep_g(r0, n, gate=None):
        rows = pl.ds(_mult(r0, 16), n)
        lane = lax.broadcasted_iota(I32, (n, 128), 1)
        for a in range(NB):
            hf = hk_s[rows, 128 * a:128 * (a + 1)].astype(F32)
            hs = delayed(hk_s, rows, a, 1, gate)
            if a == 0:
                hf = jnp.where(lane == 0, hf + dc_s[rows, :], hf)
                hs = jnp.where(lane == 1, hs + dc_s[rows, :], hs)
            wrd = pltpu.pack_elementwise([hf, hs], packed_dtype=BF16).astype(U32)
            g_s[a, rows, :] = wrd
            yield _digest([wrd])

    def phase0():
        XC = 512
        NF = CFG.get('nf', 4)
        N0 = CFG.get('n0', NF)
        cq = [cp(wq32.at[:, word_row(g // 2, g % 2), :], y_s.at[pl.ds(C * g, C)],
                 0 if g < N0 else 19 if g < NF else 1 if g < 8 else 18)
              for g in range(H)]
        cx = [cp(x_hbm.at[:, pl.ds(XC * i, XC)], x_w.at[:, pl.ds(XC * i, XC)], 22 + i) for i in range(S // XC)]
        g2 = [cp(sk_hbm, sk_ref, 2), cp(d_hbm, d_ref, 20),
              cp(ka_hbm, ka_w, 3), cp(va_hbm, va_w, 4), cp(hk_hbm, hk_w, 5)]
        order = CFG.get('order', 'A')
        if order == 'A':
            ga, gb = g2, cq[8:] + gc
        else:
            ga, gb = gc, g2 + cq[8:]
        rest = cx[1:] + cq[NF:8] + ga + gb + g3 + g3b
        for c_ in [cx[0]] + cq[:NF] + rest:
            c_.start()
        zero = pl.semaphore_read(sems.at[34])
        never = _never(zero)
        due = []
        toks = []

        def pad_rows(t):
            return jnp.concatenate([t, jnp.zeros((256 - CH, 128), t.dtype)], axis=0)

        def wq_terms(j, b, gate):
            x = y_s[C * (2 * j + b):C * (2 * j + b + 1), :]
            g16 = jnp.concatenate([_after(jnp.full((8, 128), 16, U32), gate, never)] * (C // 8), axis=0)
            gm = jnp.concatenate([_after(jnp.full((8, 128), HI_MASK, U32), gate, never)] * (C // 8), axis=0)
            lo, hi = pltpu.bitcast(x << g16, F32), pltpu.bitcast(x & gm, F32)
            blocks = [pad_rows(t).T for t in (lo[:CH], hi[:CH], lo[CH:], hi[CH:])]
            if not CFG.get('q4', 1):
                return [t.astype(BF16) for t in _rhs_terms(*blocks)]
            slot = (2 * j + b) % 2
            for n, t in enumerate(blocks):
                for k in range(2):
                    wt_s[slot, 2 * n + k] = t[:, 128 * k:128 * (k + 1)]
            quarter = [[jnp.concatenate([wt_s[slot, 2 * n + k, pl.ds(e, 32, stride=4), :] for k in range(2)], axis=1)
                        for n in range(4)] for e in range(4)]
            terms = [_rhs_terms(*q) for q in quarter]
            out = []
            for i in range(7):
                ev, od = _pack(terms[0][i], terms[2][i]), _pack(terms[1][i], terms[3][i])
                rows = [w[8 * m:8 * (m + 1)] for m in range(4) for w in (ev, od)]
                out.append(pltpu.bitcast(jnp.concatenate(rows, axis=0), BF16))
            return out

        def x_terms(jp):
            top = slice(256 * jp, 256 * jp + 128)
            bot = slice(256 * jp + 128, 256 * jp + 256)
            for i in range(7):
                xs_s[256 * (NP * i + jp) + CH:256 * (NP * i + jp + 1), :] = jnp.zeros((256 - CH, 128), BF16)
            for r in range(0, CH, 32):
                lo, hi = slice(r // 2, r // 2 + 16), slice((CH + r) // 2, (CH + r) // 2 + 16)
                blocks = [x_w[lo, top], x_w[hi, top], x_w[lo, bot], x_w[hi, bot]]
                terms = [_join(t) for t in _lhs_terms(*[_split(t) for t in blocks])]
                terms[2], terms[3] = blocks[0], blocks[3]
                for i, t in enumerate(terms):
                    xs_w[128 * (NP * i + jp) + r // 2:128 * (NP * i + jp) + r // 2 + 16, :] = t
                yield 1, _digest(terms)

        def qproj(g, jp, waits):
            j, b = groups[g]
            for c_ in waits:
                c_.wait()
            if False:
                x_terms(jp)
                x_terms(jp + 1)

            def prod(i):
                pump()
                m = _dot(_tied(wts[g][i], due, never), xs_s[256 * (NP * i + jp):256 * (NP * i + jp + 1), :])
                toks.append(m[:8])
                return m

            def emit(r, c, val):
                val = val * QSCALE
                if CFG.get('q4', 1):
                    w = [_pack(val[32 * m:32 * m + 16], val[32 * m + 16:32 * m + 32]) for m in range(4)]
                    qc_w[2 * j + c, 2 * jp + r, 64 * b:64 * (b + 1), :] = jnp.concatenate(w, axis=0)
                else:
                    qc_s[2 * j + c, 2 * jp + r, 128 * b:128 * (b + 1), :] = val.astype(BF16)

            _strassen(prod, emit)

        def column(row):
            row = jnp.concatenate([row.astype(F32), jnp.zeros((1, 512 - C), F32)], axis=1)
            return jnp.broadcast_to(row, (128, 512)).T

        consts = {}

        def make_consts():
            consts['taps'] = [column(sk_ref[j:j + 1, :]) for j in range(4)]
            dc_s[...] = column(d_ref[...].reshape(1, C))

        def gate(x):
            back = CFG.get('gback', 6)
            return _after(x, toks[-back], never) if back else x

        def prep_u(r0, n):
            rows = slice(r0, r0 + n)
            tp = [t[rows] for t in consts['taps']]
            prev = jnp.zeros((n, 128), F32)
            for sg in range(NB):
                cols = slice(128 * sg, 128 * (sg + 1))
                ksh = ((delayed(ka_s, rows, sg, 3, gate) * tp[3] + delayed(ka_s, rows, sg, 2, gate) * tp[2])
                       + (delayed(ka_s, rows, sg, 1, gate) * tp[1] + ka_s[rows, cols].astype(F32) * tp[0]))
                kv = ksh * va_s[rows, cols].astype(F32)
                wrd = pltpu.pack_elementwise([prev, kv], packed_dtype=BF16).astype(U32)
                sb_s[sg // 4, C * (sg % 4) + r0:C * (sg % 4) + r0 + n, :] = pltpu.bitcast(wrd, F32)
                prev = kv
                yield _digest([wrd])

        def words_t(b):
            for sg in range(NB):
                r0 = C * (sg % 4) + 128 * b
                if b < 3:
                    wrd = sb_s[sg // 4, r0:r0 + 128, :]
                else:
                    wrd = jnp.concatenate([sb_s[sg // 4, r0:r0 + C - 384, :], jnp.zeros((512 - C, 128), F32)], axis=0)
                wrd = gated_t(pltpu.bitcast(wrd, U32), gate)
                sa_s[b, 128 * sg:128 * (sg + 1), :] = pltpu.bitcast(wrd, F32)
                yield wrd[120:]

        def all_windows(b):
            for p in range(8):
                for j in range(8):
                    yield windows(b, p // 2, p % 2, [j], gate)[0]

        def c_terms():
            for ck in range(4):
                for half in range(2):
                    for r0 in range(0, 128, 16):
                        def blocks(z):
                            return [[[[_split(c_w[4 * K + 2 * k + half + z,
                                                  pl.ds(256 * ck + 128 * R + 64 * r + r0 // 2, 8), :])
                                       for k in range(2)] for r in range(2)] for K in range(2)] for R in range(2)]

                        if CFG.get('crl'):
                            terms = [x for o in range(7)
                                     for x in list(_terms2(_lhs_terms, blocks(zero * (o + 1))))[7 * o:7 * (o + 1)]]
                        else:
                            terms = _terms2(_lhs_terms, blocks(0))
                        acc = None
                        for o, i, t in terms:
                            t = _join(t)
                            cs_w[ck, 7 * o + i, half, r0 // 2:r0 // 2 + 8, :] = t
                            acc = _digest([t]) if acc is None else acc ^ _digest([t])
                            if i == 6:
                                yield acc
                                acc = None

        UG = CFG.get('ug', 32)

        def a_stream():
            make_consts()
            cu, ct, cg = CFG.get('costs', (3, 2, 1))
            gs = [prep_g(r0, 32, gate) for r0 in range(0, C, 32)]
            for b in range(4):
                for r0 in range(128 * b, min(C, 128 * (b + 1)), UG):
                    for v in prep_u(r0, UG):
                        yield cu * UG // 32, v
                for v in words_t(b):
                    yield ct, v
                for v in all_windows(b):
                    yield ct, v
                if CFG.get('gpos', 'end') == 'blk' or b == 3:
                    for g_ in (gs[4 * b:4 * b + 4] if CFG.get('gpos', 'end') == 'blk' else gs):
                        for v in g_:
                            yield cg, v

        cu, ct, cg = CFG.get('costs', (3, 2, 1))
        a_total = cu * 14 * NB + ct * 4 * (NB + 64) + cg * 14 * NB
        streams = []
        nprod = [0]
        later = {}
        LAG = CFG.get('lag', 0)

        def pump():
            for st_ in streams:
                gen, n, p0, p1, done = st_
                want = min(n, max(0, (nprod[0] - p0 + 1) * n // (p1 - p0)))
                while st_[4] < want:
                    cost, v = next(gen)
                    later.setdefault(nprod[0] + LAG, []).append(v)
                    st_[4] += cost
            due.extend(later.pop(nprod[0], []))
            nprod[0] += 1

        groups = [(j, b) for j in range(H // 2) for b in range(2)]
        units = [(g, jp) for c in range(0, NP, 2) for g in range(NF) for jp in (c, c + 1)]
        units += [(g, jp) for g in range(NF, len(groups)) for jp in range(NP)]
        NU = len(units)
        wts = {}
        lead = CFG.get('lead', 4)
        ua = CFG.get('ua', 32)
        ub = 8 * NP - lead
        ux = CFG.get('ux', 5)
        waits = {ux: cx[1:] + cq[NF:8], ua: ga, ub: gb}
        if N0 < NF:
            waits[2 * N0 - 1] = cq[N0:NF]
        xe = [7 * ux + 2] + [7 * NF * 2 * c - 1 for c in (1, 2, 3)]
        for c in range(3):
            streams.append([(v for jp in (2 * c + 2, 2 * c + 3) for v in x_terms(jp)), 14, xe[c], xe[c + 1], 0])
        sl = CFG.get('slack', 4)
        PA, PB, PE = 7 * ua + sl, 7 * ub + sl, 7 * NU - 2 - LAG
        c_stream = ((1, v) for v in c_terms())
        nc = 4 * 2 * 8 * 7
        if order == 'A':
            streams.append([a_stream(), a_total, PA, PE, 0])
            streams.append([c_stream, nc, PB, PE, 0])
        else:
            streams.append([c_stream, nc, PA, CFG.get('cend', PB), 0])
            streams.append([a_stream(), a_total, PB, PE, 0])

        if not CFG.get('p0', 1):
            for c_ in cq + cx + g2 + gc:
                c_.wait()
            return
        _wait([cx[0]], 'wx0')
        list(x_terms(0))
        list(x_terms(1))
        _wait(cq[:N0], 'wq0')
        first_use = {}
        for u, (g, jp) in enumerate(units):
            first_use.setdefault(g, u)
        for u, (g, jp) in enumerate(units):
            if u in waits:
                _wait(waits[u], 'wu%d' % u)
            for g_, fu in first_use.items():
                if g_ not in wts and fu - (lead if g_ >= NF else 1) <= u:
                    back = CFG.get('wback', 8)
                    wts[g_] = wq_terms(*groups[g_], toks[-back] if len(toks) >= back else None)
            qproj(g, jp, [])
        assert all(st_[4] == st_[1] for st_ in streams) and not later, streams

    phase0()

    _wait(g3, 'wg3')

    def phase1(k_s, vt_s, wx_s, *s_s):
        def extract(h, r0, o, shift, z):
            def block(n, kq, b):
                x = jnp.concatenate([wp_s[(h // 2) % 2 + z, 2 * n + b, pl.ds(256 * kq + r0 + e, 8, stride=2), :]
                                     for e in range(2)], axis=0)
                if isinstance(h, int):
                    return _lo(x) if h % 2 == 0 else _hi(x)
                return _hi(x << jnp.concatenate([shift] * 2, axis=0))

            blk = [[[[block(N, 2 * K + k, n) for n in range(2)] for k in range(2)]
                    for N in range(2)] for K in range(2)]
            terms = [_join(t) for _, _, t in list(_terms2(_rhs_terms, blk))[7 * o:7 * (o + 1)]]
            for i, t in enumerate(terms):
                wx_w[7 * o + i, r0 // 2:r0 // 2 + 8, :] = t
            return _digest(terms)

        LATE = CFG.get('late', (2, 5))
        EARLY = tuple(o for o in (0, 1, 3, 4, 6, 2, 5) if o not in LATE)
        for r0 in range(0, 256, 16):
            for o in EARLY:
                extract(0, r0, o, None, 0)

        UN = CFG.get('unroll', 1)

        def heads(it, carry):
            @pl.when(it == 1)
            def _():
                for c_ in g4:
                    c_.start()

            @pl.when(jnp.logical_and(it % 2 == 1, it < H - 1))
            def _():
                _wait(kv_copies((it + 1) // 2), 'wkv')

            @pl.when(jnp.logical_and(jnp.logical_and(it % 2 == 0, it > 0), it < H - 2))
            def _():
                for c_ in kv_copies(it // 2 + 1):
                    c_.start()

            zero = it // H
            toks = []
            due = []
            for r in range(UN):
                head(it * UN + r, None if UN % 2 else r % 2, zero, toks, due)
            return carry + zero

        def head(h, par, zero, toks, due):
            lane8 = lax.broadcasted_iota(I32, (8, 128), 1)
            sub8 = lax.broadcasted_iota(I32, (8, 128), 0)
            lane16 = lax.broadcasted_iota(I32, (16, 128), 1)
            sub16 = lax.broadcasted_iota(I32, (16, 128), 0)
            tri = (lax.broadcasted_iota(I32, (128, 128), 0) <= lax.broadcasted_iota(I32, (128, 128), 1))
            h_next = h + 1 if isinstance(h, int) else jnp.minimum(h + 1, H - 1)
            never = _never(zero)

            def after(x, tok):
                return _after(x, tok, never)

            def tied(lhs):
                return _tied(lhs, due, never)

            def tok(back):
                return toks[-back] if (back and len(toks) >= back) else None

            def chan_mm(c, gate):
                m_b = lane8 < after(128 - 2 * sub8, gate)
                gs = [jnp.broadcast_to(g_s[a, pl.ds(c, 1), :], (8, 128)) for a in range(NB)]
                bt = [pltpu.roll(jnp.where(m_b, gs[a], gs[a - 1] if a > 0 else jnp.uint32(0)), 0, 1,
                                 stride=2, stride_axis=0) for a in range(NB)]
                b1 = pltpu.bitcast(jnp.concatenate(bt[7::-1], axis=0), BF16)
                b2 = pltpu.bitcast(jnp.concatenate(bt[15:7:-1], axis=0), BF16)
                am = pltpu.bitcast(aw_s[pl.ds(c, 64, stride=PITCH), :], BF16)
                tick('C', 48)
                z1 = _dot(tied(am), b1)
                z2 = _dot(am[:64], b2)
                return c, z1[:64], z1[64:] + z2

            def chan_post(c, zlo, zhi):
                acc = car = None
                for p in range(8):
                    z = jnp.concatenate([zlo[8 * p:8 * p + 8], zhi[8 * p:8 * p + 8]], axis=0)
                    if p == 0:
                        acc = z
                    else:
                        z = pltpu.roll(z, 16 * p, 1)
                        cz = jnp.where(lane16 < 16 * p, z, 0.0)
                        acc = acc + z
                        car = cz if car is None else car + cz
                y = (acc - car) + jnp.where(sub16 > 0, pltpu.roll(car, 1, 0), 0.0)
                later(CFG.get('ly', 0), [y])
                if CFG.get('ylate'):
                    ys.append((c, y))
                else:
                    y_s[pl.ds(c, NB, stride=PITCH), :] = pltpu.bitcast(y, U32)
                if CFG.get('pd', 0):
                    due.append(y[:8])
                    due.append(y[8:])

            chans = [h * CPH + i for i in range(CPH)]
            ys, cs = [], []

            def x_stream(hh, outers):
                n = 16 * len(outers)
                for r0 in range(0, 256, 16):
                    for o in outers:
                        n -= 1
                        free = n < CFG.get('xfree', 0) and hh is h_next
                        d = extract(hh, r0, o, shift_of(hh, tok(CFG.get('xfb', 1)) if free else None), zero * (o + 1))
                        yield None if free else d

            streams = [[x_stream(h_next, EARLY), 16 * len(EARLY), 0, 0] + list(CFG['x1']),
                       [x_stream(h, LATE), 16 * len(LATE), 0, 0] + list(CFG['x2'])]

            clock, queue = [0], []

            def later(lag, vals):
                if lag:
                    queue.append((clock[0] + lag, _digest(vals)))

            def tick(kind, cycles):
                due.extend(v for t, v in queue if t <= clock[0])
                queue[:] = [q for q in queue if q[0] > clock[0]]
                clock[0] += cycles
                for st_ in streams:
                    gen, n, done, clk, kinds, c0, c1 = st_
                    if kind in kinds:
                        want = min(n, max(0, (clk - c0) * n // (c1 - c0)))
                        while st_[2] < want:
                            d = next(gen)
                            if d is not None:
                                due.append(d)
                            st_[2] += 1
                        st_[3] += cycles

            def shift_of(hh, gate):
                return after(jnp.full((8, 128), (1 - hh % 2) * 16, I32).astype(U32), gate)

            def kv_chunk(ck):
                def prod(o):
                    out = {}

                    def inner(i):
                        tick('M', 64)
                        lhs = jnp.concatenate([cs_s[ck, 7 * o + i, 0], cs_s[ck, 7 * o + i, 1]], axis=1)
                        m = _dot(tied(lhs), wx_s[7 * o + i])
                        if i == CFG.get('ti', 3):
                            toks.append(m[:8])
                        return m

                    _strassen(inner, lambda r, n, val: out.__setitem__((r, n), val))
                    return jnp.concatenate(
                        [jnp.concatenate([out[r, 0], out[r, 1]], axis=1) for r in range(2)], axis=0)

                def emit(R, N, val):
                    if N == 0:
                        rows = slice(512 * ck + 256 * R, 512 * ck + 256 * (R + 1))
                        val = val.astype(BF16)
                        k_s[0, rows, :] = val[:, :128]
                        k_s[1, rows, :] = val[:, 128:]
                    else:
                        for r in range(2):
                            for n in range(2):
                                v = val[128 * r:128 * (r + 1), 128 * n:128 * (n + 1)].T.astype(BF16)
                                vt_s[4 * ck + 2 * R + r, 128 * n:128 * (n + 1), :] = v
                                later(CFG.get('lv', 0), [v[112:]])

                return _strassen_steps(prod, emit)

            kv = [kv_chunk(ck) for ck in range(4)]

            def k_rows(r0, r1):
                return jnp.concatenate([k_s[0, r0:r1, :], k_s[1, r0:r1, :]], axis=1)

            def q_cols(r0, r1):
                return jnp.concatenate([qc_s[h, t] for t in range(r0 // 128, r1 // 128)], axis=1)

            mx, pr = {}, {}

            def qk(t):
                q0 = t * TQ
                if q0 > 0:
                    QR = CFG.get('qr', 2048)
                    rect = []
                    for r0 in range(0, q0, QR):
                        for e in CFG.get('qe', {}).get((t, r0 // QR), '').split():
                            softmax(int(e[0]), int(e[1]), True)
                        tick('Q', min(QR, q0 - r0) * 2)
                        rect.append(_dot(tied(k_rows(r0, min(q0, r0 + QR))), q_cols(q0, q0 + TQ)))
                    s_rect = jnp.concatenate(rect, axis=0) if len(rect) > 1 else rect[0]
                    toks.append(s_rect[:8, :128])
                for u in range(TQ // 128):
                    qs = q0 + u * 128
                    if u == 0:
                        for e in CFG.get('qe', {}).get((t, 'd'), '').split():
                            softmax(int(e[0]), int(e[1]), True)
                    tick('Q', 64 * (u + 1))
                    sd = _dot(tied(k_rows(q0, qs + 128)), q_cols(qs, qs + 128))
                    parts = []
                    if q0 > 0:
                        parts.append(s_rect[:, u * 128:(u + 1) * 128])
                    if u > 0:
                        parts.append(sd[:u * 128, :])
                    parts.append(jnp.where(tri, sd[u * 128:, :], NEG))
                    s = jnp.concatenate(parts, axis=0) if len(parts) > 1 else parts[0]
                    s_s[t % 2][u, 0:qs + 128, :] = s
                    mx[(t, u)] = jnp.max(s, axis=0, keepdims=True)
                toks.append(sd[:8])
                if CFG.get('clob', 1):
                    s_s[t % 2][zero, S:S + 8, :] = sd[:8]

            def softmax(t, u, deadline):
                qs = t * TQ + u * 128
                p = jnp.exp2(s_s[t % 2][u if CFG.get('clob', 1) else u + zero, 0:qs + 128, :] - mx.pop((t, u)))
                NA = CFG.get('na', 0)
                if NA:
                    accs = [None] * NA
                    for r in range(p.shape[0] // 8):
                        v = p[8 * r:8 * (r + 1)]
                        accs[r % NA] = v if accs[r % NA] is None else accs[r % NA] + v
                    while len(accs) > 1:
                        accs = [a + b for a, b in zip(accs[::2], accs[1::2])]
                    part = accs[0]
                    rl = 1.0 / jnp.sum(part, axis=0, keepdims=True)
                else:
                    rl = part = 1.0 / jnp.sum(p, axis=0, keepdims=True)
                pb = p.astype(BF16)
                pr[(t, u)] = (pb, rl)
                if deadline:
                    due.append(part)
                    if CFG.get('pk'):
                        due.append(_digest([pb]))

            def pv(t, u):
                if (t, u) not in pr:
                    softmax(t, u, False)
                p, rl = pr.pop((t, u))
                qs = t * TQ + u * 128
                vt = jnp.concatenate([vt_s[i] for i in range(qs // 128 + 1)], axis=1)
                PH = D // CFG.get('ph', 1)
                for d0 in range(0, D, PH):
                    tick('P', (qs + 128) * PH // 512)
                    ctx = _dot(tied(vt[d0:d0 + PH]), p)
                    v = (ctx * rl).astype(BF16)
                    later(CFG.get('lc', 0), [v])
                    if CFG.get('clate'):
                        cs.append((qs // 128, d0, PH, v))
                    else:
                        qc_s[h, qs // 128, d0:d0 + PH, :] = v
                toks.append(ctx[:8])

            CG, XG = CFG.get('cg', 0), CFG.get('xg', 0)
            pend = []
            def run_step(st_):
                kind, arg = st_[0], st_[1:]
                if kind == 'E':
                    softmax(int(arg[0]), int(arg[1]), True)
                    return
                old = list(pend)
                pend.clear()
                if kind == 'C':
                    for _ in range(int(arg)):
                        pend.append(chan_mm(chans.pop(0), tok(CG)))
                elif kind == 'M':
                    for o in arg[1:]:
                        kv[int(arg[0])](int(o))
                elif kind == 'Q':
                    qk(int(arg))
                elif kind == 'P':
                    for u in ([int(arg[1])] if len(arg) > 1 else range(TQ // 128)):
                        pv(int(arg[0]), u)
                for args in old:
                    chan_post(*args)

            for seg in [g for g in CFG['sched'].split('|') if g.strip()]:
                if CFG.get('scopes') and '|' in CFG['sched']:
                    with jax.named_scope('s_' + seg.split()[0]):
                        for st_ in seg.split():
                            run_step(st_)
                else:
                    for st_ in seg.split():
                        run_step(st_)
            for c, y in ys:
                y_s[pl.ds(c, NB, stride=PITCH), :] = pltpu.bitcast(y, U32)
            for t, d0, n, v in cs:
                qc_s[h, t, d0:d0 + n, :] = v
            assert all(st_[1] == st_[2] for st_ in streams), [st_[1:] for st_ in streams]
            assert CFG.get('noassert') or not chans and not pend and (not due or CFG.get('pd')) and not pr and not mx

        if CFG.get('p1', 1):
            return lax.fori_loop(0, H // UN, heads, 0)
        else:
            _wait(g3b, 'wg3b')
            for c_ in g4:
                c_.start()

            def keep(h, carry):
                r = pl.multiple_of(h * 16, 16)
                t = (qc_s[h, h, 0:16, :].astype(F32) + cs_s[h % 4, h, h % 2, 0:16, :].astype(F32)
                     + pltpu.bitcast(aw_s[pl.ds(r, 16), :] + g_s[h, pl.ds(r, 16), :], F32)
                     + wx_s[h, pl.ds(r, 16), :].astype(F32))
                y_s[pl.ds(r, 16), :] = pltpu.bitcast(t, U32)
                return carry + h // H
            return lax.fori_loop(0, H, keep, 0)

    zero_end = phase1(k_s, vt_s, wx_s, sa_s, sb_s)

    def phase2():
        _wait(g4, 'wg4')
        HH = H // 2

        def wo_block(rh, kh):
            return jnp.concatenate(
                [xs_s[C * (H * b + h) + CH * rh:C * (H * b + h) + CH * (rh + 1), :]
                 for h in range(HH * kh, HH * (kh + 1)) for b in range(2)], axis=1)

        raw = [wo_block(0, 0), wo_block(1, 0), wo_block(0, 1), wo_block(1, 1)]
        wt = [t.astype(BF16) for t in _rhs_terms(*[t.astype(F32) for t in raw])]
        wt[1], wt[4] = raw[0], raw[3]
        outs = []
        due, late = [], []
        DL = CFG.get('dl', 3)
        never = _never(zero_end)

        def put(t, b, z, opaque=False):
            o = z.T.astype(BF16)
            r0 = pl.multiple_of(zero_end * 16 + 128 * t, 16) if opaque else 128 * t
            c_s[b, pl.ds(r0, 128), :] = o
            late.append(pltpu.bitcast(o[112:], U32))

        for jp in range(CFG.get('np2', NP) if CFG.get('p2', 1) else 0):
            def ctx_block(r, kh):
                return jnp.concatenate([qc_s[h, 2 * jp + r] for h in range(HH * kh, HH * (kh + 1))], axis=0)

            craw = [ctx_block(0, 0), ctx_block(0, 1), ctx_block(1, 0), ctx_block(1, 1)]
            ct = [t.astype(BF16) for t in _lhs_terms(*[t.astype(F32) for t in craw])]
            ct[2], ct[3] = craw[0], craw[3]
            za = {}
            prev_late = list(late)
            late.clear()
            for r in range(2):
                t = 2 * jp + r
                za[r] = (pltpu.bitcast(y_s[t * PITCH:t * PITCH + C, :], F32)
                         * x_s[:, 128 * t:128 * (t + 1)].astype(F32))
                for b in range(3):
                    put(t, b, za[r][128 * b:128 * (b + 1)], opaque=(r == 0 and b == 0 and jp > 0))
            a_late = list(late)
            late.clear()
            res = {}
            count = [0]

            def prod(i):
                if count[0] == DL:
                    due.extend(prev_late)
                if count[0] == 6:
                    due.extend(a_late)
                count[0] += 1
                return _dot(_tied(wt[i], due, never), ct[i])

            _strassen(prod, lambda r, c, val: res.__setitem__((r, c), val), order=(1, 4, 3, 2, 0, 5, 6))
            for r in (1, 0):
                z = jnp.concatenate([za[r][384:], res[(r, 0)], res[(r, 1)]], axis=0)
                for b in (3, 2, 1, 0):
                    put(2 * jp + r, 3 + b, z[128 * b:128 * (b + 1)])
            rows = pl.ds(128 * jp, 128)
            for b in range(7):
                oc = cp(c_w.at[b, rows], o_hbm.at[rows, pl.ds(128 * b, 128)], 26 + jp)
                oc.start()
                outs.append(oc)
        if not CFG.get('p2', 1):
            def keep(h, carry):
                r = pl.multiple_of(h * 16, 16)
                c_s[0, pl.ds(r, 16), :] = pltpu.bitcast(y_s[pl.ds(r, 16), :], F32).astype(BF16) + qc_s[h, h, 0:16, :]
                return carry
            lax.fori_loop(0, H, keep, 0)
            oc = cp(c_w.at[0, pl.ds(0, 128)], o_hbm.at[pl.ds(0, 128), pl.ds(0, 128)], 26)
            oc.start()
            outs.append(oc)
        _wait(outs, 'wout')

    phase2()


def _tiles(w):
    rows = w.shape[0]
    return w.reshape(rows, 2, 8, 2, 128).transpose(0, 1, 3, 2, 4).reshape(rows, 32, 128)


@jax.jit
def pallas_concat_heads__ssm_conv_h3__compressed_kv_cla__prompt_kernel(
    A_q: jax.Array,
    A_k: jax.Array,
    A_v: jax.Array,
    A_shift_k: jax.Array,
    A_ssm_k: jax.Array,
    A_ssm_D: jax.Array,
    B_x: jax.Array,
    B_c_kv: jax.Array,
    B_w_q: jax.Array,
    B_w_uk: jax.Array,
    B_w_uv: jax.Array,
    B_w_o: jax.Array,
):
    hbm = pl.BlockSpec(memory_space=pltpu.HBM)
    out = pl.pallas_call(
        _kernel,
        in_specs=[hbm] * 12,
        out_specs=hbm,
        out_shape=jax.ShapeDtypeStruct((S, 2 * C), BF16),
        scratch_shapes=[
            pltpu.VMEM((8, S // 2, 128), U32),
            pltpu.VMEM((4, 49, 2, 64, 128), U32),
            pltpu.VMEM((2, 4, DC, 128), U32),
            pltpu.VMEM((H, NB, D // 2, 128), U32),
            pltpu.VMEM((64 * PITCH, 128), U32),
            pltpu.VMEM((NB, C, 128), U32),
            pltpu.VMEM((NB * PITCH, 128), U32),
            pltpu.VMEM((CH, S), U32),
            pltpu.VMEM((512, 128), F32),
            pltpu.VMEM((2, S // 2, 128), U32),
            pltpu.VMEM((NB, D // 2, 128), U32),
            pltpu.VMEM((49, DC // 8, 128), U32),
            pltpu.VMEM((TQ // 128, S + 8, 128), F32),
            pltpu.VMEM((TQ // 128, S + 8, 128), F32),
            pltpu.VMEM((CH, S), U32),
            pltpu.VMEM((7 * NP * 128, 128), U32),
            pltpu.VMEM((CH, S), U32),
            pltpu.VMEM((CH, S), U32),
            pltpu.VMEM((2, 8, 128, 128), F32),
            pltpu.VMEM((4, C), BF16),
            pltpu.VMEM((C,), BF16),
            pltpu.SemaphoreType.DMA((35,)),
        ],
        compiler_params=pltpu.CompilerParams(vmem_limit_bytes=127 * 2 ** 20),
    )(
        A_q[0].T, A_k[0].T, A_v[0].T, A_shift_k.T, A_ssm_k, A_ssm_D, B_x[0].T, B_c_kv[0],
        _tiles(B_w_q), _tiles(B_w_uk), _tiles(B_w_uv),
        jnp.swapaxes(B_w_o, 1, 2).reshape(H * C, D),
    )
    return out.reshape(1, S, 2 * C)
```

```python
import math

import jax
import jax.numpy as jnp
from jax import lax
import jax.experimental.pallas as pl
import jax.experimental.pallas.tpu as pltpu

F32 = jnp.float32
BF16 = jnp.bfloat16
U32 = jnp.uint32
I32 = jnp.int32

S = 2048
C = 448
H = 16
D = 256
DC = 1024
NB = S // 128
NP = NB // 2
CH = C // 2
PITCH = 520
CPH = C // H
TQ = 512
NT = (((1,), (1,)), ((), ()))
LOG2E = math.log2(math.e)
QSCALE = (D ** -0.5) * LOG2E
NEG = -1e9 * LOG2E
HI_MASK = 0xFFFF0000
CFG = dict(ua=30,ud=96,nf=8,n0=3,ux=13,crl=1,gback=8,slack=8,clob=0,cg=3,ph=2,late=(),x2=('P',0,1),x1=('P',2200,8190),sched='M001 C2 M034 C2 M06 M101 C2 Q0 M134 C2 M16 M201 C2 E00 E01 E02 E03 Q1 M234 C2 M26 M301 C2 E10 E11 Q2 M334 C2 E12 M36 E13 M02 C2 Q3 M05 C2 E20 M12 C2 E21 M15 C2 E22 M22 C2 E23 M25 C2 E30 M32 M35 E31 P0 P1 P2 P3')


def _wait(copies, name):
    if CFG.get('scopes'):
        with jax.named_scope(name):
            for c_ in copies:
                c_.wait()
    else:
        for c_ in copies:
            c_.wait()


def _dot(a, b):
    return jnp.dot(a, b, preferred_element_type=F32)


def _dot_nt(a, b):
    return lax.dot_general(a, b, NT, preferred_element_type=F32)


def _lo(x):
    return pltpu.bitcast(x << 16, F32)


def _hi(x):
    return pltpu.bitcast(x & jnp.uint32(HI_MASK), F32)


def _pack(even, odd):
    return pltpu.pack_elementwise([even, odd], packed_dtype=BF16).astype(U32)


def _split(words):
    return jnp.concatenate([_lo(words), _hi(words)], axis=0)


def _join(x):
    n = x.shape[0] // 2
    return _pack(x[:n], x[n:])


def _head_cols(w_s, h, rows):
    out = []
    for b in range(2):
        x = w_s[b, pl.ds(h // 2, rows, stride=8), :]
        if isinstance(h, int):
            out.append(_lo(x) if h % 2 == 0 else _hi(x))
        else:
            out.append(_hi(x << ((1 - h % 2) * 16).astype(U32)))
    return out


def _lhs_terms(a11, a12, a21, a22):
    return [a11 + a22, a21 + a22, a11, a22, a11 + a12, a21 - a11, a12 - a22]


def _rhs_terms(b11, b12, b21, b22):
    return [b11 + b22, b11, b12 - b22, b21 - b11, b22, b11 + b12, b21 + b22]


_LHS_SUMS = (0, 1, 4, 5, 6)


def _strassen_steps(prod, emit):
    uses = {(0, 0): {0: 1, 3: 1, 4: -1, 6: 1}, (0, 1): {2: 1, 4: 1},
            (1, 0): {1: 1, 3: 1}, (1, 1): {0: 1, 1: -1, 2: 1, 5: 1}}
    acc = {}
    neg = {}

    def step(i):
        m = prod(i)
        for key, terms in uses.items():
            if i not in terms:
                continue
            sign = terms.pop(i)
            if key not in acc:
                acc[key] = m
                neg[key] = sign < 0
            elif neg[key]:
                assert sign > 0
                acc[key] = m - acc[key]
                neg[key] = False
            else:
                acc[key] = acc[key] + m if sign > 0 else acc[key] - m
            if not terms:
                emit(key[0], key[1], acc.pop(key))

    return step


def _strassen(prod, emit, order=(0, 1, 3, 2, 4, 5, 6)):
    step = _strassen_steps(prod, emit)
    for i in order:
        step(i)


def _terms2(terms, blk):
    outer = {(r, k): terms(blk[0][0][r][k], blk[0][1][r][k], blk[1][0][r][k], blk[1][1][r][k])
             for r in range(2) for k in range(2)}
    for o in range(7):
        for i, t in enumerate(terms(outer[0, 0][o], outer[0, 1][o], outer[1, 0][o], outer[1, 1][o])):
            yield o, i, t


def _mult(i, n):
    return i if isinstance(i, int) else pl.multiple_of(i, n)


def _never(zero):
    return lax.broadcasted_iota(I32, (8, 128), 1) < zero


def _after(x, tok, never):
    if tok is None:
        return x
    return jnp.where(never, pltpu.bitcast(tok, x.dtype), x)


def _tied(lhs, due, never):
    if not due:
        return lhs
    t = None
    for d in due:
        d = pltpu.bitcast(jnp.broadcast_to(d, (8, 128)), U32)
        t = d if t is None else t ^ d
    due.clear()
    x = pltpu.bitcast(_after(pltpu.bitcast(lhs[:16, :128], U32), t, never), BF16)
    if lhs.shape[1] > 128:
        x = jnp.concatenate([x, lhs[:16, 128:]], axis=1)
    return jnp.concatenate([x, lhs[16:]], axis=0) if lhs.shape[0] > 16 else x


def _digest(vals):
    acc = None
    words = [v if v.dtype == U32 else pltpu.bitcast(v, U32) for v in vals]
    for r in range(words[0].shape[0] // 8):
        for w in words:
            w = w[8 * r:8 * (r + 1)]
            acc = w if acc is None else acc ^ w
    return acc


class _Packed:
    def __init__(self, ref):
        self.ref = ref

    def _index(self, idx):
        idx = idx if isinstance(idx, tuple) else (idx,)
        axis = len(self.ref.shape) - 2
        if len(idx) <= axis:
            return idx + (slice(None),) * (axis + 2 - len(idx))
        r = idx[axis]
        if isinstance(r, slice):
            r = slice(None if r.start is None else r.start // 2, None if r.stop is None else r.stop // 2)
        else:
            r = pl.ds(_mult(r.start // 2, 8), r.size // 2)
        return idx[:axis] + (r,) + idx[axis + 1:]

    def __getitem__(self, idx):
        return pltpu.bitcast(self.ref[self._index(idx)], BF16)

    def __setitem__(self, idx, val):
        self.ref[self._index(idx)] = pltpu.bitcast(val, U32)


def _kernel(qa_hbm, ka_hbm, va_hbm, sk_hbm, hk_hbm, d_hbm, x_hbm, c_hbm, wq_hbm, wk_hbm, wv_hbm, wo_hbm,
            o_hbm,
            c_s, cs_s, wp_s, qc_s, aw_s, g_s, y_s, hk_s, dc_s, k_s, vt_s, wx_s, sa_s, sb_s, x_s, xs_s, ka_s, va_s, wt_s, sk_ref, d_ref, sems):
    def cp(src, dst, i):
        return pltpu.make_async_copy(src, dst, sems.at[i])

    c_w, xs_w, x_w, ka_w, va_w, hk_w, cs_w, wx_w, qc_w = c_s, xs_s, x_s, ka_s, va_s, hk_s, cs_s, wx_s, qc_s
    c_s, cs_s, qc_s, k_s, vt_s, wx_s, xs_s, x_s, ka_s, va_s, hk_s = (
        _Packed(r) for r in (c_s, cs_s, qc_s, k_s, vt_s, wx_s, xs_s, x_s, ka_s, va_s, hk_s))
    qa_hbm, ka_hbm, va_hbm, hk_hbm, x_hbm, c_hbm, wo_hbm, o_hbm = (
        r.bitcast(U32) for r in (qa_hbm, ka_hbm, va_hbm, hk_hbm, x_hbm, c_hbm, wo_hbm, o_hbm))
    wq32 = wq_hbm.bitcast(U32)
    wk32 = wk_hbm.bitcast(U32)
    wv32 = wv_hbm.bitcast(U32)
    gc = [cp(c_hbm.at[:, pl.ds(128 * b, 128)], c_w.at[b], 8 + b) for b in range(8)]

    def word_row(pair, b):
        return 8 * (pair // 4) + 4 * b + pair % 4

    def kv_copies(pair):
        return [cp(w.at[:, word_row(pair, b), :], wp_s.at[pair % 2, 2 * n + b], 16 + pair % 2)
                for n, w in enumerate((wk32, wv32)) for b in range(2)]

    g3 = kv_copies(0)
    g3b = kv_copies(1)
    g4 = [cp(qa_hbm, x_w, 21)] + [cp(wo_hbm.at[:, pl.ds(128 * b, 128)], xs_w.at[pl.ds(H * CH * b, H * CH)], 6 + b)
                                  for b in range(2)]

    def delayed(ref, rows, sg, n, gate=None):
        cur = pltpu.bitcast(ref[rows, 128 * sg:128 * (sg + 1)], U32)
        lane = lax.broadcasted_iota(I32, (8, 128), 1)
        if gate is not None:
            lane = gate(lane)
        lane = jnp.concatenate([lane] * (cur.shape[0] // 8), axis=0)
        prev = pltpu.bitcast(ref[rows, 128 * (sg - 1):128 * sg], U32) if sg > 0 else jnp.uint32(0)
        x = pltpu.roll(jnp.where(lane < 128 - n, cur, prev), n, 1)
        return pltpu.bitcast(x, BF16).astype(F32)

    def gated_t(x, gate):
        if gate is not None:
            x = jnp.concatenate([gate(x[:8]), x[8:]], axis=0)
        return x.T

    def windows(b, q, e, js, gate=None):
        out = []
        for j in js:
            parts = []
            for sg in range(2 * j - 6, 2 * j + 2):
                if sg < 0:
                    parts.append(jnp.zeros((16, 128), U32))
                else:
                    parts.append(pltpu.bitcast(sa_s[b, pl.ds(_mult(128 * sg + 32 * q + 16 * e, 16), 16), :], U32))
            plane = 32 * (j // 4) + 8 * q + 4 * e + j % 4
            win = gated_t(jnp.concatenate(parts, axis=0), gate)
            aw_s[pl.ds(_mult(plane * PITCH + 128 * b, 8), 128), :] = win
            out.append(win[120:])
        return out

    def prep_g(r0, n, gate=None):
        rows = pl.ds(_mult(r0, 16), n)
        lane = lax.broadcasted_iota(I32, (n, 128), 1)
        for a in range(NB):
            hf = hk_s[rows, 128 * a:128 * (a + 1)].astype(F32)
            hs = delayed(hk_s, rows, a, 1, gate)
            if a == 0:
                hf = jnp.where(lane == 0, hf + dc_s[rows, :], hf)
                hs = jnp.where(lane == 1, hs + dc_s[rows, :], hs)
            wrd = pltpu.pack_elementwise([hf, hs], packed_dtype=BF16).astype(U32)
            g_s[a, rows, :] = wrd
            yield _digest([wrd])

    def extract(h, r0, o, shift, z):
        def block(n, kq, b):
            x = jnp.concatenate([wp_s[(h // 2) % 2 + z, 2 * n + b, pl.ds(256 * kq + r0 + e, 8, stride=2), :]
                                 for e in range(2)], axis=0)
            if isinstance(h, int):
                return _lo(x) if h % 2 == 0 else _hi(x)
            return _hi(x << jnp.concatenate([shift] * 2, axis=0))

        blk = [[[[block(N, 2 * K + k, n) for n in range(2)] for k in range(2)]
                for N in range(2)] for K in range(2)]
        terms = [_join(t) for _, _, t in list(_terms2(_rhs_terms, blk))[7 * o:7 * (o + 1)]]
        for i, t in enumerate(terms):
            wx_w[7 * o + i, r0 // 2:r0 // 2 + 8, :] = t
        return _digest(terms)

    def phase0():
        XC = 512
        NF = CFG.get('nf', 4)
        N0 = CFG.get('n0', NF)
        cq = [cp(wq32.at[:, word_row(g // 2, g % 2), :], y_s.at[pl.ds(C * g, C)],
                 0 if g < N0 else 19 if g < NF else 1 if g < 8 else 18)
              for g in range(H)]
        cx = [cp(x_hbm.at[:, pl.ds(XC * i, XC)], x_w.at[:, pl.ds(XC * i, XC)], 22 + i) for i in range(S // XC)]
        ga = [cp(sk_hbm, sk_ref, 2), cp(ka_hbm, ka_w, 3), cp(va_hbm, va_w, 4)]
        gb = cq[8:] + gc
        gd = [cp(d_hbm, d_ref, 20), cp(hk_hbm, hk_w, 5)] + g3
        rest = cx[1:] + cq[NF:8] + ga + gb + gd + g3b
        for c_ in [cx[0]] + cq[:NF] + rest:
            c_.start()
        zero = pl.semaphore_read(sems.at[34])
        never = _never(zero)
        due = []
        toks = []

        def pad_rows(t):
            return jnp.concatenate([t, jnp.zeros((256 - CH, 128), t.dtype)], axis=0)

        def wq_terms(j, b, gate):
            x = y_s[C * (2 * j + b):C * (2 * j + b + 1), :]
            g16 = jnp.concatenate([_after(jnp.full((8, 128), 16, U32), gate, never)] * (C // 8), axis=0)
            gm = jnp.concatenate([_after(jnp.full((8, 128), HI_MASK, U32), gate, never)] * (C // 8), axis=0)
            lo, hi = pltpu.bitcast(x << g16, F32), pltpu.bitcast(x & gm, F32)
            blocks = [pad_rows(t).T for t in (lo[:CH], hi[:CH], lo[CH:], hi[CH:])]
            if not CFG.get('q4', 1):
                return [t.astype(BF16) for t in _rhs_terms(*blocks)]
            slot = (2 * j + b) % 2
            for n, t in enumerate(blocks):
                for k in range(2):
                    wt_s[slot, 2 * n + k] = t[:, 128 * k:128 * (k + 1)]
            quarter = [[jnp.concatenate([wt_s[slot, 2 * n + k, pl.ds(e, 32, stride=4), :] for k in range(2)], axis=1)
                        for n in range(4)] for e in range(4)]
            terms = [_rhs_terms(*q) for q in quarter]
            out = []
            for i in range(7):
                ev, od = _pack(terms[0][i], terms[2][i]), _pack(terms[1][i], terms[3][i])
                rows = [w[8 * m:8 * (m + 1)] for m in range(4) for w in (ev, od)]
                out.append(pltpu.bitcast(jnp.concatenate(rows, axis=0), BF16))
            return out

        def x_terms(jp):
            top = slice(256 * jp, 256 * jp + 128)
            bot = slice(256 * jp + 128, 256 * jp + 256)
            for i in range(7):
                xs_s[256 * (NP * i + jp) + CH:256 * (NP * i + jp + 1), :] = jnp.zeros((256 - CH, 128), BF16)
            for r in range(0, CH, 32):
                lo, hi = slice(r // 2, r // 2 + 16), slice((CH + r) // 2, (CH + r) // 2 + 16)
                blocks = [x_w[lo, top], x_w[hi, top], x_w[lo, bot], x_w[hi, bot]]
                terms = [_join(t) for t in _lhs_terms(*[_split(t) for t in blocks])]
                terms[2], terms[3] = blocks[0], blocks[3]
                for i, t in enumerate(terms):
                    xs_w[128 * (NP * i + jp) + r // 2:128 * (NP * i + jp) + r // 2 + 16, :] = t
                yield 1, _digest(terms)

        def qproj(g, jp, waits):
            j, b = groups[g]
            for c_ in waits:
                c_.wait()
            if False:
                x_terms(jp)
                x_terms(jp + 1)

            def prod(i):
                pump()
                m = _dot(_tied(wts[g][i], due, never), xs_s[256 * (NP * i + jp):256 * (NP * i + jp + 1), :])
                toks.append(m[:8])
                return m

            def emit(r, c, val):
                val = val * QSCALE
                if CFG.get('q4', 1):
                    w = [_pack(val[32 * m:32 * m + 16], val[32 * m + 16:32 * m + 32]) for m in range(4)]
                    qc_w[2 * j + c, 2 * jp + r, 64 * b:64 * (b + 1), :] = jnp.concatenate(w, axis=0)
                else:
                    qc_s[2 * j + c, 2 * jp + r, 128 * b:128 * (b + 1), :] = val.astype(BF16)

            _strassen(prod, emit)

        def column(row):
            row = jnp.concatenate([row.astype(F32), jnp.zeros((1, 512 - C), F32)], axis=1)
            return jnp.broadcast_to(row, (128, 512)).T

        consts = {}

        def make_consts():
            consts['taps'] = [column(sk_ref[j:j + 1, :]) for j in range(4)]

        def gate(x):
            back = CFG.get('gback', 6)
            return _after(x, toks[-back], never) if back else x

        def prep_u(r0, n):
            rows = slice(r0, r0 + n)
            tp = [t[rows] for t in consts['taps']]
            prev = jnp.zeros((n, 128), F32)
            for sg in range(NB):
                cols = slice(128 * sg, 128 * (sg + 1))
                ksh = ((delayed(ka_s, rows, sg, 3, gate) * tp[3] + delayed(ka_s, rows, sg, 2, gate) * tp[2])
                       + (delayed(ka_s, rows, sg, 1, gate) * tp[1] + ka_s[rows, cols].astype(F32) * tp[0]))
                kv = ksh * va_s[rows, cols].astype(F32)
                wrd = pltpu.pack_elementwise([prev, kv], packed_dtype=BF16).astype(U32)
                sb_s[sg // 4, C * (sg % 4) + r0:C * (sg % 4) + r0 + n, :] = pltpu.bitcast(wrd, F32)
                prev = kv
                yield _digest([wrd])

        def words_t(b):
            for sg in range(NB):
                r0 = C * (sg % 4) + 128 * b
                if b < 3:
                    wrd = sb_s[sg // 4, r0:r0 + 128, :]
                else:
                    wrd = jnp.concatenate([sb_s[sg // 4, r0:r0 + C - 384, :], jnp.zeros((512 - C, 128), F32)], axis=0)
                wrd = gated_t(pltpu.bitcast(wrd, U32), gate)
                sa_s[b, 128 * sg:128 * (sg + 1), :] = pltpu.bitcast(wrd, F32)
                yield wrd[120:]

        def all_windows(b):
            for p in range(8):
                for j in range(8):
                    yield windows(b, p // 2, p % 2, [j], gate)[0]

        def c_terms():
            for ck in range(4):
                for half in range(2):
                    for r0 in range(0, 128, 16):
                        def blocks(z):
                            return [[[[_split(c_w[4 * K + 2 * k + half + z,
                                                  pl.ds(256 * ck + 128 * R + 64 * r + r0 // 2, 8), :])
                                       for k in range(2)] for r in range(2)] for K in range(2)] for R in range(2)]

                        if CFG.get('crl'):
                            terms = [x for o in range(7)
                                     for x in list(_terms2(_lhs_terms, blocks(zero * (o + 1))))[7 * o:7 * (o + 1)]]
                        else:
                            terms = _terms2(_lhs_terms, blocks(0))
                        acc = None
                        for o, i, t in terms:
                            t = _join(t)
                            cs_w[ck, 7 * o + i, half, r0 // 2:r0 // 2 + 8, :] = t
                            acc = _digest([t]) if acc is None else acc ^ _digest([t])
                            if i == 6:
                                yield acc
                                acc = None

        UG = CFG.get('ug', 32)

        cu, ct, cg, cx_ = CFG.get('costs', (2, 2, 1, 1))

        def a_stream():
            make_consts()
            for b in range(4):
                for r0 in range(128 * b, min(C, 128 * (b + 1)), UG):
                    for v in prep_u(r0, UG):
                        yield cu * UG // 32, v
                for v in words_t(b):
                    yield ct, v
                for v in all_windows(b):
                    yield ct, v

        def d_stream():
            dc_s[...] = column(d_ref[...].reshape(1, C))
            for r0 in range(0, C, 32):
                for v in prep_g(r0, 32, gate):
                    yield cg, v
            for r0 in range(0, 256, 16):
                for o in range(7):
                    yield cx_, extract(0, r0, o, None, zero * (o + 1))

        a_total = cu * 14 * NB + ct * 4 * (NB + 64)
        d_total = cg * 14 * NB + cx_ * 112
        streams = []
        nprod = [0]
        later = {}
        LAG = CFG.get('lag', 0)

        def pump():
            for st_ in streams:
                gen, n, p0, p1, done = st_
                want = min(n, max(0, (nprod[0] - p0 + 1) * n // (p1 - p0)))
                while st_[4] < want:
                    cost, v = next(gen)
                    later.setdefault(nprod[0] + LAG, []).append(v)
                    st_[4] += cost
            due.extend(later.pop(nprod[0], []))
            nprod[0] += 1

        groups = [(j, b) for j in range(H // 2) for b in range(2)]
        units = [(g, jp) for c in range(0, NP, 2) for g in range(NF) for jp in (c, c + 1)]
        units += [(g, jp) for g in range(NF, len(groups)) for jp in range(NP)]
        NU = len(units)
        wts = {}
        lead = CFG.get('lead', 4)
        ua = CFG.get('ua', 32)
        ub = 8 * NP - lead
        ux = CFG.get('ux', 5)
        ud = CFG.get('ud', 96)
        waits = {ux: cx[1:] + cq[NF:8], ua: ga, ub: gb, ud: gd}
        if N0 < NF:
            waits[2 * N0 - 1] = cq[N0:NF]
        xe = [7 * ux + 2] + [7 * NF * 2 * c - 1 for c in (1, 2, 3)]
        for c in range(3):
            streams.append([(v for jp in (2 * c + 2, 2 * c + 3) for v in x_terms(jp)), 14, xe[c], xe[c + 1], 0])
        sl = CFG.get('slack', 4)
        PA, PB, PE = 7 * ua + sl, 7 * ub + sl, 7 * NU - 2 - LAG
        c_stream = ((1, v) for v in c_terms())
        nc = 4 * 2 * 8 * 7
        PD = 7 * ud + sl
        streams.append([a_stream(), a_total, PA, PD + CFG.get('aext', 0), 0])
        streams.append([c_stream, nc, PB, PE, 0])
        streams.append([d_stream(), d_total, PD + CFG.get('aext', 0), PE, 0])

        if not CFG.get('p0', 1):
            for c_ in cq + cx + ga + gc + gd:
                c_.wait()
            return
        _wait([cx[0]], 'wx0')
        list(x_terms(0))
        list(x_terms(1))
        _wait(cq[:N0], 'wq0')
        first_use = {}
        for u, (g, jp) in enumerate(units):
            first_use.setdefault(g, u)
        for u, (g, jp) in enumerate(units):
            if u in waits:
                _wait(waits[u], 'wu%d' % u)
            for g_, fu in first_use.items():
                if g_ not in wts and fu - (lead if g_ >= NF else 1) <= u:
                    back = CFG.get('wback', 8)
                    wts[g_] = wq_terms(*groups[g_], toks[-back] if len(toks) >= back else None)
            qproj(g, jp, [])
        assert all(st_[4] == st_[1] for st_ in streams) and not later, streams

    phase0()


    def phase1(k_s, vt_s, wx_s, *s_s):
        LATE = CFG.get('late', (2, 5))
        EARLY = tuple(o for o in (0, 1, 3, 4, 6, 2, 5) if o not in LATE)
        UN = CFG.get('unroll', 1)

        def heads(it, carry):
            @pl.when(it == 1)
            def _():
                for c_ in g4:
                    c_.start()

            @pl.when(jnp.logical_and(it % 2 == 1, it < H - 1))
            def _():
                _wait(kv_copies((it + 1) // 2), 'wkv')

            @pl.when(jnp.logical_and(jnp.logical_and(it % 2 == 0, it > 0), it < H - 2))
            def _():
                for c_ in kv_copies(it // 2 + 1):
                    c_.start()

            zero = it // H
            toks = []
            due = []
            for r in range(UN):
                head(it * UN + r, None if UN % 2 else r % 2, zero, toks, due)
            return carry + zero

        def head(h, par, zero, toks, due):
            lane8 = lax.broadcasted_iota(I32, (8, 128), 1)
            sub8 = lax.broadcasted_iota(I32, (8, 128), 0)
            lane16 = lax.broadcasted_iota(I32, (16, 128), 1)
            sub16 = lax.broadcasted_iota(I32, (16, 128), 0)
            tri = (lax.broadcasted_iota(I32, (128, 128), 0) <= lax.broadcasted_iota(I32, (128, 128), 1))
            h_next = h + 1 if isinstance(h, int) else jnp.minimum(h + 1, H - 1)
            never = _never(zero)

            def after(x, tok):
                return _after(x, tok, never)

            def tied(lhs):
                return _tied(lhs, due, never)

            def tok(back):
                return toks[-back] if (back and len(toks) >= back) else None

            def chan_mm(c, gate):
                m_b = lane8 < after(128 - 2 * sub8, gate)
                gs = [jnp.broadcast_to(g_s[a, pl.ds(c, 1), :], (8, 128)) for a in range(NB)]
                bt = [pltpu.roll(jnp.where(m_b, gs[a], gs[a - 1] if a > 0 else jnp.uint32(0)), 0, 1,
                                 stride=2, stride_axis=0) for a in range(NB)]
                b1 = pltpu.bitcast(jnp.concatenate(bt[7::-1], axis=0), BF16)
                b2 = pltpu.bitcast(jnp.concatenate(bt[15:7:-1], axis=0), BF16)
                am = pltpu.bitcast(aw_s[pl.ds(c, 64, stride=PITCH), :], BF16)
                tick('C', 48)
                z1 = _dot(tied(am), b1)
                z2 = _dot(am[:64], b2)
                return c, z1[:64], z1[64:] + z2

            def chan_post(c, zlo, zhi):
                acc = car = None
                for p in range(8):
                    z = jnp.concatenate([zlo[8 * p:8 * p + 8], zhi[8 * p:8 * p + 8]], axis=0)
                    if p == 0:
                        acc = z
                    else:
                        z = pltpu.roll(z, 16 * p, 1)
                        cz = jnp.where(lane16 < 16 * p, z, 0.0)
                        acc = acc + z
                        car = cz if car is None else car + cz
                y = (acc - car) + jnp.where(sub16 > 0, pltpu.roll(car, 1, 0), 0.0)
                later(CFG.get('ly', 0), [y])
                if CFG.get('ylate'):
                    ys.append((c, y))
                else:
                    y_s[pl.ds(c, NB, stride=PITCH), :] = pltpu.bitcast(y, U32)
                if CFG.get('pd', 0):
                    due.append(y[:8])
                    due.append(y[8:])

            chans = [h * CPH + i for i in range(CPH)]
            ys, cs = [], []

            def x_stream(hh, outers):
                n = 16 * len(outers)
                for r0 in range(0, 256, 16):
                    for o in outers:
                        n -= 1
                        free = n < CFG.get('xfree', 0) and hh is h_next
                        d = extract(hh, r0, o, shift_of(hh, tok(CFG.get('xfb', 1)) if free else None), zero * (o + 1))
                        yield None if free else d

            streams = [[x_stream(h_next, EARLY), 16 * len(EARLY), 0, 0] + list(CFG['x1']),
                       [x_stream(h, LATE), 16 * len(LATE), 0, 0] + list(CFG['x2'])]

            clock, queue = [0], []

            def later(lag, vals):
                if lag:
                    queue.append((clock[0] + lag, _digest(vals)))

            def tick(kind, cycles):
                due.extend(v for t, v in queue if t <= clock[0])
                queue[:] = [q for q in queue if q[0] > clock[0]]
                clock[0] += cycles
                for st_ in streams:
                    gen, n, done, clk, kinds, c0, c1 = st_
                    if kind in kinds:
                        want = min(n, max(0, (clk - c0) * n // (c1 - c0)))
                        while st_[2] < want:
                            d = next(gen)
                            if d is not None:
                                due.append(d)
                            st_[2] += 1
                        st_[3] += cycles

            def shift_of(hh, gate):
                return after(jnp.full((8, 128), (1 - hh % 2) * 16, I32).astype(U32), gate)

            def kv_chunk(ck):
                def prod(o):
                    out = {}

                    def inner(i):
                        tick('M', 64)
                        lhs = jnp.concatenate([cs_s[ck, 7 * o + i, 0], cs_s[ck, 7 * o + i, 1]], axis=1)
                        m = _dot(tied(lhs), wx_s[7 * o + i])
                        if i == CFG.get('ti', 3):
                            toks.append(m[:8])
                        return m

                    _strassen(inner, lambda r, n, val: out.__setitem__((r, n), val))
                    return jnp.concatenate(
                        [jnp.concatenate([out[r, 0], out[r, 1]], axis=1) for r in range(2)], axis=0)

                def emit(R, N, val):
                    if N == 0:
                        rows = slice(512 * ck + 256 * R, 512 * ck + 256 * (R + 1))
                        val = val.astype(BF16)
                        k_s[0, rows, :] = val[:, :128]
                        k_s[1, rows, :] = val[:, 128:]
                    else:
                        for r in range(2):
                            for n in range(2):
                                v = val[128 * r:128 * (r + 1), 128 * n:128 * (n + 1)].T.astype(BF16)
                                vt_s[4 * ck + 2 * R + r, 128 * n:128 * (n + 1), :] = v
                                later(CFG.get('lv', 0), [v[112:]])

                return _strassen_steps(prod, emit)

            kv = [kv_chunk(ck) for ck in range(4)]

            def k_rows(r0, r1):
                return jnp.concatenate([k_s[0, r0:r1, :], k_s[1, r0:r1, :]], axis=1)

            def q_cols(r0, r1):
                return jnp.concatenate([qc_s[h, t] for t in range(r0 // 128, r1 // 128)], axis=1)

            mx, pr = {}, {}

            def qk(t):
                q0 = t * TQ
                if q0 > 0:
                    QR = CFG.get('qr', 2048)
                    rect = []
                    for r0 in range(0, q0, QR):
                        for e in CFG.get('qe', {}).get((t, r0 // QR), '').split():
                            softmax(int(e[0]), int(e[1]), True)
                        tick('Q', min(QR, q0 - r0) * 2)
                        rect.append(_dot(tied(k_rows(r0, min(q0, r0 + QR))), q_cols(q0, q0 + TQ)))
                    s_rect = jnp.concatenate(rect, axis=0) if len(rect) > 1 else rect[0]
                    toks.append(s_rect[:8, :128])
                for u in range(TQ // 128):
                    qs = q0 + u * 128
                    if u == 0:
                        for e in CFG.get('qe', {}).get((t, 'd'), '').split():
                            softmax(int(e[0]), int(e[1]), True)
                    tick('Q', 64 * (u + 1))
                    sd = _dot(tied(k_rows(q0, qs + 128)), q_cols(qs, qs + 128))
                    parts = []
                    if q0 > 0:
                        parts.append(s_rect[:, u * 128:(u + 1) * 128])
                    if u > 0:
                        parts.append(sd[:u * 128, :])
                    parts.append(jnp.where(tri, sd[u * 128:, :], NEG))
                    s = jnp.concatenate(parts, axis=0) if len(parts) > 1 else parts[0]
                    s_s[t % 2][u, 0:qs + 128, :] = s
                    mx[(t, u)] = jnp.max(s, axis=0, keepdims=True)
                toks.append(sd[:8])
                if CFG.get('clob', 1):
                    s_s[t % 2][zero, S:S + 8, :] = sd[:8]

            def softmax(t, u, deadline):
                qs = t * TQ + u * 128
                p = jnp.exp2(s_s[t % 2][u if CFG.get('clob', 1) else u + zero, 0:qs + 128, :] - mx.pop((t, u)))
                NA = CFG.get('na', 0)
                if NA:
                    accs = [None] * NA
                    for r in range(p.shape[0] // 8):
                        v = p[8 * r:8 * (r + 1)]
                        accs[r % NA] = v if accs[r % NA] is None else accs[r % NA] + v
                    while len(accs) > 1:
                        accs = [a + b for a, b in zip(accs[::2], accs[1::2])]
                    part = accs[0]
                    rl = 1.0 / jnp.sum(part, axis=0, keepdims=True)
                else:
                    rl = part = 1.0 / jnp.sum(p, axis=0, keepdims=True)
                pb = p.astype(BF16)
                pr[(t, u)] = (pb, rl)
                if deadline:
                    due.append(part)
                    if CFG.get('pk'):
                        due.append(_digest([pb]))

            def pv(t, u):
                if (t, u) not in pr:
                    softmax(t, u, False)
                p, rl = pr.pop((t, u))
                qs = t * TQ + u * 128
                vt = jnp.concatenate([vt_s[i] for i in range(qs // 128 + 1)], axis=1)
                PH = D // CFG.get('ph', 1)
                for d0 in range(0, D, PH):
                    tick('P', (qs + 128) * PH // 512)
                    ctx = _dot(tied(vt[d0:d0 + PH]), p)
                    v = (ctx * rl).astype(BF16)
                    later(CFG.get('lc', 0), [v])
                    if CFG.get('clate'):
                        cs.append((qs // 128, d0, PH, v))
                    else:
                        qc_s[h, qs // 128, d0:d0 + PH, :] = v
                toks.append(ctx[:8])

            CG, XG = CFG.get('cg', 0), CFG.get('xg', 0)
            pend = []
            def run_step(st_):
                kind, arg = st_[0], st_[1:]
                if kind == 'E':
                    softmax(int(arg[0]), int(arg[1]), True)
                    return
                old = list(pend)
                pend.clear()
                if kind == 'C':
                    for _ in range(int(arg)):
                        pend.append(chan_mm(chans.pop(0), tok(CG)))
                elif kind == 'M':
                    for o in arg[1:]:
                        kv[int(arg[0])](int(o))
                elif kind == 'Q':
                    qk(int(arg))
                elif kind == 'P':
                    for u in ([int(arg[1])] if len(arg) > 1 else range(TQ // 128)):
                        pv(int(arg[0]), u)
                for args in old:
                    chan_post(*args)

            for seg in [g for g in CFG['sched'].split('|') if g.strip()]:
                if CFG.get('scopes') and '|' in CFG['sched']:
                    with jax.named_scope('s_' + seg.split()[0]):
                        for st_ in seg.split():
                            run_step(st_)
                else:
                    for st_ in seg.split():
                        run_step(st_)
            for c, y in ys:
                y_s[pl.ds(c, NB, stride=PITCH), :] = pltpu.bitcast(y, U32)
            for t, d0, n, v in cs:
                qc_s[h, t, d0:d0 + n, :] = v
            assert all(st_[1] == st_[2] for st_ in streams), [st_[1:] for st_ in streams]
            assert CFG.get('noassert') or not chans and not pend and (not due or CFG.get('pd')) and not pr and not mx

        if CFG.get('p1', 1):
            return lax.fori_loop(0, H // UN, heads, 0)
        else:
            _wait(g3b, 'wg3b')
            for c_ in g4:
                c_.start()

            def keep(h, carry):
                r = pl.multiple_of(h * 16, 16)
                t = (qc_s[h, h, 0:16, :].astype(F32) + cs_s[h % 4, h, h % 2, 0:16, :].astype(F32)
                     + pltpu.bitcast(aw_s[pl.ds(r, 16), :] + g_s[h, pl.ds(r, 16), :], F32)
                     + wx_s[h, pl.ds(r, 16), :].astype(F32))
                y_s[pl.ds(r, 16), :] = pltpu.bitcast(t, U32)
                return carry + h // H
            return lax.fori_loop(0, H, keep, 0)

    zero_end = phase1(k_s, vt_s, wx_s, sa_s, sb_s)

    def phase2():
        _wait(g4, 'wg4')
        HH = H // 2

        def wo_block(rh, kh):
            return jnp.concatenate(
                [xs_s[C * (H * b + h) + CH * rh:C * (H * b + h) + CH * (rh + 1), :]
                 for h in range(HH * kh, HH * (kh + 1)) for b in range(2)], axis=1)

        raw = [wo_block(0, 0), wo_block(1, 0), wo_block(0, 1), wo_block(1, 1)]
        wt = [t.astype(BF16) for t in _rhs_terms(*[t.astype(F32) for t in raw])]
        wt[1], wt[4] = raw[0], raw[3]
        outs = []
        due, late = [], []
        DL = CFG.get('dl', 3)
        never = _never(zero_end)

        def put(t, b, z, opaque=False):
            o = z.T.astype(BF16)
            r0 = pl.multiple_of(zero_end * 16 + 128 * t, 16) if opaque else 128 * t
            c_s[b, pl.ds(r0, 128), :] = o
            late.append(pltpu.bitcast(o[112:], U32))

        for jp in range(CFG.get('np2', NP) if CFG.get('p2', 1) else 0):
            def ctx_block(r, kh):
                return jnp.concatenate([qc_s[h, 2 * jp + r] for h in range(HH * kh, HH * (kh + 1))], axis=0)

            craw = [ctx_block(0, 0), ctx_block(0, 1), ctx_block(1, 0), ctx_block(1, 1)]
            ct = [t.astype(BF16) for t in _lhs_terms(*[t.astype(F32) for t in craw])]
            ct[2], ct[3] = craw[0], craw[3]
            za = {}
            prev_late = list(late)
            late.clear()
            for r in range(2):
                t = 2 * jp + r
                za[r] = (pltpu.bitcast(y_s[t * PITCH:t * PITCH + C, :], F32)
                         * x_s[:, 128 * t:128 * (t + 1)].astype(F32))
                for b in range(3):
                    put(t, b, za[r][128 * b:128 * (b + 1)], opaque=(r == 0 and b == 0 and jp > 0))
            a_late = list(late)
            late.clear()
            res = {}
            count = [0]

            def prod(i):
                if count[0] == DL:
                    due.extend(prev_late)
                if count[0] == 6:
                    due.extend(a_late)
                count[0] += 1
                return _dot(_tied(wt[i], due, never), ct[i])

            _strassen(prod, lambda r, c, val: res.__setitem__((r, c), val), order=(1, 4, 3, 2, 0, 5, 6))
            for r in (1, 0):
                z = jnp.concatenate([za[r][384:], res[(r, 0)], res[(r, 1)]], axis=0)
                for b in (3, 2, 1, 0):
                    put(2 * jp + r, 3 + b, z[128 * b:128 * (b + 1)])
            rows = pl.ds(128 * jp, 128)
            for b in range(7):
                oc = cp(c_w.at[b, rows], o_hbm.at[rows, pl.ds(128 * b, 128)], 26 + jp)
                oc.start()
                outs.append(oc)
        if not CFG.get('p2', 1):
            def keep(h, carry):
                r = pl.multiple_of(h * 16, 16)
                c_s[0, pl.ds(r, 16), :] = pltpu.bitcast(y_s[pl.ds(r, 16), :], F32).astype(BF16) + qc_s[h, h, 0:16, :]
                return carry
            lax.fori_loop(0, H, keep, 0)
            oc = cp(c_w.at[0, pl.ds(0, 128)], o_hbm.at[pl.ds(0, 128), pl.ds(0, 128)], 26)
            oc.start()
            outs.append(oc)
        _wait(outs, 'wout')

    phase2()


def _tiles(w):
    rows = w.shape[0]
    return w.reshape(rows, 2, 8, 2, 128).transpose(0, 1, 3, 2, 4).reshape(rows, 32, 128)


@jax.jit
def pallas_concat_heads__ssm_conv_h3__compressed_kv_cla__prompt_kernel(
    A_q: jax.Array,
    A_k: jax.Array,
    A_v: jax.Array,
    A_shift_k: jax.Array,
    A_ssm_k: jax.Array,
    A_ssm_D: jax.Array,
    B_x: jax.Array,
    B_c_kv: jax.Array,
    B_w_q: jax.Array,
    B_w_uk: jax.Array,
    B_w_uv: jax.Array,
    B_w_o: jax.Array,
):
    hbm = pl.BlockSpec(memory_space=pltpu.HBM)
    out = pl.pallas_call(
        _kernel,
        in_specs=[hbm] * 12,
        out_specs=hbm,
        out_shape=jax.ShapeDtypeStruct((S, 2 * C), BF16),
        scratch_shapes=[
            pltpu.VMEM((8, S // 2, 128), U32),
            pltpu.VMEM((4, 49, 2, 64, 128), U32),
            pltpu.VMEM((2, 4, DC, 128), U32),
            pltpu.VMEM((H, NB, D // 2, 128), U32),
            pltpu.VMEM((64 * PITCH, 128), U32),
            pltpu.VMEM((NB, C, 128), U32),
            pltpu.VMEM((NB * PITCH, 128), U32),
            pltpu.VMEM((CH, S), U32),
            pltpu.VMEM((512, 128), F32),
            pltpu.VMEM((2, S // 2, 128), U32),
            pltpu.VMEM((NB, D // 2, 128), U32),
            pltpu.VMEM((49, DC // 8, 128), U32),
            pltpu.VMEM((TQ // 128, S + 8, 128), F32),
            pltpu.VMEM((TQ // 128, S + 8, 128), F32),
            pltpu.VMEM((CH, S), U32),
            pltpu.VMEM((7 * NP * 128, 128), U32),
            pltpu.VMEM((CH, S), U32),
            pltpu.VMEM((CH, S), U32),
            pltpu.VMEM((2, 8, 128, 128), F32),
            pltpu.VMEM((4, C), BF16),
            pltpu.VMEM((C,), BF16),
            pltpu.SemaphoreType.DMA((35,)),
        ],
        compiler_params=pltpu.CompilerParams(vmem_limit_bytes=127 * 2 ** 20),
    )(
        A_q[0].T, A_k[0].T, A_v[0].T, A_shift_k.T, A_ssm_k, A_ssm_D, B_x[0].T, B_c_kv[0],
        _tiles(B_w_q), _tiles(B_w_uk), _tiles(B_w_uv),
        jnp.swapaxes(B_w_o, 1, 2).reshape(H * C, D),
    )
    return out.reshape(1, S, 2 * C)
```

```python
import math

import jax
import jax.numpy as jnp
from jax import lax
import jax.experimental.pallas as pl
import jax.experimental.pallas.tpu as pltpu

F32 = jnp.float32
BF16 = jnp.bfloat16
U32 = jnp.uint32
I32 = jnp.int32

S = 2048
C = 448
H = 16
D = 256
DC = 1024
NB = S // 128
NP = NB // 2
CH = C // 2
PITCH = 520
CPH = C // H
TQ = 512
NT = (((1,), (1,)), ((), ()))
LOG2E = math.log2(math.e)
QSCALE = (D ** -0.5) * LOG2E
NEG = -1e9 * LOG2E
HI_MASK = 0xFFFF0000
CFG = dict(sq=1,cg=5,ua=30,ud=96,nf=8,n0=3,ux=13,crl=1,gback=8,slack=8,clob=0,ph=2,late=(),x2=('P',0,1),x1=('P',2200,8190),sched='M001 C2 M034 C2 M06 M101 C2 Q0 M134 C2 M16 M201 C2 E00 E01 E02 E03 Q1 M234 C2 M26 M301 C2 E10 E11 Q2 M334 C2 E12 M36 E13 M02 C2 Q3 M05 C2 E20 M12 C2 E21 M15 C2 E22 M22 C2 E23 M25 C2 E30 M32 M35 E31 P0 P1 P2 P3')


def _wait(copies, name):
    if CFG.get('scopes'):
        with jax.named_scope(name):
            for c_ in copies:
                c_.wait()
    else:
        for c_ in copies:
            c_.wait()


def _dot(a, b):
    return jnp.dot(a, b, preferred_element_type=F32)


def _dot_nt(a, b):
    return lax.dot_general(a, b, NT, preferred_element_type=F32)


def _lo(x):
    return pltpu.bitcast(x << 16, F32)


def _hi(x):
    return pltpu.bitcast(x & jnp.uint32(HI_MASK), F32)


def _pack(even, odd):
    return pltpu.pack_elementwise([even, odd], packed_dtype=BF16).astype(U32)


def _split(words):
    return jnp.concatenate([_lo(words), _hi(words)], axis=0)


def _join(x):
    n = x.shape[0] // 2
    return _pack(x[:n], x[n:])


def _head_cols(w_s, h, rows):
    out = []
    for b in range(2):
        x = w_s[b, pl.ds(h // 2, rows, stride=8), :]
        if isinstance(h, int):
            out.append(_lo(x) if h % 2 == 0 else _hi(x))
        else:
            out.append(_hi(x << ((1 - h % 2) * 16).astype(U32)))
    return out


_LHS = ((0, 1, 3), (2, 1, 3), (0,), (3,), (0, 1, 1), (2, -1, 0), (1, -1, 3))
_RHS = ((0, 1, 3), (0,), (1, -1, 3), (2, -1, 0), (3,), (0, 1, 1), (2, 1, 3))


def _term(table, i, block):
    spec = table[i]
    if len(spec) == 1:
        return block(spec[0])
    return block(spec[0]) + block(spec[2]) if spec[1] > 0 else block(spec[0]) - block(spec[2])


def _lhs_terms(*blocks):
    return [_term(_LHS, i, blocks.__getitem__) for i in range(7)]


def _rhs_terms(*blocks):
    return [_term(_RHS, i, blocks.__getitem__) for i in range(7)]


def _inner_terms(table, o, block):
    sub = [_term(table, o, lambda n: block(n, m)) for m in range(4)]
    return [_term(table, i, sub.__getitem__) for i in range(7)]


def _strassen_steps(prod, emit):
    uses = {(0, 0): {0: 1, 3: 1, 4: -1, 6: 1}, (0, 1): {2: 1, 4: 1},
            (1, 0): {1: 1, 3: 1}, (1, 1): {0: 1, 1: -1, 2: 1, 5: 1}}
    acc = {}
    neg = {}

    def step(i):
        m = prod(i)
        for key, terms in uses.items():
            if i not in terms:
                continue
            sign = terms.pop(i)
            if key not in acc:
                acc[key] = m
                neg[key] = sign < 0
            elif neg[key]:
                assert sign > 0
                acc[key] = m - acc[key]
                neg[key] = False
            else:
                acc[key] = acc[key] + m if sign > 0 else acc[key] - m
            if not terms:
                emit(key[0], key[1], acc.pop(key))

    return step


def _strassen(prod, emit, order=(0, 1, 3, 2, 4, 5, 6)):
    step = _strassen_steps(prod, emit)
    for i in order:
        step(i)


def _mult(i, n):
    return i if isinstance(i, int) else pl.multiple_of(i, n)


def _never(zero):
    return lax.broadcasted_iota(I32, (8, 128), 1) < zero


def _after(x, tok, never):
    if tok is None:
        return x
    return jnp.where(never, pltpu.bitcast(tok, x.dtype), x)


def _tied(lhs, due, never):
    if not due:
        return lhs
    t = None
    for d in due:
        d = pltpu.bitcast(jnp.broadcast_to(d, (8, 128)), U32)
        t = d if t is None else t ^ d
    due.clear()
    x = pltpu.bitcast(_after(pltpu.bitcast(lhs[:16, :128], U32), t, never), BF16)
    if lhs.shape[1] > 128:
        x = jnp.concatenate([x, lhs[:16, 128:]], axis=1)
    return jnp.concatenate([x, lhs[16:]], axis=0) if lhs.shape[0] > 16 else x


def _digest(vals):
    acc = None
    words = [v if v.dtype == U32 else pltpu.bitcast(v, U32) for v in vals]
    for r in range(words[0].shape[0] // 8):
        for w in words:
            w = w[8 * r:8 * (r + 1)]
            acc = w if acc is None else acc ^ w
    return acc


class _Packed:
    def __init__(self, ref):
        self.ref = ref

    def _index(self, idx):
        idx = idx if isinstance(idx, tuple) else (idx,)
        axis = len(self.ref.shape) - 2
        if len(idx) <= axis:
            return idx + (slice(None),) * (axis + 2 - len(idx))
        r = idx[axis]
        if isinstance(r, slice):
            r = slice(None if r.start is None else r.start // 2, None if r.stop is None else r.stop // 2)
        else:
            r = pl.ds(_mult(r.start // 2, 8), r.size // 2)
        return idx[:axis] + (r,) + idx[axis + 1:]

    def __getitem__(self, idx):
        return pltpu.bitcast(self.ref[self._index(idx)], BF16)

    def __setitem__(self, idx, val):
        self.ref[self._index(idx)] = pltpu.bitcast(val, U32)


def _kernel(qa_hbm, ka_hbm, va_hbm, sk_hbm, hk_hbm, d_hbm, x_hbm, c_hbm, wq_hbm, wk_hbm, wv_hbm, wo_hbm,
            o_hbm,
            c_s, cs_s, wp_s, qc_s, aw_s, g_s, y_s, hk_s, dc_s, k_s, kt_s, vt_s, wx_s, sa_s, sb_s, x_s, xs_s, ka_s, va_s, wt_s, sk_ref, d_ref, sems):
    def cp(src, dst, i):
        return pltpu.make_async_copy(src, dst, sems.at[i])

    c_w, xs_w, x_w, ka_w, va_w, hk_w, cs_w, wx_w, qc_w = c_s, xs_s, x_s, ka_s, va_s, hk_s, cs_s, wx_s, qc_s
    c_s, cs_s, qc_s, k_s, kt_s, vt_s, wx_s, xs_s, x_s, ka_s, va_s, hk_s = (
        _Packed(r) for r in (c_s, cs_s, qc_s, k_s, kt_s, vt_s, wx_s, xs_s, x_s, ka_s, va_s, hk_s))
    qa_hbm, ka_hbm, va_hbm, hk_hbm, x_hbm, c_hbm, wo_hbm, o_hbm = (
        r.bitcast(U32) for r in (qa_hbm, ka_hbm, va_hbm, hk_hbm, x_hbm, c_hbm, wo_hbm, o_hbm))
    wq32 = wq_hbm.bitcast(U32)
    wk32 = wk_hbm.bitcast(U32)
    wv32 = wv_hbm.bitcast(U32)
    gc = [cp(c_hbm.at[:, pl.ds(128 * b, 128)], c_w.at[b], 8 + b) for b in range(8)]

    def word_row(pair, b):
        return 8 * (pair // 4) + 4 * b + pair % 4

    def kv_copies(pair):
        return [cp(w.at[:, word_row(pair, b), :], wp_s.at[pair % 2, 2 * n + b], 16 + pair % 2)
                for n, w in enumerate((wk32, wv32)) for b in range(2)]

    g3 = kv_copies(0)
    g3b = kv_copies(1)
    g4 = [cp(qa_hbm, x_w, 21)] + [cp(wo_hbm.at[:, pl.ds(128 * b, 128)], xs_w.at[pl.ds(H * CH * b, H * CH)], 6 + b)
                                  for b in range(2)]

    def delayed(ref, rows, sg, n, gate=None):
        cur = pltpu.bitcast(ref[rows, 128 * sg:128 * (sg + 1)], U32)
        lane = lax.broadcasted_iota(I32, (8, 128), 1)
        if gate is not None:
            lane = gate(lane)
        lane = jnp.concatenate([lane] * (cur.shape[0] // 8), axis=0)
        prev = pltpu.bitcast(ref[rows, 128 * (sg - 1):128 * sg], U32) if sg > 0 else jnp.uint32(0)
        x = pltpu.roll(jnp.where(lane < 128 - n, cur, prev), n, 1)
        return pltpu.bitcast(x, BF16).astype(F32)

    def gated_t(x, gate):
        if gate is not None:
            x = jnp.concatenate([gate(x[:8]), x[8:]], axis=0)
        return x.T

    def windows(b, q, e, js, gate=None):
        out = []
        for j in js:
            parts = []
            for sg in range(2 * j - 6, 2 * j + 2):
                if sg < 0:
                    parts.append(jnp.zeros((16, 128), U32))
                else:
                    parts.append(pltpu.bitcast(sa_s[b, pl.ds(_mult(128 * sg + 32 * q + 16 * e, 16), 16), :], U32))
            plane = 32 * (j // 4) + 8 * q + 4 * e + j % 4
            win = gated_t(jnp.concatenate(parts, axis=0), gate)
            aw_s[pl.ds(_mult(plane * PITCH + 128 * b, 8), 128), :] = win
            out.append(win[120:])
        return out

    def prep_g(r0, n, gate=None):
        rows = pl.ds(_mult(r0, 16), n)
        lane = lax.broadcasted_iota(I32, (n, 128), 1)
        for a in range(NB):
            hf = hk_s[rows, 128 * a:128 * (a + 1)].astype(F32)
            hs = delayed(hk_s, rows, a, 1, gate)
            if a == 0:
                hf = jnp.where(lane == 0, hf + dc_s[rows, :], hf)
                hs = jnp.where(lane == 1, hs + dc_s[rows, :], hs)
            wrd = pltpu.pack_elementwise([hf, hs], packed_dtype=BF16).astype(U32)
            g_s[a, rows, :] = wrd
            yield _digest([wrd])

    def extract(h, r0, o, shift, z):
        def block(n, kq, b):
            x = jnp.concatenate([wp_s[(h // 2) % 2 + z, 2 * n + b, pl.ds(256 * kq + r0 + e, 8, stride=2), :]
                                 for e in range(2)], axis=0)
            if isinstance(h, int):
                return _lo(x) if h % 2 == 0 else _hi(x)
            return _hi(x << jnp.concatenate([shift] * 2, axis=0))

        terms = [_join(t) for t in _inner_terms(
            _RHS, o, lambda n, m: block(n % 2, 2 * (n // 2) + m // 2, m % 2))]
        for i, t in enumerate(terms):
            wx_w[7 * o + i, r0 // 2:r0 // 2 + 8, :] = t
        return _digest(terms)

    def phase0():
        XC = 512
        NF = CFG.get('nf', 4)
        N0 = CFG.get('n0', NF)
        cq = [cp(wq32.at[:, word_row(g // 2, g % 2), :], y_s.at[pl.ds(C * g, C)],
                 0 if g < N0 else 19 if g < NF else 1 if g < 8 else 18)
              for g in range(H)]
        cx = [cp(x_hbm.at[:, pl.ds(XC * i, XC)], x_w.at[:, pl.ds(XC * i, XC)], 22 + i) for i in range(S // XC)]
        ga = [cp(sk_hbm, sk_ref, 2), cp(ka_hbm, ka_w, 3), cp(va_hbm, va_w, 4)]
        gb = cq[8:] + gc
        gd = [cp(d_hbm, d_ref, 20), cp(hk_hbm, hk_w, 5)] + g3
        rest = cx[1:] + cq[NF:8] + ga + gb + gd + g3b
        for c_ in [cx[0]] + cq[:NF] + rest:
            c_.start()
        zero = pl.semaphore_read(sems.at[34])
        never = _never(zero)
        due = []
        toks = []

        def pad_rows(t):
            return jnp.concatenate([t, jnp.zeros((256 - CH, 128), t.dtype)], axis=0)

        def wq_terms(j, b, gate):
            x = y_s[C * (2 * j + b):C * (2 * j + b + 1), :]
            g16 = jnp.concatenate([_after(jnp.full((8, 128), 16, U32), gate, never)] * (C // 8), axis=0)
            gm = jnp.concatenate([_after(jnp.full((8, 128), HI_MASK, U32), gate, never)] * (C // 8), axis=0)
            lo, hi = pltpu.bitcast(x << g16, F32), pltpu.bitcast(x & gm, F32)
            blocks = [pad_rows(t).T for t in (lo[:CH], hi[:CH], lo[CH:], hi[CH:])]
            if not CFG.get('q4', 1):
                return [t.astype(BF16) for t in _rhs_terms(*blocks)]
            slot = (2 * j + b) % 2
            for n, t in enumerate(blocks):
                for k in range(2):
                    wt_s[slot, 2 * n + k] = t[:, 128 * k:128 * (k + 1)]
            quarter = [[jnp.concatenate([wt_s[slot, 2 * n + k, pl.ds(e, 32, stride=4), :] for k in range(2)], axis=1)
                        for n in range(4)] for e in range(4)]
            terms = [_rhs_terms(*q) for q in quarter]
            out = []
            for i in range(7):
                ev, od = _pack(terms[0][i], terms[2][i]), _pack(terms[1][i], terms[3][i])
                rows = [w[8 * m:8 * (m + 1)] for m in range(4) for w in (ev, od)]
                out.append(pltpu.bitcast(jnp.concatenate(rows, axis=0), BF16))
            return out

        def x_terms(jp):
            top = slice(256 * jp, 256 * jp + 128)
            bot = slice(256 * jp + 128, 256 * jp + 256)
            for i in range(7):
                xs_s[256 * (NP * i + jp) + CH:256 * (NP * i + jp + 1), :] = jnp.zeros((256 - CH, 128), BF16)
            for r in range(0, CH, 32):
                lo, hi = slice(r // 2, r // 2 + 16), slice((CH + r) // 2, (CH + r) // 2 + 16)
                blocks = [x_w[lo, top], x_w[hi, top], x_w[lo, bot], x_w[hi, bot]]
                terms = [_join(t) for t in _lhs_terms(*[_split(t) for t in blocks])]
                terms[2], terms[3] = blocks[0], blocks[3]
                for i, t in enumerate(terms):
                    xs_w[128 * (NP * i + jp) + r // 2:128 * (NP * i + jp) + r // 2 + 16, :] = t
                yield 1, _digest(terms)

        def qproj(g, jp, waits):
            j, b = groups[g]
            for c_ in waits:
                c_.wait()
            if False:
                x_terms(jp)
                x_terms(jp + 1)

            def prod(i):
                pump()
                m = _dot(_tied(wts[g][i], due, never), xs_s[256 * (NP * i + jp):256 * (NP * i + jp + 1), :])
                toks.append(m[:8])
                return m

            def emit(r, c, val):
                val = val * QSCALE
                if CFG.get('q4', 1):
                    w = [_pack(val[32 * m:32 * m + 16], val[32 * m + 16:32 * m + 32]) for m in range(4)]
                    qc_w[2 * j + c, 2 * jp + r, 64 * b:64 * (b + 1), :] = jnp.concatenate(w, axis=0)
                else:
                    qc_s[2 * j + c, 2 * jp + r, 128 * b:128 * (b + 1), :] = val.astype(BF16)

            _strassen(prod, emit)

        def column(row):
            row = jnp.concatenate([row.astype(F32), jnp.zeros((1, 512 - C), F32)], axis=1)
            return jnp.broadcast_to(row, (128, 512)).T

        consts = {}

        def make_consts():
            consts['taps'] = [column(sk_ref[j:j + 1, :]) for j in range(4)]

        def gate(x):
            back = CFG.get('gback', 6)
            return _after(x, toks[-back], never) if back else x

        def prep_u(r0, n):
            rows = slice(r0, r0 + n)
            tp = [t[rows] for t in consts['taps']]
            prev = jnp.zeros((n, 128), F32)
            for sg in range(NB):
                cols = slice(128 * sg, 128 * (sg + 1))
                ksh = ((delayed(ka_s, rows, sg, 3, gate) * tp[3] + delayed(ka_s, rows, sg, 2, gate) * tp[2])
                       + (delayed(ka_s, rows, sg, 1, gate) * tp[1] + ka_s[rows, cols].astype(F32) * tp[0]))
                kv = ksh * va_s[rows, cols].astype(F32)
                wrd = pltpu.pack_elementwise([prev, kv], packed_dtype=BF16).astype(U32)
                sb_s[sg // 4, C * (sg % 4) + r0:C * (sg % 4) + r0 + n, :] = pltpu.bitcast(wrd, F32)
                prev = kv
                yield _digest([wrd])

        def words_t(b):
            for sg in range(NB):
                r0 = C * (sg % 4) + 128 * b
                if b < 3:
                    wrd = sb_s[sg // 4, r0:r0 + 128, :]
                else:
                    wrd = jnp.concatenate([sb_s[sg // 4, r0:r0 + C - 384, :], jnp.zeros((512 - C, 128), F32)], axis=0)
                wrd = gated_t(pltpu.bitcast(wrd, U32), gate)
                sa_s[b, 128 * sg:128 * (sg + 1), :] = pltpu.bitcast(wrd, F32)
                yield wrd[120:]

        def all_windows(b):
            for p in range(8):
                for j in range(8):
                    yield windows(b, p // 2, p % 2, [j], gate)[0]

        def c_terms():
            for ck in range(4):
                for half in range(2):
                    for r0 in range(0, 128, 16):
                        for o in range(7):
                            def block(n, m):
                                row = 256 * ck + 128 * (n // 2) + 64 * (m // 2) + r0 // 2
                                return _split(c_w[4 * (n % 2) + 2 * (m % 2) + half + zero * (o + 1), pl.ds(row, 8), :])

                            terms = [_join(t) for t in _inner_terms(_LHS, o, block)]
                            for i, t in enumerate(terms):
                                cs_w[ck, 7 * o + i, half, r0 // 2:r0 // 2 + 8, :] = t
                            yield _digest(terms)

        UG = CFG.get('ug', 32)

        cu, ct, cg, cx_ = CFG.get('costs', (2, 2, 1, 1))

        def a_stream():
            make_consts()
            for b in range(4):
                for r0 in range(128 * b, min(C, 128 * (b + 1)), UG):
                    for v in prep_u(r0, UG):
                        yield cu * UG // 32, v
                for v in words_t(b):
                    yield ct, v
                for v in all_windows(b):
                    yield ct, v

        def d_stream():
            dc_s[...] = column(d_ref[...].reshape(1, C))
            for r0 in range(0, C, 32):
                for v in prep_g(r0, 32, gate):
                    yield cg, v
            for r0 in range(0, 256, 16):
                for o in range(7):
                    yield cx_, extract(0, r0, o, None, zero * (o + 1))

        a_total = cu * 14 * NB + ct * 4 * (NB + 64)
        d_total = cg * 14 * NB + cx_ * 112
        streams = []
        nprod = [0]
        later = {}
        LAG = CFG.get('lag', 0)

        def pump():
            for st_ in streams:
                gen, n, p0, p1, done = st_
                want = min(n, max(0, (nprod[0] - p0 + 1) * n // (p1 - p0)))
                while st_[4] < want:
                    cost, v = next(gen)
                    later.setdefault(nprod[0] + LAG, []).append(v)
                    st_[4] += cost
            due.extend(later.pop(nprod[0], []))
            nprod[0] += 1

        groups = [(j, b) for j in range(H // 2) for b in range(2)]
        units = [(g, jp) for c in range(0, NP, 2) for g in range(NF) for jp in (c, c + 1)]
        units += [(g, jp) for g in range(NF, len(groups)) for jp in range(NP)]
        NU = len(units)
        wts = {}
        lead = CFG.get('lead', 4)
        ua = CFG.get('ua', 32)
        ub = 8 * NP - lead
        ux = CFG.get('ux', 5)
        ud = CFG.get('ud', 96)
        waits = {ux: cx[1:] + cq[NF:8], ua: ga, ub: gb, ud: gd}
        if N0 < NF:
            waits[2 * N0 - 1] = cq[N0:NF]
        xe = [7 * ux + 2] + [7 * NF * 2 * c - 1 for c in (1, 2, 3)]
        for c in range(3):
            streams.append([(v for jp in (2 * c + 2, 2 * c + 3) for v in x_terms(jp)), 14, xe[c], xe[c + 1], 0])
        sl = CFG.get('slack', 4)
        PA, PB, PE = 7 * ua + sl, 7 * ub + sl, 7 * NU - 2 - LAG
        c_stream = ((1, v) for v in c_terms())
        nc = 4 * 2 * 8 * 7
        PD = 7 * ud + sl
        streams.append([a_stream(), a_total, PA, PD + CFG.get('aext', 0), 0])
        streams.append([c_stream, nc, PB, PE, 0])
        streams.append([d_stream(), d_total, PD + CFG.get('aext', 0), PE, 0])

        if not CFG.get('p0', 1):
            for c_ in cq + cx + ga + gc + gd:
                c_.wait()
            return
        _wait([cx[0]], 'wx0')
        list(x_terms(0))
        list(x_terms(1))
        _wait(cq[:N0], 'wq0')
        first_use = {}
        for u, (g, jp) in enumerate(units):
            first_use.setdefault(g, u)
        for u, (g, jp) in enumerate(units):
            if u in waits:
                _wait(waits[u], 'wu%d' % u)
            for g_, fu in first_use.items():
                if g_ not in wts and fu - (lead if g_ >= NF else 1) <= u:
                    back = CFG.get('wback', 8)
                    wts[g_] = wq_terms(*groups[g_], toks[-back] if len(toks) >= back else None)
            qproj(g, jp, [])
        assert all(st_[4] == st_[1] for st_ in streams) and not later, streams

    phase0()


    def phase1(k_s, kt_s, vt_s, wx_s, *s_s):
        LATE = CFG.get('late', (2, 5))
        EARLY = tuple(o for o in (0, 1, 3, 4, 6, 2, 5) if o not in LATE)
        UN = CFG.get('unroll', 1)

        def heads(it, carry):
            @pl.when(it == 1)
            def _():
                for c_ in g4:
                    c_.start()

            @pl.when(jnp.logical_and(it % 2 == 1, it < H - 1))
            def _():
                _wait(kv_copies((it + 1) // 2), 'wkv')

            @pl.when(jnp.logical_and(jnp.logical_and(it % 2 == 0, it > 0), it < H - 2))
            def _():
                for c_ in kv_copies(it // 2 + 1):
                    c_.start()

            zero = it // H
            toks = []
            due = []
            for r in range(UN):
                head(it * UN + r, None if UN % 2 else r % 2, zero, toks, due)
            return carry + zero

        def head(h, par, zero, toks, due):
            lane8 = lax.broadcasted_iota(I32, (8, 128), 1)
            sub8 = lax.broadcasted_iota(I32, (8, 128), 0)
            lane16 = lax.broadcasted_iota(I32, (16, 128), 1)
            sub16 = lax.broadcasted_iota(I32, (16, 128), 0)
            tri = (lax.broadcasted_iota(I32, (128, 128), 0) <= lax.broadcasted_iota(I32, (128, 128), 1))
            h_next = h + 1 if isinstance(h, int) else jnp.minimum(h + 1, H - 1)
            never = _never(zero)

            def after(x, tok):
                return _after(x, tok, never)

            def tied(lhs):
                return _tied(lhs, due, never)

            def tok(back):
                return toks[-back] if (back and len(toks) >= back) else None

            def chan_mm(c, gate):
                m_b = lane8 < after(128 - 2 * sub8, gate)
                gs = [jnp.broadcast_to(g_s[a, pl.ds(c, 1), :], (8, 128)) for a in range(NB)]
                bt = [pltpu.roll(jnp.where(m_b, gs[a], gs[a - 1] if a > 0 else jnp.uint32(0)), 0, 1,
                                 stride=2, stride_axis=0) for a in range(NB)]
                b1 = pltpu.bitcast(jnp.concatenate(bt[7::-1], axis=0), BF16)
                b2 = pltpu.bitcast(jnp.concatenate(bt[15:7:-1], axis=0), BF16)
                am = pltpu.bitcast(aw_s[pl.ds(c, 64, stride=PITCH), :], BF16)
                tick('C', 48)
                z1 = _dot(tied(am), b1)
                z2 = _dot(am[:64], b2)
                return c, z1[:64], z1[64:] + z2

            def chan_post(c, zlo, zhi):
                acc = car = None
                for p in range(8):
                    z = jnp.concatenate([zlo[8 * p:8 * p + 8], zhi[8 * p:8 * p + 8]], axis=0)
                    if p == 0:
                        acc = z
                    else:
                        z = pltpu.roll(z, 16 * p, 1)
                        cz = jnp.where(lane16 < 16 * p, z, 0.0)
                        acc = acc + z
                        car = cz if car is None else car + cz
                y = (acc - car) + jnp.where(sub16 > 0, pltpu.roll(car, 1, 0), 0.0)
                later(CFG.get('ly', 0), [y])
                if CFG.get('ylate'):
                    ys.append((c, y))
                else:
                    y_s[pl.ds(c, NB, stride=PITCH), :] = pltpu.bitcast(y, U32)
                if CFG.get('pd', 0):
                    due.append(y[:8])
                    due.append(y[8:])

            chans = [h * CPH + i for i in range(CPH)]
            ys, cs = [], []

            def x_stream(hh, outers):
                n = 16 * len(outers)
                for r0 in range(0, 256, 16):
                    for o in outers:
                        n -= 1
                        free = n < CFG.get('xfree', 0) and hh is h_next
                        d = extract(hh, r0, o, shift_of(hh, tok(CFG.get('xfb', 1)) if free else None), zero * (o + 1))
                        yield None if free else d

            streams = [[x_stream(h_next, EARLY), 16 * len(EARLY), 0, 0] + list(CFG['x1']),
                       [x_stream(h, LATE), 16 * len(LATE), 0, 0] + list(CFG['x2'])]

            clock, queue = [0], []

            def later(lag, vals):
                if lag:
                    queue.append((clock[0] + lag, _digest(vals)))

            def tick(kind, cycles):
                due.extend(v for t, v in queue if t <= clock[0])
                queue[:] = [q for q in queue if q[0] > clock[0]]
                clock[0] += cycles
                for st_ in streams:
                    gen, n, done, clk, kinds, c0, c1 = st_
                    if kind in kinds:
                        want = min(n, max(0, (clk - c0) * n // (c1 - c0)))
                        while st_[2] < want:
                            d = next(gen)
                            if d is not None:
                                due.append(d)
                            st_[2] += 1
                        st_[3] += cycles

            def shift_of(hh, gate):
                return after(jnp.full((8, 128), (1 - hh % 2) * 16, I32).astype(U32), gate)

            def kv_chunk(ck):
                def prod(o):
                    out = {}

                    def inner(i):
                        tick('M', 64)
                        lhs = jnp.concatenate([cs_s[ck, 7 * o + i, 0], cs_s[ck, 7 * o + i, 1]], axis=1)
                        m = _dot(tied(lhs), wx_s[7 * o + i])
                        if i == CFG.get('ti', 3):
                            toks.append(m[:8])
                        return m

                    _strassen(inner, lambda r, n, val: out.__setitem__((r, n), val))
                    return jnp.concatenate(
                        [jnp.concatenate([out[r, 0], out[r, 1]], axis=1) for r in range(2)], axis=0)

                def emit(R, N, val):
                    if N == 0:
                        rows = slice(512 * ck + 256 * R, 512 * ck + 256 * (R + 1))
                        if CFG.get('sq') and 2 * ck + R < NP - 1:
                            blocks = [val[:128, :128], val[:128, 128:], val[128:, :128], val[128:, 128:]]
                            for i in (0, 1, 4, 5, 6):
                                kt_s[i, 2 * ck + R] = _term(_LHS, i, blocks.__getitem__).astype(BF16)
                        val = val.astype(BF16)
                        k_s[0, rows, :] = val[:, :128]
                        k_s[1, rows, :] = val[:, 128:]
                    else:
                        for r in range(2):
                            for n in range(2):
                                v = val[128 * r:128 * (r + 1), 128 * n:128 * (n + 1)].T.astype(BF16)
                                vt_s[4 * ck + 2 * R + r, 128 * n:128 * (n + 1), :] = v
                                later(CFG.get('lv', 0), [v[112:]])

                return _strassen_steps(prod, emit)

            kv = [kv_chunk(ck) for ck in range(4)]

            def k_rows(r0, r1):
                return jnp.concatenate([k_s[0, r0:r1, :], k_s[1, r0:r1, :]], axis=1)

            def q_cols(r0, r1):
                return jnp.concatenate([qc_s[h, t] for t in range(r0 // 128, r1 // 128)], axis=1)

            mx, pr = {}, {}

            def qk_strassen(t):
                buf = s_s[t % 2]
                for e in range(2):
                    jq = 2 * t + e
                    run = [None, None]

                    def put(n, r0, val):
                        buf[2 * e + n, r0:r0 + val.shape[0], :] = val
                        for r in range(0, val.shape[0], 8):
                            v = val[r:r + 8]
                            run[n] = v if run[n] is None else jnp.maximum(run[n], v)

                    if jq > 0:
                        raw = [qc_w[h, 2 * jq + n % 2, 64 * (n // 2):64 * (n // 2 + 1), :] for n in range(4)]
                        full = [_split(w) for w in raw]
                        qt = [pltpu.bitcast(raw[_RHS[i][0]] if len(_RHS[i]) == 1
                                            else _join(_term(_RHS, i, full.__getitem__)), BF16) for i in range(7)]
                    KB = CFG.get('kb', 1)
                    for jp0 in range(0, jq, KB):
                        jps = range(jp0, min(jq, jp0 + KB))
                        for x in CFG.get('qe', {}).get((jq, jp0), '').split():
                            softmax(int(x[0]), int(x[1]), True)

                        def prod(i):
                            tick('Q', 32 * len(jps))
                            if i == 2:
                                lhs = [k_s[0, 256 * jp:256 * jp + 128, :] for jp in jps]
                            elif i == 3:
                                lhs = [k_s[1, 256 * jp + 128:256 * jp + 256, :] for jp in jps]
                            else:
                                lhs = [kt_s[i, jp] for jp in jps]
                            m = _dot(tied(jnp.concatenate(lhs, axis=0)), qt[i])
                            if i == 3:
                                toks.append(m[:8])
                            return m

                        def emit(r, n, val):
                            for k, jp in enumerate(jps):
                                put(n, 256 * jp + 128 * r, val[128 * k:128 * (k + 1)])

                        _strassen(prod, emit)
                    q0 = 256 * jq
                    for n in range(2):
                        tick('Q', 64 * (n + 1))
                        sd = _dot(tied(k_rows(q0, q0 + 128 * (n + 1))), qc_s[h, 2 * jq + n])
                        if n:
                            put(n, q0, sd[:128])
                        put(n, q0 + 128 * n, jnp.where(tri, sd[128 * n:], NEG))
                        mx[(t, 2 * e + n)] = jnp.max(run[n], axis=0, keepdims=True)
                    toks.append(sd[:8])

            def qk(t):
                if CFG.get('sq'):
                    return qk_strassen(t)
                q0 = t * TQ
                if q0 > 0:
                    QR = CFG.get('qr', 2048)
                    rect = []
                    for r0 in range(0, q0, QR):
                        for e in CFG.get('qe', {}).get((t, r0 // QR), '').split():
                            softmax(int(e[0]), int(e[1]), True)
                        tick('Q', min(QR, q0 - r0) * 2)
                        rect.append(_dot(tied(k_rows(r0, min(q0, r0 + QR))), q_cols(q0, q0 + TQ)))
                    s_rect = jnp.concatenate(rect, axis=0) if len(rect) > 1 else rect[0]
                    toks.append(s_rect[:8, :128])
                for u in range(TQ // 128):
                    qs = q0 + u * 128
                    if u == 0:
                        for e in CFG.get('qe', {}).get((t, 'd'), '').split():
                            softmax(int(e[0]), int(e[1]), True)
                    tick('Q', 64 * (u + 1))
                    sd = _dot(tied(k_rows(q0, qs + 128)), q_cols(qs, qs + 128))
                    parts = []
                    if q0 > 0:
                        parts.append(s_rect[:, u * 128:(u + 1) * 128])
                    if u > 0:
                        parts.append(sd[:u * 128, :])
                    parts.append(jnp.where(tri, sd[u * 128:, :], NEG))
                    s = jnp.concatenate(parts, axis=0) if len(parts) > 1 else parts[0]
                    s_s[t % 2][u, 0:qs + 128, :] = s
                    mx[(t, u)] = jnp.max(s, axis=0, keepdims=True)
                toks.append(sd[:8])
                if CFG.get('clob', 1):
                    s_s[t % 2][zero, S:S + 8, :] = sd[:8]

            def softmax(t, u, deadline):
                qs = t * TQ + u * 128
                p = jnp.exp2(s_s[t % 2][u if CFG.get('clob', 1) else u + zero, 0:qs + 128, :] - mx.pop((t, u)))
                NA = CFG.get('na', 0)
                if NA:
                    accs = [None] * NA
                    for r in range(p.shape[0] // 8):
                        v = p[8 * r:8 * (r + 1)]
                        accs[r % NA] = v if accs[r % NA] is None else accs[r % NA] + v
                    while len(accs) > 1:
                        accs = [a + b for a, b in zip(accs[::2], accs[1::2])]
                    part = accs[0]
                    rl = 1.0 / jnp.sum(part, axis=0, keepdims=True)
                else:
                    rl = part = 1.0 / jnp.sum(p, axis=0, keepdims=True)
                pb = p.astype(BF16)
                pr[(t, u)] = (pb, rl)
                if deadline:
                    due.append(part)
                    if CFG.get('pk'):
                        due.append(_digest([pb]))

            def pv(t, u):
                if (t, u) not in pr:
                    softmax(t, u, False)
                p, rl = pr.pop((t, u))
                qs = t * TQ + u * 128
                vt = jnp.concatenate([vt_s[i] for i in range(qs // 128 + 1)], axis=1)
                PH = D // CFG.get('ph', 1)
                for d0 in range(0, D, PH):
                    tick('P', (qs + 128) * PH // 512)
                    ctx = _dot(tied(vt[d0:d0 + PH]), p)
                    v = (ctx * rl).astype(BF16)
                    later(CFG.get('lc', 0), [v])
                    if CFG.get('clate'):
                        cs.append((qs // 128, d0, PH, v))
                    else:
                        qc_s[h, qs // 128, d0:d0 + PH, :] = v
                toks.append(ctx[:8])

            CG, XG = CFG.get('cg', 0), CFG.get('xg', 0)
            pend = []
            def run_step(st_):
                kind, arg = st_[0], st_[1:]
                if kind == 'E':
                    softmax(int(arg[0]), int(arg[1]), True)
                    return
                old = list(pend)
                pend.clear()
                if kind == 'C':
                    for _ in range(int(arg)):
                        pend.append(chan_mm(chans.pop(0), tok(CG)))
                elif kind == 'M':
                    for o in arg[1:]:
                        kv[int(arg[0])](int(o))
                elif kind == 'Q':
                    qk(int(arg))
                elif kind == 'P':
                    for u in ([int(arg[1])] if len(arg) > 1 else range(TQ // 128)):
                        pv(int(arg[0]), u)
                for args in old:
                    chan_post(*args)

            for seg in [g for g in CFG['sched'].split('|') if g.strip()]:
                if CFG.get('scopes') and '|' in CFG['sched']:
                    with jax.named_scope('s_' + seg.split()[0]):
                        for st_ in seg.split():
                            run_step(st_)
                else:
                    for st_ in seg.split():
                        run_step(st_)
            for c, y in ys:
                y_s[pl.ds(c, NB, stride=PITCH), :] = pltpu.bitcast(y, U32)
            for t, d0, n, v in cs:
                qc_s[h, t, d0:d0 + n, :] = v
            assert all(st_[1] == st_[2] for st_ in streams), [st_[1:] for st_ in streams]
            assert CFG.get('noassert') or not chans and not pend and (not due or CFG.get('pd')) and not pr and not mx

        if CFG.get('p1', 1):
            return lax.fori_loop(0, H // UN, heads, 0)
        else:
            _wait(g3b, 'wg3b')
            for c_ in g4:
                c_.start()

            def keep(h, carry):
                r = pl.multiple_of(h * 16, 16)
                t = (qc_s[h, h, 0:16, :].astype(F32) + cs_s[h % 4, h, h % 2, 0:16, :].astype(F32)
                     + pltpu.bitcast(aw_s[pl.ds(r, 16), :] + g_s[h, pl.ds(r, 16), :], F32)
                     + wx_s[h, pl.ds(r, 16), :].astype(F32))
                y_s[pl.ds(r, 16), :] = pltpu.bitcast(t, U32)
                return carry + h // H
            return lax.fori_loop(0, H, keep, 0)

    zero_end = phase1(k_s, kt_s, vt_s, wx_s, sa_s, sb_s)

    def phase2():
        _wait(g4, 'wg4')
        HH = H // 2

        def wo_block(rh, kh):
            return jnp.concatenate(
                [xs_s[C * (H * b + h) + CH * rh:C * (H * b + h) + CH * (rh + 1), :]
                 for h in range(HH * kh, HH * (kh + 1)) for b in range(2)], axis=1)

        raw = [wo_block(0, 0), wo_block(1, 0), wo_block(0, 1), wo_block(1, 1)]
        wt = [t.astype(BF16) for t in _rhs_terms(*[t.astype(F32) for t in raw])]
        wt[1], wt[4] = raw[0], raw[3]
        outs = []
        due, late = [], []
        DL = CFG.get('dl', 3)
        never = _never(zero_end)

        def put(t, b, z, opaque=False):
            o = z.T.astype(BF16)
            r0 = pl.multiple_of(zero_end * 16 + 128 * t, 16) if opaque else 128 * t
            c_s[b, pl.ds(r0, 128), :] = o
            late.append(pltpu.bitcast(o[112:], U32))

        for jp in range(CFG.get('np2', NP) if CFG.get('p2', 1) else 0):
            def ctx_block(r, kh):
                return jnp.concatenate([qc_s[h, 2 * jp + r] for h in range(HH * kh, HH * (kh + 1))], axis=0)

            craw = [ctx_block(0, 0), ctx_block(0, 1), ctx_block(1, 0), ctx_block(1, 1)]
            ct = [t.astype(BF16) for t in _lhs_terms(*[t.astype(F32) for t in craw])]
            ct[2], ct[3] = craw[0], craw[3]
            za = {}
            prev_late = list(late)
            late.clear()
            for r in range(2):
                t = 2 * jp + r
                za[r] = (pltpu.bitcast(y_s[t * PITCH:t * PITCH + C, :], F32)
                         * x_s[:, 128 * t:128 * (t + 1)].astype(F32))
                for b in range(3):
                    put(t, b, za[r][128 * b:128 * (b + 1)], opaque=(r == 0 and b == 0 and jp > 0))
            a_late = list(late)
            late.clear()
            res = {}
            count = [0]

            def prod(i):
                if count[0] == DL:
                    due.extend(prev_late)
                if count[0] == 6:
                    due.extend(a_late)
                count[0] += 1
                return _dot(_tied(wt[i], due, never), ct[i])

            _strassen(prod, lambda r, c, val: res.__setitem__((r, c), val), order=(1, 4, 3, 2, 0, 5, 6))
            for r in (1, 0):
                z = jnp.concatenate([za[r][384:], res[(r, 0)], res[(r, 1)]], axis=0)
                for b in (3, 2, 1, 0):
                    put(2 * jp + r, 3 + b, z[128 * b:128 * (b + 1)])
            rows = pl.ds(128 * jp, 128)
            for b in range(7):
                oc = cp(c_w.at[b, rows], o_hbm.at[rows, pl.ds(128 * b, 128)], 26 + jp)
                oc.start()
                outs.append(oc)
        if not CFG.get('p2', 1):
            def keep(h, carry):
                r = pl.multiple_of(h * 16, 16)
                c_s[0, pl.ds(r, 16), :] = pltpu.bitcast(y_s[pl.ds(r, 16), :], F32).astype(BF16) + qc_s[h, h, 0:16, :]
                return carry
            lax.fori_loop(0, H, keep, 0)
            oc = cp(c_w.at[0, pl.ds(0, 128)], o_hbm.at[pl.ds(0, 128), pl.ds(0, 128)], 26)
            oc.start()
            outs.append(oc)
        _wait(outs, 'wout')

    phase2()


def _tiles(w):
    rows = w.shape[0]
    return w.reshape(rows, 2, 8, 2, 128).transpose(0, 1, 3, 2, 4).reshape(rows, 32, 128)


@jax.jit
def pallas_concat_heads__ssm_conv_h3__compressed_kv_cla__prompt_kernel(
    A_q: jax.Array,
    A_k: jax.Array,
    A_v: jax.Array,
    A_shift_k: jax.Array,
    A_ssm_k: jax.Array,
    A_ssm_D: jax.Array,
    B_x: jax.Array,
    B_c_kv: jax.Array,
    B_w_q: jax.Array,
    B_w_uk: jax.Array,
    B_w_uv: jax.Array,
    B_w_o: jax.Array,
):
    hbm = pl.BlockSpec(memory_space=pltpu.HBM)
    out = pl.pallas_call(
        _kernel,
        in_specs=[hbm] * 12,
        out_specs=hbm,
        out_shape=jax.ShapeDtypeStruct((S, 2 * C), BF16),
        scratch_shapes=[
            pltpu.VMEM((8, S // 2, 128), U32),
            pltpu.VMEM((4, 49, 2, 64, 128), U32),
            pltpu.VMEM((2, 4, DC, 128), U32),
            pltpu.VMEM((H, NB, D // 2, 128), U32),
            pltpu.VMEM((64 * PITCH, 128), U32),
            pltpu.VMEM((NB, C, 128), U32),
            pltpu.VMEM((NB * PITCH, 128), U32),
            pltpu.VMEM((CH, S), U32),
            pltpu.VMEM((512, 128), F32),
            pltpu.VMEM((2, S // 2, 128), U32),
            pltpu.VMEM((7, NP, 64, 128), U32),
            pltpu.VMEM((NB, D // 2, 128), U32),
            pltpu.VMEM((49, DC // 8, 128), U32),
            pltpu.VMEM((TQ // 128, S + 8, 128), F32),
            pltpu.VMEM((TQ // 128, S + 8, 128), F32),
            pltpu.VMEM((CH, S), U32),
            pltpu.VMEM((7 * NP * 128, 128), U32),
            pltpu.VMEM((CH, S), U32),
            pltpu.VMEM((CH, S), U32),
            pltpu.VMEM((2, 8, 128, 128), F32),
            pltpu.VMEM((4, C), BF16),
            pltpu.VMEM((C,), BF16),
            pltpu.SemaphoreType.DMA((35,)),
        ],
        compiler_params=pltpu.CompilerParams(vmem_limit_bytes=127 * 2 ** 20),
    )(
        A_q[0].T, A_k[0].T, A_v[0].T, A_shift_k.T, A_ssm_k, A_ssm_D, B_x[0].T, B_c_kv[0],
        _tiles(B_w_q), _tiles(B_w_uk), _tiles(B_w_uv),
        jnp.swapaxes(B_w_o, 1, 2).reshape(H * C, D),
    )
    return out.reshape(1, S, 2 * C)
```

```python
import math

import jax
import jax.numpy as jnp
from jax import lax
import jax.experimental.pallas as pl
import jax.experimental.pallas.tpu as pltpu

F32 = jnp.float32
BF16 = jnp.bfloat16
U32 = jnp.uint32
I32 = jnp.int32

S = 2048
C = 448
H = 16
D = 256
DC = 1024
NB = S // 128
NP = NB // 2
CH = C // 2
PITCH = 520
CPH = C // H
TQ = 512
NT = (((1,), (1,)), ((), ()))
LOG2E = math.log2(math.e)
QSCALE = (D ** -0.5) * LOG2E
NEG = -1e9 * LOG2E
HI_MASK = 0xFFFF0000
CFG = dict(ua=30,ud=96,nf=8,n0=3,ux=13,gback=8,slack=8,late=(),x2=('P',0,1),mh=2,qh=2,cg=5,mw=2,lw=2,x1=('P',1500,7580),sched='M001 C2 M034 C2 M06 M101 C2 Q01 M134 C2 M16 M201 C2 Q23 M234 C2 M26 M301 C2 E0 E1 E2 Q45 M334 C2 M36 E3 M02 C2 Q67 M05 C2 E4 M12 C2 E5012 M15 C2 E5345 M22 C2 E6012 M25 C2 E63456 M32 M35 P01234567')


def _wait(copies, name):
    if CFG.get('scopes'):
        with jax.named_scope(name):
            for c_ in copies:
                c_.wait()
    else:
        for c_ in copies:
            c_.wait()


def _dot(a, b):
    return jnp.dot(a, b, preferred_element_type=F32)


def _dot_nt(a, b):
    return lax.dot_general(a, b, NT, preferred_element_type=F32)


def _lo(x):
    return pltpu.bitcast(x << 16, F32)


def _hi(x):
    return pltpu.bitcast(x & jnp.uint32(HI_MASK), F32)


def _pack(even, odd):
    return pltpu.pack_elementwise([even, odd], packed_dtype=BF16).astype(U32)


def _split(words):
    return jnp.concatenate([_lo(words), _hi(words)], axis=0)


def _join32(x):
    return jnp.concatenate([_pack(x[m:m + 16], x[m + 16:m + 32]) for m in range(0, x.shape[0], 32)], axis=0)


def _join(x):
    n = x.shape[0] // 2
    return _pack(x[:n], x[n:])


def _head_cols(w_s, h, rows):
    out = []
    for b in range(2):
        x = w_s[b, pl.ds(h // 2, rows, stride=8), :]
        if isinstance(h, int):
            out.append(_lo(x) if h % 2 == 0 else _hi(x))
        else:
            out.append(_hi(x << ((1 - h % 2) * 16).astype(U32)))
    return out


_LHS = ((0, 1, 3), (2, 1, 3), (0,), (3,), (0, 1, 1), (2, -1, 0), (1, -1, 3))
_RHS = ((0, 1, 3), (0,), (1, -1, 3), (2, -1, 0), (3,), (0, 1, 1), (2, 1, 3))


def _term(table, i, block):
    spec = table[i]
    if len(spec) == 1:
        return block(spec[0])
    return block(spec[0]) + block(spec[2]) if spec[1] > 0 else block(spec[0]) - block(spec[2])


def _lhs_terms(*blocks):
    return [_term(_LHS, i, blocks.__getitem__) for i in range(7)]


def _rhs_terms(*blocks):
    return [_term(_RHS, i, blocks.__getitem__) for i in range(7)]


def _inner_terms(table, o, block):
    sub = [_term(table, o, lambda n: block(n, m)) for m in range(4)]
    return [_term(table, i, sub.__getitem__) for i in range(7)]


def _strassen_steps(prod, emit):
    uses = {(0, 0): {0: 1, 3: 1, 4: -1, 6: 1}, (0, 1): {2: 1, 4: 1},
            (1, 0): {1: 1, 3: 1}, (1, 1): {0: 1, 1: -1, 2: 1, 5: 1}}
    acc = {}
    neg = {}

    def step(i):
        m = prod(i)
        for key, terms in uses.items():
            if i not in terms:
                continue
            sign = terms.pop(i)
            if key not in acc:
                acc[key] = m
                neg[key] = sign < 0
            elif neg[key]:
                assert sign > 0
                acc[key] = m - acc[key]
                neg[key] = False
            else:
                acc[key] = acc[key] + m if sign > 0 else acc[key] - m
            if not terms:
                emit(key[0], key[1], acc.pop(key))

    return step


def _strassen(prod, emit, order=(0, 1, 3, 2, 4, 5, 6)):
    step = _strassen_steps(prod, emit)
    for i in order:
        step(i)


def _mult(i, n):
    return i if isinstance(i, int) else pl.multiple_of(i, n)


def _never(zero):
    return lax.broadcasted_iota(I32, (8, 128), 1) < zero


def _after(x, tok, never):
    if tok is None:
        return x
    return jnp.where(never, pltpu.bitcast(tok, x.dtype), x)


def _tied(lhs, due, never):
    if not due:
        return lhs
    t = None
    for d in due:
        d = pltpu.bitcast(jnp.broadcast_to(d, (8, 128)), U32)
        t = d if t is None else t ^ d
    due.clear()
    x = pltpu.bitcast(_after(pltpu.bitcast(lhs[:16, :128], U32), t, never), BF16)
    if lhs.shape[1] > 128:
        x = jnp.concatenate([x, lhs[:16, 128:]], axis=1)
    return jnp.concatenate([x, lhs[16:]], axis=0) if lhs.shape[0] > 16 else x


def _digest(vals):
    acc = None
    words = [v if v.dtype == U32 else pltpu.bitcast(v, U32) for v in vals]
    for r in range(words[0].shape[0] // 8):
        for w in words:
            w = w[8 * r:8 * (r + 1)]
            acc = w if acc is None else acc ^ w
    return acc


class _Packed:
    def __init__(self, ref):
        self.ref = ref

    def _index(self, idx):
        idx = idx if isinstance(idx, tuple) else (idx,)
        axis = len(self.ref.shape) - 2
        if len(idx) <= axis:
            return idx + (slice(None),) * (axis + 2 - len(idx))
        r = idx[axis]
        if isinstance(r, slice):
            r = slice(None if r.start is None else r.start // 2, None if r.stop is None else r.stop // 2)
        else:
            r = pl.ds(_mult(r.start // 2, 8), r.size // 2)
        return idx[:axis] + (r,) + idx[axis + 1:]

    def __getitem__(self, idx):
        return pltpu.bitcast(self.ref[self._index(idx)], BF16)

    def __setitem__(self, idx, val):
        self.ref[self._index(idx)] = pltpu.bitcast(val, U32)


def _kernel(qa_hbm, ka_hbm, va_hbm, sk_hbm, hk_hbm, d_hbm, x_hbm, c_hbm, wq_hbm, wk_hbm, wv_hbm, wo_hbm,
            o_hbm,
            c_s, cs_s, wp_s, qc_s, aw_s, g_s, y_s, hk_s, dc_s, k_s, kt_s, vt_s, vx_s, wx_s, sa_s, sb_s, x_s, xs_s, ka_s, va_s, wt_s, sk_ref, d_ref, sems):
    def cp(src, dst, i):
        return pltpu.make_async_copy(src, dst, sems.at[i])

    c_w, xs_w, x_w, ka_w, va_w, hk_w, cs_w, wx_w, qc_w = c_s, xs_s, x_s, ka_s, va_s, hk_s, cs_s, wx_s, qc_s
    k_w, kt_w = k_s, kt_s
    c_s, cs_s, qc_s, k_s, kt_s, vt_s, vx_s, wx_s, xs_s, x_s, ka_s, va_s, hk_s = (
        _Packed(r) for r in (c_s, cs_s, qc_s, k_s, kt_s, vt_s, vx_s, wx_s, xs_s, x_s, ka_s, va_s, hk_s))
    qa_hbm, ka_hbm, va_hbm, hk_hbm, x_hbm, c_hbm, wo_hbm, o_hbm = (
        r.bitcast(U32) for r in (qa_hbm, ka_hbm, va_hbm, hk_hbm, x_hbm, c_hbm, wo_hbm, o_hbm))
    wq32 = wq_hbm.bitcast(U32)
    wk32 = wk_hbm.bitcast(U32)
    wv32 = wv_hbm.bitcast(U32)
    gc = [cp(c_hbm.at[:, pl.ds(128 * b, 128)], c_w.at[b], 8 + b) for b in range(8)]

    def word_row(pair, b):
        return 8 * (pair // 4) + 4 * b + pair % 4

    def kv_copies(pair):
        return [cp(w.at[:, word_row(pair, b), :], wp_s.at[pair % 2, 2 * n + b], 16 + pair % 2)
                for n, w in enumerate((wk32, wv32)) for b in range(2)]

    g3 = kv_copies(0)
    g3b = kv_copies(1)
    g4 = [cp(qa_hbm, x_w, 21)] + [cp(wo_hbm.at[:, pl.ds(128 * b, 128)], xs_w.at[pl.ds(H * CH * b, H * CH)], 6 + b)
                                  for b in range(2)]

    def delayed(ref, rows, sg, n, gate=None):
        cur = pltpu.bitcast(ref[rows, 128 * sg:128 * (sg + 1)], U32)
        lane = lax.broadcasted_iota(I32, (8, 128), 1)
        if gate is not None:
            lane = gate(lane)
        lane = jnp.concatenate([lane] * (cur.shape[0] // 8), axis=0)
        prev = pltpu.bitcast(ref[rows, 128 * (sg - 1):128 * sg], U32) if sg > 0 else jnp.uint32(0)
        x = pltpu.roll(jnp.where(lane < 128 - n, cur, prev), n, 1)
        return pltpu.bitcast(x, BF16).astype(F32)

    def gated_t(x, gate):
        if gate is not None:
            x = jnp.concatenate([gate(x[:8]), x[8:]], axis=0)
        return x.T

    def windows(b, q, e, js, gate=None):
        out = []
        for j in js:
            parts = []
            for sg in range(2 * j - 6, 2 * j + 2):
                if sg < 0:
                    parts.append(jnp.zeros((16, 128), U32))
                else:
                    parts.append(pltpu.bitcast(sb_s[pl.ds(S * b + 128 * sg + 32 * q + 16 * e, 16), :], U32))
            plane = 32 * (j // 4) + 8 * q + 4 * e + j % 4
            win = gated_t(jnp.concatenate(parts, axis=0), gate)
            aw_s[pl.ds(_mult(plane * PITCH + 128 * b, 8), 128), :] = win
            out.append(win[120:])
        return out

    def prep_g(r0, n, gate=None):
        rows = pl.ds(_mult(r0, 16), n)
        lane = lax.broadcasted_iota(I32, (n, 128), 1)
        for a in range(NB):
            hf = hk_s[rows, 128 * a:128 * (a + 1)].astype(F32)
            hs = delayed(hk_s, rows, a, 1, gate)
            if a == 0:
                hf = jnp.where(lane == 0, hf + dc_s[rows, :], hf)
                hs = jnp.where(lane == 1, hs + dc_s[rows, :], hs)
            wrd = pltpu.pack_elementwise([hf, hs], packed_dtype=BF16).astype(U32)
            g_s[a, rows, :] = wrd
            yield _digest([wrd])

    def extract(h, r0, o, shift, z):
        def block(n, kq, b):
            x = jnp.concatenate([wp_s[(h // 2) % 2 + z, 2 * n + b, pl.ds(256 * kq + r0 + e, 8, stride=2), :]
                                 for e in range(2)], axis=0)
            if isinstance(h, int):
                return _lo(x) if h % 2 == 0 else _hi(x)
            return _hi(x << jnp.concatenate([shift] * 2, axis=0))

        terms = [_join(t) for t in _inner_terms(
            _RHS, o, lambda n, m: block(n % 2, 2 * (n // 2) + m // 2, m % 2))]
        for i, t in enumerate(terms):
            wx_w[7 * o + i, r0 // 2:r0 // 2 + 8, :] = t
        return _digest(terms)

    def phase0():
        XC = 512
        NF = CFG.get('nf', 4)
        N0 = CFG.get('n0', NF)
        cq = [cp(wq32.at[:, word_row(g // 2, g % 2), :], y_s.at[pl.ds(C * g, C)],
                 0 if g < N0 else 19 if g < NF else 1 if g < 8 else 18)
              for g in range(H)]
        cx = [cp(x_hbm.at[:, pl.ds(XC * i, XC)], x_w.at[:, pl.ds(XC * i, XC)], 22 + i) for i in range(S // XC)]
        ga = [cp(sk_hbm, sk_ref, 2), cp(ka_hbm, ka_w, 3), cp(va_hbm, va_w, 4)]
        gb = cq[8:] + gc
        gd = [cp(d_hbm, d_ref, 20), cp(hk_hbm, hk_w, 5)] + g3
        rest = cx[1:] + cq[NF:8] + ga + gb + gd + g3b
        for c_ in [cx[0]] + cq[:NF] + rest:
            c_.start()
        zero = pl.semaphore_read(sems.at[34])
        never = _never(zero)
        due = []
        toks = []

        def pad_rows(t):
            return jnp.concatenate([t, jnp.zeros((256 - CH, 128), t.dtype)], axis=0)

        def wq_terms(j, b, gate):
            x = y_s[C * (2 * j + b):C * (2 * j + b + 1), :]
            g16 = jnp.concatenate([_after(jnp.full((8, 128), 16, U32), gate, never)] * (C // 8), axis=0)
            gm = jnp.concatenate([_after(jnp.full((8, 128), HI_MASK, U32), gate, never)] * (C // 8), axis=0)
            lo, hi = pltpu.bitcast(x << g16, F32), pltpu.bitcast(x & gm, F32)
            blocks = [pad_rows(t).T for t in (lo[:CH], hi[:CH], lo[CH:], hi[CH:])]
            if not CFG.get('q4', 1):
                return [t.astype(BF16) for t in _rhs_terms(*blocks)]
            slot = (2 * j + b) % 2
            for n, t in enumerate(blocks):
                for k in range(2):
                    wt_s[slot, 2 * n + k] = t[:, 128 * k:128 * (k + 1)]
            quarter = [[jnp.concatenate([wt_s[slot, 2 * n + k, pl.ds(e, 32, stride=4), :] for k in range(2)], axis=1)
                        for n in range(4)] for e in range(4)]
            terms = [_rhs_terms(*q) for q in quarter]
            out = []
            for i in range(7):
                ev, od = _pack(terms[0][i], terms[2][i]), _pack(terms[1][i], terms[3][i])
                rows = [w[8 * m:8 * (m + 1)] for m in range(4) for w in (ev, od)]
                out.append(pltpu.bitcast(jnp.concatenate(rows, axis=0), BF16))
            return out

        def x_terms(jp):
            top = slice(256 * jp, 256 * jp + 128)
            bot = slice(256 * jp + 128, 256 * jp + 256)
            for i in range(7):
                xs_s[256 * (NP * i + jp) + CH:256 * (NP * i + jp + 1), :] = jnp.zeros((256 - CH, 128), BF16)
            for r in range(0, CH, 32):
                lo, hi = slice(r // 2, r // 2 + 16), slice((CH + r) // 2, (CH + r) // 2 + 16)
                blocks = [x_w[lo, top], x_w[hi, top], x_w[lo, bot], x_w[hi, bot]]
                terms = [_join(t) for t in _lhs_terms(*[_split(t) for t in blocks])]
                terms[2], terms[3] = blocks[0], blocks[3]
                for i, t in enumerate(terms):
                    xs_w[128 * (NP * i + jp) + r // 2:128 * (NP * i + jp) + r // 2 + 16, :] = t
                yield 1, _digest(terms)

        def qproj(g, jp, waits):
            j, b = groups[g]
            for c_ in waits:
                c_.wait()
            if False:
                x_terms(jp)
                x_terms(jp + 1)

            def prod(i):
                pump()
                m = _dot(_tied(wts[g][i], due, never), xs_s[256 * (NP * i + jp):256 * (NP * i + jp + 1), :])
                toks.append(m[:8])
                return m

            def emit(r, c, val):
                val = val * QSCALE
                if CFG.get('q4', 1):
                    qc_w[2 * j + c, 2 * jp + r, 64 * b:64 * (b + 1), :] = _join32(val)
                else:
                    qc_s[2 * j + c, 2 * jp + r, 128 * b:128 * (b + 1), :] = val.astype(BF16)

            _strassen(prod, emit)

        def column(row):
            row = jnp.concatenate([row.astype(F32), jnp.zeros((1, 512 - C), F32)], axis=1)
            return jnp.broadcast_to(row, (128, 512)).T

        consts = {}

        def make_consts():
            consts['taps'] = [column(sk_ref[j:j + 1, :]) for j in range(4)]

        def gate(x):
            back = CFG.get('gback', 6)
            return _after(x, toks[-back], never) if back else x

        def prep_u(r0, n):
            rows = slice(r0, r0 + n)
            tp = [t[rows] for t in consts['taps']]
            prev = jnp.zeros((n, 128), F32)
            for sg in range(NB):
                cols = slice(128 * sg, 128 * (sg + 1))
                ksh = ((delayed(ka_s, rows, sg, 3, gate) * tp[3] + delayed(ka_s, rows, sg, 2, gate) * tp[2])
                       + (delayed(ka_s, rows, sg, 1, gate) * tp[1] + ka_s[rows, cols].astype(F32) * tp[0]))
                kv = ksh * va_s[rows, cols].astype(F32)
                wrd = pltpu.pack_elementwise([prev, kv], packed_dtype=BF16).astype(U32)
                sa_s[C * sg + r0:C * sg + r0 + n, :] = pltpu.bitcast(wrd, F32)
                prev = kv
                yield _digest([wrd])

        def words_t(b):
            for sg in range(NB):
                r0 = C * sg + 128 * b
                if b < 3:
                    wrd = sa_s[r0:r0 + 128, :]
                else:
                    wrd = jnp.concatenate([sa_s[r0:r0 + C - 384, :], jnp.zeros((512 - C, 128), F32)], axis=0)
                wrd = gated_t(pltpu.bitcast(wrd, U32), gate)
                sb_s[S * b + 128 * sg:S * b + 128 * (sg + 1), :] = pltpu.bitcast(wrd, F32)
                yield wrd[120:]

        def all_windows(b):
            for p in range(8):
                for j in range(8):
                    yield windows(b, p // 2, p % 2, [j], gate)[0]

        def c_terms():
            for ck in range(4):
                for half in range(2):
                    for r0 in range(0, 128, 16):
                        for o in range(7):
                            def block(n, m):
                                row = 256 * ck + 128 * (n // 2) + 64 * (m // 2) + 16 * (r0 // 32)
                                col = 4 * (n % 2) + 2 * (m % 2) + half + zero * (o + 1)
                                w = jnp.concatenate([c_w[col, pl.ds(row + e, 8, stride=2), :] for e in range(2)], axis=0)
                                return _hi(w) if r0 % 32 else _lo(w)

                            terms = [_join(t) for t in _inner_terms(_LHS, o, block)]
                            for i, t in enumerate(terms):
                                cs_w[ck, 7 * o + i, half, r0 // 2:r0 // 2 + 8, :] = t
                            yield _digest(terms)

        UG = CFG.get('ug', 32)

        cu, ct, cg, cx_ = CFG.get('costs', (2, 2, 1, 1))

        def a_stream():
            make_consts()
            for b in range(4):
                for r0 in range(128 * b, min(C, 128 * (b + 1)), UG):
                    for v in prep_u(r0, UG):
                        yield cu * UG // 32, v
                for v in words_t(b):
                    yield ct, v
                for v in all_windows(b):
                    yield ct, v

        def d_stream():
            dc_s[...] = column(d_ref[...].reshape(1, C))
            for r0 in range(0, C, 32):
                for v in prep_g(r0, 32, gate):
                    yield cg, v
            for r0 in range(0, 256, 16):
                for o in range(7):
                    yield cx_, extract(0, r0, o, None, zero * (o + 1))

        a_total = cu * 14 * NB + ct * 4 * (NB + 64)
        d_total = cg * 14 * NB + cx_ * 112
        streams = []
        nprod = [0]
        later = {}
        LAG = CFG.get('lag', 0)

        def pump():
            for st_ in streams:
                gen, n, p0, p1, done = st_
                want = min(n, max(0, (nprod[0] - p0 + 1) * n // (p1 - p0)))
                while st_[4] < want:
                    cost, v = next(gen)
                    later.setdefault(nprod[0] + LAG, []).append(v)
                    st_[4] += cost
            due.extend(later.pop(nprod[0], []))
            nprod[0] += 1

        groups = [(j, b) for j in range(H // 2) for b in range(2)]
        units = [(g, jp) for c in range(0, NP, 2) for g in range(NF) for jp in (c, c + 1)]
        units += [(g, jp) for g in range(NF, len(groups)) for jp in range(NP)]
        NU = len(units)
        wts = {}
        lead = CFG.get('lead', 4)
        ua = CFG.get('ua', 32)
        ub = 8 * NP - lead
        ux = CFG.get('ux', 5)
        ud = CFG.get('ud', 96)
        waits = {ux: cx[1:] + cq[NF:8], ua: ga, ub: gb, ud: gd}
        if N0 < NF:
            waits[2 * N0 - 1] = cq[N0:NF]
        xe = [7 * ux + 2] + [7 * NF * 2 * c - 1 for c in (1, 2, 3)]
        for c in range(3):
            streams.append([(v for jp in (2 * c + 2, 2 * c + 3) for v in x_terms(jp)), 14, xe[c], xe[c + 1], 0])
        sl = CFG.get('slack', 4)
        PA, PB, PE = 7 * ua + sl, 7 * ub + sl, 7 * NU - 2 - LAG
        c_stream = ((1, v) for v in c_terms())
        nc = 4 * 2 * 8 * 7
        PD = 7 * ud + sl
        streams.append([a_stream(), a_total, PA, PD + CFG.get('aext', 0), 0])
        streams.append([c_stream, nc, PB, PE, 0])
        streams.append([d_stream(), d_total, PD + CFG.get('aext', 0), PE, 0])

        if not CFG.get('p0', 1):
            for c_ in cq + cx + ga + gc + gd:
                c_.wait()
            return
        _wait([cx[0]], 'wx0')
        list(x_terms(0))
        list(x_terms(1))
        _wait(cq[:N0], 'wq0')
        first_use = {}
        for u, (g, jp) in enumerate(units):
            first_use.setdefault(g, u)
        for u, (g, jp) in enumerate(units):
            if u in waits:
                _wait(waits[u], 'wu%d' % u)
            for g_, fu in first_use.items():
                if g_ not in wts and fu - (lead if g_ >= NF else 1) <= u:
                    back = CFG.get('wback', 8)
                    wts[g_] = wq_terms(*groups[g_], toks[-back] if len(toks) >= back else None)
            qproj(g, jp, [])
        assert all(st_[4] == st_[1] for st_ in streams) and not later, streams

    phase0()


    def phase1(k_s, kt_s, vt_s, vx_s, wx_s, *s_s):
        LATE = CFG.get('late', (2, 5))
        EARLY = tuple(o for o in (0, 1, 3, 4, 6, 2, 5) if o not in LATE)
        UN = CFG.get('unroll', 1)

        def heads(it, carry):
            @pl.when(it == 1)
            def _():
                for c_ in g4:
                    c_.start()

            @pl.when(jnp.logical_and(it % 2 == 1, it < H - 1))
            def _():
                _wait(kv_copies((it + 1) // 2), 'wkv')

            @pl.when(jnp.logical_and(jnp.logical_and(it % 2 == 0, it > 0), it < H - 2))
            def _():
                for c_ in kv_copies(it // 2 + 1):
                    c_.start()

            zero = it // H
            toks = []
            due = []
            for r in range(UN):
                head(it * UN + r, None if UN % 2 else r % 2, zero, toks, due)
            return carry + zero

        def head(h, par, zero, toks, due):
            lane8 = lax.broadcasted_iota(I32, (8, 128), 1)
            sub8 = lax.broadcasted_iota(I32, (8, 128), 0)
            lane16 = lax.broadcasted_iota(I32, (16, 128), 1)
            sub16 = lax.broadcasted_iota(I32, (16, 128), 0)
            tri = (lax.broadcasted_iota(I32, (128, 128), 0) <= lax.broadcasted_iota(I32, (128, 128), 1))
            h_next = h + 1 if isinstance(h, int) else jnp.minimum(h + 1, H - 1)
            never = _never(zero)

            def after(x, tok):
                return _after(x, tok, never)

            def tied(lhs):
                return _tied(lhs, due, never)

            def tok(back):
                return toks[-back] if (back and len(toks) >= back) else None

            def chan_mm(c, gate):
                m_b = lane8 < after(128 - 2 * sub8, gate)
                gs = [jnp.broadcast_to(g_s[a, pl.ds(c, 1), :], (8, 128)) for a in range(NB)]
                bt = [pltpu.roll(jnp.where(m_b, gs[a], gs[a - 1] if a > 0 else jnp.uint32(0)), 0, 1,
                                 stride=2, stride_axis=0) for a in range(NB)]
                b1 = pltpu.bitcast(jnp.concatenate(bt[7::-1], axis=0), BF16)
                b2 = pltpu.bitcast(jnp.concatenate(bt[15:7:-1], axis=0), BF16)
                am = pltpu.bitcast(aw_s[pl.ds(c, 64, stride=PITCH), :], BF16)
                tick('C', 48)
                z1 = _dot(tied(am), b1)
                z2 = _dot(am[:64], b2)
                return c, z1[:64], z1[64:] + z2

            def chan_post(c, zlo, zhi):
                acc = car = None
                for p in range(8):
                    z = jnp.concatenate([zlo[8 * p:8 * p + 8], zhi[8 * p:8 * p + 8]], axis=0)
                    if p == 0:
                        acc = z
                    else:
                        z = pltpu.roll(z, 16 * p, 1)
                        cz = jnp.where(lane16 < 16 * p, z, 0.0)
                        acc = acc + z
                        car = cz if car is None else car + cz
                y = (acc - car) + jnp.where(sub16 > 0, pltpu.roll(car, 1, 0), 0.0)
                later(CFG.get('ly', 0), [y])
                if CFG.get('ylate'):
                    ys.append((c, y))
                else:
                    y_s[pl.ds(c, NB, stride=PITCH), :] = pltpu.bitcast(y, U32)
                if CFG.get('pd', 0):
                    due.append(y[:8])
                    due.append(y[8:])

            chans = [h * CPH + i for i in range(CPH)]
            ys, cs = [], []

            def x_stream(hh, outers):
                n = 16 * len(outers)
                for r0 in range(0, 256, 16):
                    for o in outers:
                        n -= 1
                        free = n < CFG.get('xfree', 0) and hh is h_next
                        d = extract(hh, r0, o, shift_of(hh, tok(CFG.get('xfb', 1)) if free else None), zero * (o + 1))
                        yield None if free else d

            streams = [[x_stream(h_next, EARLY), 16 * len(EARLY), 0, 0] + list(CFG['x1']),
                       [x_stream(h, LATE), 16 * len(LATE), 0, 0] + list(CFG['x2'])]

            clock, queue = [0], []

            def later(lag, vals):
                if lag:
                    queue.append((clock[0] + lag, _digest(vals)))

            def tick(kind, cycles):
                due.extend(v for t, v in queue if t <= clock[0])
                queue[:] = [q for q in queue if q[0] > clock[0]]
                clock[0] += cycles
                for st_ in streams:
                    gen, n, done, clk, kinds, c0, c1 = st_
                    if kind in kinds:
                        want = min(n, max(0, (clk - c0) * n // (c1 - c0)))
                        while st_[2] < want:
                            d = next(gen)
                            if d is not None:
                                due.append(d)
                            st_[2] += 1
                        st_[3] += cycles

            def shift_of(hh, gate):
                return after(jnp.full((8, 128), (1 - hh % 2) * 16, I32).astype(U32), gate)

            def kv_chunk(ck):
                def prod(o):
                    MH = 128 // CFG.get('mh', 1)
                    out = {}
                    for r0 in range(0, 128, MH):
                        def inner(i):
                            tick('M', MH // 2)
                            lhs = jnp.concatenate([cs_s[ck, 7 * o + i, k, r0:r0 + MH, :] for k in range(2)], axis=1)
                            m = _dot(tied(lhs), wx_s[7 * o + i])
                            if i == CFG.get('ti', 3) and r0 == 0:
                                toks.append(m[:8])
                            return m

                        _strassen(inner, lambda r, n, val: out.__setitem__((r, n, r0), val))
                    return jnp.concatenate(
                        [jnp.concatenate([out[r, 0, r0], out[r, 1, r0]], axis=1)
                         for r in range(2) for r0 in range(0, 128, MH)], axis=0)

                def emit(R, N, val):
                    if N == 0:
                        rows = slice(512 * ck + 256 * R, 512 * ck + 256 * (R + 1))
                        if 2 * ck + R < NP - 1:
                            blocks = [val[:128, :128], val[:128, 128:], val[128:, :128], val[128:, 128:]]
                            for i in (0, 1, 4, 5, 6):
                                kt_w[i, 2 * ck + R] = _join32(_term(_LHS, i, blocks.__getitem__))
                        for n in range(2):
                            k_w[n, 256 * ck + 128 * R:256 * ck + 128 * (R + 1), :] = _join32(val[:, 128 * n:128 * (n + 1)])
                    else:
                        blocks = [val[128 * r:128 * (r + 1), 128 * n:128 * (n + 1)].T
                                  for n in range(2) for r in range(2)]
                        for m, v in enumerate(blocks):
                            vt_s[4 * ck + 2 * R + m % 2, 128 * (m // 2):128 * (m // 2 + 1), :] = v.astype(BF16)
                        if 2 * ck + R < NP - 1:
                            for i in (0, 1, 4, 5, 6):
                                vx_s[i, 2 * ck + R] = _term(_LHS, i, blocks.__getitem__).astype(BF16)

                return _strassen_steps(prod, emit)

            kv = [kv_chunk(ck) for ck in range(4)]

            def k_rows(r0, r1):
                return jnp.concatenate([k_s[0, r0:r1, :], k_s[1, r0:r1, :]], axis=1)

            def q_cols(r0, r1):
                return jnp.concatenate([qc_s[h, t] for t in range(r0 // 128, r1 // 128)], axis=1)

            mx, pr = {}, {}

            def s_at(u, r0):
                t = u // 4
                first = [v for v in range(u) if (v // 4) % 2 == t % 2]
                return s_s[t % 2], 128 * sum(v + 1 for v in first) + r0

            def qk(jq):
                run = [None, None]

                def put(n, r0, val):
                    buf, row = s_at(2 * jq + n, r0)
                    buf[row:row + val.shape[0], :] = val
                    vs = [val[r:r + 8] for r in range(0, val.shape[0], 8)]
                    def fold(op, xs, ways):
                        accs = xs[:ways]
                        for k, x in enumerate(xs[ways:]):
                            accs[k % ways] = op(accs[k % ways], x)
                        while len(accs) > 1:
                            accs = [op(a, b) for a, b in zip(accs[::2], accs[1::2])]
                        return accs[0]

                    m = fold(jnp.maximum, list(vs), CFG.get('mw', 1))
                    if run[n] is not None:
                        m = jnp.maximum(m, run[n][0])
                    if CFG.get('lsep'):
                        run[n] = (m, None)
                        return
                    l = fold(jnp.add, [jnp.exp2(v - m) for v in vs], CFG.get('lw', 1))
                    if run[n] is not None:
                        l = l + run[n][1] * jnp.exp2(run[n][0] - m)
                    run[n] = (m, l)

                if jq > 0:
                    raw = [qc_w[h, 2 * jq + n % 2, 64 * (n // 2):64 * (n // 2 + 1), :] for n in range(4)]
                    full = [_split(w) for w in raw]
                    qt = [pltpu.bitcast(raw[_RHS[i][0]] if len(_RHS[i]) == 1
                                        else _join(_term(_RHS, i, full.__getitem__)), BF16) for i in range(7)]
                QH = 128 // CFG.get('qh', 1)

                def diag():
                    q0 = 256 * jq
                    for n in range(2):
                        tick('Q', 64 * (n + 1))
                        sd = _dot(tied(k_rows(q0, q0 + 128 * (n + 1))), qc_s[h, 2 * jq + n])
                        sd = jnp.concatenate([sd[:128 * n], jnp.where(tri, sd[128 * n:], NEG)], axis=0) if n else (
                            jnp.where(tri, sd, NEG))
                        for r0 in range(0, 128 * (n + 1), QH):
                            put(n, q0 + r0, sd[r0:r0 + QH])
                    toks.append(sd[:8])

                if CFG.get('dfirst'):
                    diag()
                for jp in range(jq):
                    for r0 in range(0, 128, QH):
                        def prod(i):
                            tick('Q', QH // 4)
                            if i == 2:
                                lhs = k_s[0, 256 * jp + r0:256 * jp + r0 + QH, :]
                            elif i == 3:
                                lhs = k_s[1, 256 * jp + 128 + r0:256 * jp + 128 + r0 + QH, :]
                            else:
                                lhs = kt_s[i, jp, r0:r0 + QH, :]
                            m = _dot(tied(lhs), qt[i])
                            if i == 3 and r0 == 0:
                                toks.append(m[:8])
                            return m

                        _strassen(prod, lambda r, n, val: put(n, 256 * jp + 128 * r + r0, val))
                if not CFG.get('dfirst'):
                    diag()
                for n in range(2):
                    m, l = run[n]
                    top = jnp.max(m, axis=0, keepdims=True)
                    if CFG.get('lsep'):
                        tops[2 * jq + n] = top
                        continue
                    tot = jnp.sum(l * jnp.exp2(m - top), axis=0, keepdims=True)
                    mx[2 * jq + n] = top + jnp.log2(tot)

            tops = {}

            def denom(u, deadline):
                buf, row = s_at(u, 0)
                x = buf[pl.ds(pl.multiple_of(row + 16 * zero, 8), 128 * (u + 1)), :]
                e = jnp.exp2(x - tops[u])
                ways = CFG.get('dw', 1)
                accs = [e[8 * k:8 * (k + 1)] for k in range(ways)]
                for k in range(ways, e.shape[0] // 8):
                    accs[k % ways] = accs[k % ways] + e[8 * k:8 * (k + 1)]
                while len(accs) > 1:
                    accs = [a + b for a, b in zip(accs[::2], accs[1::2])]
                tot = jnp.sum(accs[0], axis=0, keepdims=True)
                mx[u] = tops[u] + jnp.log2(tot)
                if deadline:
                    due.append(tot)

            def probs(u, r0):
                buf, row = s_at(u, r0)
                x = jnp.concatenate([buf[pl.ds(row + e + zero, 8, stride=4), :] for e in (0, 2)], axis=0)
                return jnp.exp2(x - mx[u])

            def softmax(jq, jps, deadline):
                for u in (2 * jq, 2 * jq + 1):
                    if u not in mx:
                        denom(u, False)
                starts = [r + e for r in range(0, 256, 32) for e in range(2)]
                for jp in jps:
                    if jp == jq:
                        out = [jnp.concatenate([_join(probs(2 * jq + n, 256 * jq + r)) for r in starts[:8 * (n + 1)]],
                                               axis=0) for n in range(2)]
                    else:
                        parts = []
                        for r in starts[:8]:
                            blocks = [probs(2 * jq + m % 2, 256 * jp + 128 * (m // 2) + r) for m in range(4)]
                            parts.append([_join(t) for t in _rhs_terms(*blocks)])
                        out = [jnp.concatenate([p[i] for p in parts], axis=0) for i in range(7)]
                    pr[jq, jp] = out
                    if deadline:
                        due.append(_digest([out[0]]) ^ _digest([out[1]]) if jp == jq else _digest(out))

            def pv(jq):
                softmax(jq, [jp for jp in range(jq + 1) if (jq, jp) not in pr], False)
                diag = pr.pop((jq, jq))
                ps = [pr.pop((jq, jp)) for jp in range(jq)]
                base = []
                for n in range(2):
                    tick('P', 64 * (n + 1))
                    vt = jnp.concatenate([vt_s[2 * jq + i] for i in range(n + 1)], axis=1)
                    base.append(_dot(tied(vt), pltpu.bitcast(diag[n], BF16)))

                def emit(r, n, val):
                    val = base[n][128 * r:128 * (r + 1)] if val is None else val + base[n][128 * r:128 * (r + 1)]
                    qc_s[h, 2 * jq + n, 128 * r:128 * (r + 1), :] = val.astype(BF16)

                def prod(i):
                    tick('P', 32 * jq)
                    if i == 2:
                        lhs = [vt_s[2 * jp, 0:128, :] for jp in range(jq)]
                    elif i == 3:
                        lhs = [vt_s[2 * jp + 1, 128:256, :] for jp in range(jq)]
                    else:
                        lhs = [vx_s[i, jp] for jp in range(jq)]
                    rhs = pltpu.bitcast(jnp.concatenate([p[i] for p in ps], axis=0), BF16)
                    return _dot(tied(jnp.concatenate(lhs, axis=1)), rhs)

                if jq:
                    _strassen(prod, emit)
                else:
                    for r in range(2):
                        for n in range(2):
                            emit(r, n, None)

            CG, XG = CFG.get('cg', 0), CFG.get('xg', 0)
            pend = []
            def run_step(st_):
                kind, arg = st_[0], st_[1:]
                if kind == 'L':
                    for x in arg:
                        denom(int(x, 16), True)
                    return
                if kind == 'E':
                    jq = int(arg[0])
                    softmax(jq, [int(x) for x in arg[1:]] if arg[1:] else range(jq + 1), True)
                    return
                old = list(pend)
                pend.clear()
                if kind == 'C':
                    for _ in range(int(arg)):
                        pend.append(chan_mm(chans.pop(0), tok(CG)))
                elif kind == 'M':
                    for o in arg[1:]:
                        kv[int(arg[0])](int(o))
                elif kind == 'Q':
                    for x in arg:
                        qk(int(x))
                elif kind == 'P':
                    for x in arg:
                        pv(int(x))
                for args in old:
                    chan_post(*args)

            for seg in [g for g in CFG['sched'].split('|') if g.strip()]:
                if CFG.get('scopes') and '|' in CFG['sched']:
                    with jax.named_scope('s_' + seg.split()[0]):
                        for st_ in seg.split():
                            run_step(st_)
                else:
                    for st_ in seg.split():
                        run_step(st_)
            for c, y in ys:
                y_s[pl.ds(c, NB, stride=PITCH), :] = pltpu.bitcast(y, U32)
            for t, d0, n, v in cs:
                qc_s[h, t, d0:d0 + n, :] = v
            assert all(st_[1] == st_[2] for st_ in streams), [st_[1:] for st_ in streams]
            assert CFG.get('noassert') or not chans and not pend and (not due or CFG.get('pd')) and not pr

        if CFG.get('p1', 1):
            return lax.fori_loop(0, H // UN, heads, 0)
        else:
            _wait(g3b, 'wg3b')
            for c_ in g4:
                c_.start()

            def keep(h, carry):
                r = pl.multiple_of(h * 16, 16)
                t = (qc_s[h, h, 0:16, :].astype(F32) + cs_s[h % 4, h, h % 2, 0:16, :].astype(F32)
                     + pltpu.bitcast(aw_s[pl.ds(r, 16), :] + g_s[h, pl.ds(r, 16), :], F32)
                     + wx_s[h, pl.ds(r, 16), :].astype(F32))
                y_s[pl.ds(r, 16), :] = pltpu.bitcast(t, U32)
                return carry + h // H
            return lax.fori_loop(0, H, keep, 0)

    zero_end = phase1(k_s, kt_s, vt_s, vx_s, wx_s, sa_s, sb_s)

    def phase2():
        _wait(g4, 'wg4')
        HH = H // 2

        def wo_block(rh, kh):
            return jnp.concatenate(
                [xs_s[C * (H * b + h) + CH * rh:C * (H * b + h) + CH * (rh + 1), :]
                 for h in range(HH * kh, HH * (kh + 1)) for b in range(2)], axis=1)

        raw = [wo_block(0, 0), wo_block(1, 0), wo_block(0, 1), wo_block(1, 1)]
        wt = [t.astype(BF16) for t in _rhs_terms(*[t.astype(F32) for t in raw])]
        wt[1], wt[4] = raw[0], raw[3]
        outs = []
        due, late = [], []
        DL = CFG.get('dl', 3)
        never = _never(zero_end)

        def put(t, b, z, opaque=False):
            o = z.T.astype(BF16)
            r0 = pl.multiple_of(zero_end * 16 + 128 * t, 16) if opaque else 128 * t
            c_s[b, pl.ds(r0, 128), :] = o
            late.append(pltpu.bitcast(o[112:], U32))

        for jp in range(CFG.get('np2', NP) if CFG.get('p2', 1) else 0):
            def ctx_block(r, kh):
                return jnp.concatenate([qc_s[h, 2 * jp + r] for h in range(HH * kh, HH * (kh + 1))], axis=0)

            craw = [ctx_block(0, 0), ctx_block(0, 1), ctx_block(1, 0), ctx_block(1, 1)]
            ct = [t.astype(BF16) for t in _lhs_terms(*[t.astype(F32) for t in craw])]
            ct[2], ct[3] = craw[0], craw[3]
            za = {}
            prev_late = list(late)
            late.clear()
            for r in range(2):
                t = 2 * jp + r
                za[r] = (pltpu.bitcast(y_s[t * PITCH:t * PITCH + C, :], F32)
                         * x_s[:, 128 * t:128 * (t + 1)].astype(F32))
                for b in range(3):
                    put(t, b, za[r][128 * b:128 * (b + 1)], opaque=(r == 0 and b == 0 and jp > 0))
            a_late = list(late)
            late.clear()
            res = {}
            count = [0]

            def prod(i):
                if count[0] == DL:
                    due.extend(prev_late)
                if count[0] == 6:
                    due.extend(a_late)
                count[0] += 1
                return _dot(_tied(wt[i], due, never), ct[i])

            _strassen(prod, lambda r, c, val: res.__setitem__((r, c), val), order=(1, 4, 3, 2, 0, 5, 6))
            for r in (1, 0):
                z = jnp.concatenate([za[r][384:], res[(r, 0)], res[(r, 1)]], axis=0)
                for b in (3, 2, 1, 0):
                    put(2 * jp + r, 3 + b, z[128 * b:128 * (b + 1)])
            rows = pl.ds(128 * jp, 128)
            for b in range(7):
                oc = cp(c_w.at[b, rows], o_hbm.at[rows, pl.ds(128 * b, 128)], 26 + jp)
                oc.start()
                outs.append(oc)
        if not CFG.get('p2', 1):
            def keep(h, carry):
                r = pl.multiple_of(h * 16, 16)
                c_s[0, pl.ds(r, 16), :] = pltpu.bitcast(y_s[pl.ds(r, 16), :], F32).astype(BF16) + qc_s[h, h, 0:16, :]
                return carry
            lax.fori_loop(0, H, keep, 0)
            oc = cp(c_w.at[0, pl.ds(0, 128)], o_hbm.at[pl.ds(0, 128), pl.ds(0, 128)], 26)
            oc.start()
            outs.append(oc)
        _wait(outs, 'wout')

    phase2()


def _tiles(w):
    rows = w.shape[0]
    return w.reshape(rows, 2, 8, 2, 128).transpose(0, 1, 3, 2, 4).reshape(rows, 32, 128)


@jax.jit
def pallas_concat_heads__ssm_conv_h3__compressed_kv_cla__prompt_kernel(
    A_q: jax.Array,
    A_k: jax.Array,
    A_v: jax.Array,
    A_shift_k: jax.Array,
    A_ssm_k: jax.Array,
    A_ssm_D: jax.Array,
    B_x: jax.Array,
    B_c_kv: jax.Array,
    B_w_q: jax.Array,
    B_w_uk: jax.Array,
    B_w_uv: jax.Array,
    B_w_o: jax.Array,
):
    hbm = pl.BlockSpec(memory_space=pltpu.HBM)
    out = pl.pallas_call(
        _kernel,
        in_specs=[hbm] * 12,
        out_specs=hbm,
        out_shape=jax.ShapeDtypeStruct((S, 2 * C), BF16),
        scratch_shapes=[
            pltpu.VMEM((8, S // 2, 128), U32),
            pltpu.VMEM((4, 49, 2, 64, 128), U32),
            pltpu.VMEM((2, 4, DC, 128), U32),
            pltpu.VMEM((H, NB, D // 2, 128), U32),
            pltpu.VMEM((64 * PITCH, 128), U32),
            pltpu.VMEM((NB, C, 128), U32),
            pltpu.VMEM((NB * PITCH, 128), U32),
            pltpu.VMEM((CH, S), U32),
            pltpu.VMEM((512, 128), F32),
            pltpu.VMEM((2, S // 2, 128), U32),
            pltpu.VMEM((7, NP, 64, 128), U32),
            pltpu.VMEM((NB, D // 2, 128), U32),
            pltpu.VMEM((7, NP, 64, 128), U32),
            pltpu.VMEM((49, DC // 8, 128), U32),
            pltpu.VMEM((4 * C * 4, 128), F32),
            pltpu.VMEM((84 * 128, 128), F32),
            pltpu.VMEM((CH, S), U32),
            pltpu.VMEM((7 * NP * 128, 128), U32),
            pltpu.VMEM((CH, S), U32),
            pltpu.VMEM((CH, S), U32),
            pltpu.VMEM((2, 8, 128, 128), F32),
            pltpu.VMEM((4, C), BF16),
            pltpu.VMEM((C,), BF16),
            pltpu.SemaphoreType.DMA((35,)),
        ],
        compiler_params=pltpu.CompilerParams(vmem_limit_bytes=127 * 2 ** 20),
    )(
        A_q[0].T, A_k[0].T, A_v[0].T, A_shift_k.T, A_ssm_k, A_ssm_D, B_x[0].T, B_c_kv[0],
        _tiles(B_w_q), _tiles(B_w_uk), _tiles(B_w_uv),
        jnp.swapaxes(B_w_o, 1, 2).reshape(H * C, D),
    )
    return out.reshape(1, S, 2 * C)
```

```python
import math

import jax
import jax.numpy as jnp
from jax import lax
import jax.experimental.pallas as pl
import jax.experimental.pallas.tpu as pltpu

F32 = jnp.float32
BF16 = jnp.bfloat16
U32 = jnp.uint32
I32 = jnp.int32

S = 2048
C = 448
H = 16
D = 256
DC = 1024
NB = S // 128
NP = NB // 2
CH = C // 2
PITCH = 520
CPH = C // H
TQ = 512
NT = (((1,), (1,)), ((), ()))
LOG2E = math.log2(math.e)
QSCALE = (D ** -0.5) * LOG2E
NEG = -1e9 * LOG2E
HI_MASK = 0xFFFF0000
CFG = dict(ua=30,ud=96,nf=8,n0=3,ux=13,gback=8,slack=8,nsc=1,oo=(1,4,3,6,0,2,5),ro=(0,1),bo=(0,1,2,3),late=(),x2=('P',0,1),mh=2,qh=2,mw=2,lw=2,cg=5,x1=('P',1500,7580),sched='M001 C2 M034 C2 M06 M101 C2 Q01 M134 C2 M16 M201 C2 Q23 M234 C2 M26 M301 C2 E0 E1 E2 Q45 M334 C2 M36 E3 M02 C2 Q67 M05 C2 M12 C2 E4 M15 C2 E5012 M22 C2 E5345 M25 C2 M32 E6012 M35 E63456 P01234567')


def _wait(copies, name):
    if CFG.get('scopes'):
        with jax.named_scope(name):
            for c_ in copies:
                c_.wait()
    else:
        for c_ in copies:
            c_.wait()


def _dot(a, b):
    return jnp.dot(a, b, preferred_element_type=F32)


def _dot_nt(a, b):
    return lax.dot_general(a, b, NT, preferred_element_type=F32)


def _lo(x):
    return pltpu.bitcast(x << 16, F32)


def _hi(x):
    return pltpu.bitcast(x & jnp.uint32(HI_MASK), F32)


def _pack(even, odd):
    return pltpu.pack_elementwise([even, odd], packed_dtype=BF16).astype(U32)


def _split(words):
    return jnp.concatenate([_lo(words), _hi(words)], axis=0)


def _join32(x):
    return jnp.concatenate([_pack(x[m:m + 16], x[m + 16:m + 32]) for m in range(0, x.shape[0], 32)], axis=0)


def _join16(x):
    return jnp.concatenate([_pack(x[m:m + 8], x[m + 8:m + 16]) for m in range(0, x.shape[0], 16)], axis=0)


def _join(x):
    n = x.shape[0] // 2
    return _pack(x[:n], x[n:])


def _head_cols(w_s, h, rows):
    out = []
    for b in range(2):
        x = w_s[b, pl.ds(h // 2, rows, stride=8), :]
        if isinstance(h, int):
            out.append(_lo(x) if h % 2 == 0 else _hi(x))
        else:
            out.append(_hi(x << ((1 - h % 2) * 16).astype(U32)))
    return out


_LHS = ((0, 1, 3), (2, 1, 3), (0,), (3,), (0, 1, 1), (2, -1, 0), (1, -1, 3))
_RHS = ((0, 1, 3), (0,), (1, -1, 3), (2, -1, 0), (3,), (0, 1, 1), (2, 1, 3))


def _term(table, i, block):
    spec = table[i]
    if len(spec) == 1:
        return block(spec[0])
    return block(spec[0]) + block(spec[2]) if spec[1] > 0 else block(spec[0]) - block(spec[2])


def _lhs_terms(*blocks):
    return [_term(_LHS, i, blocks.__getitem__) for i in range(7)]


def _rhs_terms(*blocks):
    return [_term(_RHS, i, blocks.__getitem__) for i in range(7)]


def _inner_terms(table, o, block):
    sub = [_term(table, o, lambda n: block(n, m)) for m in range(4)]
    return [_term(table, i, sub.__getitem__) for i in range(7)]


def _strassen_steps(prod, emit):
    uses = {(0, 0): {0: 1, 3: 1, 4: -1, 6: 1}, (0, 1): {2: 1, 4: 1},
            (1, 0): {1: 1, 3: 1}, (1, 1): {0: 1, 1: -1, 2: 1, 5: 1}}
    acc = {}
    neg = {}

    def step(i):
        m = prod(i)
        for key, terms in uses.items():
            if i not in terms:
                continue
            sign = terms.pop(i)
            if key not in acc:
                acc[key] = m
                neg[key] = sign < 0
            elif neg[key]:
                assert sign > 0
                acc[key] = m - acc[key]
                neg[key] = False
            else:
                acc[key] = acc[key] + m if sign > 0 else acc[key] - m
            if not terms:
                emit(key[0], key[1], acc.pop(key))

    return step


def _strassen(prod, emit, order=(0, 1, 3, 2, 4, 5, 6)):
    step = _strassen_steps(prod, emit)
    for i in order:
        step(i)


def _mult(i, n):
    return i if isinstance(i, int) else pl.multiple_of(i, n)


def _never(zero):
    return lax.broadcasted_iota(I32, (8, 128), 1) < zero


def _after(x, tok, never):
    if tok is None:
        return x
    return jnp.where(never, pltpu.bitcast(tok, x.dtype), x)


def _tied(lhs, due, never):
    if not due:
        return lhs
    t = None
    for d in due:
        d = pltpu.bitcast(jnp.broadcast_to(d, (8, 128)), U32)
        t = d if t is None else t ^ d
    due.clear()
    x = pltpu.bitcast(_after(pltpu.bitcast(lhs[:16, :128], U32), t, never), BF16)
    if lhs.shape[1] > 128:
        x = jnp.concatenate([x, lhs[:16, 128:]], axis=1)
    return jnp.concatenate([x, lhs[16:]], axis=0) if lhs.shape[0] > 16 else x


def _digest(vals):
    acc = None
    words = [v if v.dtype == U32 else pltpu.bitcast(v, U32) for v in vals]
    for r in range(words[0].shape[0] // 8):
        for w in words:
            w = w[8 * r:8 * (r + 1)]
            acc = w if acc is None else acc ^ w
    return acc


class _Packed:
    def __init__(self, ref):
        self.ref = ref

    def _index(self, idx):
        idx = idx if isinstance(idx, tuple) else (idx,)
        axis = len(self.ref.shape) - 2
        if len(idx) <= axis:
            return idx + (slice(None),) * (axis + 2 - len(idx))
        r = idx[axis]
        if isinstance(r, slice):
            r = slice(None if r.start is None else r.start // 2, None if r.stop is None else r.stop // 2)
        else:
            r = pl.ds(_mult(r.start // 2, 8), r.size // 2)
        return idx[:axis] + (r,) + idx[axis + 1:]

    def __getitem__(self, idx):
        return pltpu.bitcast(self.ref[self._index(idx)], BF16)

    def __setitem__(self, idx, val):
        self.ref[self._index(idx)] = pltpu.bitcast(val, U32)


def _kernel(qa_hbm, ka_hbm, va_hbm, sk_hbm, hk_hbm, d_hbm, x_hbm, c_hbm, wq_hbm, wk_hbm, wv_hbm, wo_hbm,
            o_hbm,
            c_s, cs_s, wp_s, qc_s, aw_s, g_s, y_s, hk_s, dc_s, k_s, kt_s, vt_s, vx_s, wx_s, sa_s, sb_s, x_s, xs_s, ka_s, va_s, wt_s, out_s, sk_ref, d_ref, sems):
    def cp(src, dst, i):
        return pltpu.make_async_copy(src, dst, sems.at[i])

    c_w, xs_w, x_w, ka_w, va_w, hk_w, cs_w, wx_w, qc_w = c_s, xs_s, x_s, ka_s, va_s, hk_s, cs_s, wx_s, qc_s
    k_w, kt_w, vt_w, vx_w = k_s, kt_s, vt_s, vx_s
    c_s, cs_s, qc_s, k_s, kt_s, vt_s, vx_s, wx_s, xs_s, x_s, ka_s, va_s, hk_s = (
        _Packed(r) for r in (c_s, cs_s, qc_s, k_s, kt_s, vt_s, vx_s, wx_s, xs_s, x_s, ka_s, va_s, hk_s))
    qa_hbm, ka_hbm, va_hbm, hk_hbm, x_hbm, c_hbm, wo_hbm = (
        r.bitcast(U32) for r in (qa_hbm, ka_hbm, va_hbm, hk_hbm, x_hbm, c_hbm, wo_hbm))
    wq32 = wq_hbm.bitcast(U32)
    wk32 = wk_hbm.bitcast(U32)
    wv32 = wv_hbm.bitcast(U32)
    gc = [cp(c_hbm.at[:, pl.ds(128 * b, 128)], c_w.at[b], 8 + b) for b in range(8)]

    def word_row(pair, b):
        return 8 * (pair // 4) + 4 * b + pair % 4

    def kv_copies(pair):
        return [cp(w.at[:, word_row(pair, b), :], wp_s.at[pair % 2, 2 * n + b], 16 + pair % 2)
                for n, w in enumerate((wk32, wv32)) for b in range(2)]

    g3 = kv_copies(0)
    g3b = kv_copies(1)
    g4 = [cp(qa_hbm, x_w, 21)] + [cp(wo_hbm.at[:, pl.ds(128 * b, 128)], xs_w.at[pl.ds(H * CH * b, H * CH)], 6 + b)
                                  for b in range(2)]

    def delayed(ref, rows, sg, n, gate=None):
        cur = pltpu.bitcast(ref[rows, 128 * sg:128 * (sg + 1)], U32)
        lane = lax.broadcasted_iota(I32, (8, 128), 1)
        if gate is not None:
            lane = gate(lane)
        lane = jnp.concatenate([lane] * (cur.shape[0] // 8), axis=0)
        prev = pltpu.bitcast(ref[rows, 128 * (sg - 1):128 * sg], U32) if sg > 0 else jnp.uint32(0)
        x = pltpu.roll(jnp.where(lane < 128 - n, cur, prev), n, 1)
        return pltpu.bitcast(x, BF16).astype(F32)

    def gated_t(x, gate):
        if gate is not None:
            x = jnp.concatenate([gate(x[:8]), x[8:]], axis=0)
        return x.T

    def windows(b, q, e, js, gate=None):
        out = []
        for j in js:
            parts = []
            for sg in range(2 * j - 6, 2 * j + 2):
                if sg < 0:
                    parts.append(jnp.zeros((16, 128), U32))
                else:
                    parts.append(pltpu.bitcast(sb_s[pl.ds(S * b + 128 * sg + 32 * q + 16 * e, 16), :], U32))
            plane = 32 * (j // 4) + 8 * q + 4 * e + j % 4
            win = gated_t(jnp.concatenate(parts, axis=0), gate)
            aw_s[pl.ds(_mult(plane * PITCH + 128 * b, 8), 128), :] = win
            out.append(win[120:])
        return out

    def prep_g(r0, n, gate=None):
        rows = pl.ds(_mult(r0, 16), n)
        lane = lax.broadcasted_iota(I32, (n, 128), 1)
        for a in range(NB):
            hf = hk_s[rows, 128 * a:128 * (a + 1)].astype(F32)
            hs = delayed(hk_s, rows, a, 1, gate)
            if a == 0:
                hf = jnp.where(lane == 0, hf + dc_s[rows, :], hf)
                hs = jnp.where(lane == 1, hs + dc_s[rows, :], hs)
            wrd = pltpu.pack_elementwise([hf, hs], packed_dtype=BF16).astype(U32)
            g_s[a, rows, :] = wrd
            yield _digest([wrd])

    def extract(h, r0, o, shift, z):
        def block(n, kq, b):
            x = jnp.concatenate([wp_s[(h // 2) % 2 + z, 2 * n + b, pl.ds(256 * kq + r0 + e, 8, stride=2), :]
                                 for e in range(2)], axis=0)
            if isinstance(h, int):
                return _lo(x) if h % 2 == 0 else _hi(x)
            return _hi(x << jnp.concatenate([shift] * 2, axis=0))

        terms = [_join(t) for t in _inner_terms(
            _RHS, o, lambda n, m: block(n % 2, 2 * (n // 2) + m // 2, m % 2))]
        for i, t in enumerate(terms):
            wx_w[7 * o + i, r0 // 2:r0 // 2 + 8, :] = t
        return _digest(terms)

    def phase0():
        XC = 512
        NF = CFG.get('nf', 4)
        N0 = CFG.get('n0', NF)
        N1 = CFG.get('n1', N0)
        cq = [cp(wq32.at[:, word_row(g // 2, g % 2), :], y_s.at[pl.ds(C * g, C)],
                 0 if g < N0 else 35 if g < N1 else 19 if g < NF else 1 if g < 8 else 18)
              for g in range(H)]
        cx = [cp(x_hbm.at[:, pl.ds(XC * i, XC)], x_w.at[:, pl.ds(XC * i, XC)], 22 + i) for i in range(S // XC)]
        ga = [cp(sk_hbm, sk_ref, 2), cp(ka_hbm, ka_w, 3), cp(va_hbm, va_w, 4)]
        gb = cq[8:] + gc
        gd = [cp(d_hbm, d_ref, 20), cp(hk_hbm, hk_w, 5)] + g3
        rest = cx[1:] + cq[NF:8] + ga + gb + gd + g3b
        for c_ in [cx[0]] + cq[:NF] + rest:
            c_.start()
        zero = pl.semaphore_read(sems.at[34])
        never = _never(zero)
        due = []
        toks = []

        def pad_rows(t):
            return jnp.concatenate([t, jnp.zeros((256 - CH, 128), t.dtype)], axis=0)

        def wq_terms(j, b, gate):
            x = y_s[C * (2 * j + b):C * (2 * j + b + 1), :]
            g16 = jnp.concatenate([_after(jnp.full((8, 128), 16, U32), gate, never)] * (C // 8), axis=0)
            gm = jnp.concatenate([_after(jnp.full((8, 128), HI_MASK, U32), gate, never)] * (C // 8), axis=0)
            lo, hi = pltpu.bitcast(x << g16, F32), pltpu.bitcast(x & gm, F32)
            blocks = [pad_rows(t).T for t in (lo[:CH], hi[:CH], lo[CH:], hi[CH:])]
            if not CFG.get('q4', 1):
                return [t.astype(BF16) for t in _rhs_terms(*blocks)]
            slot = (2 * j + b) % 2
            for n, t in enumerate(blocks):
                for k in range(2):
                    wt_s[slot, 2 * n + k] = t[:, 128 * k:128 * (k + 1)]
            quarter = [[jnp.concatenate([wt_s[slot, 2 * n + k, pl.ds(e, 32, stride=4), :] for k in range(2)], axis=1)
                        for n in range(4)] for e in range(4)]
            terms = [_rhs_terms(*q) for q in quarter]
            out = []
            for i in range(7):
                ev, od = _pack(terms[0][i], terms[2][i]), _pack(terms[1][i], terms[3][i])
                rows = [w[8 * m:8 * (m + 1)] for m in range(4) for w in (ev, od)]
                out.append(pltpu.bitcast(jnp.concatenate(rows, axis=0), BF16))
            return out

        def x_terms(jp):
            top = slice(256 * jp, 256 * jp + 128)
            bot = slice(256 * jp + 128, 256 * jp + 256)
            for i in range(7):
                xs_s[256 * (NP * i + jp) + CH:256 * (NP * i + jp + 1), :] = jnp.zeros((256 - CH, 128), BF16)
            for r in range(0, CH, 32):
                lo, hi = slice(r // 2, r // 2 + 16), slice((CH + r) // 2, (CH + r) // 2 + 16)
                blocks = [x_w[lo, top], x_w[hi, top], x_w[lo, bot], x_w[hi, bot]]
                terms = [_join(t) for t in _lhs_terms(*[_split(t) for t in blocks])]
                terms[2], terms[3] = blocks[0], blocks[3]
                for i, t in enumerate(terms):
                    xs_w[128 * (NP * i + jp) + r // 2:128 * (NP * i + jp) + r // 2 + 16, :] = t
                yield 1, _digest(terms)

        def qproj(g, jp, waits):
            j, b = groups[g]
            for c_ in waits:
                c_.wait()
            if False:
                x_terms(jp)
                x_terms(jp + 1)

            XH = 128 // CFG.get('xh', 1)
            for r0 in range(0, 128, XH):
                def prod(i):
                    if r0 == 0 or True:
                        pump()
                    m = _dot(_tied(wts[g][i][r0:r0 + XH], due, never),
                             xs_s[256 * (NP * i + jp):256 * (NP * i + jp + 1), :])
                    toks.append(m[:8])
                    return m

                def emit(r, c, val):
                    w0 = 64 * b + r0 // 2
                    qc_w[2 * j + c, 2 * jp + r, w0:w0 + XH // 2, :] = _join32(val * QSCALE)

                _strassen(prod, emit)

        def column(row):
            row = jnp.concatenate([row.astype(F32), jnp.zeros((1, 512 - C), F32)], axis=1)
            return jnp.broadcast_to(row, (128, 512)).T

        consts = {}

        def make_consts():
            consts['taps'] = [column(sk_ref[j:j + 1, :]) for j in range(4)]

        def gate(x):
            back = CFG.get('gback', 6)
            return _after(x, toks[-back], never) if back else x

        def prep_u(r0, n):
            rows = slice(r0, r0 + n)
            tp = [t[rows] for t in consts['taps']]
            prev = jnp.zeros((n, 128), F32)
            for sg in range(NB):
                cols = slice(128 * sg, 128 * (sg + 1))
                ksh = ((delayed(ka_s, rows, sg, 3, gate) * tp[3] + delayed(ka_s, rows, sg, 2, gate) * tp[2])
                       + (delayed(ka_s, rows, sg, 1, gate) * tp[1] + ka_s[rows, cols].astype(F32) * tp[0]))
                kv = ksh * va_s[rows, cols].astype(F32)
                wrd = pltpu.pack_elementwise([prev, kv], packed_dtype=BF16).astype(U32)
                sa_s[C * sg + r0:C * sg + r0 + n, :] = pltpu.bitcast(wrd, F32)
                prev = kv
                yield _digest([wrd])

        def words_t(b):
            for sg in range(NB):
                r0 = C * sg + 128 * b
                if b < 3:
                    wrd = sa_s[r0:r0 + 128, :]
                else:
                    wrd = jnp.concatenate([sa_s[r0:r0 + C - 384, :], jnp.zeros((512 - C, 128), F32)], axis=0)
                wrd = gated_t(pltpu.bitcast(wrd, U32), gate)
                sb_s[S * b + 128 * sg:S * b + 128 * (sg + 1), :] = pltpu.bitcast(wrd, F32)
                yield wrd[120:]

        def all_windows(b):
            for p in range(8):
                for j in range(8):
                    yield windows(b, p // 2, p % 2, [j], gate)[0]

        def c_terms():
            for ck in range(4):
                for half in range(2):
                    for r0 in range(0, 128, 16):
                        for o in range(7):
                            def block(n, m):
                                row = 256 * ck + 128 * (n // 2) + 64 * (m // 2) + 16 * (r0 // 32)
                                col = 4 * (n % 2) + 2 * (m % 2) + half + zero * (o + 1)
                                w = jnp.concatenate([c_w[col, pl.ds(row + e, 8, stride=2), :] for e in range(2)], axis=0)
                                return _hi(w) if r0 % 32 else _lo(w)

                            terms = [_join(t) for t in _inner_terms(_LHS, o, block)]
                            for i, t in enumerate(terms):
                                cs_w[ck, 7 * o + i, half, r0 // 2:r0 // 2 + 8, :] = t
                            yield _digest(terms)

        UG = CFG.get('ug', 32)

        cu, ct, cg, cx_ = CFG.get('costs', (2, 2, 1, 1))

        def a_stream():
            make_consts()
            for b in range(4):
                for r0 in range(128 * b, min(C, 128 * (b + 1)), UG):
                    for v in prep_u(r0, UG):
                        yield cu * UG // 32, v
                for v in words_t(b):
                    yield ct, v
                for v in all_windows(b):
                    yield ct, v

        def d_stream():
            dc_s[...] = column(d_ref[...].reshape(1, C))
            for r0 in range(0, C, 32):
                for v in prep_g(r0, 32, gate):
                    yield cg, v
            for r0 in range(0, 256, 16):
                for o in range(7):
                    yield cx_, extract(0, r0, o, None, zero * (o + 1))

        a_total = cu * 14 * NB + ct * 4 * (NB + 64)
        d_total = cg * 14 * NB + cx_ * 112
        streams = []
        nprod = [0]
        later = {}
        LAG = CFG.get('lag', 0)

        def pump():
            for st_ in streams:
                gen, n, p0, p1, done = st_
                want = min(n, max(0, (nprod[0] - p0 + 1) * n // (p1 - p0)))
                while st_[4] < want:
                    cost, v = next(gen)
                    later.setdefault(nprod[0] + LAG, []).append(v)
                    st_[4] += cost
            due.extend(later.pop(nprod[0], []))
            nprod[0] += 1

        groups = [(j, b) for j in range(H // 2) for b in range(2)]
        units = [(g, jp) for c in range(0, NP, 2) for g in range(NF) for jp in (c, c + 1)]
        units += [(g, jp) for g in range(NF, len(groups)) for jp in range(NP)]
        NU = len(units)
        wts = {}
        lead = CFG.get('lead', 4)
        ua = CFG.get('ua', 32)
        ub = 8 * NP - lead
        ux = CFG.get('ux', 5)
        ud = CFG.get('ud', 96)
        waits = {ux: cx[1:] + cq[NF:8], ua: ga, ub: gb, ud: gd}
        if N0 < N1:
            waits[2 * N0 - 1] = cq[N0:N1]
        if N1 < NF:
            waits[2 * N1 - 1] = cq[N1:NF]
        PU = 7 * CFG.get('xh', 1)
        xe = [PU * ux + 2] + [PU * NF * 2 * c - 1 for c in (1, 2, 3)]
        for c in range(3):
            streams.append([(v for jp in (2 * c + 2, 2 * c + 3) for v in x_terms(jp)), 14, xe[c], xe[c + 1], 0])
        sl = CFG.get('slack', 4)
        PA, PB, PE = PU * ua + sl, PU * ub + sl, PU * NU - 2 - LAG
        c_stream = ((1, v) for v in c_terms())
        nc = 4 * 2 * 8 * 7
        PD = PU * ud + sl
        streams.append([a_stream(), a_total, PA, PD + CFG.get('aext', 0), 0])
        streams.append([c_stream, nc, PB, PE, 0])
        streams.append([d_stream(), d_total, PD + CFG.get('aext', 0), PE, 0])

        if not CFG.get('p0', 1):
            for c_ in cq + cx + ga + gc + gd:
                c_.wait()
            return
        _wait([cx[0]], 'wx0')
        list(x_terms(0))
        list(x_terms(1))
        _wait(cq[:N0], 'wq0')
        first_use = {}
        for u, (g, jp) in enumerate(units):
            first_use.setdefault(g, u)
        for u, (g, jp) in enumerate(units):
            if u in waits:
                _wait(waits[u], 'wu%d' % u)
            for g_, fu in first_use.items():
                if g_ not in wts and fu - (lead if g_ >= NF else 1) <= u:
                    back = CFG.get('wback', 8)
                    wts[g_] = wq_terms(*groups[g_], toks[-back] if len(toks) >= back else None)
            qproj(g, jp, [])
        assert all(st_[4] == st_[1] for st_ in streams) and not later, streams

    phase0()


    def phase1(k_s, kt_s, vt_s, vx_s, wx_s, *s_s):
        LATE = CFG.get('late', (2, 5))
        EARLY = tuple(o for o in (0, 1, 3, 4, 6, 2, 5) if o not in LATE)
        UN = CFG.get('unroll', 1)

        def heads(it, carry):
            @pl.when(it == 1)
            def _():
                for c_ in g4:
                    c_.start()

            @pl.when(jnp.logical_and(it % 2 == 1, it < H - 1))
            def _():
                _wait(kv_copies((it + 1) // 2), 'wkv')

            @pl.when(jnp.logical_and(jnp.logical_and(it % 2 == 0, it > 0), it < H - 2))
            def _():
                for c_ in kv_copies(it // 2 + 1):
                    c_.start()

            zero = it // H
            toks = []
            due = []
            for r in range(UN):
                head(it * UN + r, None if UN % 2 else r % 2, zero, toks, due)
            return carry + zero

        def head(h, par, zero, toks, due):
            lane8 = lax.broadcasted_iota(I32, (8, 128), 1)
            sub8 = lax.broadcasted_iota(I32, (8, 128), 0)
            lane16 = lax.broadcasted_iota(I32, (16, 128), 1)
            sub16 = lax.broadcasted_iota(I32, (16, 128), 0)
            tri = (lax.broadcasted_iota(I32, (128, 128), 0) <= lax.broadcasted_iota(I32, (128, 128), 1))
            h_next = h + 1 if isinstance(h, int) else jnp.minimum(h + 1, H - 1)
            never = _never(zero)

            def after(x, tok):
                return _after(x, tok, never)

            def tied(lhs):
                return _tied(lhs, due, never)

            def tok(back):
                return toks[-back] if (back and len(toks) >= back) else None

            def chan_mm(c, gate):
                m_b = lane8 < after(128 - 2 * sub8, gate)
                gs = [jnp.broadcast_to(g_s[a, pl.ds(c, 1), :], (8, 128)) for a in range(NB)]
                bt = [pltpu.roll(jnp.where(m_b, gs[a], gs[a - 1] if a > 0 else jnp.uint32(0)), 0, 1,
                                 stride=2, stride_axis=0) for a in range(NB)]
                b1 = pltpu.bitcast(jnp.concatenate(bt[7::-1], axis=0), BF16)
                b2 = pltpu.bitcast(jnp.concatenate(bt[15:7:-1], axis=0), BF16)
                am = pltpu.bitcast(aw_s[pl.ds(c, 64, stride=PITCH), :], BF16)
                tick('C', 48)
                z1 = _dot(tied(am), b1)
                z2 = _dot(am[:64], b2)
                return c, z1[:64], z1[64:] + z2

            def chan_post(c, zlo, zhi):
                acc = car = None
                for p in range(8):
                    z = jnp.concatenate([zlo[8 * p:8 * p + 8], zhi[8 * p:8 * p + 8]], axis=0)
                    if p == 0:
                        acc = z
                    else:
                        z = pltpu.roll(z, 16 * p, 1)
                        cz = jnp.where(lane16 < 16 * p, z, 0.0)
                        acc = acc + z
                        car = cz if car is None else car + cz
                y = (acc - car) + jnp.where(sub16 > 0, pltpu.roll(car, 1, 0), 0.0)
                later(CFG.get('ly', 0), [y])
                if CFG.get('ylate'):
                    ys.append((c, y))
                else:
                    y_s[pl.ds(c, NB, stride=PITCH), :] = pltpu.bitcast(y, U32)
                if CFG.get('pd', 0):
                    due.append(y[:8])
                    due.append(y[8:])

            chans = [h * CPH + i for i in range(CPH)]
            ys, cs = [], []

            def x_stream(hh, outers):
                n = 16 * len(outers)
                for r0 in range(0, 256, 16):
                    for o in outers:
                        n -= 1
                        free = n < CFG.get('xfree', 0) and hh is h_next
                        d = extract(hh, r0, o, shift_of(hh, tok(CFG.get('xfb', 1)) if free else None), zero * (o + 1))
                        yield None if free else d

            streams = [[x_stream(h_next, EARLY), 16 * len(EARLY), 0, 0] + list(CFG['x1']),
                       [x_stream(h, LATE), 16 * len(LATE), 0, 0] + list(CFG['x2'])]

            clock, queue = [0], []

            def later(lag, vals):
                if lag:
                    queue.append((clock[0] + lag, _digest(vals)))

            def tick(kind, cycles):
                due.extend(v for t, v in queue if t <= clock[0])
                queue[:] = [q for q in queue if q[0] > clock[0]]
                clock[0] += cycles
                for st_ in streams:
                    gen, n, done, clk, kinds, c0, c1 = st_
                    if kind in kinds:
                        want = min(n, max(0, (clk - c0) * n // (c1 - c0)))
                        while st_[2] < want:
                            d = next(gen)
                            if d is not None:
                                due.append(d)
                            st_[2] += 1
                        st_[3] += cycles

            def shift_of(hh, gate):
                return after(jnp.full((8, 128), (1 - hh % 2) * 16, I32).astype(U32), gate)

            def kv_chunk(ck):
                def prod(o):
                    MH = 128 // CFG.get('mh', 1)
                    out = {}
                    for r0 in range(0, 128, MH):
                        def inner(i):
                            tick('M', MH // 2)
                            lhs = jnp.concatenate([cs_s[ck, 7 * o + i, k, r0:r0 + MH, :] for k in range(2)], axis=1)
                            m = _dot(tied(lhs), wx_s[7 * o + i])
                            if i == CFG.get('ti', 3) and r0 == 0:
                                toks.append(m[:8])
                            return m

                        _strassen(inner, lambda r, n, val: out.__setitem__((r, n, r0), val))
                    return jnp.concatenate(
                        [jnp.concatenate([out[r, 0, r0], out[r, 1, r0]], axis=1)
                         for r in range(2) for r0 in range(0, 128, MH)], axis=0)

                def emit(R, N, val):
                    if N == 0:
                        rows = slice(512 * ck + 256 * R, 512 * ck + 256 * (R + 1))
                        outs = []
                        if 2 * ck + R < NP - 1:
                            blocks = [val[:128, :128], val[:128, 128:], val[128:, :128], val[128:, 128:]]
                            for i in (0, 1, 4, 5, 6):
                                outs.append(_join32(_term(_LHS, i, blocks.__getitem__)))
                                kt_w[i, 2 * ck + R] = outs[-1]
                        for n in range(2):
                            w = _join32(val[:, 128 * n:128 * (n + 1)])
                            k_w[n, 256 * ck + 128 * R:256 * ck + 128 * (R + 1), :] = w
                            outs += [w[:64], w[64:]]
                        later(CFG.get('lk', 0), outs)
                    else:
                        blocks = [val[128 * r:128 * (r + 1), 128 * n:128 * (n + 1)].T
                                  for n in range(2) for r in range(2)]
                        outs = [v.astype(BF16) for v in blocks]
                        for m, v in enumerate(outs):
                            vt_s[4 * ck + 2 * R + m % 2, 128 * (m // 2):128 * (m // 2 + 1), :] = v
                        if 2 * ck + R < NP - 1:
                            for i in (0, 1, 4, 5, 6):
                                outs.append(_term(_LHS, i, blocks.__getitem__).astype(BF16))
                                vx_s[i, 2 * ck + R] = outs[-1]
                        later(CFG.get('lv', 0), outs)

                return _strassen_steps(prod, emit)

            kv = [kv_chunk(ck) for ck in range(4)]

            def k_rows(r0, r1):
                return jnp.concatenate([k_s[0, r0:r1, :], k_s[1, r0:r1, :]], axis=1)

            def q_cols(r0, r1):
                return jnp.concatenate([qc_s[h, t] for t in range(r0 // 128, r1 // 128)], axis=1)

            mx, pr = {}, {}

            def s_at(u, r0):
                t = u // 4
                first = [v for v in range(u) if (v // 4) % 2 == t % 2]
                return s_s[t % 2], 128 * sum(v + 1 for v in first) + r0

            def qk(jq):
                run = [None, None]

                def put(n, r0, val):
                    buf, row = s_at(2 * jq + n, r0)
                    buf[row:row + val.shape[0], :] = val
                    vs = [val[r:r + 8] for r in range(0, val.shape[0], 8)]
                    def fold(op, xs, ways):
                        accs = xs[:ways]
                        for k, x in enumerate(xs[ways:]):
                            accs[k % ways] = op(accs[k % ways], x)
                        while len(accs) > 1:
                            accs = [op(a, b) for a, b in zip(accs[::2], accs[1::2])]
                        return accs[0]

                    m = fold(jnp.maximum, list(vs), CFG.get('mw', 1))
                    if run[n] is not None:
                        m = jnp.maximum(m, run[n][0])
                    if CFG.get('lsep'):
                        run[n] = (m, None)
                        return
                    l = fold(jnp.add, [jnp.exp2(v - m) for v in vs], CFG.get('lw', 1))
                    if run[n] is not None:
                        l = l + run[n][1] * jnp.exp2(run[n][0] - m)
                    run[n] = (m, l)

                if jq > 0:
                    raw = [qc_w[h, 2 * jq + n % 2, 64 * (n // 2):64 * (n // 2 + 1), :] for n in range(4)]
                    full = [_split(w) for w in raw]
                    qt = [pltpu.bitcast(raw[_RHS[i][0]] if len(_RHS[i]) == 1
                                        else _join(_term(_RHS, i, full.__getitem__)), BF16) for i in range(7)]
                QH = 128 // CFG.get('qh', 1)

                def diag():
                    q0 = 256 * jq
                    for n in range(2):
                        tick('Q', 64 * (n + 1))
                        sd = _dot(tied(k_rows(q0, q0 + 128 * (n + 1))), qc_s[h, 2 * jq + n])
                        sd = jnp.concatenate([sd[:128 * n], jnp.where(tri, sd[128 * n:], NEG)], axis=0) if n else (
                            jnp.where(tri, sd, NEG))
                        for r0 in range(0, 128 * (n + 1), QH):
                            put(n, q0 + r0, sd[r0:r0 + QH])
                    toks.append(sd[:8])

                if CFG.get('dfirst'):
                    diag()
                for jp in range(jq):
                    for r0 in range(0, 128, QH):
                        def prod(i):
                            tick('Q', QH // 4)
                            if i == 2:
                                lhs = k_s[0, 256 * jp + r0:256 * jp + r0 + QH, :]
                            elif i == 3:
                                lhs = k_s[1, 256 * jp + 128 + r0:256 * jp + 128 + r0 + QH, :]
                            else:
                                lhs = kt_s[i, jp, r0:r0 + QH, :]
                            m = _dot(tied(lhs), qt[i])
                            if i == 3 and r0 == 0:
                                toks.append(m[:8])
                            return m

                        _strassen(prod, lambda r, n, val: put(n, 256 * jp + 128 * r + r0, val))
                if not CFG.get('dfirst'):
                    diag()
                for n in range(2):
                    m, l = run[n]
                    top = jnp.max(m, axis=0, keepdims=True)
                    if CFG.get('lsep'):
                        tops[2 * jq + n] = top
                        continue
                    tot = jnp.sum(l * jnp.exp2(m - top), axis=0, keepdims=True)
                    mx[2 * jq + n] = top + jnp.log2(tot)

            tops = {}

            def denom(u, deadline):
                buf, row = s_at(u, 0)
                x = buf[pl.ds(pl.multiple_of(row + 16 * zero, 8), 128 * (u + 1)), :]
                e = jnp.exp2(x - tops[u])
                ways = CFG.get('dw', 1)
                accs = [e[8 * k:8 * (k + 1)] for k in range(ways)]
                for k in range(ways, e.shape[0] // 8):
                    accs[k % ways] = accs[k % ways] + e[8 * k:8 * (k + 1)]
                while len(accs) > 1:
                    accs = [a + b for a, b in zip(accs[::2], accs[1::2])]
                tot = jnp.sum(accs[0], axis=0, keepdims=True)
                mx[u] = tops[u] + jnp.log2(tot)
                if deadline:
                    due.append(tot)

            def probs(u, r0):
                buf, row = s_at(u, r0)
                x = jnp.concatenate([buf[pl.ds(row + e + zero, 8, stride=4), :] for e in (0, 2)], axis=0)
                return jnp.exp2(x - mx[u])

            def softmax(jq, jps, deadline):
                for u in (2 * jq, 2 * jq + 1):
                    if u not in mx:
                        denom(u, False)
                starts = [r + e for r in range(0, 256, 32) for e in range(2)]
                for jp in jps:
                    if jp == jq:
                        out = [jnp.concatenate([_join(probs(2 * jq + n, 256 * jq + r)) for r in starts[:8 * (n + 1)]],
                                               axis=0) for n in range(2)]
                    else:
                        parts = []
                        for r in starts[:8]:
                            blocks = [probs(2 * jq + m % 2, 256 * jp + 128 * (m // 2) + r) for m in range(4)]
                            parts.append([_join(t) for t in _rhs_terms(*blocks)])
                        out = [jnp.concatenate([p[i] for p in parts], axis=0) for i in range(7)]
                    pr[jq, jp] = out
                    if deadline:
                        due.append(_digest([out[0]]) ^ _digest([out[1]]) if jp == jq else _digest(out))

            def pv(jq):
                softmax(jq, [jp for jp in range(jq + 1) if (jq, jp) not in pr], False)
                diag = pr.pop((jq, jq))
                ps = [pr.pop((jq, jp)) for jp in range(jq)]
                base = []
                for n in range(2):
                    tick('P', 64 * (n + 1))
                    vt = jnp.concatenate([vt_s[2 * jq + i] for i in range(n + 1)], axis=1)
                    base.append(_dot(tied(vt), pltpu.bitcast(diag[n], BF16)))

                def emit(r, n, val):
                    val = base[n][128 * r:128 * (r + 1)] if val is None else val + base[n][128 * r:128 * (r + 1)]
                    qc_s[h, 2 * jq + n, 128 * r:128 * (r + 1), :] = val.astype(BF16)

                def prod(i):
                    tick('P', 32 * jq)
                    if i == 2:
                        lhs = [vt_s[2 * jp, 0:128, :] for jp in range(jq)]
                    elif i == 3:
                        lhs = [vt_s[2 * jp + 1, 128:256, :] for jp in range(jq)]
                    else:
                        lhs = [vx_s[i, jp] for jp in range(jq)]
                    rhs = pltpu.bitcast(jnp.concatenate([p[i] for p in ps], axis=0), BF16)
                    return _dot(tied(jnp.concatenate(lhs, axis=1)), rhs)

                if jq:
                    _strassen(prod, emit)
                else:
                    for r in range(2):
                        for n in range(2):
                            emit(r, n, None)

            CG, XG = CFG.get('cg', 0), CFG.get('xg', 0)
            pend = []
            def run_step(st_):
                kind, arg = st_[0], st_[1:]
                if kind == 'L':
                    for x in arg:
                        denom(int(x, 16), True)
                    return
                if kind == 'E':
                    jq = int(arg[0])
                    softmax(jq, [int(x) for x in arg[1:]] if arg[1:] else range(jq + 1), True)
                    return
                old = list(pend)
                pend.clear()
                if kind == 'C':
                    for _ in range(int(arg)):
                        pend.append(chan_mm(chans.pop(0), tok(CG)))
                elif kind == 'M':
                    for o in arg[1:]:
                        kv[int(arg[0])](int(o))
                elif kind == 'Q':
                    for x in arg:
                        qk(int(x))
                elif kind == 'P':
                    for x in arg:
                        pv(int(x))
                for args in old:
                    chan_post(*args)

            for seg in [g for g in CFG['sched'].split('|') if g.strip()]:
                if CFG.get('scopes') and '|' in CFG['sched']:
                    with jax.named_scope('s_' + seg.split()[0]):
                        for st_ in seg.split():
                            run_step(st_)
                else:
                    for st_ in seg.split():
                        run_step(st_)
            for c, y in ys:
                y_s[pl.ds(c, NB, stride=PITCH), :] = pltpu.bitcast(y, U32)
            for t, d0, n, v in cs:
                qc_s[h, t, d0:d0 + n, :] = v
            assert all(st_[1] == st_[2] for st_ in streams), [st_[1:] for st_ in streams]
            assert CFG.get('noassert') or not chans and not pend and (not due or CFG.get('pd')) and not pr

        if CFG.get('p1', 1):
            return lax.fori_loop(0, H // UN, heads, 0)
        else:
            _wait(g3b, 'wg3b')
            for c_ in g4:
                c_.start()

            def keep(h, carry):
                r = pl.multiple_of(h * 16, 16)
                t = (qc_s[h, h, 0:16, :].astype(F32) + cs_s[h % 4, h, h % 2, 0:16, :].astype(F32)
                     + pltpu.bitcast(aw_s[pl.ds(r, 16), :] + g_s[h, pl.ds(r, 16), :], F32)
                     + wx_s[h, pl.ds(r, 16), :].astype(F32))
                y_s[pl.ds(r, 16), :] = pltpu.bitcast(t, U32)
                return carry + h // H
            return lax.fori_loop(0, H, keep, 0)

    zero_end = phase1(k_s, kt_s, vt_s, vx_s, wx_s, sa_s, sb_s)

    def phase2():
        _wait(g4, 'wg4')
        HH = H // 2

        def wo_block(rh, kh):
            rows = [(C * (H * b + h) + CH * rh) // 2 for h in range(HH * kh, HH * (kh + 1)) for b in range(2)]
            return jnp.concatenate([xs_w[r:r + CH // 2, :] for r in rows], axis=1)

        raw = [wo_block(0, 0), wo_block(1, 0), wo_block(0, 1), wo_block(1, 1)]
        full = [_split(w) for w in raw]
        wt = [pltpu.bitcast(raw[_RHS[i][0]] if len(_RHS[i]) == 1 else _join(_term(_RHS, i, full.__getitem__)), BF16)
              for i in range(7)]
        outs = []
        due, late = [], []
        DL = CFG.get('dl', 3)
        never = _never(zero_end)

        def put(t, b, z, opaque=False):
            z = z.T
            r0 = pl.multiple_of(zero_end * 16 + 128 * t, 16) if opaque else 128 * t
            out_s[pl.ds(r0, 128), 128 * b:128 * (b + 1)] = z.astype(BF16)
            late.append(z[120:])

        for jp in range(CFG.get('np2', NP) if CFG.get('p2', 1) else 0):
            def ctx_block(r, kh):
                return jnp.concatenate([qc_w[h, 2 * jp + r] for h in range(HH * kh, HH * (kh + 1))], axis=0)

            craw = [ctx_block(0, 0), ctx_block(0, 1), ctx_block(1, 0), ctx_block(1, 1)]
            cfull = [_split(w) for w in craw]
            ct = [pltpu.bitcast(craw[_LHS[i][0]] if len(_LHS[i]) == 1
                                else _join(_term(_LHS, i, cfull.__getitem__)), BF16) for i in range(7)]
            za = {}
            prev_late = list(late)
            late.clear()
            for r in range(2):
                t = 2 * jp + r
                za[r] = (pltpu.bitcast(y_s[t * PITCH:t * PITCH + C, :], F32)
                         * x_s[:, 128 * t:128 * (t + 1)].astype(F32))
                for b in range(3):
                    put(t, b, za[r][128 * b:128 * (b + 1)], opaque=(r == 0 and b == 0 and jp > 0))
            a_late = list(late)
            late.clear()
            res = {}
            count = [0]

            def prod(i):
                if count[0] == DL:
                    due.extend(prev_late)
                if count[0] == 6:
                    due.extend(a_late)
                count[0] += 1
                return _dot(_tied(wt[i], due, never), ct[i])

            _strassen(prod, lambda r, c, val: res.__setitem__((r, c), val), order=CFG.get('oo', (1, 4, 3, 2, 0, 5, 6)))
            for r in CFG.get('ro', (1, 0)):
                z = jnp.concatenate([za[r][384:], res[(r, 0)], res[(r, 1)]], axis=0)
                for b in CFG.get('bo', (3, 2, 1, 0)):
                    put(2 * jp + r, 3 + b, z[128 * b:128 * (b + 1)])
            rows = pl.ds(256 * jp, 256)
            oc = cp(out_s.at[rows], o_hbm.at[rows], 26 + jp)
            oc.start()
            outs.append(oc)
        if not CFG.get('p2', 1):
            def keep(h, carry):
                r = pl.multiple_of(h * 16, 16)
                out_s[pl.ds(r, 16), 0:128] = pltpu.bitcast(y_s[pl.ds(r, 16), :], F32).astype(BF16) + qc_s[h, h, 0:16, :]
                return carry
            lax.fori_loop(0, H, keep, 0)
            oc = cp(out_s.at[pl.ds(0, 256)], o_hbm.at[pl.ds(0, 256)], 26)
            oc.start()
            outs.append(oc)
        _wait(outs, 'wout')

    phase2()


def _tiles(w):
    rows = w.shape[0]
    return w.reshape(rows, 2, 8, 2, 128).transpose(0, 1, 3, 2, 4).reshape(rows, 32, 128)


@jax.jit
def pallas_concat_heads__ssm_conv_h3__compressed_kv_cla__prompt_kernel(
    A_q: jax.Array,
    A_k: jax.Array,
    A_v: jax.Array,
    A_shift_k: jax.Array,
    A_ssm_k: jax.Array,
    A_ssm_D: jax.Array,
    B_x: jax.Array,
    B_c_kv: jax.Array,
    B_w_q: jax.Array,
    B_w_uk: jax.Array,
    B_w_uv: jax.Array,
    B_w_o: jax.Array,
):
    hbm = pl.BlockSpec(memory_space=pltpu.HBM)
    out = pl.pallas_call(
        _kernel,
        in_specs=[hbm] * 12,
        out_specs=hbm,
        out_shape=jax.ShapeDtypeStruct((S, 2 * C), BF16),
        scratch_shapes=[
            pltpu.VMEM((8, S // 2, 128), U32),
            pltpu.VMEM((4, 49, 2, 64, 128), U32),
            pltpu.VMEM((2, 4, DC, 128), U32),
            pltpu.VMEM((H, NB, D // 2, 128), U32),
            pltpu.VMEM((64 * PITCH, 128), U32),
            pltpu.VMEM((NB, C, 128), U32),
            pltpu.VMEM((NB * PITCH, 128), U32),
            pltpu.VMEM((CH, S), U32),
            pltpu.VMEM((512, 128), F32),
            pltpu.VMEM((2, S // 2, 128), U32),
            pltpu.VMEM((7, NP, 64, 128), U32),
            pltpu.VMEM((NB, D // 2, 128), U32),
            pltpu.VMEM((7, NP, 64, 128), U32),
            pltpu.VMEM((49, DC // 8, 128), U32),
            pltpu.VMEM((4 * C * 4, 128), F32),
            pltpu.VMEM((84 * 128, 128), F32),
            pltpu.VMEM((CH, S), U32),
            pltpu.VMEM((7 * NP * 128, 128), U32),
            pltpu.VMEM((CH, S), U32),
            pltpu.VMEM((CH, S), U32),
            pltpu.VMEM((2, 8, 128, 128), F32),
            pltpu.VMEM((S, 2 * C), BF16),
            pltpu.VMEM((4, C), BF16),
            pltpu.VMEM((C,), BF16),
            pltpu.SemaphoreType.DMA((36,)),
        ],
        compiler_params=pltpu.CompilerParams(
            vmem_limit_bytes=127 * 2 ** 20, disable_semaphore_checks=bool(CFG.get('nsc')),
            disable_bounds_checks=bool(CFG.get('nbc'))),
    )(
        A_q[0].T, A_k[0].T, A_v[0].T, A_shift_k.T, A_ssm_k, A_ssm_D, B_x[0].T, B_c_kv[0],
        _tiles(B_w_q), _tiles(B_w_uk), _tiles(B_w_uv),
        jnp.swapaxes(B_w_o, 1, 2).reshape(H * C, D),
    )
    return out.reshape(1, S, 2 * C)
```

```python
import math

import jax
import jax.numpy as jnp
from jax import lax
import jax.experimental.pallas as pl
import jax.experimental.pallas.tpu as pltpu

F32 = jnp.float32
BF16 = jnp.bfloat16
U32 = jnp.uint32
I32 = jnp.int32

S = 2048
C = 448
H = 16
D = 256
DC = 1024
NB = S // 128
NP = NB // 2
CH = C // 2
PITCH = 520
CPH = C // H
TQ = 512
NT = (((1,), (1,)), ((), ()))
LOG2E = math.log2(math.e)
QSCALE = (D ** -0.5) * LOG2E
NEG = -1e9 * LOG2E
HI_MASK = 0xFFFF0000
CFG = dict(ua=30,ud=96,nf=8,n0=3,ux=13,gback=8,slack=8,lag=8,lagA=3,nsc=1,oo=(1,4,3,6,0,2,5),ro=(0,1),bo=(0,1,2,3),late=(),x2=('P',0,1),mh=2,qh=2,mw=2,lw=2,cg=5,x1=('P',1500,7580),sched='M001 C2 M034 C2 M06 M101 C2 Q01 M134 C2 M16 M201 C2 Q23 M234 C2 M26 M301 C2 E0 E1 E2 Q45 M334 C2 M36 E3 M02 C2 Q67 M05 C2 M12 C2 E4 M15 C2 E5012 M22 C2 E5345 M25 C2 M32 E6012 M35 E63456 P01234567')


def _wait(copies, name):
    if CFG.get('scopes'):
        with jax.named_scope(name):
            for c_ in copies:
                c_.wait()
    else:
        for c_ in copies:
            c_.wait()


def _dot(a, b):
    return jnp.dot(a, b, preferred_element_type=F32)


def _dot_nt(a, b):
    return lax.dot_general(a, b, NT, preferred_element_type=F32)


def _lo(x):
    return pltpu.bitcast(x << 16, F32)


def _hi(x):
    return pltpu.bitcast(x & jnp.uint32(HI_MASK), F32)


def _pack(even, odd):
    return pltpu.pack_elementwise([even, odd], packed_dtype=BF16).astype(U32)


def _split(words):
    return jnp.concatenate([_lo(words), _hi(words)], axis=0)


def _join32(x):
    return jnp.concatenate([_pack(x[m:m + 16], x[m + 16:m + 32]) for m in range(0, x.shape[0], 32)], axis=0)


def _join16(x):
    return jnp.concatenate([_pack(x[m:m + 8], x[m + 8:m + 16]) for m in range(0, x.shape[0], 16)], axis=0)


def _join(x):
    n = x.shape[0] // 2
    return _pack(x[:n], x[n:])


def _head_cols(w_s, h, rows):
    out = []
    for b in range(2):
        x = w_s[b, pl.ds(h // 2, rows, stride=8), :]
        if isinstance(h, int):
            out.append(_lo(x) if h % 2 == 0 else _hi(x))
        else:
            out.append(_hi(x << ((1 - h % 2) * 16).astype(U32)))
    return out


_LHS = ((0, 1, 3), (2, 1, 3), (0,), (3,), (0, 1, 1), (2, -1, 0), (1, -1, 3))
_RHS = ((0, 1, 3), (0,), (1, -1, 3), (2, -1, 0), (3,), (0, 1, 1), (2, 1, 3))


def _term(table, i, block):
    spec = table[i]
    if len(spec) == 1:
        return block(spec[0])
    return block(spec[0]) + block(spec[2]) if spec[1] > 0 else block(spec[0]) - block(spec[2])


def _lhs_terms(*blocks):
    return [_term(_LHS, i, blocks.__getitem__) for i in range(7)]


def _rhs_terms(*blocks):
    return [_term(_RHS, i, blocks.__getitem__) for i in range(7)]


def _inner_terms(table, o, block):
    sub = [_term(table, o, lambda n: block(n, m)) for m in range(4)]
    return [_term(table, i, sub.__getitem__) for i in range(7)]


def _strassen_steps(prod, emit):
    uses = {(0, 0): {0: 1, 3: 1, 4: -1, 6: 1}, (0, 1): {2: 1, 4: 1},
            (1, 0): {1: 1, 3: 1}, (1, 1): {0: 1, 1: -1, 2: 1, 5: 1}}
    acc = {}
    neg = {}

    def step(i):
        m = prod(i)
        for key, terms in uses.items():
            if i not in terms:
                continue
            sign = terms.pop(i)
            if key not in acc:
                acc[key] = m
                neg[key] = sign < 0
            elif neg[key]:
                assert sign > 0
                acc[key] = m - acc[key]
                neg[key] = False
            else:
                acc[key] = acc[key] + m if sign > 0 else acc[key] - m
            if not terms:
                emit(key[0], key[1], acc.pop(key))

    return step


def _strassen(prod, emit, order=(0, 1, 3, 2, 4, 5, 6)):
    step = _strassen_steps(prod, emit)
    for i in order:
        step(i)


def _mult(i, n):
    return i if isinstance(i, int) else pl.multiple_of(i, n)


def _never(zero):
    return lax.broadcasted_iota(I32, (8, 128), 1) < zero


def _after(x, tok, never):
    if tok is None:
        return x
    return jnp.where(never, pltpu.bitcast(tok, x.dtype), x)


def _tied(lhs, due, never):
    if not due:
        return lhs
    t = None
    for d in due:
        d = pltpu.bitcast(jnp.broadcast_to(d, (8, 128)), U32)
        t = d if t is None else t ^ d
    due.clear()
    x = pltpu.bitcast(_after(pltpu.bitcast(lhs[:16, :128], U32), t, never), BF16)
    if lhs.shape[1] > 128:
        x = jnp.concatenate([x, lhs[:16, 128:]], axis=1)
    return jnp.concatenate([x, lhs[16:]], axis=0) if lhs.shape[0] > 16 else x


def _digest(vals):
    acc = None
    words = [v if v.dtype == U32 else pltpu.bitcast(v, U32) for v in vals]
    for r in range(words[0].shape[0] // 8):
        for w in words:
            w = w[8 * r:8 * (r + 1)]
            acc = w if acc is None else acc ^ w
    return acc


class _Packed:
    def __init__(self, ref):
        self.ref = ref

    def _index(self, idx):
        idx = idx if isinstance(idx, tuple) else (idx,)
        axis = len(self.ref.shape) - 2
        if len(idx) <= axis:
            return idx + (slice(None),) * (axis + 2 - len(idx))
        r = idx[axis]
        if isinstance(r, slice):
            r = slice(None if r.start is None else r.start // 2, None if r.stop is None else r.stop // 2)
        else:
            r = pl.ds(_mult(r.start // 2, 8), r.size // 2)
        return idx[:axis] + (r,) + idx[axis + 1:]

    def __getitem__(self, idx):
        return pltpu.bitcast(self.ref[self._index(idx)], BF16)

    def __setitem__(self, idx, val):
        self.ref[self._index(idx)] = pltpu.bitcast(val, U32)


def _kernel(qa_hbm, ka_hbm, va_hbm, sk_hbm, hk_hbm, d_hbm, x_hbm, c_hbm, wq_hbm, wk_hbm, wv_hbm, wo_hbm,
            o_hbm,
            c_s, cs_s, wp_s, qc_s, aw_s, g_s, y_s, hk_s, dc_s, k_s, kt_s, vt_s, vx_s, wx_s, sa_s, sb_s, x_s, xs_s, ka_s, va_s, wt_s, out_s, sk_ref, d_ref, sems):
    def cp(src, dst, i):
        return pltpu.make_async_copy(src, dst, sems.at[i])

    c_w, xs_w, x_w, ka_w, va_w, hk_w, cs_w, wx_w, qc_w = c_s, xs_s, x_s, ka_s, va_s, hk_s, cs_s, wx_s, qc_s
    k_w, kt_w, vt_w, vx_w = k_s, kt_s, vt_s, vx_s
    c_s, cs_s, qc_s, k_s, kt_s, vt_s, vx_s, wx_s, xs_s, x_s, ka_s, va_s, hk_s = (
        _Packed(r) for r in (c_s, cs_s, qc_s, k_s, kt_s, vt_s, vx_s, wx_s, xs_s, x_s, ka_s, va_s, hk_s))
    qa_hbm, ka_hbm, va_hbm, hk_hbm, x_hbm, c_hbm, wo_hbm = (
        r.bitcast(U32) for r in (qa_hbm, ka_hbm, va_hbm, hk_hbm, x_hbm, c_hbm, wo_hbm))
    wq32 = wq_hbm.bitcast(U32)
    wk32 = wk_hbm.bitcast(U32)
    wv32 = wv_hbm.bitcast(U32)
    gc = [cp(c_hbm.at[:, pl.ds(128 * b, 128)], c_w.at[b], 8 + b) for b in range(8)]

    def word_row(pair, b):
        return 8 * (pair // 4) + 4 * b + pair % 4

    def kv_copies(pair):
        return [cp(w.at[:, word_row(pair, b), :], wp_s.at[pair % 2, 2 * n + b], 16 + pair % 2)
                for n, w in enumerate((wk32, wv32)) for b in range(2)]

    g3 = kv_copies(0)
    g3b = kv_copies(1)
    g4 = [cp(qa_hbm, x_w, 21)] + [cp(wo_hbm.at[:, pl.ds(128 * b, 128)], xs_w.at[pl.ds(H * CH * b, H * CH)], 6 + b)
                                  for b in range(2)]

    def delayed(ref, rows, sg, n, gate=None):
        cur = pltpu.bitcast(ref[rows, 128 * sg:128 * (sg + 1)], U32)
        lane = lax.broadcasted_iota(I32, (8, 128), 1)
        if gate is not None:
            lane = gate(lane)
        lane = jnp.concatenate([lane] * (cur.shape[0] // 8), axis=0)
        prev = pltpu.bitcast(ref[rows, 128 * (sg - 1):128 * sg], U32) if sg > 0 else jnp.uint32(0)
        x = pltpu.roll(jnp.where(lane < 128 - n, cur, prev), n, 1)
        return pltpu.bitcast(x, BF16).astype(F32)

    def gated_t(x, gate):
        if gate is not None:
            x = jnp.concatenate([gate(x[:8]), x[8:]], axis=0)
        return x.T

    def windows(b, q, e, js, gate=None):
        out = []
        for j in js:
            parts = []
            for sg in range(2 * j - 6, 2 * j + 2):
                if sg < 0:
                    parts.append(jnp.zeros((16, 128), U32))
                else:
                    parts.append(pltpu.bitcast(sb_s[pl.ds(S * b + 128 * sg + 32 * q + 16 * e, 16), :], U32))
            plane = 32 * (j // 4) + 8 * q + 4 * e + j % 4
            win = gated_t(jnp.concatenate(parts, axis=0), gate)
            aw_s[pl.ds(_mult(plane * PITCH + 128 * b, 8), 128), :] = win
            out.append(win[120:])
        return out

    def prep_g(r0, n, gate=None):
        rows = pl.ds(_mult(r0, 16), n)
        lane = lax.broadcasted_iota(I32, (n, 128), 1)
        for a in range(NB):
            hf = hk_s[rows, 128 * a:128 * (a + 1)].astype(F32)
            hs = delayed(hk_s, rows, a, 1, gate)
            if a == 0:
                hf = jnp.where(lane == 0, hf + dc_s[rows, :], hf)
                hs = jnp.where(lane == 1, hs + dc_s[rows, :], hs)
            wrd = pltpu.pack_elementwise([hf, hs], packed_dtype=BF16).astype(U32)
            g_s[a, rows, :] = wrd
            yield _digest([wrd])

    def extract(h, r0, o, shift, z):
        def block(n, kq, b):
            x = jnp.concatenate([wp_s[(h // 2) % 2 + z, 2 * n + b, pl.ds(256 * kq + r0 + e, 8, stride=2), :]
                                 for e in range(2)], axis=0)
            if isinstance(h, int):
                return _lo(x) if h % 2 == 0 else _hi(x)
            return _hi(x << jnp.concatenate([shift] * 2, axis=0))

        terms = [_join(t) for t in _inner_terms(
            _RHS, o, lambda n, m: block(n % 2, 2 * (n // 2) + m // 2, m % 2))]
        for i, t in enumerate(terms):
            wx_w[7 * o + i, r0 // 2:r0 // 2 + 8, :] = t
        return _digest(terms)

    def phase0():
        XC = 512
        NF = CFG.get('nf', 4)
        N0 = CFG.get('n0', NF)
        N1 = CFG.get('n1', N0)
        cq = [cp(wq32.at[:, word_row(g // 2, g % 2), :], y_s.at[pl.ds(C * g, C)],
                 0 if g < N0 else 35 if g < N1 else 19 if g < NF else 1 if g < 8 else 18)
              for g in range(H)]
        cx = [cp(x_hbm.at[:, pl.ds(XC * i, XC)], x_w.at[:, pl.ds(XC * i, XC)], 22 + i) for i in range(S // XC)]
        ga = [cp(sk_hbm, sk_ref, 2), cp(ka_hbm, ka_w, 3), cp(va_hbm, va_w, 4)]
        gb = cq[8:] + gc
        gd = [cp(d_hbm, d_ref, 20), cp(hk_hbm, hk_w, 5)] + g3
        if CFG.get('merge'):
            ga, gb, gd = ga + cq[8:], [], gc + gd
        rest = cx[1:] + cq[NF:8] + ga
        if not CFG.get('jit', 1) or not CFG.get('p0', 1):
            rest = rest + gb + gd + g3b
        for c_ in [cx[0]] + cq[:NF] + rest:
            c_.start()
        zero = pl.semaphore_read(sems.at[34])
        never = _never(zero)
        due = []
        toks = []

        def pad_rows(t):
            return jnp.concatenate([t, jnp.zeros((256 - CH, 128), t.dtype)], axis=0)

        def wq_terms(j, b, gate):
            x = y_s[C * (2 * j + b):C * (2 * j + b + 1), :]
            g16 = jnp.concatenate([_after(jnp.full((8, 128), 16, U32), gate, never)] * (C // 8), axis=0)
            gm = jnp.concatenate([_after(jnp.full((8, 128), HI_MASK, U32), gate, never)] * (C // 8), axis=0)
            lo, hi = pltpu.bitcast(x << g16, F32), pltpu.bitcast(x & gm, F32)
            blocks = [pad_rows(t).T for t in (lo[:CH], hi[:CH], lo[CH:], hi[CH:])]
            if not CFG.get('q4', 1):
                return [t.astype(BF16) for t in _rhs_terms(*blocks)]
            slot = (2 * j + b) % 2
            for n, t in enumerate(blocks):
                for k in range(2):
                    wt_s[slot, 2 * n + k] = t[:, 128 * k:128 * (k + 1)]
            quarter = [[jnp.concatenate([wt_s[slot, 2 * n + k, pl.ds(e, 32, stride=4), :] for k in range(2)], axis=1)
                        for n in range(4)] for e in range(4)]
            terms = [_rhs_terms(*q) for q in quarter]
            out = []
            for i in range(7):
                ev, od = _pack(terms[0][i], terms[2][i]), _pack(terms[1][i], terms[3][i])
                rows = [w[8 * m:8 * (m + 1)] for m in range(4) for w in (ev, od)]
                out.append(pltpu.bitcast(jnp.concatenate(rows, axis=0), BF16))
            return out

        def x_terms(jp):
            top = slice(256 * jp, 256 * jp + 128)
            bot = slice(256 * jp + 128, 256 * jp + 256)
            for i in range(7):
                xs_s[256 * (NP * i + jp) + CH:256 * (NP * i + jp + 1), :] = jnp.zeros((256 - CH, 128), BF16)
            for r in range(0, CH, 32):
                lo, hi = slice(r // 2, r // 2 + 16), slice((CH + r) // 2, (CH + r) // 2 + 16)
                blocks = [x_w[lo, top], x_w[hi, top], x_w[lo, bot], x_w[hi, bot]]
                terms = [_join(t) for t in _lhs_terms(*[_split(t) for t in blocks])]
                terms[2], terms[3] = blocks[0], blocks[3]
                for i, t in enumerate(terms):
                    xs_w[128 * (NP * i + jp) + r // 2:128 * (NP * i + jp) + r // 2 + 16, :] = t
                yield 1, _digest(terms)

        def qproj(g, jp, waits):
            j, b = groups[g]
            for c_ in waits:
                c_.wait()
            if False:
                x_terms(jp)
                x_terms(jp + 1)

            XH = 128 // CFG.get('xh', 1)
            for r0 in range(0, 128, XH):
                def prod(i):
                    if r0 == 0 or True:
                        pump()
                    m = _dot(_tied(wts[g][i][r0:r0 + XH], due, never),
                             xs_s[256 * (NP * i + jp):256 * (NP * i + jp + 1), :])
                    toks.append(m[:8])
                    return m

                def emit(r, c, val):
                    w0 = 64 * b + r0 // 2
                    qc_w[2 * j + c, 2 * jp + r, w0:w0 + XH // 2, :] = _join32(val * QSCALE)

                _strassen(prod, emit)

        def column(row):
            row = jnp.concatenate([row.astype(F32), jnp.zeros((1, 512 - C), F32)], axis=1)
            return jnp.broadcast_to(row, (128, 512)).T

        consts = {}

        def make_consts():
            consts['taps'] = [column(sk_ref[j:j + 1, :]) for j in range(4)]

        def gate(x):
            back = CFG.get('gback', 6)
            return _after(x, toks[-back], never) if back else x

        def prep_u(r0, n):
            rows = slice(r0, r0 + n)
            tp = [t[rows] for t in consts['taps']]
            prev = jnp.zeros((n, 128), F32)
            for sg in range(NB):
                cols = slice(128 * sg, 128 * (sg + 1))
                ksh = ((delayed(ka_s, rows, sg, 3, gate) * tp[3] + delayed(ka_s, rows, sg, 2, gate) * tp[2])
                       + (delayed(ka_s, rows, sg, 1, gate) * tp[1] + ka_s[rows, cols].astype(F32) * tp[0]))
                kv = ksh * va_s[rows, cols].astype(F32)
                wrd = pltpu.pack_elementwise([prev, kv], packed_dtype=BF16).astype(U32)
                sa_s[C * sg + r0:C * sg + r0 + n, :] = pltpu.bitcast(wrd, F32)
                prev = kv
                yield _digest([wrd])

        def words_t(b):
            for sg in range(NB):
                r0 = C * sg + 128 * b
                if b < 3:
                    wrd = sa_s[r0:r0 + 128, :]
                else:
                    wrd = jnp.concatenate([sa_s[r0:r0 + C - 384, :], jnp.zeros((512 - C, 128), F32)], axis=0)
                wrd = gated_t(pltpu.bitcast(wrd, U32), gate)
                sb_s[S * b + 128 * sg:S * b + 128 * (sg + 1), :] = pltpu.bitcast(wrd, F32)
                yield wrd[120:]

        def all_windows(b):
            for p in range(8):
                for j in range(8):
                    yield windows(b, p // 2, p % 2, [j], gate)[0]

        def c_terms():
            for ck in range(4):
                for half in range(2):
                    for r0 in range(0, 128, 16):
                        for o in range(7):
                            def block(n, m):
                                row = 256 * ck + 128 * (n // 2) + 64 * (m // 2) + 16 * (r0 // 32)
                                col = 4 * (n % 2) + 2 * (m % 2) + half + zero * (o + 1)
                                w = jnp.concatenate([c_w[col, pl.ds(row + e, 8, stride=2), :] for e in range(2)], axis=0)
                                return _hi(w) if r0 % 32 else _lo(w)

                            terms = [_join(t) for t in _inner_terms(_LHS, o, block)]
                            for i, t in enumerate(terms):
                                cs_w[ck, 7 * o + i, half, r0 // 2:r0 // 2 + 8, :] = t
                            yield _digest(terms)

        UG = CFG.get('ug', 32)

        cu, ct, cg, cx_ = CFG.get('costs', (2, 2, 1, 1))

        def a_stream():
            make_consts()
            for b in range(4):
                for r0 in range(128 * b, min(C, 128 * (b + 1)), UG):
                    for v in prep_u(r0, UG):
                        yield cu * UG // 32, v
                for v in words_t(b):
                    yield ct, v
                for v in all_windows(b):
                    yield ct, v

        def d_stream():
            dc_s[...] = column(d_ref[...].reshape(1, C))
            for r0 in range(0, C, 32):
                for v in prep_g(r0, 32, gate):
                    yield cg, v
            for r0 in range(0, 256, 16):
                for o in range(7):
                    yield cx_, extract(0, r0, o, None, zero * (o + 1))

        a_total = cu * 14 * NB + ct * 4 * (NB + 64)
        d_total = cg * 14 * NB + cx_ * 112
        streams = []
        nprod = [0]
        later = {}
        LAG = CFG.get('lag', 0)

        def pump():
            for st_ in streams:
                gen, n, p0, p1, done = st_[:5]
                want = min(n, max(0, (nprod[0] - p0 + 1) * n // (p1 - p0)))
                while st_[4] < want:
                    cost, v = next(gen)
                    later.setdefault(nprod[0] + (st_[5] if len(st_) > 5 else LAG), []).append(v)
                    st_[4] += cost
            due.extend(later.pop(nprod[0], []))
            nprod[0] += 1

        groups = [(j, b) for j in range(H // 2) for b in range(2)]
        units = [(g, jp) for c in range(0, NP, 2) for g in range(NF) for jp in (c, c + 1)]
        units += [(g, jp) for g in range(NF, len(groups)) for jp in range(NP)]
        NU = len(units)
        wts = {}
        lead = CFG.get('lead', 4)
        ua = CFG.get('ua', 32)
        ub = 8 * NP - lead
        ux = CFG.get('ux', 5)
        ud = CFG.get('ud', 96)
        waits = {ux: cx[1:] + cq[NF:8], ua: ga, ud: gd}
        if gb:
            waits[ub] = gb
        else:
            ub = ud
        if N0 < N1:
            waits[2 * N0 - 1] = cq[N0:N1]
        if N1 < NF:
            waits[2 * N1 - 1] = cq[N1:NF]
        PU = 7 * CFG.get('xh', 1)
        xe = [PU * ux + 2] + [PU * NF * 2 * c - 1 for c in (1, 2, 3)]
        for c in range(3):
            streams.append([(v for jp in (2 * c + 2, 2 * c + 3) for v in x_terms(jp)), 14, xe[c], xe[c + 1], 0])
        sl = CFG.get('slack', 4)
        PA, PB, PE = PU * ua + sl, PU * ub + sl, PU * NU - 2 - LAG
        c_stream = ((1, v) for v in c_terms())
        nc = 4 * 2 * 8 * 7
        PD = PU * ud + sl
        streams.append([a_stream(), a_total, PA, PD + CFG.get('aext', 0), 0, CFG.get('lagA', LAG)])
        streams.append([c_stream, nc, PB, PE, 0])
        streams.append([d_stream(), d_total, PD + CFG.get('dext', CFG.get('aext', 0)), PE, 0])

        if not CFG.get('p0', 1):
            for c_ in cq[:8] + cx + ga + gb + gd:
                c_.wait()
            return
        _wait([cx[0]], 'wx0')
        list(x_terms(0))
        list(x_terms(1))
        _wait(cq[:N0], 'wq0')
        first_use = {}
        for u, (g, jp) in enumerate(units):
            first_use.setdefault(g, u)
        for u, (g, jp) in enumerate(units):
            if u in waits:
                if CFG.get('jit', 1):
                    for c_ in {ux: gb, ua: gd, ub: g3b}.get(u, []):
                        c_.start()
                _wait(waits[u], 'wu%d' % u)
            for g_, fu in first_use.items():
                if g_ not in wts and fu - (lead if g_ >= NF else 1) <= u:
                    back = CFG.get('wback', 8)
                    wts[g_] = wq_terms(*groups[g_], toks[-back] if len(toks) >= back else None)
            qproj(g, jp, [])
        assert all(st_[4] == st_[1] for st_ in streams) and not later, streams

    phase0()


    def phase1(k_s, kt_s, vt_s, vx_s, wx_s, *s_s):
        LATE = CFG.get('late', (2, 5))
        EARLY = tuple(o for o in (0, 1, 3, 4, 6, 2, 5) if o not in LATE)
        UN = CFG.get('unroll', 1)

        def heads(it, carry):
            @pl.when(it == 1)
            def _():
                for c_ in g4:
                    c_.start()

            if UN == 1:
                @pl.when(jnp.logical_and(it % 2 == 1, it < H - 1))
                def _():
                    _wait(kv_copies((it + 1) // 2), 'wkv')

                @pl.when(jnp.logical_and(jnp.logical_and(it % 2 == 0, it > 0), it < H - 2))
                def _():
                    for c_ in kv_copies(it // 2 + 1):
                        c_.start()
            else:
                @pl.when(it == 0)
                def _():
                    _wait(kv_copies(1), 'wkv')

            zero = it // H
            toks = []
            due = []
            for r in range(UN):
                head(it * UN + r, None if UN % 2 else r % 2, zero, toks, due)
            return carry + zero

        def head(h, par, zero, toks, due):
            lane8 = lax.broadcasted_iota(I32, (8, 128), 1)
            sub8 = lax.broadcasted_iota(I32, (8, 128), 0)
            lane16 = lax.broadcasted_iota(I32, (16, 128), 1)
            sub16 = lax.broadcasted_iota(I32, (16, 128), 0)
            tri = (lax.broadcasted_iota(I32, (128, 128), 0) <= lax.broadcasted_iota(I32, (128, 128), 1))
            h_next = h + 1 if isinstance(h, int) else jnp.minimum(h + 1, H - 1)
            never = _never(zero)

            def after(x, tok):
                return _after(x, tok, never)

            def tied(lhs):
                return _tied(lhs, due, never)

            def tok(back):
                return toks[-back] if (back and len(toks) >= back) else None

            def chan_mm(c, gate):
                m_b = lane8 < after(128 - 2 * sub8, gate)
                gs = [jnp.broadcast_to(g_s[a, pl.ds(c, 1), :], (8, 128)) for a in range(NB)]
                bt = [pltpu.roll(jnp.where(m_b, gs[a], gs[a - 1] if a > 0 else jnp.uint32(0)), 0, 1,
                                 stride=2, stride_axis=0) for a in range(NB)]
                b1 = pltpu.bitcast(jnp.concatenate(bt[7::-1], axis=0), BF16)
                b2 = pltpu.bitcast(jnp.concatenate(bt[15:7:-1], axis=0), BF16)
                am = pltpu.bitcast(aw_s[pl.ds(c, 64, stride=PITCH), :], BF16)
                tick('C', 48)
                z1 = _dot(tied(am), b1)
                z2 = _dot(am[:64], b2)
                return c, z1[:64], z1[64:] + z2

            def chan_post(c, zlo, zhi):
                acc = car = None
                for p in range(8):
                    z = jnp.concatenate([zlo[8 * p:8 * p + 8], zhi[8 * p:8 * p + 8]], axis=0)
                    if p == 0:
                        acc = z
                    else:
                        z = pltpu.roll(z, 16 * p, 1)
                        cz = jnp.where(lane16 < 16 * p, z, 0.0)
                        acc = acc + z
                        car = cz if car is None else car + cz
                y = (acc - car) + jnp.where(sub16 > 0, pltpu.roll(car, 1, 0), 0.0)
                later(CFG.get('ly', 0), [y])
                if CFG.get('ylate'):
                    ys.append((c, y))
                else:
                    y_s[pl.ds(c, NB, stride=PITCH), :] = pltpu.bitcast(y, U32)
                if CFG.get('pd', 0):
                    due.append(y[:8])
                    due.append(y[8:])

            chans = [h * CPH + i for i in range(CPH)]
            ys, cs = [], []

            def x_stream(hh, outers):
                n = 16 * len(outers)
                for r0 in range(0, 256, 16):
                    for o in outers:
                        n -= 1
                        free = n < CFG.get('xfree', 0) and hh is h_next
                        d = extract(hh, r0, o, shift_of(hh, tok(CFG.get('xfb', 1)) if free else None), zero * (o + 1))
                        yield None if free else d

            streams = [[x_stream(h_next, EARLY), 16 * len(EARLY), 0, 0] + list(CFG['x1']),
                       [x_stream(h, LATE), 16 * len(LATE), 0, 0] + list(CFG['x2'])]

            clock, queue = [0], []

            def later(lag, vals):
                if lag:
                    queue.append((clock[0] + lag, _digest(vals)))

            def tick(kind, cycles):
                clock[0] += cycles
                due.extend(v for t, v in queue if t <= clock[0] - cycles)
                queue[:] = [q for q in queue if q[0] > clock[0] - cycles]
                for st_ in streams:
                    gen, n, done, clk, kinds, c0, c1 = st_
                    if kind in kinds:
                        want = min(n, max(0, (clk - c0) * n // (c1 - c0)))
                        while st_[2] < want:
                            d = next(gen)
                            if d is not None:
                                if CFG.get('lx'):
                                    queue.append((clock[0] + CFG['lx'], d))
                                else:
                                    due.append(d)
                            st_[2] += 1
                        st_[3] += cycles

            def shift_of(hh, gate):
                return after(jnp.full((8, 128), (1 - hh % 2) * 16, I32).astype(U32), gate)

            def kv_chunk(ck):
                def prod(o):
                    MH = 128 // CFG.get('mh', 1)
                    out = {}
                    for r0 in range(0, 128, MH):
                        def inner(i):
                            tick('M', MH // 2)
                            lhs = jnp.concatenate([cs_s[ck, 7 * o + i, k, r0:r0 + MH, :] for k in range(2)], axis=1)
                            m = _dot(tied(lhs), wx_s[7 * o + i])
                            if i == CFG.get('ti', 3) and r0 == 0:
                                toks.append(m[:8])
                            return m

                        _strassen(inner, lambda r, n, val: out.__setitem__((r, n, r0), val))
                    return jnp.concatenate(
                        [jnp.concatenate([out[r, 0, r0], out[r, 1, r0]], axis=1)
                         for r in range(2) for r0 in range(0, 128, MH)], axis=0)

                def emit(R, N, val):
                    if N == 0:
                        rows = slice(512 * ck + 256 * R, 512 * ck + 256 * (R + 1))
                        outs = []
                        if 2 * ck + R < NP - 1:
                            blocks = [val[:128, :128], val[:128, 128:], val[128:, :128], val[128:, 128:]]
                            for i in (0, 1, 4, 5, 6):
                                outs.append(_join32(_term(_LHS, i, blocks.__getitem__)))
                                kt_w[i, 2 * ck + R] = outs[-1]
                        for n in range(2):
                            w = _join32(val[:, 128 * n:128 * (n + 1)])
                            k_w[n, 256 * ck + 128 * R:256 * ck + 128 * (R + 1), :] = w
                            outs += [w[:64], w[64:]]
                        later(CFG.get('lk', 0), outs)
                    else:
                        blocks = [val[128 * r:128 * (r + 1), 128 * n:128 * (n + 1)].T
                                  for n in range(2) for r in range(2)]
                        outs = [v.astype(BF16) for v in blocks]
                        for m, v in enumerate(outs):
                            vt_s[4 * ck + 2 * R + m % 2, 128 * (m // 2):128 * (m // 2 + 1), :] = v
                        if 2 * ck + R < NP - 1:
                            for i in (0, 1, 4, 5, 6):
                                outs.append(_term(_LHS, i, blocks.__getitem__).astype(BF16))
                                vx_s[i, 2 * ck + R] = outs[-1]
                        later(CFG.get('lv', 0), outs)

                return _strassen_steps(prod, emit)

            kv = [kv_chunk(ck) for ck in range(4)]

            def k_rows(r0, r1):
                return jnp.concatenate([k_s[0, r0:r1, :], k_s[1, r0:r1, :]], axis=1)

            def q_cols(r0, r1):
                return jnp.concatenate([qc_s[h, t] for t in range(r0 // 128, r1 // 128)], axis=1)

            mx, pr = {}, {}

            def s_at(u, r0):
                t = u // 4
                first = [v for v in range(u) if (v // 4) % 2 == t % 2]
                return s_s[t % 2], 128 * sum(v + 1 for v in first) + r0

            def qk(jq):
                run = [None, None]

                def put(n, r0, val):
                    buf, row = s_at(2 * jq + n, r0)
                    buf[row:row + val.shape[0], :] = val
                    vs = [val[r:r + 8] for r in range(0, val.shape[0], 8)]
                    def fold(op, xs, ways):
                        accs = xs[:ways]
                        for k, x in enumerate(xs[ways:]):
                            accs[k % ways] = op(accs[k % ways], x)
                        while len(accs) > 1:
                            accs = [op(a, b) for a, b in zip(accs[::2], accs[1::2])]
                        return accs[0]

                    m = fold(jnp.maximum, list(vs), CFG.get('mw', 1))
                    if run[n] is not None:
                        m = jnp.maximum(m, run[n][0])
                    if CFG.get('lsep'):
                        run[n] = (m, None)
                        return
                    l = fold(jnp.add, [jnp.exp2(v - m) for v in vs], CFG.get('lw', 1))
                    if run[n] is not None:
                        l = l + run[n][1] * jnp.exp2(run[n][0] - m)
                    run[n] = (m, l)

                if jq > 0:
                    raw = [qc_w[h, 2 * jq + n % 2, 64 * (n // 2):64 * (n // 2 + 1), :] for n in range(4)]
                    full = [_split(w) for w in raw]
                    qt = [pltpu.bitcast(raw[_RHS[i][0]] if len(_RHS[i]) == 1
                                        else _join(_term(_RHS, i, full.__getitem__)), BF16) for i in range(7)]
                QH = 128 // CFG.get('qh', 1)

                def diag():
                    q0 = 256 * jq
                    for n in range(2):
                        tick('Q', 64 * (n + 1))
                        sd = _dot(tied(k_rows(q0, q0 + 128 * (n + 1))), qc_s[h, 2 * jq + n])
                        sd = jnp.concatenate([sd[:128 * n], jnp.where(tri, sd[128 * n:], NEG)], axis=0) if n else (
                            jnp.where(tri, sd, NEG))
                        for r0 in range(0, 128 * (n + 1), QH):
                            put(n, q0 + r0, sd[r0:r0 + QH])
                    toks.append(sd[:8])

                if CFG.get('dfirst'):
                    diag()
                for jp in range(jq):
                    for r0 in range(0, 128, QH):
                        def prod(i):
                            tick('Q', QH // 4)
                            if i == 2:
                                lhs = k_s[0, 256 * jp + r0:256 * jp + r0 + QH, :]
                            elif i == 3:
                                lhs = k_s[1, 256 * jp + 128 + r0:256 * jp + 128 + r0 + QH, :]
                            else:
                                lhs = kt_s[i, jp, r0:r0 + QH, :]
                            m = _dot(tied(lhs), qt[i])
                            if i == 3 and r0 == 0:
                                toks.append(m[:8])
                            return m

                        _strassen(prod, lambda r, n, val: put(n, 256 * jp + 128 * r + r0, val))
                if not CFG.get('dfirst'):
                    diag()
                for n in range(2):
                    m, l = run[n]
                    top = jnp.max(m, axis=0, keepdims=True)
                    if CFG.get('lsep'):
                        tops[2 * jq + n] = top
                        continue
                    tot = jnp.sum(l * jnp.exp2(m - top), axis=0, keepdims=True)
                    mx[2 * jq + n] = top + jnp.log2(tot)

            tops = {}

            def denom(u, deadline):
                buf, row = s_at(u, 0)
                x = buf[pl.ds(pl.multiple_of(row + 16 * zero, 8), 128 * (u + 1)), :]
                e = jnp.exp2(x - tops[u])
                ways = CFG.get('dw', 1)
                accs = [e[8 * k:8 * (k + 1)] for k in range(ways)]
                for k in range(ways, e.shape[0] // 8):
                    accs[k % ways] = accs[k % ways] + e[8 * k:8 * (k + 1)]
                while len(accs) > 1:
                    accs = [a + b for a, b in zip(accs[::2], accs[1::2])]
                tot = jnp.sum(accs[0], axis=0, keepdims=True)
                mx[u] = tops[u] + jnp.log2(tot)
                if deadline:
                    due.append(tot)

            def probs(u, r0):
                buf, row = s_at(u, r0)
                x = jnp.concatenate([buf[pl.ds(row + e + zero, 8, stride=4), :] for e in (0, 2)], axis=0)
                return jnp.exp2(x - mx[u])

            def softmax(jq, jps, deadline):
                for u in (2 * jq, 2 * jq + 1):
                    if u not in mx:
                        denom(u, False)
                starts = [r + e for r in range(0, 256, 32) for e in range(2)]
                for jp in jps:
                    if jp == jq:
                        out = [jnp.concatenate([_join(probs(2 * jq + n, 256 * jq + r)) for r in starts[:8 * (n + 1)]],
                                               axis=0) for n in range(2)]
                    else:
                        parts = []
                        for r in starts[:8]:
                            blocks = [probs(2 * jq + m % 2, 256 * jp + 128 * (m // 2) + r) for m in range(4)]
                            parts.append([_join(t) for t in _rhs_terms(*blocks)])
                        out = [jnp.concatenate([p[i] for p in parts], axis=0) for i in range(7)]
                    pr[jq, jp] = out
                    if deadline:
                        d = _digest([out[0]]) ^ _digest([out[1]]) if jp == jq else _digest(out)
                        if CFG.get('le'):
                            queue.append((clock[0] + CFG['le'], d))
                        else:
                            due.append(d)

            def pv(jq):
                softmax(jq, [jp for jp in range(jq + 1) if (jq, jp) not in pr], False)
                diag = pr.pop((jq, jq))
                ps = [pr.pop((jq, jp)) for jp in range(jq)]
                base = []
                for n in range(2):
                    tick('P', 64 * (n + 1))
                    vt = jnp.concatenate([vt_s[2 * jq + i] for i in range(n + 1)], axis=1)
                    base.append(_dot(tied(vt), pltpu.bitcast(diag[n], BF16)))

                def emit(r, n, val):
                    val = base[n][128 * r:128 * (r + 1)] if val is None else val + base[n][128 * r:128 * (r + 1)]
                    qc_s[h, 2 * jq + n, 128 * r:128 * (r + 1), :] = val.astype(BF16)

                def prod(i):
                    tick('P', 32 * jq)
                    if i == 2:
                        lhs = [vt_s[2 * jp, 0:128, :] for jp in range(jq)]
                    elif i == 3:
                        lhs = [vt_s[2 * jp + 1, 128:256, :] for jp in range(jq)]
                    else:
                        lhs = [vx_s[i, jp] for jp in range(jq)]
                    rhs = pltpu.bitcast(jnp.concatenate([p[i] for p in ps], axis=0), BF16)
                    return _dot(tied(jnp.concatenate(lhs, axis=1)), rhs)

                if jq:
                    _strassen(prod, emit)
                else:
                    for r in range(2):
                        for n in range(2):
                            emit(r, n, None)

            CG, XG = CFG.get('cg', 0), CFG.get('xg', 0)
            pend = []
            def run_step(st_):
                kind, arg = st_[0], st_[1:]
                if kind == 'L':
                    for x in arg:
                        denom(int(x, 16), True)
                    return
                if kind == 'E':
                    jq = int(arg[0])
                    softmax(jq, [int(x) for x in arg[1:]] if arg[1:] else range(jq + 1), True)
                    return
                old = list(pend)
                pend.clear()
                if kind == 'C':
                    for _ in range(int(arg)):
                        pend.append(chan_mm(chans.pop(0), tok(CG)))
                elif kind == 'M':
                    for o in arg[1:]:
                        kv[int(arg[0])](int(o))
                elif kind == 'Q':
                    for x in arg:
                        qk(int(x))
                elif kind == 'P':
                    for x in arg:
                        pv(int(x))
                for args in old:
                    chan_post(*args)

            for seg in [g for g in CFG['sched'].split('|') if g.strip()]:
                if CFG.get('scopes') and '|' in CFG['sched']:
                    with jax.named_scope('s_' + seg.split()[0]):
                        for st_ in seg.split():
                            run_step(st_)
                else:
                    for st_ in seg.split():
                        run_step(st_)
            for c, y in ys:
                y_s[pl.ds(c, NB, stride=PITCH), :] = pltpu.bitcast(y, U32)
            for t, d0, n, v in cs:
                qc_s[h, t, d0:d0 + n, :] = v
            assert all(st_[1] == st_[2] for st_ in streams), [st_[1:] for st_ in streams]
            assert CFG.get('noassert') or not chans and not pend and (not due or CFG.get('pd')) and not pr

        if CFG.get('p1', 1):
            return lax.fori_loop(0, H // UN, heads, 0)
        else:
            _wait(g3b, 'wg3b')
            if CFG.get('p2', 1):
                for c_ in g4:
                    c_.start()

            def keep(h, carry):
                r = pl.multiple_of(h * 16, 16)
                t = (qc_s[h, h, 0:16, :].astype(F32) + cs_s[h % 4, h, h % 2, 0:16, :].astype(F32)
                     + pltpu.bitcast(aw_s[pl.ds(r, 16), :] + g_s[h, pl.ds(r, 16), :], F32)
                     + wx_s[h, pl.ds(r, 16), :].astype(F32))
                y_s[pl.ds(r, 16), :] = pltpu.bitcast(t, U32)
                return carry + h // H
            return lax.fori_loop(0, H, keep, 0)

    zero_end = phase1(k_s, kt_s, vt_s, vx_s, wx_s, sa_s, sb_s)

    def phase2():
        if CFG.get('p2', 1) or CFG.get('p1', 1):
            _wait(g4, 'wg4')
        HH = H // 2

        def wo_block(rh, kh):
            rows = [(C * (H * b + h) + CH * rh) // 2 for h in range(HH * kh, HH * (kh + 1)) for b in range(2)]
            return jnp.concatenate([xs_w[r:r + CH // 2, :] for r in rows], axis=1)

        raw = [wo_block(0, 0), wo_block(1, 0), wo_block(0, 1), wo_block(1, 1)]
        full = [_split(w) for w in raw]
        wt = [pltpu.bitcast(raw[_RHS[i][0]] if len(_RHS[i]) == 1 else _join(_term(_RHS, i, full.__getitem__)), BF16)
              for i in range(7)]
        outs = []
        due, late = [], []
        DL = CFG.get('dl', 3)
        never = _never(zero_end)

        def put(t, b, z, opaque=False):
            z = z.T
            r0 = pl.multiple_of(zero_end * 16 + 128 * t, 16) if opaque else 128 * t
            out_s[pl.ds(r0, 128), 128 * b:128 * (b + 1)] = z.astype(BF16)
            late.append(z[120:])

        for jp in range(CFG.get('np2', NP) if CFG.get('p2', 1) else 0):
            def ctx_block(r, kh):
                return jnp.concatenate([qc_w[h, 2 * jp + r] for h in range(HH * kh, HH * (kh + 1))], axis=0)

            craw = [ctx_block(0, 0), ctx_block(0, 1), ctx_block(1, 0), ctx_block(1, 1)]
            cfull = [_split(w) for w in craw]
            ct = [pltpu.bitcast(craw[_LHS[i][0]] if len(_LHS[i]) == 1
                                else _join(_term(_LHS, i, cfull.__getitem__)), BF16) for i in range(7)]
            za = {}
            prev_late = list(late)
            late.clear()
            for r in range(2):
                t = 2 * jp + r
                za[r] = (pltpu.bitcast(y_s[t * PITCH:t * PITCH + C, :], F32)
                         * x_s[:, 128 * t:128 * (t + 1)].astype(F32))
                for b in range(3):
                    put(t, b, za[r][128 * b:128 * (b + 1)], opaque=(r == 0 and b == 0 and jp > 0))
            a_late = list(late)
            late.clear()
            res = {}
            count = [0]

            def prod(i):
                if count[0] == DL:
                    due.extend(prev_late)
                if count[0] == 6:
                    due.extend(a_late)
                count[0] += 1
                return _dot(_tied(wt[i], due, never), ct[i])

            _strassen(prod, lambda r, c, val: res.__setitem__((r, c), val), order=CFG.get('oo', (1, 4, 3, 2, 0, 5, 6)))
            for r in CFG.get('ro', (1, 0)):
                z = jnp.concatenate([za[r][384:], res[(r, 0)], res[(r, 1)]], axis=0)
                for b in CFG.get('bo', (3, 2, 1, 0)):
                    put(2 * jp + r, 3 + b, z[128 * b:128 * (b + 1)])
            rows = pl.ds(256 * jp, 256)
            oc = cp(out_s.at[rows], o_hbm.at[rows], 26 + jp)
            oc.start()
            outs.append(oc)
        if not CFG.get('p2', 1):
            def keep(h, carry):
                r = pl.multiple_of(h * 16, 16)
                out_s[pl.ds(r, 16), 0:128] = pltpu.bitcast(y_s[pl.ds(r, 16), :], F32).astype(BF16) + qc_s[h, h, 0:16, :]
                return carry
            lax.fori_loop(0, H, keep, 0)
            oc = cp(out_s.at[pl.ds(0, 256)], o_hbm.at[pl.ds(0, 256)], 26)
            oc.start()
            outs.append(oc)
        _wait(outs, 'wout')

    phase2()


def _tiles(w):
    rows = w.shape[0]
    return w.reshape(rows, 2, 8, 2, 128).transpose(0, 1, 3, 2, 4).reshape(rows, 32, 128)


@jax.jit
def pallas_concat_heads__ssm_conv_h3__compressed_kv_cla__prompt_kernel(
    A_q: jax.Array,
    A_k: jax.Array,
    A_v: jax.Array,
    A_shift_k: jax.Array,
    A_ssm_k: jax.Array,
    A_ssm_D: jax.Array,
    B_x: jax.Array,
    B_c_kv: jax.Array,
    B_w_q: jax.Array,
    B_w_uk: jax.Array,
    B_w_uv: jax.Array,
    B_w_o: jax.Array,
):
    hbm = pl.BlockSpec(memory_space=pltpu.HBM)
    out = pl.pallas_call(
        _kernel,
        in_specs=[hbm] * 12,
        out_specs=hbm,
        out_shape=jax.ShapeDtypeStruct((S, 2 * C), BF16),
        scratch_shapes=[
            pltpu.VMEM((8, S // 2, 128), U32),
            pltpu.VMEM((4, 49, 2, 64, 128), U32),
            pltpu.VMEM((2, 4, DC, 128), U32),
            pltpu.VMEM((H, NB, D // 2, 128), U32),
            pltpu.VMEM((64 * PITCH, 128), U32),
            pltpu.VMEM((NB, C, 128), U32),
            pltpu.VMEM((NB * PITCH, 128), U32),
            pltpu.VMEM((CH, S), U32),
            pltpu.VMEM((512, 128), F32),
            pltpu.VMEM((2, S // 2, 128), U32),
            pltpu.VMEM((7, NP, 64, 128), U32),
            pltpu.VMEM((NB, D // 2, 128), U32),
            pltpu.VMEM((7, NP, 64, 128), U32),
            pltpu.VMEM((49, DC // 8, 128), U32),
            pltpu.VMEM((4 * C * 4, 128), F32),
            pltpu.VMEM((84 * 128, 128), F32),
            pltpu.VMEM((CH, S), U32),
            pltpu.VMEM((7 * NP * 128, 128), U32),
            pltpu.VMEM((CH, S), U32),
            pltpu.VMEM((CH, S), U32),
            pltpu.VMEM((2, 8, 128, 128), F32),
            pltpu.VMEM((S, 2 * C), BF16),
            pltpu.VMEM((4, C), BF16),
            pltpu.VMEM((C,), BF16),
            pltpu.SemaphoreType.DMA((36,)),
        ],
        compiler_params=pltpu.CompilerParams(
            vmem_limit_bytes=127 * 2 ** 20, disable_semaphore_checks=bool(CFG.get('nsc')),
            disable_bounds_checks=bool(CFG.get('nbc'))),
    )(
        A_q[0].T, A_k[0].T, A_v[0].T, A_shift_k.T, A_ssm_k, A_ssm_D, B_x[0].T, B_c_kv[0],
        _tiles(B_w_q), _tiles(B_w_uk), _tiles(B_w_uv),
        jnp.swapaxes(B_w_o, 1, 2).reshape(H * C, D),
    )
    return out.reshape(1, S, 2 * C)
```

```python
import math

import jax
import jax.numpy as jnp
from jax import lax
import jax.experimental.pallas as pl
import jax.experimental.pallas.tpu as pltpu

F32 = jnp.float32
BF16 = jnp.bfloat16
U32 = jnp.uint32
I32 = jnp.int32

S = 2048
C = 448
H = 16
D = 256
DC = 1024
NB = S // 128
NP = NB // 2
CH = C // 2
PITCH = 520
CPH = C // H
TQ = 512
NT = (((1,), (1,)), ((), ()))
LOG2E = math.log2(math.e)
QSCALE = (D ** -0.5) * LOG2E
NEG = -1e9 * LOG2E
HI_MASK = 0xFFFF0000
CFG = dict(ua=30,ud=96,nf=8,n0=3,ux=13,gback=8,slack=8,lag=8,lagU=8,lagT=3,nsc=1,oo=(1,4,3,6,0,2,5),ro=(0,1),bo=(0,1,2,3),late=(),x2=('P',0,1),mh=2,qh=2,mw=2,lw=2,cg=5,x1=('P',1500,7580),sched='M001 C2 M034 C2 M06 M101 C2 Q01 M134 C2 M16 M201 C2 Q23 M234 C2 M26 M301 C2 E0 E1 E2 Q45 M334 C2 M36 E3 M02 C2 Q67 M05 C2 M12 C2 E4 M15 C2 E5012 M22 C2 E5345 M25 C2 M32 E6012 M35 E63456 P01234567')


def _wait(copies, name):
    if CFG.get('scopes'):
        with jax.named_scope(name):
            for c_ in copies:
                c_.wait()
    else:
        for c_ in copies:
            c_.wait()


def _dot(a, b):
    return jnp.dot(a, b, preferred_element_type=F32)


def _dot_nt(a, b):
    return lax.dot_general(a, b, NT, preferred_element_type=F32)


def _lo(x):
    return pltpu.bitcast(x << 16, F32)


def _hi(x):
    return pltpu.bitcast(x & jnp.uint32(HI_MASK), F32)


def _pack(even, odd):
    return pltpu.pack_elementwise([even, odd], packed_dtype=BF16).astype(U32)


def _split(words):
    return jnp.concatenate([_lo(words), _hi(words)], axis=0)


def _join32(x):
    return jnp.concatenate([_pack(x[m:m + 16], x[m + 16:m + 32]) for m in range(0, x.shape[0], 32)], axis=0)


def _join16(x):
    return jnp.concatenate([_pack(x[m:m + 8], x[m + 8:m + 16]) for m in range(0, x.shape[0], 16)], axis=0)


def _join(x):
    n = x.shape[0] // 2
    return _pack(x[:n], x[n:])


def _head_cols(w_s, h, rows):
    out = []
    for b in range(2):
        x = w_s[b, pl.ds(h // 2, rows, stride=8), :]
        if isinstance(h, int):
            out.append(_lo(x) if h % 2 == 0 else _hi(x))
        else:
            out.append(_hi(x << ((1 - h % 2) * 16).astype(U32)))
    return out


_LHS = ((0, 1, 3), (2, 1, 3), (0,), (3,), (0, 1, 1), (2, -1, 0), (1, -1, 3))
_RHS = ((0, 1, 3), (0,), (1, -1, 3), (2, -1, 0), (3,), (0, 1, 1), (2, 1, 3))


def _term(table, i, block):
    spec = table[i]
    if len(spec) == 1:
        return block(spec[0])
    return block(spec[0]) + block(spec[2]) if spec[1] > 0 else block(spec[0]) - block(spec[2])


def _lhs_terms(*blocks):
    return [_term(_LHS, i, blocks.__getitem__) for i in range(7)]


def _rhs_terms(*blocks):
    return [_term(_RHS, i, blocks.__getitem__) for i in range(7)]


def _inner_terms(table, o, block):
    sub = [_term(table, o, lambda n: block(n, m)) for m in range(4)]
    return [_term(table, i, sub.__getitem__) for i in range(7)]


def _strassen_steps(prod, emit):
    uses = {(0, 0): {0: 1, 3: 1, 4: -1, 6: 1}, (0, 1): {2: 1, 4: 1},
            (1, 0): {1: 1, 3: 1}, (1, 1): {0: 1, 1: -1, 2: 1, 5: 1}}
    acc = {}
    neg = {}

    def step(i):
        m = prod(i)
        for key, terms in uses.items():
            if i not in terms:
                continue
            sign = terms.pop(i)
            if key not in acc:
                acc[key] = m
                neg[key] = sign < 0
            elif neg[key]:
                assert sign > 0
                acc[key] = m - acc[key]
                neg[key] = False
            else:
                acc[key] = acc[key] + m if sign > 0 else acc[key] - m
            if not terms:
                emit(key[0], key[1], acc.pop(key))

    return step


def _strassen(prod, emit, order=(0, 1, 3, 2, 4, 5, 6)):
    step = _strassen_steps(prod, emit)
    for i in order:
        step(i)


def _mult(i, n):
    return i if isinstance(i, int) else pl.multiple_of(i, n)


def _never(zero):
    return lax.broadcasted_iota(I32, (8, 128), 1) < zero


def _after(x, tok, never):
    if tok is None:
        return x
    return jnp.where(never, pltpu.bitcast(tok, x.dtype), x)


def _tied(lhs, due, never):
    if not due:
        return lhs
    t = None
    for d in due:
        d = pltpu.bitcast(jnp.broadcast_to(d, (8, 128)), U32)
        t = d if t is None else t ^ d
    due.clear()
    x = pltpu.bitcast(_after(pltpu.bitcast(lhs[:16, :128], U32), t, never), BF16)
    if lhs.shape[1] > 128:
        x = jnp.concatenate([x, lhs[:16, 128:]], axis=1)
    return jnp.concatenate([x, lhs[16:]], axis=0) if lhs.shape[0] > 16 else x


def _digest(vals):
    acc = None
    words = [v if v.dtype == U32 else pltpu.bitcast(v, U32) for v in vals]
    for r in range(words[0].shape[0] // 8):
        for w in words:
            w = w[8 * r:8 * (r + 1)]
            acc = w if acc is None else acc ^ w
    return acc


class _Packed:
    def __init__(self, ref):
        self.ref = ref

    def _index(self, idx):
        idx = idx if isinstance(idx, tuple) else (idx,)
        axis = len(self.ref.shape) - 2
        if len(idx) <= axis:
            return idx + (slice(None),) * (axis + 2 - len(idx))
        r = idx[axis]
        if isinstance(r, slice):
            r = slice(None if r.start is None else r.start // 2, None if r.stop is None else r.stop // 2)
        else:
            r = pl.ds(_mult(r.start // 2, 8), r.size // 2)
        return idx[:axis] + (r,) + idx[axis + 1:]

    def __getitem__(self, idx):
        return pltpu.bitcast(self.ref[self._index(idx)], BF16)

    def __setitem__(self, idx, val):
        self.ref[self._index(idx)] = pltpu.bitcast(val, U32)


def _kernel(qa_hbm, ka_hbm, va_hbm, sk_hbm, hk_hbm, d_hbm, x_hbm, c_hbm, wq_hbm, wk_hbm, wv_hbm, wo_hbm,
            o_hbm,
            c_s, cs_s, wp_s, qc_s, aw_s, g_s, y_s, hk_s, dc_s, k_s, kt_s, vt_s, vx_s, wx_s, sa_s, sb_s, x_s, xs_s, ka_s, va_s, wt_s, out_s, sk_ref, d_ref, sems):
    def cp(src, dst, i):
        return pltpu.make_async_copy(src, dst, sems.at[i])

    c_w, xs_w, x_w, ka_w, va_w, hk_w, cs_w, wx_w, qc_w = c_s, xs_s, x_s, ka_s, va_s, hk_s, cs_s, wx_s, qc_s
    k_w, kt_w, vt_w, vx_w = k_s, kt_s, vt_s, vx_s
    c_s, cs_s, qc_s, k_s, kt_s, vt_s, vx_s, wx_s, xs_s, x_s, ka_s, va_s, hk_s = (
        _Packed(r) for r in (c_s, cs_s, qc_s, k_s, kt_s, vt_s, vx_s, wx_s, xs_s, x_s, ka_s, va_s, hk_s))
    qa_hbm, ka_hbm, va_hbm, hk_hbm, x_hbm, c_hbm, wo_hbm = (
        r.bitcast(U32) for r in (qa_hbm, ka_hbm, va_hbm, hk_hbm, x_hbm, c_hbm, wo_hbm))
    wq32 = wq_hbm.bitcast(U32)
    wk32 = wk_hbm.bitcast(U32)
    wv32 = wv_hbm.bitcast(U32)
    gc = [cp(c_hbm.at[:, pl.ds(128 * b, 128)], c_w.at[b], 8 + b) for b in range(8)]

    def word_row(pair, b):
        return 8 * (pair // 4) + 4 * b + pair % 4

    def kv_copies(pair):
        return [cp(w.at[:, word_row(pair, b), :], wp_s.at[pair % 2, 2 * n + b], 16 + pair % 2)
                for n, w in enumerate((wk32, wv32)) for b in range(2)]

    g3 = kv_copies(0)
    g3b = kv_copies(1)
    g4 = [cp(qa_hbm, x_w, 21)] + [cp(wo_hbm.at[:, pl.ds(128 * b, 128)], xs_w.at[pl.ds(H * CH * b, H * CH)], 6 + b)
                                  for b in range(2)]

    def delayed(ref, rows, sg, n, gate=None):
        cur = pltpu.bitcast(ref[rows, 128 * sg:128 * (sg + 1)], U32)
        lane = lax.broadcasted_iota(I32, (8, 128), 1)
        if gate is not None:
            lane = gate(lane)
        lane = jnp.concatenate([lane] * (cur.shape[0] // 8), axis=0)
        prev = pltpu.bitcast(ref[rows, 128 * (sg - 1):128 * sg], U32) if sg > 0 else jnp.uint32(0)
        x = pltpu.roll(jnp.where(lane < 128 - n, cur, prev), n, 1)
        return pltpu.bitcast(x, BF16).astype(F32)

    def gated_t(x, gate):
        if gate is not None:
            x = jnp.concatenate([gate(x[:8]), x[8:]], axis=0)
        return x.T

    def windows(b, q, e, js, gate=None):
        out = []
        for j in js:
            parts = []
            for sg in range(2 * j - 6, 2 * j + 2):
                if sg < 0:
                    parts.append(jnp.zeros((16, 128), U32))
                else:
                    parts.append(pltpu.bitcast(sb_s[pl.ds(S * b + 128 * sg + 32 * q + 16 * e, 16), :], U32))
            plane = 32 * (j // 4) + 8 * q + 4 * e + j % 4
            win = gated_t(jnp.concatenate(parts, axis=0), gate)
            aw_s[pl.ds(_mult(plane * PITCH + 128 * b, 8), 128), :] = win
            out.append(win[120:])
        return out

    def prep_g(r0, n, gate=None):
        rows = pl.ds(_mult(r0, 16), n)
        lane = lax.broadcasted_iota(I32, (n, 128), 1)
        for a in range(NB):
            hf = hk_s[rows, 128 * a:128 * (a + 1)].astype(F32)
            hs = delayed(hk_s, rows, a, 1, gate)
            if a == 0:
                hf = jnp.where(lane == 0, hf + dc_s[rows, :], hf)
                hs = jnp.where(lane == 1, hs + dc_s[rows, :], hs)
            wrd = pltpu.pack_elementwise([hf, hs], packed_dtype=BF16).astype(U32)
            g_s[a, rows, :] = wrd
            yield _digest([wrd])

    def extract(h, r0, o, shift, z):
        def block(n, kq, b):
            x = jnp.concatenate([wp_s[(h // 2) % 2 + z, 2 * n + b, pl.ds(256 * kq + r0 + e, 8, stride=2), :]
                                 for e in range(2)], axis=0)
            if isinstance(h, int):
                return _lo(x) if h % 2 == 0 else _hi(x)
            return _hi(x << jnp.concatenate([shift] * 2, axis=0))

        terms = [_join(t) for t in _inner_terms(
            _RHS, o, lambda n, m: block(n % 2, 2 * (n // 2) + m // 2, m % 2))]
        for i, t in enumerate(terms):
            wx_w[7 * o + i, r0 // 2:r0 // 2 + 8, :] = t
        return _digest(terms)

    def phase0():
        XC = 512
        NF = CFG.get('nf', 4)
        N0 = CFG.get('n0', NF)
        N1 = CFG.get('n1', N0)
        cq = [cp(wq32.at[:, word_row(g // 2, g % 2), :], y_s.at[pl.ds(C * g, C)],
                 0 if g < N0 else 35 if g < N1 else 19 if g < NF else 1 if g < 8 else 18)
              for g in range(H)]
        cx = [cp(x_hbm.at[:, pl.ds(XC * i, XC)], x_w.at[:, pl.ds(XC * i, XC)], 22 + i) for i in range(S // XC)]
        ga = [cp(sk_hbm, sk_ref, 2), cp(ka_hbm, ka_w, 3), cp(va_hbm, va_w, 4)]
        gb = cq[8:] + gc
        gd = [cp(d_hbm, d_ref, 20), cp(hk_hbm, hk_w, 5)] + g3
        if CFG.get('merge'):
            ga, gb, gd = ga + cq[8:], [], gc + gd
        rest = cx[1:] + cq[NF:8] + ga
        if not CFG.get('jit', 1) or not CFG.get('p0', 1):
            rest = rest + gb + gd + g3b
        for c_ in [cx[0]] + cq[:NF] + rest:
            c_.start()
        zero = pl.semaphore_read(sems.at[34])
        never = _never(zero)
        due = []
        toks = []

        def pad_rows(t):
            return jnp.concatenate([t, jnp.zeros((256 - CH, 128), t.dtype)], axis=0)

        def wq_terms(j, b, gate):
            x = y_s[C * (2 * j + b):C * (2 * j + b + 1), :]
            g16 = jnp.concatenate([_after(jnp.full((8, 128), 16, U32), gate, never)] * (C // 8), axis=0)
            gm = jnp.concatenate([_after(jnp.full((8, 128), HI_MASK, U32), gate, never)] * (C // 8), axis=0)
            lo, hi = pltpu.bitcast(x << g16, F32), pltpu.bitcast(x & gm, F32)
            blocks = [pad_rows(t).T for t in (lo[:CH], hi[:CH], lo[CH:], hi[CH:])]
            if not CFG.get('q4', 1):
                return [t.astype(BF16) for t in _rhs_terms(*blocks)]
            slot = (2 * j + b) % 2
            for n, t in enumerate(blocks):
                for k in range(2):
                    wt_s[slot, 2 * n + k] = t[:, 128 * k:128 * (k + 1)]
            quarter = [[jnp.concatenate([wt_s[slot, 2 * n + k, pl.ds(e, 32, stride=4), :] for k in range(2)], axis=1)
                        for n in range(4)] for e in range(4)]
            terms = [_rhs_terms(*q) for q in quarter]
            out = []
            for i in range(7):
                ev, od = _pack(terms[0][i], terms[2][i]), _pack(terms[1][i], terms[3][i])
                rows = [w[8 * m:8 * (m + 1)] for m in range(4) for w in (ev, od)]
                out.append(pltpu.bitcast(jnp.concatenate(rows, axis=0), BF16))
            return out

        def x_terms(jp):
            top = slice(256 * jp, 256 * jp + 128)
            bot = slice(256 * jp + 128, 256 * jp + 256)
            for i in range(7):
                xs_s[256 * (NP * i + jp) + CH:256 * (NP * i + jp + 1), :] = jnp.zeros((256 - CH, 128), BF16)
            for r in range(0, CH, 32):
                lo, hi = slice(r // 2, r // 2 + 16), slice((CH + r) // 2, (CH + r) // 2 + 16)
                blocks = [x_w[lo, top], x_w[hi, top], x_w[lo, bot], x_w[hi, bot]]
                terms = [_join(t) for t in _lhs_terms(*[_split(t) for t in blocks])]
                terms[2], terms[3] = blocks[0], blocks[3]
                for i, t in enumerate(terms):
                    xs_w[128 * (NP * i + jp) + r // 2:128 * (NP * i + jp) + r // 2 + 16, :] = t
                yield 1, _digest(terms)

        def qproj(g, jp, waits):
            j, b = groups[g]
            for c_ in waits:
                c_.wait()
            if False:
                x_terms(jp)
                x_terms(jp + 1)

            XH = 128 // CFG.get('xh', 1)
            for r0 in range(0, 128, XH):
                def prod(i):
                    if r0 == 0 or True:
                        pump()
                    m = _dot(_tied(wts[g][i][r0:r0 + XH], due, never),
                             xs_s[256 * (NP * i + jp):256 * (NP * i + jp + 1), :])
                    toks.append(m[:8])
                    return m

                def emit(r, c, val):
                    w0 = 64 * b + r0 // 2
                    qc_w[2 * j + c, 2 * jp + r, w0:w0 + XH // 2, :] = _join32(val * QSCALE)

                _strassen(prod, emit)

        def column(row):
            row = jnp.concatenate([row.astype(F32), jnp.zeros((1, 512 - C), F32)], axis=1)
            return jnp.broadcast_to(row, (128, 512)).T

        consts = {}

        def make_consts():
            consts['taps'] = [column(sk_ref[j:j + 1, :]) for j in range(4)]

        def gate(x):
            back = CFG.get('gback', 6)
            return _after(x, toks[-back], never) if back else x

        def prep_u(r0, n):
            rows = slice(r0, r0 + n)
            tp = [t[rows] for t in consts['taps']]
            prev = jnp.zeros((n, 128), F32)
            for sg in range(NB):
                cols = slice(128 * sg, 128 * (sg + 1))
                ksh = ((delayed(ka_s, rows, sg, 3, gate) * tp[3] + delayed(ka_s, rows, sg, 2, gate) * tp[2])
                       + (delayed(ka_s, rows, sg, 1, gate) * tp[1] + ka_s[rows, cols].astype(F32) * tp[0]))
                kv = ksh * va_s[rows, cols].astype(F32)
                wrd = pltpu.pack_elementwise([prev, kv], packed_dtype=BF16).astype(U32)
                sa_s[C * sg + r0:C * sg + r0 + n, :] = pltpu.bitcast(wrd, F32)
                prev = kv
                yield _digest([wrd])

        def words_t(b):
            for sg in range(NB):
                r0 = C * sg + 128 * b
                if b < 3:
                    wrd = sa_s[r0:r0 + 128, :]
                else:
                    wrd = jnp.concatenate([sa_s[r0:r0 + C - 384, :], jnp.zeros((512 - C, 128), F32)], axis=0)
                wrd = gated_t(pltpu.bitcast(wrd, U32), gate)
                sb_s[S * b + 128 * sg:S * b + 128 * (sg + 1), :] = pltpu.bitcast(wrd, F32)
                yield wrd[120:]

        def all_windows(b):
            for p in range(8):
                for j in range(8):
                    yield windows(b, p // 2, p % 2, [j], gate)[0]

        def c_terms():
            for ck in range(4):
                for half in range(2):
                    for r0 in range(0, 128, 16):
                        for o in range(7):
                            def block(n, m):
                                row = 256 * ck + 128 * (n // 2) + 64 * (m // 2) + 16 * (r0 // 32)
                                col = 4 * (n % 2) + 2 * (m % 2) + half + zero * (o + 1)
                                w = jnp.concatenate([c_w[col, pl.ds(row + e, 8, stride=2), :] for e in range(2)], axis=0)
                                return _hi(w) if r0 % 32 else _lo(w)

                            terms = [_join(t) for t in _inner_terms(_LHS, o, block)]
                            for i, t in enumerate(terms):
                                cs_w[ck, 7 * o + i, half, r0 // 2:r0 // 2 + 8, :] = t
                            yield _digest(terms)

        UG = CFG.get('ug', 32)

        cu, ct, cg, cx_ = CFG.get('costs', (2, 2, 1, 1))

        def a_stream():
            make_consts()
            for b in range(4):
                for r0 in range(128 * b, min(C, 128 * (b + 1)), UG):
                    for v in prep_u(r0, UG):
                        yield cu * UG // 32, v, CFG.get('lagU', CFG.get('lagA', LAG))
                for v in words_t(b):
                    yield ct, v, CFG.get('lagT', CFG.get('lagA', LAG))
                for v in all_windows(b):
                    yield ct, v, CFG.get('lagT', CFG.get('lagA', LAG))

        def d_stream():
            dc_s[...] = column(d_ref[...].reshape(1, C))
            for r0 in range(0, C, 32):
                for v in prep_g(r0, 32, gate):
                    yield cg, v
            for r0 in range(0, 256, 16):
                for o in range(7):
                    yield cx_, extract(0, r0, o, None, zero * (o + 1))

        a_total = cu * 14 * NB + ct * 4 * (NB + 64)
        d_total = cg * 14 * NB + cx_ * 112
        streams = []
        nprod = [0]
        later = {}
        LAG = CFG.get('lag', 0)

        def pump():
            for st_ in streams:
                gen, n, p0, p1, done = st_[:5]
                want = min(n, max(0, (nprod[0] - p0 + 1) * n // (p1 - p0)))
                while st_[4] < want:
                    cost, v, *lag = next(gen)
                    later.setdefault(nprod[0] + (lag[0] if lag else LAG), []).append(v)
                    st_[4] += cost
            due.extend(later.pop(nprod[0], []))
            nprod[0] += 1

        groups = [(j, b) for j in range(H // 2) for b in range(2)]
        units = [(g, jp) for c in range(0, NP, 2) for g in range(NF) for jp in (c, c + 1)]
        units += [(g, jp) for g in range(NF, len(groups)) for jp in range(NP)]
        NU = len(units)
        wts = {}
        lead = CFG.get('lead', 4)
        ua = CFG.get('ua', 32)
        ub = 8 * NP - lead
        ux = CFG.get('ux', 5)
        ud = CFG.get('ud', 96)
        waits = {ux: cx[1:] + cq[NF:8], ua: ga, ud: gd}
        if gb:
            waits[ub] = gb
        else:
            ub = ud
        if N0 < N1:
            waits[2 * N0 - 1] = cq[N0:N1]
        if N1 < NF:
            waits[2 * N1 - 1] = cq[N1:NF]
        PU = 7 * CFG.get('xh', 1)
        xe = [PU * ux + 2] + [PU * NF * 2 * c - 1 for c in (1, 2, 3)]
        for c in range(3):
            streams.append([(v for jp in (2 * c + 2, 2 * c + 3) for v in x_terms(jp)), 14, xe[c], xe[c + 1], 0])
        sl = CFG.get('slack', 4)
        PA, PB, PE = PU * ua + sl, PU * ub + sl, PU * NU - 2 - LAG
        c_stream = ((1, v) for v in c_terms())
        nc = 4 * 2 * 8 * 7
        PD = PU * ud + sl
        streams.append([a_stream(), a_total, PA, PD + CFG.get('aext', 0), 0, CFG.get('lagA', LAG)])
        streams.append([c_stream, nc, PB, PE, 0])
        streams.append([d_stream(), d_total, PD + CFG.get('dext', CFG.get('aext', 0)), PE, 0])

        if not CFG.get('p0', 1):
            for c_ in cq[:8] + cx + ga + gb + gd:
                c_.wait()
            return
        _wait([cx[0]], 'wx0')
        list(x_terms(0))
        list(x_terms(1))
        _wait(cq[:N0], 'wq0')
        first_use = {}
        for u, (g, jp) in enumerate(units):
            first_use.setdefault(g, u)
        for u, (g, jp) in enumerate(units):
            if u in waits:
                if CFG.get('jit', 1):
                    for c_ in {ux: gb, ua: gd, ub: g3b}.get(u, []):
                        c_.start()
                _wait(waits[u], 'wu%d' % u)
            for g_, fu in first_use.items():
                if g_ not in wts and fu - (lead if g_ >= NF else 1) <= u:
                    back = CFG.get('wback', 8)
                    wts[g_] = wq_terms(*groups[g_], toks[-back] if len(toks) >= back else None)
            qproj(g, jp, [])
        assert all(st_[4] == st_[1] for st_ in streams) and not later, streams

    phase0()


    def phase1(k_s, kt_s, vt_s, vx_s, wx_s, *s_s):
        LATE = CFG.get('late', (2, 5))
        EARLY = tuple(o for o in (0, 1, 3, 4, 6, 2, 5) if o not in LATE)
        UN = CFG.get('unroll', 1)

        def heads(it, carry):
            @pl.when(it == 1)
            def _():
                for c_ in g4:
                    c_.start()

            if UN == 1:
                @pl.when(jnp.logical_and(it % 2 == 1, it < H - 1))
                def _():
                    _wait(kv_copies((it + 1) // 2), 'wkv')

                @pl.when(jnp.logical_and(jnp.logical_and(it % 2 == 0, it > 0), it < H - 2))
                def _():
                    for c_ in kv_copies(it // 2 + 1):
                        c_.start()
            else:
                @pl.when(it == 0)
                def _():
                    _wait(kv_copies(1), 'wkv')

            zero = it // H
            toks = []
            due = []
            for r in range(UN):
                head(it * UN + r, None if UN % 2 else r % 2, zero, toks, due)
            return carry + zero

        def head(h, par, zero, toks, due):
            lane8 = lax.broadcasted_iota(I32, (8, 128), 1)
            sub8 = lax.broadcasted_iota(I32, (8, 128), 0)
            lane16 = lax.broadcasted_iota(I32, (16, 128), 1)
            sub16 = lax.broadcasted_iota(I32, (16, 128), 0)
            tri = (lax.broadcasted_iota(I32, (128, 128), 0) <= lax.broadcasted_iota(I32, (128, 128), 1))
            h_next = h + 1 if isinstance(h, int) else jnp.minimum(h + 1, H - 1)
            never = _never(zero)

            def after(x, tok):
                return _after(x, tok, never)

            def tied(lhs):
                return _tied(lhs, due, never)

            def tok(back):
                return toks[-back] if (back and len(toks) >= back) else None

            def chan_mm(c, gate):
                m_b = lane8 < after(128 - 2 * sub8, gate)
                gs = [jnp.broadcast_to(g_s[a, pl.ds(c, 1), :], (8, 128)) for a in range(NB)]
                bt = [pltpu.roll(jnp.where(m_b, gs[a], gs[a - 1] if a > 0 else jnp.uint32(0)), 0, 1,
                                 stride=2, stride_axis=0) for a in range(NB)]
                b1 = pltpu.bitcast(jnp.concatenate(bt[7::-1], axis=0), BF16)
                b2 = pltpu.bitcast(jnp.concatenate(bt[15:7:-1], axis=0), BF16)
                am = pltpu.bitcast(aw_s[pl.ds(c, 64, stride=PITCH), :], BF16)
                tick('C', 48)
                z1 = _dot(tied(am), b1)
                z2 = _dot(am[:64], b2)
                return c, z1[:64], z1[64:] + z2

            def chan_post(c, zlo, zhi):
                acc = car = None
                for p in range(8):
                    z = jnp.concatenate([zlo[8 * p:8 * p + 8], zhi[8 * p:8 * p + 8]], axis=0)
                    if p == 0:
                        acc = z
                    else:
                        z = pltpu.roll(z, 16 * p, 1)
                        cz = jnp.where(lane16 < 16 * p, z, 0.0)
                        acc = acc + z
                        car = cz if car is None else car + cz
                y = (acc - car) + jnp.where(sub16 > 0, pltpu.roll(car, 1, 0), 0.0)
                later(CFG.get('ly', 0), [y])
                if CFG.get('ylate'):
                    ys.append((c, y))
                else:
                    y_s[pl.ds(c, NB, stride=PITCH), :] = pltpu.bitcast(y, U32)
                if CFG.get('pd', 0):
                    due.append(y[:8])
                    due.append(y[8:])

            chans = [h * CPH + i for i in range(CPH)]
            ys, cs = [], []

            def x_stream(hh, outers):
                n = 16 * len(outers)
                for r0 in range(0, 256, 16):
                    for o in outers:
                        n -= 1
                        free = n < CFG.get('xfree', 0) and hh is h_next
                        d = extract(hh, r0, o, shift_of(hh, tok(CFG.get('xfb', 1)) if free else None), zero * (o + 1))
                        yield None if free else d

            streams = [[x_stream(h_next, EARLY), 16 * len(EARLY), 0, 0] + list(CFG['x1']),
                       [x_stream(h, LATE), 16 * len(LATE), 0, 0] + list(CFG['x2'])]

            clock, queue = [0], []

            def later(lag, vals):
                if lag:
                    queue.append((clock[0] + lag, _digest(vals)))

            def tick(kind, cycles):
                clock[0] += cycles
                due.extend(v for t, v in queue if t <= clock[0] - cycles)
                queue[:] = [q for q in queue if q[0] > clock[0] - cycles]
                for st_ in streams:
                    gen, n, done, clk, kinds, c0, c1 = st_
                    if kind in kinds:
                        want = min(n, max(0, (clk - c0) * n // (c1 - c0)))
                        while st_[2] < want:
                            d = next(gen)
                            if d is not None:
                                if CFG.get('lx'):
                                    queue.append((clock[0] + CFG['lx'], d))
                                else:
                                    due.append(d)
                            st_[2] += 1
                        st_[3] += cycles

            def shift_of(hh, gate):
                return after(jnp.full((8, 128), (1 - hh % 2) * 16, I32).astype(U32), gate)

            def kv_chunk(ck):
                def prod(o):
                    MH = 128 // CFG.get('mh', 1)
                    out = {}
                    for r0 in range(0, 128, MH):
                        def inner(i):
                            tick('M', MH // 2)
                            lhs = jnp.concatenate([cs_s[ck, 7 * o + i, k, r0:r0 + MH, :] for k in range(2)], axis=1)
                            m = _dot(tied(lhs), wx_s[7 * o + i])
                            if i == CFG.get('ti', 3) and r0 == 0:
                                toks.append(m[:8])
                            return m

                        _strassen(inner, lambda r, n, val: out.__setitem__((r, n, r0), val))
                    return jnp.concatenate(
                        [jnp.concatenate([out[r, 0, r0], out[r, 1, r0]], axis=1)
                         for r in range(2) for r0 in range(0, 128, MH)], axis=0)

                def emit(R, N, val):
                    if N == 0:
                        rows = slice(512 * ck + 256 * R, 512 * ck + 256 * (R + 1))
                        outs = []
                        if 2 * ck + R < NP - 1:
                            blocks = [val[:128, :128], val[:128, 128:], val[128:, :128], val[128:, 128:]]
                            for i in (0, 1, 4, 5, 6):
                                outs.append(_join32(_term(_LHS, i, blocks.__getitem__)))
                                kt_w[i, 2 * ck + R] = outs[-1]
                        for n in range(2):
                            w = _join32(val[:, 128 * n:128 * (n + 1)])
                            k_w[n, 256 * ck + 128 * R:256 * ck + 128 * (R + 1), :] = w
                            outs += [w[:64], w[64:]]
                        later(CFG.get('lk', 0), outs)
                    else:
                        blocks = [val[128 * r:128 * (r + 1), 128 * n:128 * (n + 1)].T
                                  for n in range(2) for r in range(2)]
                        outs = [v.astype(BF16) for v in blocks]
                        for m, v in enumerate(outs):
                            vt_s[4 * ck + 2 * R + m % 2, 128 * (m // 2):128 * (m // 2 + 1), :] = v
                        if 2 * ck + R < NP - 1:
                            for i in (0, 1, 4, 5, 6):
                                outs.append(_term(_LHS, i, blocks.__getitem__).astype(BF16))
                                vx_s[i, 2 * ck + R] = outs[-1]
                        later(CFG.get('lv', 0), outs)

                return _strassen_steps(prod, emit)

            kv = [kv_chunk(ck) for ck in range(4)]

            def k_rows(r0, r1):
                return jnp.concatenate([k_s[0, r0:r1, :], k_s[1, r0:r1, :]], axis=1)

            def q_cols(r0, r1):
                return jnp.concatenate([qc_s[h, t] for t in range(r0 // 128, r1 // 128)], axis=1)

            mx, pr = {}, {}

            def s_at(u, r0):
                t = u // 4
                first = [v for v in range(u) if (v // 4) % 2 == t % 2]
                return s_s[t % 2], 128 * sum(v + 1 for v in first) + r0

            def qk(jq):
                run = [None, None]

                def put(n, r0, val):
                    buf, row = s_at(2 * jq + n, r0)
                    buf[row:row + val.shape[0], :] = val
                    vs = [val[r:r + 8] for r in range(0, val.shape[0], 8)]
                    def fold(op, xs, ways):
                        accs = xs[:ways]
                        for k, x in enumerate(xs[ways:]):
                            accs[k % ways] = op(accs[k % ways], x)
                        while len(accs) > 1:
                            accs = [op(a, b) for a, b in zip(accs[::2], accs[1::2])]
                        return accs[0]

                    m = fold(jnp.maximum, list(vs), CFG.get('mw', 1))
                    if run[n] is not None:
                        m = jnp.maximum(m, run[n][0])
                    if CFG.get('lsep'):
                        run[n] = (m, None)
                        return
                    l = fold(jnp.add, [jnp.exp2(v - m) for v in vs], CFG.get('lw', 1))
                    if run[n] is not None:
                        l = l + run[n][1] * jnp.exp2(run[n][0] - m)
                    run[n] = (m, l)

                if jq > 0:
                    raw = [qc_w[h, 2 * jq + n % 2, 64 * (n // 2):64 * (n // 2 + 1), :] for n in range(4)]
                    full = [_split(w) for w in raw]
                    qt = [pltpu.bitcast(raw[_RHS[i][0]] if len(_RHS[i]) == 1
                                        else _join(_term(_RHS, i, full.__getitem__)), BF16) for i in range(7)]
                QH = 128 // CFG.get('qh', 1)

                def diag():
                    q0 = 256 * jq
                    for n in range(2):
                        tick('Q', 64 * (n + 1))
                        sd = _dot(tied(k_rows(q0, q0 + 128 * (n + 1))), qc_s[h, 2 * jq + n])
                        sd = jnp.concatenate([sd[:128 * n], jnp.where(tri, sd[128 * n:], NEG)], axis=0) if n else (
                            jnp.where(tri, sd, NEG))
                        for r0 in range(0, 128 * (n + 1), QH):
                            put(n, q0 + r0, sd[r0:r0 + QH])
                    toks.append(sd[:8])

                if CFG.get('dfirst'):
                    diag()
                for jp in range(jq):
                    for r0 in range(0, 128, QH):
                        def prod(i):
                            tick('Q', QH // 4)
                            if i == 2:
                                lhs = k_s[0, 256 * jp + r0:256 * jp + r0 + QH, :]
                            elif i == 3:
                                lhs = k_s[1, 256 * jp + 128 + r0:256 * jp + 128 + r0 + QH, :]
                            else:
                                lhs = kt_s[i, jp, r0:r0 + QH, :]
                            m = _dot(tied(lhs), qt[i])
                            if i == 3 and r0 == 0:
                                toks.append(m[:8])
                            return m

                        _strassen(prod, lambda r, n, val: put(n, 256 * jp + 128 * r + r0, val))
                if not CFG.get('dfirst'):
                    diag()
                for n in range(2):
                    m, l = run[n]
                    top = jnp.max(m, axis=0, keepdims=True)
                    if CFG.get('lsep'):
                        tops[2 * jq + n] = top
                        continue
                    tot = jnp.sum(l * jnp.exp2(m - top), axis=0, keepdims=True)
                    mx[2 * jq + n] = top + jnp.log2(tot)

            tops = {}

            def denom(u, deadline):
                buf, row = s_at(u, 0)
                x = buf[pl.ds(pl.multiple_of(row + 16 * zero, 8), 128 * (u + 1)), :]
                e = jnp.exp2(x - tops[u])
                ways = CFG.get('dw', 1)
                accs = [e[8 * k:8 * (k + 1)] for k in range(ways)]
                for k in range(ways, e.shape[0] // 8):
                    accs[k % ways] = accs[k % ways] + e[8 * k:8 * (k + 1)]
                while len(accs) > 1:
                    accs = [a + b for a, b in zip(accs[::2], accs[1::2])]
                tot = jnp.sum(accs[0], axis=0, keepdims=True)
                mx[u] = tops[u] + jnp.log2(tot)
                if deadline:
                    due.append(tot)

            def probs(u, r0):
                buf, row = s_at(u, r0)
                x = jnp.concatenate([buf[pl.ds(row + e + zero, 8, stride=4), :] for e in (0, 2)], axis=0)
                return jnp.exp2(x - mx[u])

            def softmax(jq, jps, deadline):
                for u in (2 * jq, 2 * jq + 1):
                    if u not in mx:
                        denom(u, False)
                starts = [r + e for r in range(0, 256, 32) for e in range(2)]
                for jp in jps:
                    if jp == jq:
                        out = [jnp.concatenate([_join(probs(2 * jq + n, 256 * jq + r)) for r in starts[:8 * (n + 1)]],
                                               axis=0) for n in range(2)]
                    else:
                        parts = []
                        for r in starts[:8]:
                            blocks = [probs(2 * jq + m % 2, 256 * jp + 128 * (m // 2) + r) for m in range(4)]
                            parts.append([_join(t) for t in _rhs_terms(*blocks)])
                        out = [jnp.concatenate([p[i] for p in parts], axis=0) for i in range(7)]
                    pr[jq, jp] = out
                    if deadline:
                        d = _digest([out[0]]) ^ _digest([out[1]]) if jp == jq else _digest(out)
                        if CFG.get('le'):
                            queue.append((clock[0] + CFG['le'], d))
                        else:
                            due.append(d)

            def pv(jq):
                softmax(jq, [jp for jp in range(jq + 1) if (jq, jp) not in pr], False)
                diag = pr.pop((jq, jq))
                ps = [pr.pop((jq, jp)) for jp in range(jq)]
                base = []
                for n in range(2):
                    tick('P', 64 * (n + 1))
                    vt = jnp.concatenate([vt_s[2 * jq + i] for i in range(n + 1)], axis=1)
                    base.append(_dot(tied(vt), pltpu.bitcast(diag[n], BF16)))

                def emit(r, n, val):
                    val = base[n][128 * r:128 * (r + 1)] if val is None else val + base[n][128 * r:128 * (r + 1)]
                    qc_s[h, 2 * jq + n, 128 * r:128 * (r + 1), :] = val.astype(BF16)

                def prod(i):
                    tick('P', 32 * jq)
                    if i == 2:
                        lhs = [vt_s[2 * jp, 0:128, :] for jp in range(jq)]
                    elif i == 3:
                        lhs = [vt_s[2 * jp + 1, 128:256, :] for jp in range(jq)]
                    else:
                        lhs = [vx_s[i, jp] for jp in range(jq)]
                    rhs = pltpu.bitcast(jnp.concatenate([p[i] for p in ps], axis=0), BF16)
                    return _dot(tied(jnp.concatenate(lhs, axis=1)), rhs)

                if jq:
                    _strassen(prod, emit)
                else:
                    for r in range(2):
                        for n in range(2):
                            emit(r, n, None)

            CG, XG = CFG.get('cg', 0), CFG.get('xg', 0)
            pend = []
            def run_step(st_):
                kind, arg = st_[0], st_[1:]
                if kind == 'L':
                    for x in arg:
                        denom(int(x, 16), True)
                    return
                if kind == 'E':
                    jq = int(arg[0])
                    softmax(jq, [int(x) for x in arg[1:]] if arg[1:] else range(jq + 1), True)
                    return
                old = list(pend)
                pend.clear()
                if kind == 'C':
                    for _ in range(int(arg)):
                        pend.append(chan_mm(chans.pop(0), tok(CG)))
                elif kind == 'M':
                    for o in arg[1:]:
                        kv[int(arg[0])](int(o))
                elif kind == 'Q':
                    for x in arg:
                        qk(int(x))
                elif kind == 'P':
                    for x in arg:
                        pv(int(x))
                for args in old:
                    chan_post(*args)

            for seg in [g for g in CFG['sched'].split('|') if g.strip()]:
                if CFG.get('scopes') and '|' in CFG['sched']:
                    with jax.named_scope('s_' + seg.split()[0]):
                        for st_ in seg.split():
                            run_step(st_)
                else:
                    for st_ in seg.split():
                        run_step(st_)
            for c, y in ys:
                y_s[pl.ds(c, NB, stride=PITCH), :] = pltpu.bitcast(y, U32)
            for t, d0, n, v in cs:
                qc_s[h, t, d0:d0 + n, :] = v
            assert all(st_[1] == st_[2] for st_ in streams), [st_[1:] for st_ in streams]
            assert CFG.get('noassert') or not chans and not pend and (not due or CFG.get('pd')) and not pr

        if CFG.get('p1', 1):
            return lax.fori_loop(0, H // UN, heads, 0)
        else:
            _wait(g3b, 'wg3b')
            if CFG.get('p2', 1):
                for c_ in g4:
                    c_.start()

            def keep(h, carry):
                r = pl.multiple_of(h * 16, 16)
                t = (qc_s[h, h, 0:16, :].astype(F32) + cs_s[h % 4, h, h % 2, 0:16, :].astype(F32)
                     + pltpu.bitcast(aw_s[pl.ds(r, 16), :] + g_s[h, pl.ds(r, 16), :], F32)
                     + wx_s[h, pl.ds(r, 16), :].astype(F32))
                y_s[pl.ds(r, 16), :] = pltpu.bitcast(t, U32)
                return carry + h // H
            return lax.fori_loop(0, H, keep, 0)

    zero_end = phase1(k_s, kt_s, vt_s, vx_s, wx_s, sa_s, sb_s)

    def phase2():
        if CFG.get('p2', 1) or CFG.get('p1', 1):
            _wait(g4, 'wg4')
        HH = H // 2

        def wo_block(rh, kh):
            rows = [(C * (H * b + h) + CH * rh) // 2 for h in range(HH * kh, HH * (kh + 1)) for b in range(2)]
            return jnp.concatenate([xs_w[r:r + CH // 2, :] for r in rows], axis=1)

        raw = [wo_block(0, 0), wo_block(1, 0), wo_block(0, 1), wo_block(1, 1)]
        full = [_split(w) for w in raw]
        wt = [pltpu.bitcast(raw[_RHS[i][0]] if len(_RHS[i]) == 1 else _join(_term(_RHS, i, full.__getitem__)), BF16)
              for i in range(7)]
        outs = []
        due, late = [], []
        DL = CFG.get('dl', 3)
        never = _never(zero_end)

        def put(t, b, z, opaque=False):
            z = z.T
            r0 = pl.multiple_of(zero_end * 16 + 128 * t, 16) if opaque else 128 * t
            out_s[pl.ds(r0, 128), 128 * b:128 * (b + 1)] = z.astype(BF16)
            late.append(z[120:])

        for jp in range(CFG.get('np2', NP) if CFG.get('p2', 1) else 0):
            def ctx_block(r, kh):
                return jnp.concatenate([qc_w[h, 2 * jp + r] for h in range(HH * kh, HH * (kh + 1))], axis=0)

            craw = [ctx_block(0, 0), ctx_block(0, 1), ctx_block(1, 0), ctx_block(1, 1)]
            cfull = [_split(w) for w in craw]
            ct = [pltpu.bitcast(craw[_LHS[i][0]] if len(_LHS[i]) == 1
                                else _join(_term(_LHS, i, cfull.__getitem__)), BF16) for i in range(7)]
            za = {}
            prev_late = list(late)
            late.clear()
            for r in range(2):
                t = 2 * jp + r
                za[r] = (pltpu.bitcast(y_s[t * PITCH:t * PITCH + C, :], F32)
                         * x_s[:, 128 * t:128 * (t + 1)].astype(F32))
                for b in range(3):
                    put(t, b, za[r][128 * b:128 * (b + 1)], opaque=(r == 0 and b == 0 and jp > 0))
            a_late = list(late)
            late.clear()
            res = {}
            count = [0]

            def prod(i):
                if count[0] == DL:
                    due.extend(prev_late)
                if count[0] == 6:
                    due.extend(a_late)
                count[0] += 1
                return _dot(_tied(wt[i], due, never), ct[i])

            _strassen(prod, lambda r, c, val: res.__setitem__((r, c), val), order=CFG.get('oo', (1, 4, 3, 2, 0, 5, 6)))
            for r in CFG.get('ro', (1, 0)):
                z = jnp.concatenate([za[r][384:], res[(r, 0)], res[(r, 1)]], axis=0)
                for b in CFG.get('bo', (3, 2, 1, 0)):
                    put(2 * jp + r, 3 + b, z[128 * b:128 * (b + 1)])
            rows = pl.ds(256 * jp, 256)
            oc = cp(out_s.at[rows], o_hbm.at[rows], 26 + jp)
            oc.start()
            outs.append(oc)
        if not CFG.get('p2', 1):
            def keep(h, carry):
                r = pl.multiple_of(h * 16, 16)
                out_s[pl.ds(r, 16), 0:128] = pltpu.bitcast(y_s[pl.ds(r, 16), :], F32).astype(BF16) + qc_s[h, h, 0:16, :]
                return carry
            lax.fori_loop(0, H, keep, 0)
            oc = cp(out_s.at[pl.ds(0, 256)], o_hbm.at[pl.ds(0, 256)], 26)
            oc.start()
            outs.append(oc)
        _wait(outs, 'wout')

    phase2()


def _tiles(w):
    rows = w.shape[0]
    return w.reshape(rows, 2, 8, 2, 128).transpose(0, 1, 3, 2, 4).reshape(rows, 32, 128)


@jax.jit
def pallas_concat_heads__ssm_conv_h3__compressed_kv_cla__prompt_kernel(
    A_q: jax.Array,
    A_k: jax.Array,
    A_v: jax.Array,
    A_shift_k: jax.Array,
    A_ssm_k: jax.Array,
    A_ssm_D: jax.Array,
    B_x: jax.Array,
    B_c_kv: jax.Array,
    B_w_q: jax.Array,
    B_w_uk: jax.Array,
    B_w_uv: jax.Array,
    B_w_o: jax.Array,
):
    hbm = pl.BlockSpec(memory_space=pltpu.HBM)
    out = pl.pallas_call(
        _kernel,
        in_specs=[hbm] * 12,
        out_specs=hbm,
        out_shape=jax.ShapeDtypeStruct((S, 2 * C), BF16),
        scratch_shapes=[
            pltpu.VMEM((8, S // 2, 128), U32),
            pltpu.VMEM((4, 49, 2, 64, 128), U32),
            pltpu.VMEM((2, 4, DC, 128), U32),
            pltpu.VMEM((H, NB, D // 2, 128), U32),
            pltpu.VMEM((64 * PITCH, 128), U32),
            pltpu.VMEM((NB, C, 128), U32),
            pltpu.VMEM((NB * PITCH, 128), U32),
            pltpu.VMEM((CH, S), U32),
            pltpu.VMEM((512, 128), F32),
            pltpu.VMEM((2, S // 2, 128), U32),
            pltpu.VMEM((7, NP, 64, 128), U32),
            pltpu.VMEM((NB, D // 2, 128), U32),
            pltpu.VMEM((7, NP, 64, 128), U32),
            pltpu.VMEM((49, DC // 8, 128), U32),
            pltpu.VMEM((4 * C * 4, 128), F32),
            pltpu.VMEM((84 * 128, 128), F32),
            pltpu.VMEM((CH, S), U32),
            pltpu.VMEM((7 * NP * 128, 128), U32),
            pltpu.VMEM((CH, S), U32),
            pltpu.VMEM((CH, S), U32),
            pltpu.VMEM((2, 8, 128, 128), F32),
            pltpu.VMEM((S, 2 * C), BF16),
            pltpu.VMEM((4, C), BF16),
            pltpu.VMEM((C,), BF16),
            pltpu.SemaphoreType.DMA((36,)),
        ],
        compiler_params=pltpu.CompilerParams(
            vmem_limit_bytes=127 * 2 ** 20, disable_semaphore_checks=bool(CFG.get('nsc')),
            disable_bounds_checks=bool(CFG.get('nbc'))),
    )(
        A_q[0].T, A_k[0].T, A_v[0].T, A_shift_k.T, A_ssm_k, A_ssm_D, B_x[0].T, B_c_kv[0],
        _tiles(B_w_q), _tiles(B_w_uk), _tiles(B_w_uv),
        jnp.swapaxes(B_w_o, 1, 2).reshape(H * C, D),
    )
    return out.reshape(1, S, 2 * C)
```

```python
import math

import jax
import jax.numpy as jnp
from jax import lax
import jax.experimental.pallas as pl
import jax.experimental.pallas.tpu as pltpu

F32 = jnp.float32
BF16 = jnp.bfloat16
U32 = jnp.uint32
I32 = jnp.int32

S = 2048
C = 448
H = 16
D = 256
DC = 1024
NB = S // 128
NP = NB // 2
CH = C // 2
PITCH = 520
CPH = C // H
LOG2E = math.log2(math.e)
QSCALE = (D ** -0.5) * LOG2E
NEG = -1e9 * LOG2E
HI_MASK = 0xFFFF0000

HEAD_STEPS = ("M001 C2 M034 C2 M06 M101 C2 Q01 M134 C2 M16 M201 C2 Q23 M234 C2 M26 M301 C2 E0 E1 E2 Q45 M334 C2 "
              "M36 E3 M02 C2 Q67 M05 C2 M12 C2 E4 M15 C2 E5012 M22 C2 E5345 M25 C2 M32 E6012 M35 E63456 P01234567")


def _dot(a, b):
    return jnp.dot(a, b, preferred_element_type=F32)


def _lo(x):
    return pltpu.bitcast(x << 16, F32)


def _hi(x):
    return pltpu.bitcast(x & jnp.uint32(HI_MASK), F32)


def _pack(even, odd):
    return pltpu.pack_elementwise([even, odd], packed_dtype=BF16).astype(U32)


def _split(words):
    return jnp.concatenate([_lo(words), _hi(words)], axis=0)


def _join(x):
    n = x.shape[0] // 2
    return _pack(x[:n], x[n:])


def _join32(x):
    return jnp.concatenate([_pack(x[m:m + 16], x[m + 16:m + 32]) for m in range(0, x.shape[0], 32)], axis=0)


_LHS = ((0, 1, 3), (2, 1, 3), (0,), (3,), (0, 1, 1), (2, -1, 0), (1, -1, 3))
_RHS = ((0, 1, 3), (0,), (1, -1, 3), (2, -1, 0), (3,), (0, 1, 1), (2, 1, 3))
_SUMS = (0, 1, 4, 5, 6)


def _term(table, i, block):
    spec = table[i]
    if len(spec) == 1:
        return block(spec[0])
    return block(spec[0]) + block(spec[2]) if spec[1] > 0 else block(spec[0]) - block(spec[2])


def _terms(table, blocks):
    return [_term(table, i, blocks.__getitem__) for i in range(7)]


def _word_terms(table, words):
    full = [_split(w) for w in words]
    return [pltpu.bitcast(words[table[i][0]] if len(table[i]) == 1
                          else _join(_term(table, i, full.__getitem__)), BF16) for i in range(7)]


def _inner_terms(table, o, block):
    return _terms(table, [_term(table, o, lambda n: block(n, m)) for m in range(4)])


def _strassen_steps(prod, emit):
    uses = {(0, 0): {0: 1, 3: 1, 4: -1, 6: 1}, (0, 1): {2: 1, 4: 1},
            (1, 0): {1: 1, 3: 1}, (1, 1): {0: 1, 1: -1, 2: 1, 5: 1}}
    acc = {}
    neg = {}

    def step(i):
        m = prod(i)
        for key, terms in uses.items():
            if i not in terms:
                continue
            sign = terms.pop(i)
            if key not in acc:
                acc[key] = m
                neg[key] = sign < 0
            elif neg[key]:
                assert sign > 0
                acc[key] = m - acc[key]
                neg[key] = False
            else:
                acc[key] = acc[key] + m if sign > 0 else acc[key] - m
            if not terms:
                emit(key[0], key[1], acc.pop(key))

    return step


def _strassen(prod, emit, order=(0, 1, 3, 2, 4, 5, 6)):
    step = _strassen_steps(prod, emit)
    for i in order:
        step(i)


def _never(zero):
    return lax.broadcasted_iota(I32, (8, 128), 1) < zero


def _after(x, tok, never):
    if tok is None:
        return x
    return jnp.where(never, pltpu.bitcast(tok, x.dtype), x)


def _tied(lhs, due, never):
    if not due:
        return lhs
    t = None
    for d in due:
        d = pltpu.bitcast(jnp.broadcast_to(d, (8, 128)), U32)
        t = d if t is None else t ^ d
    due.clear()
    x = pltpu.bitcast(_after(pltpu.bitcast(lhs[:16, :128], U32), t, never), BF16)
    if lhs.shape[1] > 128:
        x = jnp.concatenate([x, lhs[:16, 128:]], axis=1)
    return jnp.concatenate([x, lhs[16:]], axis=0)


def _digest(words):
    acc = None
    for r in range(words[0].shape[0] // 8):
        for w in words:
            w = w[8 * r:8 * (r + 1)]
            acc = w if acc is None else acc ^ w
    return acc


def _fold(op, xs):
    accs = list(xs[:2])
    for k, x in enumerate(xs[2:]):
        accs[k % 2] = op(accs[k % 2], x)
    return op(accs[0], accs[1])


class _Packed:
    def __init__(self, ref):
        self.ref = ref

    def _index(self, idx):
        idx = idx if isinstance(idx, tuple) else (idx,)
        axis = len(self.ref.shape) - 2
        if len(idx) <= axis:
            return idx + (slice(None),) * (axis + 2 - len(idx))
        r = idx[axis]
        r = slice(None if r.start is None else r.start // 2, None if r.stop is None else r.stop // 2)
        return idx[:axis] + (r,) + idx[axis + 1:]

    def __getitem__(self, idx):
        return pltpu.bitcast(self.ref[self._index(idx)], BF16)

    def __setitem__(self, idx, val):
        self.ref[self._index(idx)] = pltpu.bitcast(val, U32)


def _start(copies):
    for c_ in copies:
        c_.start()


def _wait(copies):
    for c_ in copies:
        c_.wait()


def _kernel(qa_hbm, ka_hbm, va_hbm, sk_hbm, hk_hbm, d_hbm, x_hbm, c_hbm, wq_hbm, wk_hbm, wv_hbm, wo_hbm,
            o_hbm,
            c_w, cs_w, wp_s, qc_w, aw_s, g_s, y_s, hk_w, dc_s, k_w, kt_w, vt_w, vx_w, wx_w, sa_s, sb_s,
            x_w, xs_w, ka_w, va_w, wt_s, out_s, sk_ref, d_ref, sems):
    def cp(src, dst, i):
        return pltpu.make_async_copy(src, dst, sems.at[i])

    cs_s, qc_s, k_s, kt_s, vt_s, vx_s, wx_s, xs_s, x_s, ka_s, va_s, hk_s = (
        _Packed(r) for r in (cs_w, qc_w, k_w, kt_w, vt_w, vx_w, wx_w, xs_w, x_w, ka_w, va_w, hk_w))
    qa_hbm, ka_hbm, va_hbm, hk_hbm, x_hbm, c_hbm, wo_hbm, wq_hbm, wk_hbm, wv_hbm = (
        r.bitcast(U32)
        for r in (qa_hbm, ka_hbm, va_hbm, hk_hbm, x_hbm, c_hbm, wo_hbm, wq_hbm, wk_hbm, wv_hbm))

    def word_row(pair, b):
        return 8 * (pair // 4) + 4 * b + pair % 4

    def kv_copies(pair):
        return [cp(w.at[:, word_row(pair, b), :], wp_s.at[pair % 2, 2 * n + b], 16 + pair % 2)
                for n, w in enumerate((wk_hbm, wv_hbm)) for b in range(2)]

    late_copies = [cp(qa_hbm, x_w, 21)] + [
        cp(wo_hbm.at[:, pl.ds(128 * b, 128)], xs_w.at[pl.ds(H * CH * b, H * CH)], 6 + b) for b in range(2)]

    def extract(h, r0, o, shift, z):
        def block(n, kq, b):
            x = jnp.concatenate([wp_s[(h // 2) % 2 + z, 2 * n + b, pl.ds(256 * kq + r0 + e, 8, stride=2), :]
                                 for e in range(2)], axis=0)
            if isinstance(h, int):
                return _lo(x) if h % 2 == 0 else _hi(x)
            return _hi(x << jnp.concatenate([shift] * 2, axis=0))

        terms = [_join(t) for t in _inner_terms(
            _RHS, o, lambda n, m: block(n % 2, 2 * (n // 2) + m // 2, m % 2))]
        for i, t in enumerate(terms):
            wx_w[7 * o + i, r0 // 2:r0 // 2 + 8, :] = t
        return _digest(terms)

    def phase0():
        N0, NF = 3, 8
        UX, UA, UB, UD = 13, 30, 60, 96
        LAG, LAG_T, BACK, SLACK = 8, 3, 8, 8
        cq = [cp(wq_hbm.at[:, word_row(g // 2, g % 2), :], y_s.at[pl.ds(C * g, C)],
                 0 if g < N0 else 19 if g < NF else 18) for g in range(H)]
        cx = [cp(x_hbm.at[:, pl.ds(512 * i, 512)], x_w.at[:, pl.ds(512 * i, 512)], 22 + i) for i in range(4)]
        ga = [cp(sk_hbm, sk_ref, 2), cp(ka_hbm, ka_w, 3), cp(va_hbm, va_w, 4)]
        gb = cq[NF:] + [cp(c_hbm.at[:, pl.ds(128 * b, 128)], c_w.at[b], 8 + b) for b in range(8)]
        gd = [cp(d_hbm, d_ref, 20), cp(hk_hbm, hk_w, 5)] + kv_copies(0)
        _start(cx[:1] + cq[:NF] + cx[1:] + ga)
        zero = pl.semaphore_read(sems.at[34])
        never = _never(zero)
        due = []
        toks = []

        def gate(x):
            return _after(x, toks[-BACK], never)

        def w_terms(j, b):
            tok = toks[-BACK] if len(toks) >= BACK else None
            x = y_s[C * (2 * j + b):C * (2 * j + b + 1), :]
            g16 = jnp.concatenate([_after(jnp.full((8, 128), 16, U32), tok, never)] * (C // 8), axis=0)
            gm = jnp.concatenate([_after(jnp.full((8, 128), HI_MASK, U32), tok, never)] * (C // 8), axis=0)
            lo, hi = pltpu.bitcast(x << g16, F32), pltpu.bitcast(x & gm, F32)
            pad = jnp.zeros((256 - CH, 128), F32)
            blocks = [jnp.concatenate([t, pad], axis=0).T for t in (lo[:CH], hi[:CH], lo[CH:], hi[CH:])]
            for n, t in enumerate(blocks):
                for k in range(2):
                    wt_s[b, 2 * n + k] = t[:, 128 * k:128 * (k + 1)]
            quarter = [[jnp.concatenate([wt_s[b, 2 * n + k, pl.ds(e, 32, stride=4), :] for k in range(2)], axis=1)
                        for n in range(4)] for e in range(4)]
            terms = [_terms(_RHS, q) for q in quarter]
            out = []
            for i in range(7):
                ev, od = _pack(terms[0][i], terms[2][i]), _pack(terms[1][i], terms[3][i])
                rows = [w[8 * m:8 * (m + 1)] for m in range(4) for w in (ev, od)]
                out.append(pltpu.bitcast(jnp.concatenate(rows, axis=0), BF16))
            return out

        def x_terms(jp):
            top = slice(256 * jp, 256 * jp + 128)
            bot = slice(256 * jp + 128, 256 * jp + 256)
            for i in range(7):
                xs_s[256 * (NP * i + jp) + CH:256 * (NP * i + jp + 1), :] = jnp.zeros((256 - CH, 128), BF16)
            for r in range(0, CH // 2, 16):
                lo, hi = slice(r, r + 16), slice(CH // 2 + r, CH // 2 + r + 16)
                blocks = [x_w[lo, top], x_w[hi, top], x_w[lo, bot], x_w[hi, bot]]
                terms = [_join(t) for t in _terms(_LHS, [_split(t) for t in blocks])]
                terms[2], terms[3] = blocks[0], blocks[3]
                for i, t in enumerate(terms):
                    xs_w[128 * (NP * i + jp) + r:128 * (NP * i + jp) + r + 16, :] = t
                yield 1, _digest(terms), LAG

        def column(row):
            row = jnp.concatenate([row.astype(F32), jnp.zeros((1, 512 - C), F32)], axis=1)
            return jnp.broadcast_to(row, (128, 512)).T

        def delayed(ref, rows, sg, n):
            cur = pltpu.bitcast(ref[rows, 128 * sg:128 * (sg + 1)], U32)
            lane = jnp.concatenate([gate(lax.broadcasted_iota(I32, (8, 128), 1))] * (cur.shape[0] // 8), axis=0)
            prev = pltpu.bitcast(ref[rows, 128 * (sg - 1):128 * sg], U32) if sg > 0 else jnp.uint32(0)
            x = pltpu.roll(jnp.where(lane < 128 - n, cur, prev), n, 1)
            return pltpu.bitcast(x, BF16).astype(F32)

        def transposed(x):
            return jnp.concatenate([gate(x[:8]), x[8:]], axis=0).T

        def conv_inputs():
            taps = [column(sk_ref[j:j + 1, :]) for j in range(4)]
            for b in range(4):
                for r0 in range(128 * b, min(C, 128 * (b + 1)), 32):
                    rows = slice(r0, r0 + 32)
                    tp = [t[rows] for t in taps]
                    prev = jnp.zeros((32, 128), F32)
                    for sg in range(NB):
                        cols = slice(128 * sg, 128 * (sg + 1))
                        ksh = ((delayed(ka_s, rows, sg, 3) * tp[3] + delayed(ka_s, rows, sg, 2) * tp[2])
                               + (delayed(ka_s, rows, sg, 1) * tp[1] + ka_s[rows, cols].astype(F32) * tp[0]))
                        kv = ksh * va_s[rows, cols].astype(F32)
                        wrd = _pack(prev, kv)
                        sa_s[C * sg + r0:C * sg + r0 + 32, :] = pltpu.bitcast(wrd, F32)
                        prev = kv
                        yield 2, _digest([wrd]), LAG
                for sg in range(NB):
                    r0 = C * sg + 128 * b
                    if b < 3:
                        wrd = sa_s[r0:r0 + 128, :]
                    else:
                        wrd = jnp.concatenate([sa_s[r0:r0 + C - 384, :], jnp.zeros((512 - C, 128), F32)], axis=0)
                    wrd = transposed(pltpu.bitcast(wrd, U32))
                    sb_s[S * b + 128 * sg:S * b + 128 * (sg + 1), :] = pltpu.bitcast(wrd, F32)
                    yield 2, wrd[120:], LAG_T
                for p in range(8):
                    for j in range(8):
                        parts = [jnp.zeros((16, 128), U32) if sg < 0 else
                                 pltpu.bitcast(sb_s[pl.ds(S * b + 128 * sg + 16 * p, 16), :], U32)
                                 for sg in range(2 * j - 6, 2 * j + 2)]
                        plane = 32 * (j // 4) + 4 * p + j % 4
                        win = transposed(jnp.concatenate(parts, axis=0))
                        aw_s[pl.ds(plane * PITCH + 128 * b, 128), :] = win
                        yield 2, win[120:], LAG_T

        def conv_filter_and_first_head():
            dc_s[...] = column(d_ref[...].reshape(1, C))
            lane = lax.broadcasted_iota(I32, (32, 128), 1)
            for r0 in range(0, C, 32):
                rows = slice(r0, r0 + 32)
                for a in range(NB):
                    hf = hk_s[rows, 128 * a:128 * (a + 1)].astype(F32)
                    hs = delayed(hk_s, rows, a, 1)
                    if a == 0:
                        hf = jnp.where(lane == 0, hf + dc_s[rows, :], hf)
                        hs = jnp.where(lane == 1, hs + dc_s[rows, :], hs)
                    wrd = _pack(hf, hs)
                    g_s[a, rows, :] = wrd
                    yield 1, _digest([wrd]), LAG
            for r0 in range(0, 256, 16):
                for o in range(7):
                    yield 1, extract(0, r0, o, None, zero * (o + 1)), LAG

        def c_terms():
            for ck in range(4):
                for half in range(2):
                    for r0 in range(0, 128, 16):
                        for o in range(7):
                            def block(n, m):
                                row = 256 * ck + 128 * (n // 2) + 64 * (m // 2) + 16 * (r0 // 32)
                                col = 4 * (n % 2) + 2 * (m % 2) + half + zero * (o + 1)
                                w = jnp.concatenate([c_w[col, pl.ds(row + e, 8, stride=2), :] for e in range(2)],
                                                    axis=0)
                                return _hi(w) if r0 % 32 else _lo(w)

                            terms = [_join(t) for t in _inner_terms(_LHS, o, block)]
                            for i, t in enumerate(terms):
                                cs_w[ck, 7 * o + i, half, r0 // 2:r0 // 2 + 8, :] = t
                            yield 1, _digest(terms), LAG

        units = [(g, jp) for c in range(0, NP, 2) for g in range(NF) for jp in (c, c + 1)]
        units += [(g, jp) for g in range(NF, H) for jp in range(NP)]
        last = 7 * len(units) - 2 - LAG
        xe = [7 * UX + 2] + [14 * NF * c - 1 for c in (1, 2, 3)]
        streams = [[(v for jp in (2 * c + 2, 2 * c + 3) for v in x_terms(jp)), 14, xe[c], xe[c + 1], 0]
                   for c in range(3)]
        streams += [[conv_inputs(), 2 * (14 * NB + 4 * (NB + 64)), 7 * UA + SLACK, 7 * UD + SLACK, 0],
                    [c_terms(), 448, 7 * UB + SLACK, last, 0],
                    [conv_filter_and_first_head(), 14 * NB + 112, 7 * UD + SLACK, last, 0]]
        later = {}

        def pump():
            n = len(toks)
            for st in streams:
                want = min(st[1], max(0, (n - st[2] + 1) * st[1] // (st[3] - st[2])))
                while st[4] < want:
                    cost, v, lag = next(st[0])
                    later.setdefault(n + lag, []).append(v)
                    st[4] += cost
            due.extend(later.pop(n, []))

        starts = {UX: gb, UA: gd, UB: kv_copies(1)}
        waits = {2 * N0 - 1: cq[N0:NF], UX: cx[1:], UA: ga, UB: gb, UD: gd}
        _wait(cx[:1])
        list(x_terms(0))
        list(x_terms(1))
        _wait(cq[:N0])
        wts = {}
        for u, (g, jp) in enumerate(units):
            _start(starts.get(u, []))
            _wait(waits.get(u, []))
            for g_ in range(H):
                if g_ not in wts and units.index((g_, 0)) - (4 if g_ >= NF else 1) <= u:
                    wts[g_] = w_terms(g_ // 2, g_ % 2)

            def prod(i):
                pump()
                m = _dot(_tied(wts[g][i], due, never), xs_s[256 * (NP * i + jp):256 * (NP * i + jp + 1), :])
                toks.append(m[:8])
                return m

            def emit(r, c, val):
                qc_w[2 * (g // 2) + c, 2 * jp + r, 64 * (g % 2):64 * (g % 2 + 1), :] = _join32(val * QSCALE)

            _strassen(prod, emit)
        assert all(st[4] == st[1] for st in streams) and not later

    phase0()

    def head(h, carry):
        @pl.when(h == 1)
        def _():
            _start(late_copies)

        @pl.when(jnp.logical_and(h % 2 == 1, h < H - 1))
        def _():
            _wait(kv_copies((h + 1) // 2))

        @pl.when(jnp.logical_and(jnp.logical_and(h % 2 == 0, h > 0), h < H - 2))
        def _():
            _start(kv_copies(h // 2 + 1))

        zero = h // H
        toks = []
        due = []
        lane8 = lax.broadcasted_iota(I32, (8, 128), 1)
        sub8 = lax.broadcasted_iota(I32, (8, 128), 0)
        lane16 = lax.broadcasted_iota(I32, (16, 128), 1)
        sub16 = lax.broadcasted_iota(I32, (16, 128), 0)
        tri = (lax.broadcasted_iota(I32, (128, 128), 0) <= lax.broadcasted_iota(I32, (128, 128), 1))
        h_next = jnp.minimum(h + 1, H - 1)
        never = _never(zero)

        def tied(lhs):
            return _tied(lhs, due, never)

        def chan_mm(c):
            m_b = lane8 < _after(128 - 2 * sub8, toks[-5] if len(toks) >= 5 else None, never)
            gs = [jnp.broadcast_to(g_s[a, pl.ds(c, 1), :], (8, 128)) for a in range(NB)]
            bt = [pltpu.roll(jnp.where(m_b, gs[a], gs[a - 1] if a > 0 else jnp.uint32(0)), 0, 1,
                             stride=2, stride_axis=0) for a in range(NB)]
            b1 = pltpu.bitcast(jnp.concatenate(bt[7::-1], axis=0), BF16)
            b2 = pltpu.bitcast(jnp.concatenate(bt[15:7:-1], axis=0), BF16)
            am = pltpu.bitcast(aw_s[pl.ds(c, 64, stride=PITCH), :], BF16)
            z1 = _dot(tied(am), b1)
            z2 = _dot(am[:64], b2)
            return c, z1[:64], z1[64:] + z2

        def chan_post(c, zlo, zhi):
            acc = car = None
            for p in range(8):
                z = jnp.concatenate([zlo[8 * p:8 * p + 8], zhi[8 * p:8 * p + 8]], axis=0)
                if p == 0:
                    acc = z
                else:
                    z = pltpu.roll(z, 16 * p, 1)
                    cz = jnp.where(lane16 < 16 * p, z, 0.0)
                    acc = acc + z
                    car = cz if car is None else car + cz
            y = (acc - car) + jnp.where(sub16 > 0, pltpu.roll(car, 1, 0), 0.0)
            y_s[pl.ds(c, NB, stride=PITCH), :] = pltpu.bitcast(y, U32)

        def next_weights():
            for r0 in range(0, 256, 16):
                for o in (0, 1, 3, 4, 6, 2, 5):
                    shift = jnp.full((8, 128), (1 - h_next % 2) * 16, I32).astype(U32)
                    yield extract(h_next, r0, o, shift, zero * (o + 1))

        weights, done, clock = next_weights(), [0], [0]

        def tick(cycles):
            while done[0] < min(112, max(0, (clock[0] - 1500) * 112 // 6080)):
                due.append(next(weights))
                done[0] += 1
            clock[0] += cycles

        def kv_chunk(ck):
            def prod(o):
                out = {}
                for r0 in (0, 64):
                    def inner(i):
                        lhs = jnp.concatenate([cs_s[ck, 7 * o + i, k, r0:r0 + 64, :] for k in range(2)], axis=1)
                        m = _dot(tied(lhs), wx_s[7 * o + i])
                        if i == 3 and r0 == 0:
                            toks.append(m[:8])
                        return m

                    _strassen(inner, lambda r, n, val: out.__setitem__((r, n, r0), val))
                return jnp.concatenate([jnp.concatenate([out[r, 0, r0], out[r, 1, r0]], axis=1)
                                        for r in range(2) for r0 in (0, 64)], axis=0)

            def emit(r, n, val):
                jp = 2 * ck + r
                if n == 0:
                    if jp < NP - 1:
                        blocks = [val[:128, :128], val[:128, 128:], val[128:, :128], val[128:, 128:]]
                        for i in _SUMS:
                            kt_w[i, jp] = _join32(_term(_LHS, i, blocks.__getitem__))
                    for k in range(2):
                        k_w[k, 128 * jp:128 * (jp + 1), :] = _join32(val[:, 128 * k:128 * (k + 1)])
                else:
                    blocks = [val[128 * t:128 * (t + 1), 128 * k:128 * (k + 1)].T
                              for k in range(2) for t in range(2)]
                    outs = [v.astype(BF16) for v in blocks]
                    for m, v in enumerate(outs):
                        vt_s[2 * jp + m % 2, 128 * (m // 2):128 * (m // 2 + 1), :] = v
                    if jp < NP - 1:
                        for i in _SUMS:
                            vx_s[i, jp] = _term(_LHS, i, blocks.__getitem__).astype(BF16)

            return _strassen_steps(prod, emit)

        kv = [kv_chunk(ck) for ck in range(4)]
        lse, pr = {}, {}

        def s_at(u, r0):
            first = [v for v in range(u) if (v // 4) % 2 == (u // 4) % 2]
            return (sa_s, sb_s)[(u // 4) % 2], 128 * sum(v + 1 for v in first) + r0

        def qk(jq):
            run = [None, None]

            def put(n, r0, val):
                buf, row = s_at(2 * jq + n, r0)
                buf[row:row + 64, :] = val
                vs = [val[r:r + 8] for r in range(0, 64, 8)]
                m = _fold(jnp.maximum, vs)
                if run[n] is not None:
                    m = jnp.maximum(m, run[n][0])
                l = _fold(jnp.add, [jnp.exp2(v - m) for v in vs])
                if run[n] is not None:
                    l = l + run[n][1] * jnp.exp2(run[n][0] - m)
                run[n] = (m, l)

            if jq > 0:
                qt = _word_terms(_RHS, [qc_w[h, 2 * jq + n % 2, 64 * (n // 2):64 * (n // 2 + 1), :]
                                        for n in range(4)])
            for jp in range(jq):
                for r0 in (0, 64):
                    def prod(i):
                        if i == 2:
                            lhs = k_s[0, 256 * jp + r0:256 * jp + r0 + 64, :]
                        elif i == 3:
                            lhs = k_s[1, 256 * jp + 128 + r0:256 * jp + 128 + r0 + 64, :]
                        else:
                            lhs = kt_s[i, jp, r0:r0 + 64, :]
                        m = _dot(tied(lhs), qt[i])
                        if i == 3 and r0 == 0:
                            toks.append(m[:8])
                        return m

                    _strassen(prod, lambda r, n, val: put(n, 256 * jp + 128 * r + r0, val))
            q0 = 256 * jq
            for n in range(2):
                rows = slice(q0, q0 + 128 * (n + 1))
                sd = _dot(tied(jnp.concatenate([k_s[0, rows, :], k_s[1, rows, :]], axis=1)), qc_s[h, 2 * jq + n])
                last = jnp.where(tri, sd[128 * n:], NEG)
                sd = jnp.concatenate([sd[:128], last], axis=0) if n else last
                for r0 in range(0, 128 * (n + 1), 64):
                    put(n, q0 + r0, sd[r0:r0 + 64])
            toks.append(sd[:8])
            for n in range(2):
                m, l = run[n]
                top = jnp.max(m, axis=0, keepdims=True)
                lse[2 * jq + n] = top + jnp.log2(jnp.sum(l * jnp.exp2(m - top), axis=0, keepdims=True))

        def probs(u, r0):
            buf, row = s_at(u, r0)
            x = jnp.concatenate([buf[pl.ds(row + e + zero, 8, stride=4), :] for e in (0, 2)], axis=0)
            return jnp.exp2(x - lse[u])

        def softmax(jq, jps, deadline):
            starts = [r + e for r in range(0, 256, 32) for e in range(2)]
            for jp in jps:
                if jp == jq:
                    out = [jnp.concatenate([_join(probs(2 * jq + n, 256 * jq + r)) for r in starts[:8 * (n + 1)]],
                                           axis=0) for n in range(2)]
                else:
                    parts = []
                    for r in starts[:8]:
                        blocks = [probs(2 * jq + m % 2, 256 * jp + 128 * (m // 2) + r) for m in range(4)]
                        parts.append([_join(t) for t in _terms(_RHS, blocks)])
                    out = [jnp.concatenate([p[i] for p in parts], axis=0) for i in range(7)]
                pr[jq, jp] = out
                if deadline:
                    due.append(_digest(out[:1]) ^ _digest(out[1:]) if jp == jq else _digest(out))

        def pv(jq):
            softmax(jq, [jp for jp in range(jq + 1) if (jq, jp) not in pr], False)
            diag = pr.pop((jq, jq))
            ps = [pr.pop((jq, jp)) for jp in range(jq)]
            base = []
            for n in range(2):
                tick(64 * (n + 1))
                vt = jnp.concatenate([vt_s[2 * jq + i] for i in range(n + 1)], axis=1)
                base.append(_dot(tied(vt), pltpu.bitcast(diag[n], BF16)))

            def emit(r, n, val):
                val = base[n][128 * r:128 * (r + 1)] if val is None else val + base[n][128 * r:128 * (r + 1)]
                qc_s[h, 2 * jq + n, 128 * r:128 * (r + 1), :] = val.astype(BF16)

            def prod(i):
                tick(32 * jq)
                if i == 2:
                    lhs = [vt_s[2 * jp, 0:128, :] for jp in range(jq)]
                elif i == 3:
                    lhs = [vt_s[2 * jp + 1, 128:256, :] for jp in range(jq)]
                else:
                    lhs = [vx_s[i, jp] for jp in range(jq)]
                rhs = pltpu.bitcast(jnp.concatenate([p[i] for p in ps], axis=0), BF16)
                return _dot(tied(jnp.concatenate(lhs, axis=1)), rhs)

            if jq:
                _strassen(prod, emit)
            else:
                for r in range(2):
                    for n in range(2):
                        emit(r, n, None)

        chans = [h * CPH + i for i in range(CPH)]
        pend = []
        for step in HEAD_STEPS.split():
            kind, arg = step[0], [int(x) for x in step[1:]]
            if kind == 'E':
                softmax(arg[0], arg[1:] or range(arg[0] + 1), True)
                continue
            old, pend = pend, []
            if kind == 'C':
                pend = [chan_mm(chans.pop(0)) for _ in range(arg[0])]
            elif kind == 'M':
                for o in arg[1:]:
                    kv[arg[0]](o)
            else:
                for jq in arg:
                    (qk if kind == 'Q' else pv)(jq)
            for args in old:
                chan_post(*args)
        assert done[0] == 112 and not (chans or pend or due or pr)
        return carry + zero

    zero_end = lax.fori_loop(0, H, head, 0)

    _wait(late_copies)
    HH = H // 2

    def wo_block(rh, kh):
        rows = [(C * (H * b + h) + CH * rh) // 2 for h in range(HH * kh, HH * (kh + 1)) for b in range(2)]
        return jnp.concatenate([xs_w[r:r + CH // 2, :] for r in rows], axis=1)

    wt = _word_terms(_RHS, [wo_block(0, 0), wo_block(1, 0), wo_block(0, 1), wo_block(1, 1)])
    outs = []
    due, late = [], []
    never = _never(zero_end)

    def put(t, b, z, opaque=False):
        z = z.T
        r0 = pl.multiple_of(zero_end * 16 + 128 * t, 16) if opaque else 128 * t
        out_s[pl.ds(r0, 128), 128 * b:128 * (b + 1)] = z.astype(BF16)
        late.append(z[120:])

    for jp in range(NP):
        ct = _word_terms(_LHS, [jnp.concatenate([qc_w[h, 2 * jp + r] for h in range(HH * kh, HH * (kh + 1))], axis=0)
                                for r in range(2) for kh in range(2)])
        za = {}
        dues = {3: list(late)}
        late.clear()
        for r in range(2):
            t = 2 * jp + r
            za[r] = (pltpu.bitcast(y_s[t * PITCH:t * PITCH + C, :], F32)
                     * x_s[:, 128 * t:128 * (t + 1)].astype(F32))
            for b in range(3):
                put(t, b, za[r][128 * b:128 * (b + 1)], opaque=(r == 0 and b == 0 and jp > 0))
        dues[6] = list(late)
        late.clear()
        res = {}
        step = _strassen_steps(lambda i: _dot(_tied(wt[i], due, never), ct[i]),
                               lambda r, c, val: res.__setitem__((r, c), val))
        for n, i in enumerate((1, 4, 3, 6, 0, 2, 5)):
            due.extend(dues.get(n, []))
            step(i)
        for r in range(2):
            z = jnp.concatenate([za[r][384:], res[r, 0], res[r, 1]], axis=0)
            for b in range(4):
                put(2 * jp + r, 3 + b, z[128 * b:128 * (b + 1)])
        rows = pl.ds(256 * jp, 256)
        outs.append(cp(out_s.at[rows], o_hbm.at[rows], 26 + jp))
        outs[-1].start()
    _wait(outs)


def _tiles(w):
    rows = w.shape[0]
    return w.reshape(rows, 2, 8, 2, 128).transpose(0, 1, 3, 2, 4).reshape(rows, 32, 128)


@jax.jit
def pallas_concat_heads__ssm_conv_h3__compressed_kv_cla__prompt_kernel(
    A_q: jax.Array,
    A_k: jax.Array,
    A_v: jax.Array,
    A_shift_k: jax.Array,
    A_ssm_k: jax.Array,
    A_ssm_D: jax.Array,
    B_x: jax.Array,
    B_c_kv: jax.Array,
    B_w_q: jax.Array,
    B_w_uk: jax.Array,
    B_w_uv: jax.Array,
    B_w_o: jax.Array,
):
    hbm = pl.BlockSpec(memory_space=pltpu.HBM)
    out = pl.pallas_call(
        _kernel,
        in_specs=[hbm] * 12,
        out_specs=hbm,
        out_shape=jax.ShapeDtypeStruct((S, 2 * C), BF16),
        scratch_shapes=[
            pltpu.VMEM((8, S // 2, 128), U32),
            pltpu.VMEM((4, 49, 2, 64, 128), U32),
            pltpu.VMEM((2, 4, DC, 128), U32),
            pltpu.VMEM((H, NB, D // 2, 128), U32),
            pltpu.VMEM((64 * PITCH, 128), U32),
            pltpu.VMEM((NB, C, 128), U32),
            pltpu.VMEM((NB * PITCH, 128), U32),
            pltpu.VMEM((CH, S), U32),
            pltpu.VMEM((512, 128), F32),
            pltpu.VMEM((2, S // 2, 128), U32),
            pltpu.VMEM((7, NP, 64, 128), U32),
            pltpu.VMEM((NB, D // 2, 128), U32),
            pltpu.VMEM((7, NP, 64, 128), U32),
            pltpu.VMEM((49, DC // 8, 128), U32),
            pltpu.VMEM((NB * C, 128), F32),
            pltpu.VMEM((84 * 128, 128), F32),
            pltpu.VMEM((CH, S), U32),
            pltpu.VMEM((7 * NP * 128, 128), U32),
            pltpu.VMEM((CH, S), U32),
            pltpu.VMEM((CH, S), U32),
            pltpu.VMEM((2, 8, 128, 128), F32),
            pltpu.VMEM((S, 2 * C), BF16),
            pltpu.VMEM((4, C), BF16),
            pltpu.VMEM((C,), BF16),
            pltpu.SemaphoreType.DMA((36,)),
        ],
        compiler_params=pltpu.CompilerParams(vmem_limit_bytes=127 * 2 ** 20, disable_semaphore_checks=True),
    )(
        A_q[0].T, A_k[0].T, A_v[0].T, A_shift_k.T, A_ssm_k, A_ssm_D, B_x[0].T, B_c_kv[0],
        _tiles(B_w_q), _tiles(B_w_uk), _tiles(B_w_uv),
        jnp.swapaxes(B_w_o, 1, 2).reshape(H * C, D),
    )
    return out.reshape(1, S, 2 * C)
```

```python
import math

import jax
import jax.numpy as jnp
from jax import lax
import jax.experimental.pallas as pl
import jax.experimental.pallas.tpu as pltpu

F32 = jnp.float32
BF16 = jnp.bfloat16
U32 = jnp.uint32
I32 = jnp.int32

S = 2048
C = 448
H = 16
D = 256
DC = 1024
NB = S // 128
NP = NB // 2
CH = C // 2
PITCH = 520
CPH = C // H
LOG2E = math.log2(math.e)
QSCALE = (D ** -0.5) * LOG2E
NEG = -1e9 * LOG2E
HI_MASK = 0xFFFF0000

HEAD_STEPS = ("M001 C2 M034 C2 M06 M101 C2 Q01 M134 C2 M16 M201 C2 Q23 M234 C2 M26 M301 C2 E0 E1 E2 Q45 M334 C2 "
              "M36 E3 M02 C2 Q67 M05 C2 M12 C2 E4 M15 C2 E5012 M22 C2 E5345 M25 C2 M32 E6012 M35 E63456 P01234567")


def _dot(a, b):
    return jnp.dot(a, b, preferred_element_type=F32)


def _lo(x):
    return pltpu.bitcast(x << 16, F32)


def _hi(x):
    return pltpu.bitcast(x & jnp.uint32(HI_MASK), F32)


def _pack(even, odd):
    return pltpu.pack_elementwise([even, odd], packed_dtype=BF16).astype(U32)


def _split(words):
    return jnp.concatenate([_lo(words), _hi(words)], axis=0)


def _join(x):
    n = x.shape[0] // 2
    return _pack(x[:n], x[n:])


def _join32(x):
    return jnp.concatenate([_pack(x[m:m + 16], x[m + 16:m + 32]) for m in range(0, x.shape[0], 32)], axis=0)


_LHS = ((0, 1, 3), (2, 1, 3), (0,), (3,), (0, 1, 1), (2, -1, 0), (1, -1, 3))
_RHS = ((0, 1, 3), (0,), (1, -1, 3), (2, -1, 0), (3,), (0, 1, 1), (2, 1, 3))
_SUMS = (0, 1, 4, 5, 6)


def _term(table, i, block):
    spec = table[i]
    if len(spec) == 1:
        return block(spec[0])
    return block(spec[0]) + block(spec[2]) if spec[1] > 0 else block(spec[0]) - block(spec[2])


def _terms(table, blocks):
    return [_term(table, i, blocks.__getitem__) for i in range(7)]


def _word_terms(table, words):
    full = [_split(w) for w in words]
    return [pltpu.bitcast(words[table[i][0]] if len(table[i]) == 1
                          else _join(_term(table, i, full.__getitem__)), BF16) for i in range(7)]


def _inner_terms(table, o, block):
    return _terms(table, [_term(table, o, lambda n: block(n, m)) for m in range(4)])


def _strassen_steps(prod, emit):
    uses = {(0, 0): {0: 1, 3: 1, 4: -1, 6: 1}, (0, 1): {2: 1, 4: 1},
            (1, 0): {1: 1, 3: 1}, (1, 1): {0: 1, 1: -1, 2: 1, 5: 1}}
    acc = {}
    neg = {}

    def step(i):
        m = prod(i)
        for key, terms in uses.items():
            if i not in terms:
                continue
            sign = terms.pop(i)
            if key not in acc:
                acc[key] = m
                neg[key] = sign < 0
            elif neg[key]:
                assert sign > 0
                acc[key] = m - acc[key]
                neg[key] = False
            else:
                acc[key] = acc[key] + m if sign > 0 else acc[key] - m
            if not terms:
                emit(key[0], key[1], acc.pop(key))

    return step


def _strassen(prod, emit, order=(0, 1, 3, 2, 4, 5, 6)):
    step = _strassen_steps(prod, emit)
    for i in order:
        step(i)


def _never(zero):
    return lax.broadcasted_iota(I32, (8, 128), 1) < zero


def _after(x, tok, never):
    if tok is None:
        return x
    return jnp.where(never, pltpu.bitcast(tok, x.dtype), x)


def _tied(lhs, due, never):
    if not due:
        return lhs
    t = None
    for d in due:
        d = pltpu.bitcast(jnp.broadcast_to(d, (8, 128)), U32)
        t = d if t is None else t ^ d
    due.clear()
    x = pltpu.bitcast(_after(pltpu.bitcast(lhs[:16, :128], U32), t, never), BF16)
    if lhs.shape[1] > 128:
        x = jnp.concatenate([x, lhs[:16, 128:]], axis=1)
    return jnp.concatenate([x, lhs[16:]], axis=0)


def _digest(words):
    acc = None
    for r in range(words[0].shape[0] // 8):
        for w in words:
            w = w[8 * r:8 * (r + 1)]
            acc = w if acc is None else acc ^ w
    return acc


def _fold(op, xs):
    accs = list(xs[:2])
    for k, x in enumerate(xs[2:]):
        accs[k % 2] = op(accs[k % 2], x)
    return op(accs[0], accs[1])


class _Packed:
    def __init__(self, ref):
        self.ref = ref

    def _index(self, idx):
        idx = idx if isinstance(idx, tuple) else (idx,)
        axis = len(self.ref.shape) - 2
        if len(idx) <= axis:
            return idx + (slice(None),) * (axis + 2 - len(idx))
        r = idx[axis]
        r = slice(None if r.start is None else r.start // 2, None if r.stop is None else r.stop // 2)
        return idx[:axis] + (r,) + idx[axis + 1:]

    def __getitem__(self, idx):
        return pltpu.bitcast(self.ref[self._index(idx)], BF16)

    def __setitem__(self, idx, val):
        self.ref[self._index(idx)] = pltpu.bitcast(val, U32)


def _start(copies):
    for c_ in copies:
        c_.start()


def _wait(copies):
    for c_ in copies:
        c_.wait()


def _kernel(qa_hbm, ka_hbm, va_hbm, sk_hbm, hk_hbm, d_hbm, x_hbm, c_hbm, wq_hbm, wk_hbm, wv_hbm, wo_hbm,
            o_hbm,
            c_w, cs_w, wp_s, qc_w, aw_s, g_s, y_s, hk_w, dc_s, k_w, kt_w, vt_w, vx_w, wx_w, sa_s, sb_s,
            x_w, xs_w, ka_w, va_w, wt_s, out_s, sk_ref, d_ref, sems):
    def cp(src, dst, i):
        return pltpu.make_async_copy(src, dst, sems.at[i])

    cs_s, qc_s, k_s, kt_s, vt_s, vx_s, wx_s, xs_s, x_s, ka_s, va_s, hk_s = (
        _Packed(r) for r in (cs_w, qc_w, k_w, kt_w, vt_w, vx_w, wx_w, xs_w, x_w, ka_w, va_w, hk_w))
    qa_hbm, ka_hbm, va_hbm, hk_hbm, x_hbm, c_hbm, wo_hbm, wq_hbm, wk_hbm, wv_hbm = (
        r.bitcast(U32)
        for r in (qa_hbm, ka_hbm, va_hbm, hk_hbm, x_hbm, c_hbm, wo_hbm, wq_hbm, wk_hbm, wv_hbm))

    def word_row(pair, b):
        return 8 * (pair // 4) + 4 * b + pair % 4

    def kv_copies(pair):
        return [cp(w.at[:, word_row(pair, b), :], wp_s.at[pair % 2, 2 * n + b], 16 + pair % 2)
                for n, w in enumerate((wk_hbm, wv_hbm)) for b in range(2)]

    late_copies = [cp(qa_hbm, x_w, 21)] + [
        cp(wo_hbm.at[:, pl.ds(128 * b, 128)], xs_w.at[pl.ds(H * CH * b, H * CH)], 6 + b) for b in range(2)]

    def extract(h, r0, o, shift, z):
        def block(n, kq, b):
            x = jnp.concatenate([wp_s[(h // 2) % 2 + z, 2 * n + b, pl.ds(256 * kq + r0 + e, 8, stride=2), :]
                                 for e in range(2)], axis=0)
            if isinstance(h, int):
                return _lo(x) if h % 2 == 0 else _hi(x)
            return _hi(x << jnp.concatenate([shift] * 2, axis=0))

        terms = [_join(t) for t in _inner_terms(
            _RHS, o, lambda n, m: block(n % 2, 2 * (n // 2) + m // 2, m % 2))]
        for i, t in enumerate(terms):
            wx_w[7 * o + i, r0 // 2:r0 // 2 + 8, :] = t
        return _digest(terms)

    def phase0():
        U1, U2, UX, UA, UB, UD = 1, 3, 10, 33, 60, 98
        LAG, LAG_U, LAG_T, BACK, BACK_W, SLACK = 12, 8, 4, 10, 8, 12
        cq = [cp(wq_hbm.at[:, word_row(g // 2, g % 2), :], y_s.at[pl.ds(C * g, C)],
                 (0, 35, 35, 19, 19, 1, 1, 1)[g] if g < 8 else 18) for g in range(H)]
        cx = [cp(x_hbm.at[:, pl.ds(512 * i, 512)], x_w.at[:, pl.ds(512 * i, 512)], 22 + i) for i in range(4)]
        ga = cq[5:8] + [cp(sk_hbm, sk_ref, 2), cp(ka_hbm, ka_w, 3), cp(va_hbm, va_w, 4)]
        gb = cq[8:] + [cp(c_hbm.at[:, pl.ds(128 * b, 128)], c_w.at[b], 8 + b) for b in range(8)]
        gd = [cp(d_hbm, d_ref, 20), cp(hk_hbm, hk_w, 5)] + kv_copies(0)
        _start(cx[:1] + cq[:3] + cx[1:2] + cq[3:5] + cx[2:] + ga)
        zero = pl.semaphore_read(sems.at[34])
        never = _never(zero)
        due = []
        toks = []

        def gate(x):
            return _after(x, toks[-BACK], never)

        def w_terms(j, b):
            tok = toks[-BACK_W] if len(toks) >= BACK_W else None
            x = y_s[C * (2 * j + b):C * (2 * j + b + 1), :]
            g16 = jnp.concatenate([_after(jnp.full((8, 128), 16, U32), tok, never)] * (C // 8), axis=0)
            gm = jnp.concatenate([_after(jnp.full((8, 128), HI_MASK, U32), tok, never)] * (C // 8), axis=0)
            lo, hi = pltpu.bitcast(x << g16, F32), pltpu.bitcast(x & gm, F32)
            pad = jnp.zeros((256 - CH, 128), F32)
            blocks = [jnp.concatenate([t, pad], axis=0).T for t in (lo[:CH], hi[:CH], lo[CH:], hi[CH:])]
            for n, t in enumerate(blocks):
                for k in range(2):
                    wt_s[b, 2 * n + k] = t[:, 128 * k:128 * (k + 1)]
            quarter = [[jnp.concatenate([wt_s[b, 2 * n + k, pl.ds(e, 32, stride=4), :] for k in range(2)], axis=1)
                        for n in range(4)] for e in range(4)]
            terms = [_terms(_RHS, q) for q in quarter]
            out = []
            for i in range(7):
                ev, od = _pack(terms[0][i], terms[2][i]), _pack(terms[1][i], terms[3][i])
                rows = [w[8 * m:8 * (m + 1)] for m in range(4) for w in (ev, od)]
                out.append(pltpu.bitcast(jnp.concatenate(rows, axis=0), BF16))
            return out

        def x_terms(jp):
            top = slice(256 * jp, 256 * jp + 128)
            bot = slice(256 * jp + 128, 256 * jp + 256)
            for i in range(7):
                xs_s[256 * (NP * i + jp) + CH:256 * (NP * i + jp + 1), :] = jnp.zeros((256 - CH, 128), BF16)
            for r in range(0, CH // 2, 16):
                lo, hi = slice(r, r + 16), slice(CH // 2 + r, CH // 2 + r + 16)
                blocks = [x_w[lo, top], x_w[hi, top], x_w[lo, bot], x_w[hi, bot]]
                terms = [_join(t) for t in _terms(_LHS, [_split(t) for t in blocks])]
                terms[2], terms[3] = blocks[0], blocks[3]
                for i, t in enumerate(terms):
                    xs_w[128 * (NP * i + jp) + r:128 * (NP * i + jp) + r + 16, :] = t
                yield 1, _digest(terms), LAG

        def column(row):
            row = jnp.concatenate([row.astype(F32), jnp.zeros((1, 512 - C), F32)], axis=1)
            return jnp.broadcast_to(row, (128, 512)).T

        def delayed(ref, rows, sg, n):
            cur = pltpu.bitcast(ref[rows, 128 * sg:128 * (sg + 1)], U32)
            lane = jnp.concatenate([gate(lax.broadcasted_iota(I32, (8, 128), 1))] * (cur.shape[0] // 8), axis=0)
            prev = pltpu.bitcast(ref[rows, 128 * (sg - 1):128 * sg], U32) if sg > 0 else jnp.uint32(0)
            x = pltpu.roll(jnp.where(lane < 128 - n, cur, prev), n, 1)
            return pltpu.bitcast(x, BF16).astype(F32)

        def transposed(x):
            return jnp.concatenate([gate(x[:8]), x[8:]], axis=0).T

        def conv_inputs():
            taps = [column(sk_ref[j:j + 1, :]) for j in range(4)]
            for b in range(4):
                for r0 in range(128 * b, min(C, 128 * (b + 1)), 32):
                    rows = slice(r0, r0 + 32)
                    tp = [t[rows] for t in taps]
                    prev = jnp.zeros((32, 128), F32)
                    for sg in range(NB):
                        cols = slice(128 * sg, 128 * (sg + 1))
                        ksh = ((delayed(ka_s, rows, sg, 3) * tp[3] + delayed(ka_s, rows, sg, 2) * tp[2])
                               + (delayed(ka_s, rows, sg, 1) * tp[1] + ka_s[rows, cols].astype(F32) * tp[0]))
                        kv = ksh * va_s[rows, cols].astype(F32)
                        wrd = _pack(prev, kv)
                        sa_s[C * sg + r0:C * sg + r0 + 32, :] = pltpu.bitcast(wrd, F32)
                        prev = kv
                        yield 2, _digest([wrd]), LAG_U
                for sg in range(NB):
                    r0 = C * sg + 128 * b
                    if b < 3:
                        wrd = sa_s[r0:r0 + 128, :]
                    else:
                        wrd = jnp.concatenate([sa_s[r0:r0 + C - 384, :], jnp.zeros((512 - C, 128), F32)], axis=0)
                    wrd = transposed(pltpu.bitcast(wrd, U32))
                    sb_s[S * b + 128 * sg:S * b + 128 * (sg + 1), :] = pltpu.bitcast(wrd, F32)
                    yield 3, wrd[120:], LAG_T
                for p in range(8):
                    for j in range(8):
                        parts = [jnp.zeros((16, 128), U32) if sg < 0 else
                                 pltpu.bitcast(sb_s[pl.ds(S * b + 128 * sg + 16 * p, 16), :], U32)
                                 for sg in range(2 * j - 6, 2 * j + 2)]
                        plane = 32 * (j // 4) + 4 * p + j % 4
                        win = transposed(jnp.concatenate(parts, axis=0))
                        aw_s[pl.ds(plane * PITCH + 128 * b, 128), :] = win
                        yield 3, win[120:], LAG_T

        def conv_filter_and_first_head():
            dc_s[...] = column(d_ref[...].reshape(1, C))
            lane = lax.broadcasted_iota(I32, (32, 128), 1)
            for r0 in range(0, C, 32):
                rows = slice(r0, r0 + 32)
                for a in range(NB):
                    hf = hk_s[rows, 128 * a:128 * (a + 1)].astype(F32)
                    hs = delayed(hk_s, rows, a, 1)
                    if a == 0:
                        hf = jnp.where(lane == 0, hf + dc_s[rows, :], hf)
                        hs = jnp.where(lane == 1, hs + dc_s[rows, :], hs)
                    wrd = _pack(hf, hs)
                    g_s[a, rows, :] = wrd
                    yield 1, _digest([wrd]), LAG
            for r0 in range(0, 256, 16):
                for o in range(7):
                    yield 2, extract(0, r0, o, None, zero * (o + 1)), LAG

        def c_terms():
            for ck in range(4):
                for half in range(2):
                    for r0 in range(0, 128, 16):
                        for o in range(7):
                            def block(n, m):
                                row = 256 * ck + 128 * (n // 2) + 64 * (m // 2) + 16 * (r0 // 32)
                                col = 4 * (n % 2) + 2 * (m % 2) + half + zero * (o + 1)
                                w = jnp.concatenate([c_w[col, pl.ds(row + e, 8, stride=2), :] for e in range(2)],
                                                    axis=0)
                                return _hi(w) if r0 % 32 else _lo(w)

                            terms = [_join(t) for t in _inner_terms(_LHS, o, block)]
                            for i, t in enumerate(terms):
                                cs_w[ck, 7 * o + i, half, r0 // 2:r0 // 2 + 8, :] = t
                            yield 1, _digest(terms), LAG

        units = [(g, jp) for g in range(3) for jp in (0, 1)] + [(g, jp) for g in range(3) for jp in (2, 3)]
        units += [(g, jp) for g in (3, 4) for jp in range(4)] + [(g, jp) for g in range(5) for jp in range(4, NP)]
        units += [(g, jp) for g in range(5, H) for jp in range(NP)]
        last = 7 * len(units) - 2 - LAG
        streams = [[(v for jp in (2, 3) for v in x_terms(jp)), 14, 7 * U2 + 1, 7 * 6 - 1, 0],
                   [(v for jp in range(4, NP) for v in x_terms(jp)), 28, 7 * UX + 2, 7 * 20 - 1 - LAG, 0],
                   [conv_inputs(), 2 * 14 * NB + 3 * 4 * (NB + 64), 7 * UA + SLACK, 7 * UD + SLACK, 0],
                   [c_terms(), 448, 7 * UB + SLACK, last, 0],
                   [conv_filter_and_first_head(), 14 * NB + 2 * 112, 7 * UD + SLACK, last, 0]]
        later = {}

        def pump():
            n = len(toks)
            for st in streams:
                want = min(st[1], max(0, (n - st[2] + 1) * st[1] // (st[3] - st[2])))
                while st[4] < want:
                    cost, v, lag = next(st[0])
                    later.setdefault(n + lag, []).append(v)
                    st[4] += cost
            due.extend(later.pop(n, []))

        starts = {UX: gb, UA: gd, UB: kv_copies(1)}
        waits = {U1: cq[1:3], U2: cx[1:2], UX: cq[3:5] + cx[2:], UA: ga, UB: gb, UD: gd}
        _wait(cx[:1])
        list(x_terms(0))
        list(x_terms(1))
        _wait(cq[:1])
        wts = {}
        for u, (g, jp) in enumerate(units):
            _start(starts.get(u, []))
            _wait(waits.get(u, []))
            for g_ in range(H):
                if g_ not in wts and units.index((g_, 0)) - (4 if g_ >= 5 else 1) <= u:
                    wts[g_] = w_terms(g_ // 2, g_ % 2)

            def prod(i):
                pump()
                m = _dot(_tied(wts[g][i], due, never), xs_s[256 * (NP * i + jp):256 * (NP * i + jp + 1), :])
                toks.append(m[:8])
                return m

            def emit(r, c, val):
                qc_w[2 * (g // 2) + c, 2 * jp + r, 64 * (g % 2):64 * (g % 2 + 1), :] = _join32(val * QSCALE)

            _strassen(prod, emit)
        assert all(st[4] == st[1] for st in streams) and not later

    phase0()

    def head(h, carry):
        @pl.when(h == 1)
        def _():
            _start(late_copies)

        @pl.when(jnp.logical_and(h % 2 == 1, h < H - 1))
        def _():
            _wait(kv_copies((h + 1) // 2))

        @pl.when(jnp.logical_and(jnp.logical_and(h % 2 == 0, h > 0), h < H - 2))
        def _():
            _start(kv_copies(h // 2 + 1))

        zero = h // H
        toks = []
        due = []
        lane8 = lax.broadcasted_iota(I32, (8, 128), 1)
        sub8 = lax.broadcasted_iota(I32, (8, 128), 0)
        lane16 = lax.broadcasted_iota(I32, (16, 128), 1)
        sub16 = lax.broadcasted_iota(I32, (16, 128), 0)
        tri = (lax.broadcasted_iota(I32, (128, 128), 0) <= lax.broadcasted_iota(I32, (128, 128), 1))
        h_next = jnp.minimum(h + 1, H - 1)
        never = _never(zero)

        def tied(lhs):
            return _tied(lhs, due, never)

        def chan_mm(c):
            m_b = lane8 < _after(128 - 2 * sub8, toks[-5] if len(toks) >= 5 else None, never)
            gs = [jnp.broadcast_to(g_s[a, pl.ds(c, 1), :], (8, 128)) for a in range(NB)]
            bt = [pltpu.roll(jnp.where(m_b, gs[a], gs[a - 1] if a > 0 else jnp.uint32(0)), 0, 1,
                             stride=2, stride_axis=0) for a in range(NB)]
            b1 = pltpu.bitcast(jnp.concatenate(bt[7::-1], axis=0), BF16)
            b2 = pltpu.bitcast(jnp.concatenate(bt[15:7:-1], axis=0), BF16)
            am = pltpu.bitcast(aw_s[pl.ds(c, 64, stride=PITCH), :], BF16)
            z1 = _dot(tied(am), b1)
            z2 = _dot(am[:64], b2)
            return c, z1[:64], z1[64:] + z2

        def chan_post(c, zlo, zhi):
            acc = car = None
            for p in range(8):
                z = jnp.concatenate([zlo[8 * p:8 * p + 8], zhi[8 * p:8 * p + 8]], axis=0)
                if p == 0:
                    acc = z
                else:
                    z = pltpu.roll(z, 16 * p, 1)
                    cz = jnp.where(lane16 < 16 * p, z, 0.0)
                    acc = acc + z
                    car = cz if car is None else car + cz
            y = (acc - car) + jnp.where(sub16 > 0, pltpu.roll(car, 1, 0), 0.0)
            y_s[pl.ds(c, NB, stride=PITCH), :] = pltpu.bitcast(y, U32)

        def next_weights():
            for r0 in range(0, 256, 16):
                for o in (0, 1, 3, 4, 6, 2, 5):
                    shift = jnp.full((8, 128), (1 - h_next % 2) * 16, I32).astype(U32)
                    yield extract(h_next, r0, o, shift, zero * (o + 1))

        weights, done, clock = next_weights(), [0], [0]

        def tick(cycles):
            while done[0] < min(112, max(0, (clock[0] - 1500) * 112 // 6080)):
                due.append(next(weights))
                done[0] += 1
            clock[0] += cycles

        def kv_chunk(ck):
            def prod(o):
                out = {}
                for r0 in (0, 64):
                    def inner(i):
                        lhs = jnp.concatenate([cs_s[ck, 7 * o + i, k, r0:r0 + 64, :] for k in range(2)], axis=1)
                        m = _dot(tied(lhs), wx_s[7 * o + i])
                        if i == 3 and r0 == 0:
                            toks.append(m[:8])
                        return m

                    _strassen(inner, lambda r, n, val: out.__setitem__((r, n, r0), val))
                return jnp.concatenate([jnp.concatenate([out[r, 0, r0], out[r, 1, r0]], axis=1)
                                        for r in range(2) for r0 in (0, 64)], axis=0)

            def emit(r, n, val):
                jp = 2 * ck + r
                if n == 0:
                    if jp < NP - 1:
                        blocks = [val[:128, :128], val[:128, 128:], val[128:, :128], val[128:, 128:]]
                        for i in _SUMS:
                            kt_w[i, jp] = _join32(_term(_LHS, i, blocks.__getitem__))
                    for k in range(2):
                        k_w[k, 128 * jp:128 * (jp + 1), :] = _join32(val[:, 128 * k:128 * (k + 1)])
                else:
                    blocks = [val[128 * t:128 * (t + 1), 128 * k:128 * (k + 1)].T
                              for k in range(2) for t in range(2)]
                    outs = [v.astype(BF16) for v in blocks]
                    for m, v in enumerate(outs):
                        vt_s[2 * jp + m % 2, 128 * (m // 2):128 * (m // 2 + 1), :] = v
                    if jp < NP - 1:
                        for i in _SUMS:
                            vx_s[i, jp] = _term(_LHS, i, blocks.__getitem__).astype(BF16)

            return _strassen_steps(prod, emit)

        kv = [kv_chunk(ck) for ck in range(4)]
        lse, pr = {}, {}

        def s_at(u, r0):
            first = [v for v in range(u) if (v // 4) % 2 == (u // 4) % 2]
            return (sa_s, sb_s)[(u // 4) % 2], 128 * sum(v + 1 for v in first) + r0

        def qk(jq):
            run = [None, None]

            def put(n, r0, val):
                buf, row = s_at(2 * jq + n, r0)
                buf[row:row + 64, :] = val
                vs = [val[r:r + 8] for r in range(0, 64, 8)]
                m = _fold(jnp.maximum, vs)
                if run[n] is not None:
                    m = jnp.maximum(m, run[n][0])
                l = _fold(jnp.add, [jnp.exp2(v - m) for v in vs])
                if run[n] is not None:
                    l = l + run[n][1] * jnp.exp2(run[n][0] - m)
                run[n] = (m, l)

            if jq > 0:
                qt = _word_terms(_RHS, [qc_w[h, 2 * jq + n % 2, 64 * (n // 2):64 * (n // 2 + 1), :]
                                        for n in range(4)])
            for jp in range(jq):
                for r0 in (0, 64):
                    def prod(i):
                        if i == 2:
                            lhs = k_s[0, 256 * jp + r0:256 * jp + r0 + 64, :]
                        elif i == 3:
                            lhs = k_s[1, 256 * jp + 128 + r0:256 * jp + 128 + r0 + 64, :]
                        else:
                            lhs = kt_s[i, jp, r0:r0 + 64, :]
                        m = _dot(tied(lhs), qt[i])
                        if i == 3 and r0 == 0:
                            toks.append(m[:8])
                        return m

                    _strassen(prod, lambda r, n, val: put(n, 256 * jp + 128 * r + r0, val))
            q0 = 256 * jq
            for n in range(2):
                rows = slice(q0, q0 + 128 * (n + 1))
                sd = _dot(tied(jnp.concatenate([k_s[0, rows, :], k_s[1, rows, :]], axis=1)), qc_s[h, 2 * jq + n])
                last = jnp.where(tri, sd[128 * n:], NEG)
                sd = jnp.concatenate([sd[:128], last], axis=0) if n else last
                for r0 in range(0, 128 * (n + 1), 64):
                    put(n, q0 + r0, sd[r0:r0 + 64])
            toks.append(sd[:8])
            for n in range(2):
                m, l = run[n]
                top = jnp.max(m, axis=0, keepdims=True)
                lse[2 * jq + n] = top + jnp.log2(jnp.sum(l * jnp.exp2(m - top), axis=0, keepdims=True))

        def probs(u, r0):
            buf, row = s_at(u, r0)
            x = jnp.concatenate([buf[pl.ds(row + e + zero, 8, stride=4), :] for e in (0, 2)], axis=0)
            return jnp.exp2(x - lse[u])

        def softmax(jq, jps, deadline):
            starts = [r + e for r in range(0, 256, 32) for e in range(2)]
            for jp in jps:
                if jp == jq:
                    out = [jnp.concatenate([_join(probs(2 * jq + n, 256 * jq + r)) for r in starts[:8 * (n + 1)]],
                                           axis=0) for n in range(2)]
                else:
                    parts = []
                    for r in starts[:8]:
                        blocks = [probs(2 * jq + m % 2, 256 * jp + 128 * (m // 2) + r) for m in range(4)]
                        parts.append([_join(t) for t in _terms(_RHS, blocks)])
                    out = [jnp.concatenate([p[i] for p in parts], axis=0) for i in range(7)]
                pr[jq, jp] = out
                if deadline:
                    due.append(_digest(out[:1]) ^ _digest(out[1:]) if jp == jq else _digest(out))

        def pv(jq):
            softmax(jq, [jp for jp in range(jq + 1) if (jq, jp) not in pr], False)
            diag = pr.pop((jq, jq))
            ps = [pr.pop((jq, jp)) for jp in range(jq)]
            base = []
            for n in range(2):
                tick(64 * (n + 1))
                vt = jnp.concatenate([vt_s[2 * jq + i] for i in range(n + 1)], axis=1)
                base.append(_dot(tied(vt), pltpu.bitcast(diag[n], BF16)))

            def emit(r, n, val):
                val = base[n][128 * r:128 * (r + 1)] if val is None else val + base[n][128 * r:128 * (r + 1)]
                qc_s[h, 2 * jq + n, 128 * r:128 * (r + 1), :] = val.astype(BF16)

            def prod(i):
                tick(32 * jq)
                if i == 2:
                    lhs = [vt_s[2 * jp, 0:128, :] for jp in range(jq)]
                elif i == 3:
                    lhs = [vt_s[2 * jp + 1, 128:256, :] for jp in range(jq)]
                else:
                    lhs = [vx_s[i, jp] for jp in range(jq)]
                rhs = pltpu.bitcast(jnp.concatenate([p[i] for p in ps], axis=0), BF16)
                return _dot(tied(jnp.concatenate(lhs, axis=1)), rhs)

            if jq:
                _strassen(prod, emit)
            else:
                for r in range(2):
                    for n in range(2):
                        emit(r, n, None)

        chans = [h * CPH + i for i in range(CPH)]
        pend = []
        for step in HEAD_STEPS.split():
            kind, arg = step[0], [int(x) for x in step[1:]]
            if kind == 'E':
                softmax(arg[0], arg[1:] or range(arg[0] + 1), True)
                continue
            old, pend = pend, []
            if kind == 'C':
                pend = [chan_mm(chans.pop(0)) for _ in range(arg[0])]
            elif kind == 'M':
                for o in arg[1:]:
                    kv[arg[0]](o)
            else:
                for jq in arg:
                    (qk if kind == 'Q' else pv)(jq)
            for args in old:
                chan_post(*args)
        assert done[0] == 112 and not (chans or pend or due or pr)
        return carry + zero

    zero_end = lax.fori_loop(0, H, head, 0)

    _wait(late_copies)
    HH = H // 2

    def wo_block(rh, kh):
        rows = [(C * (H * b + h) + CH * rh) // 2 for h in range(HH * kh, HH * (kh + 1)) for b in range(2)]
        return jnp.concatenate([xs_w[r:r + CH // 2, :] for r in rows], axis=1)

    wt = _word_terms(_RHS, [wo_block(0, 0), wo_block(1, 0), wo_block(0, 1), wo_block(1, 1)])
    outs = []
    due, late = [], []
    never = _never(zero_end)

    def put(t, b, z, opaque=False):
        z = z.T
        r0 = pl.multiple_of(zero_end * 16 + 128 * t, 16) if opaque else 128 * t
        out_s[pl.ds(r0, 128), 128 * b:128 * (b + 1)] = z.astype(BF16)
        late.append(z[120:])

    for jp in range(NP):
        ct = _word_terms(_LHS, [jnp.concatenate([qc_w[h, 2 * jp + r] for h in range(HH * kh, HH * (kh + 1))], axis=0)
                                for r in range(2) for kh in range(2)])
        za = {}
        dues = {3: list(late)}
        late.clear()
        for r in range(2):
            t = 2 * jp + r
            za[r] = (pltpu.bitcast(y_s[t * PITCH:t * PITCH + C, :], F32)
                     * x_s[:, 128 * t:128 * (t + 1)].astype(F32))
            for b in range(3):
                put(t, b, za[r][128 * b:128 * (b + 1)], opaque=(r == 0 and b == 0 and jp > 0))
        dues[6] = list(late)
        late.clear()
        res = {}
        step = _strassen_steps(lambda i: _dot(_tied(wt[i], due, never), ct[i]),
                               lambda r, c, val: res.__setitem__((r, c), val))
        for n, i in enumerate((1, 4, 3, 6, 0, 2, 5)):
            due.extend(dues.get(n, []))
            step(i)
        for r in range(2):
            z = jnp.concatenate([za[r][384:], res[r, 0], res[r, 1]], axis=0)
            for b in range(4):
                put(2 * jp + r, 3 + b, z[128 * b:128 * (b + 1)])
        rows = pl.ds(256 * jp, 256)
        outs.append(cp(out_s.at[rows], o_hbm.at[rows], 26 + jp))
        outs[-1].start()
    _wait(outs)


def _tiles(w):
    rows = w.shape[0]
    return w.reshape(rows, 2, 8, 2, 128).transpose(0, 1, 3, 2, 4).reshape(rows, 32, 128)


@jax.jit
def pallas_concat_heads__ssm_conv_h3__compressed_kv_cla__prompt_kernel(
    A_q: jax.Array,
    A_k: jax.Array,
    A_v: jax.Array,
    A_shift_k: jax.Array,
    A_ssm_k: jax.Array,
    A_ssm_D: jax.Array,
    B_x: jax.Array,
    B_c_kv: jax.Array,
    B_w_q: jax.Array,
    B_w_uk: jax.Array,
    B_w_uv: jax.Array,
    B_w_o: jax.Array,
):
    hbm = pl.BlockSpec(memory_space=pltpu.HBM)
    out = pl.pallas_call(
        _kernel,
        in_specs=[hbm] * 12,
        out_specs=hbm,
        out_shape=jax.ShapeDtypeStruct((S, 2 * C), BF16),
        scratch_shapes=[
            pltpu.VMEM((8, S // 2, 128), U32),
            pltpu.VMEM((4, 49, 2, 64, 128), U32),
            pltpu.VMEM((2, 4, DC, 128), U32),
            pltpu.VMEM((H, NB, D // 2, 128), U32),
            pltpu.VMEM((64 * PITCH, 128), U32),
            pltpu.VMEM((NB, C, 128), U32),
            pltpu.VMEM((NB * PITCH, 128), U32),
            pltpu.VMEM((CH, S), U32),
            pltpu.VMEM((512, 128), F32),
            pltpu.VMEM((2, S // 2, 128), U32),
            pltpu.VMEM((7, NP, 64, 128), U32),
            pltpu.VMEM((NB, D // 2, 128), U32),
            pltpu.VMEM((7, NP, 64, 128), U32),
            pltpu.VMEM((49, DC // 8, 128), U32),
            pltpu.VMEM((NB * C, 128), F32),
            pltpu.VMEM((84 * 128, 128), F32),
            pltpu.VMEM((CH, S), U32),
            pltpu.VMEM((7 * NP * 128, 128), U32),
            pltpu.VMEM((CH, S), U32),
            pltpu.VMEM((CH, S), U32),
            pltpu.VMEM((2, 8, 128, 128), F32),
            pltpu.VMEM((S, 2 * C), BF16),
            pltpu.VMEM((4, C), BF16),
            pltpu.VMEM((C,), BF16),
            pltpu.SemaphoreType.DMA((36,)),
        ],
        compiler_params=pltpu.CompilerParams(vmem_limit_bytes=127 * 2 ** 20, disable_semaphore_checks=True),
    )(
        A_q[0].T, A_k[0].T, A_v[0].T, A_shift_k.T, A_ssm_k, A_ssm_D, B_x[0].T, B_c_kv[0],
        _tiles(B_w_q), _tiles(B_w_uk), _tiles(B_w_uv),
        jnp.swapaxes(B_w_o, 1, 2).reshape(H * C, D),
    )
    return out.reshape(1, S, 2 * C)
```

```python
import math

import jax
import jax.numpy as jnp
from jax import lax
import jax.experimental.pallas as pl
import jax.experimental.pallas.tpu as pltpu

F32 = jnp.float32
BF16 = jnp.bfloat16
U32 = jnp.uint32
I32 = jnp.int32

S = 2048
C = 448
H = 16
D = 256
DC = 1024
NB = S // 128
NP = NB // 2
CH = C // 2
PITCH = 520
CPH = C // H
LOG2E = math.log2(math.e)
QSCALE = (D ** -0.5) * LOG2E
NEG = -1e9 * LOG2E
HI_MASK = 0xFFFF0000

HEAD_STEPS = ("M001 C2 M034 C2 M06 M101 C2 Q01 M134 C2 M16 M201 C2 Q23 M234 C2 M26 M301 C2 E0 E1 E2 Q45 M334 C2 "
              "M36 E3 M02 C2 Q67 M05 C2 M12 C2 E4 M15 C2 E5012 M22 C2 E5345 M25 C2 M32 E6012 M35 E63456 P01234567")


def _dot(a, b):
    return jnp.dot(a, b, preferred_element_type=F32)


def _lo(x):
    return pltpu.bitcast(x << 16, F32)


def _hi(x):
    return pltpu.bitcast(x & jnp.uint32(HI_MASK), F32)


def _pack(even, odd):
    return pltpu.pack_elementwise([even, odd], packed_dtype=BF16).astype(U32)


def _split(words):
    return jnp.concatenate([_lo(words), _hi(words)], axis=0)


def _join(x):
    n = x.shape[0] // 2
    return _pack(x[:n], x[n:])


def _join32(x):
    return jnp.concatenate([_pack(x[m:m + 16], x[m + 16:m + 32]) for m in range(0, x.shape[0], 32)], axis=0)


_LHS = ((0, 1, 3), (2, 1, 3), (0,), (3,), (0, 1, 1), (2, -1, 0), (1, -1, 3))
_RHS = ((0, 1, 3), (0,), (1, -1, 3), (2, -1, 0), (3,), (0, 1, 1), (2, 1, 3))
_SUMS = (0, 1, 4, 5, 6)


def _term(table, i, block):
    spec = table[i]
    if len(spec) == 1:
        return block(spec[0])
    return block(spec[0]) + block(spec[2]) if spec[1] > 0 else block(spec[0]) - block(spec[2])


def _terms(table, blocks):
    return [_term(table, i, blocks.__getitem__) for i in range(7)]


def _word_terms(table, words):
    full = [_split(w) for w in words]
    return [pltpu.bitcast(words[table[i][0]] if len(table[i]) == 1
                          else _join(_term(table, i, full.__getitem__)), BF16) for i in range(7)]


def _inner_terms(table, o, block):
    return _terms(table, [_term(table, o, lambda n: block(n, m)) for m in range(4)])


def _strassen_steps(prod, emit):
    uses = {(0, 0): {0: 1, 3: 1, 4: -1, 6: 1}, (0, 1): {2: 1, 4: 1},
            (1, 0): {1: 1, 3: 1}, (1, 1): {0: 1, 1: -1, 2: 1, 5: 1}}
    acc = {}
    neg = {}

    def step(i):
        m = prod(i)
        for key, terms in uses.items():
            if i not in terms:
                continue
            sign = terms.pop(i)
            if key not in acc:
                acc[key] = m
                neg[key] = sign < 0
            elif neg[key]:
                assert sign > 0
                acc[key] = m - acc[key]
                neg[key] = False
            else:
                acc[key] = acc[key] + m if sign > 0 else acc[key] - m
            if not terms:
                emit(key[0], key[1], acc.pop(key))

    return step


def _strassen(prod, emit, order=(0, 1, 3, 2, 4, 5, 6)):
    step = _strassen_steps(prod, emit)
    for i in order:
        step(i)


def _never(zero):
    return lax.broadcasted_iota(I32, (8, 128), 1) < zero


def _after(x, tok, never):
    if tok is None:
        return x
    return jnp.where(never, pltpu.bitcast(tok, x.dtype), x)


def _tied(lhs, due, never):
    if not due:
        return lhs
    t = None
    for d in due:
        d = pltpu.bitcast(jnp.broadcast_to(d, (8, 128)), U32)
        t = d if t is None else t ^ d
    due.clear()
    x = pltpu.bitcast(_after(pltpu.bitcast(lhs[:16, :128], U32), t, never), BF16)
    if lhs.shape[1] > 128:
        x = jnp.concatenate([x, lhs[:16, 128:]], axis=1)
    return jnp.concatenate([x, lhs[16:]], axis=0)


def _digest(words):
    acc = None
    for r in range(words[0].shape[0] // 8):
        for w in words:
            w = w[8 * r:8 * (r + 1)]
            acc = w if acc is None else acc ^ w
    return acc


def _fold(op, xs):
    accs = list(xs[:2])
    for k, x in enumerate(xs[2:]):
        accs[k % 2] = op(accs[k % 2], x)
    return op(accs[0], accs[1])


class _Packed:
    def __init__(self, ref):
        self.ref = ref

    def _index(self, idx):
        idx = idx if isinstance(idx, tuple) else (idx,)
        axis = len(self.ref.shape) - 2
        if len(idx) <= axis:
            return idx + (slice(None),) * (axis + 2 - len(idx))
        r = idx[axis]
        r = slice(None if r.start is None else r.start // 2, None if r.stop is None else r.stop // 2)
        return idx[:axis] + (r,) + idx[axis + 1:]

    def __getitem__(self, idx):
        return pltpu.bitcast(self.ref[self._index(idx)], BF16)

    def __setitem__(self, idx, val):
        self.ref[self._index(idx)] = pltpu.bitcast(val, U32)


def _start(copies):
    for c_ in copies:
        c_.start()


def _wait(copies):
    for c_ in copies:
        c_.wait()


def _kernel(qa_hbm, ka_hbm, va_hbm, sk_hbm, hk_hbm, d_hbm, x_hbm, c_hbm, wq_hbm, wk_hbm, wv_hbm, wo_hbm,
            o_hbm,
            c_w, cs_w, wp_s, qc_w, aw_s, g_s, y_s, hk_w, dc_s, k_w, kt_w, vt_w, vx_w, wx_w, sa_s, sb_s,
            x_w, xs_w, ka_w, va_w, wt_s, out_s, sk_ref, d_ref, idle_sem, sems):
    def cp(src, dst, i):
        return pltpu.make_async_copy(src, dst, sems.at[i])

    cs_s, qc_s, k_s, kt_s, vt_s, vx_s, wx_s, xs_s, x_s, ka_s, va_s, hk_s = (
        _Packed(r) for r in (cs_w, qc_w, k_w, kt_w, vt_w, vx_w, wx_w, xs_w, x_w, ka_w, va_w, hk_w))
    qa_hbm, ka_hbm, va_hbm, hk_hbm, x_hbm, c_hbm, wo_hbm, wq_hbm, wk_hbm, wv_hbm = (
        r.bitcast(U32)
        for r in (qa_hbm, ka_hbm, va_hbm, hk_hbm, x_hbm, c_hbm, wo_hbm, wq_hbm, wk_hbm, wv_hbm))

    def word_row(pair, b):
        return 8 * (pair // 4) + 4 * b + pair % 4

    def kv_copies(pair):
        src = min(pair, H // 2 - 1) if isinstance(pair, int) else jnp.minimum(pair, H // 2 - 1)
        return [cp(w.at[:, word_row(src, b), :], wp_s.at[pair % 2, 2 * n + b], 16 + pair % 2)
                for n, w in enumerate((wk_hbm, wv_hbm)) for b in range(2)]

    late_copies = [cp(qa_hbm, x_w, 21)] + [
        cp(wo_hbm.at[:, pl.ds(128 * b, 128)], xs_w.at[pl.ds(H * CH * b, H * CH)], 6 + b) for b in range(2)]

    def extract(h, r0, o, shift, z):
        def block(n, kq, b):
            x = jnp.concatenate([wp_s[(h // 2) % 2 + z, 2 * n + b, pl.ds(256 * kq + r0 + e, 8, stride=2), :]
                                 for e in range(2)], axis=0)
            if isinstance(h, int):
                return _lo(x) if h % 2 == 0 else _hi(x)
            return _hi(x << jnp.concatenate([shift] * 2, axis=0))

        terms = [_join(t) for t in _inner_terms(
            _RHS, o, lambda n, m: block(n % 2, 2 * (n // 2) + m // 2, m % 2))]
        for i, t in enumerate(terms):
            wx_w[7 * o + i, r0 // 2:r0 // 2 + 8, :] = t
        return _digest(terms)

    def phase0():
        U1, U2, UX, UA, UB, UD = 1, 3, 10, 32, 60, 100
        LAG, LAG_U, LAG_T, BACK, BACK_W, SLACK = 12, 6, 4, 10, 4, 8
        cq = [cp(wq_hbm.at[:, word_row(g // 2, g % 2), :], y_s.at[pl.ds(C * g, C)],
                 (0, 35, 35, 19, 19, 1, 1, 1)[g] if g < 8 else 18) for g in range(H)]
        cx = [cp(x_hbm.at[:, pl.ds(512 * i, 512)], x_w.at[:, pl.ds(512 * i, 512)], 22 + i) for i in range(4)]
        ga = cq[5:8] + [cp(sk_hbm, sk_ref, 2), cp(ka_hbm, ka_w, 3), cp(va_hbm, va_w, 4)]
        gb = cq[8:] + [cp(c_hbm.at[:, pl.ds(128 * b, 128)], c_w.at[b], 8 + b) for b in range(8)]
        gd = [cp(d_hbm, d_ref, 20), cp(hk_hbm, hk_w, 5)] + kv_copies(0)
        zero = pl.semaphore_read(idle_sem)
        _start(cx[:1] + cq[:3] + cx[1:2] + cq[3:5] + cx[2:] + ga)
        never = _never(zero)
        due = []
        toks = []

        def gate(x):
            return _after(x, toks[-BACK], never)

        def w_terms(j, b):
            tok = toks[-BACK_W] if len(toks) >= BACK_W else None
            x = y_s[C * (2 * j + b):C * (2 * j + b + 1), :]
            g16 = jnp.concatenate([_after(jnp.full((8, 128), 16, U32), tok, never)] * (C // 8), axis=0)
            gm = jnp.concatenate([_after(jnp.full((8, 128), HI_MASK, U32), tok, never)] * (C // 8), axis=0)
            lo, hi = pltpu.bitcast(x << g16, F32), pltpu.bitcast(x & gm, F32)
            pad = jnp.zeros((256 - CH, 128), F32)
            blocks = [jnp.concatenate([t, pad], axis=0).T for t in (lo[:CH], hi[:CH], lo[CH:], hi[CH:])]
            for n, t in enumerate(blocks):
                for k in range(2):
                    wt_s[b, 2 * n + k] = t[:, 128 * k:128 * (k + 1)]
            quarter = [[jnp.concatenate([wt_s[b, 2 * n + k, pl.ds(e, 32, stride=4), :] for k in range(2)], axis=1)
                        for n in range(4)] for e in range(4)]
            terms = [_terms(_RHS, q) for q in quarter]
            out = []
            for i in range(7):
                ev, od = _pack(terms[0][i], terms[2][i]), _pack(terms[1][i], terms[3][i])
                rows = [w[8 * m:8 * (m + 1)] for m in range(4) for w in (ev, od)]
                out.append(pltpu.bitcast(jnp.concatenate(rows, axis=0), BF16))
            return out

        def x_terms(jp):
            top = slice(256 * jp, 256 * jp + 128)
            bot = slice(256 * jp + 128, 256 * jp + 256)
            for i in range(7):
                xs_s[256 * (NP * i + jp) + CH:256 * (NP * i + jp + 1), :] = jnp.zeros((256 - CH, 128), BF16)
            for r in range(0, CH // 2, 16):
                lo, hi = slice(r, r + 16), slice(CH // 2 + r, CH // 2 + r + 16)
                blocks = [x_w[lo, top], x_w[hi, top], x_w[lo, bot], x_w[hi, bot]]
                terms = [_join(t) for t in _terms(_LHS, [_split(t) for t in blocks])]
                terms[2], terms[3] = blocks[0], blocks[3]
                for i, t in enumerate(terms):
                    xs_w[128 * (NP * i + jp) + r:128 * (NP * i + jp) + r + 16, :] = t
                yield 1, _digest(terms), LAG

        def column(row):
            row = jnp.concatenate([row.astype(F32), jnp.zeros((1, 512 - C), F32)], axis=1)
            return jnp.broadcast_to(row, (128, 512)).T

        def delayed(ref, rows, sg, n):
            cur = pltpu.bitcast(ref[rows, 128 * sg:128 * (sg + 1)], U32)
            lane = jnp.concatenate([gate(lax.broadcasted_iota(I32, (8, 128), 1))] * (cur.shape[0] // 8), axis=0)
            prev = pltpu.bitcast(ref[rows, 128 * (sg - 1):128 * sg], U32) if sg > 0 else jnp.uint32(0)
            x = pltpu.roll(jnp.where(lane < 128 - n, cur, prev), n, 1)
            return pltpu.bitcast(x, BF16).astype(F32)

        def transposed(x):
            return jnp.concatenate([gate(x[:8]), x[8:]], axis=0).T

        def conv_inputs():
            taps = [column(sk_ref[j:j + 1, :]) for j in range(4)]
            for b in range(4):
                for r0 in range(128 * b, min(C, 128 * (b + 1)), 32):
                    rows = slice(r0, r0 + 32)
                    tp = [t[rows] for t in taps]
                    prev = jnp.zeros((32, 128), F32)
                    for sg in range(NB):
                        cols = slice(128 * sg, 128 * (sg + 1))
                        ksh = ((delayed(ka_s, rows, sg, 3) * tp[3] + delayed(ka_s, rows, sg, 2) * tp[2])
                               + (delayed(ka_s, rows, sg, 1) * tp[1] + ka_s[rows, cols].astype(F32) * tp[0]))
                        kv = ksh * va_s[rows, cols].astype(F32)
                        wrd = _pack(prev, kv)
                        sa_s[C * sg + r0:C * sg + r0 + 32, :] = pltpu.bitcast(wrd, F32)
                        prev = kv
                        yield 2, _digest([wrd]), LAG_U
                for sg in range(NB):
                    r0 = C * sg + 128 * b
                    if b < 3:
                        wrd = sa_s[r0:r0 + 128, :]
                    else:
                        wrd = jnp.concatenate([sa_s[r0:r0 + C - 384, :], jnp.zeros((512 - C, 128), F32)], axis=0)
                    wrd = transposed(pltpu.bitcast(wrd, U32))
                    sb_s[S * b + 128 * sg:S * b + 128 * (sg + 1), :] = pltpu.bitcast(wrd, F32)
                    yield 4, wrd[120:], LAG_T
                for p in range(8):
                    for j in range(8):
                        parts = [jnp.zeros((16, 128), U32) if sg < 0 else
                                 pltpu.bitcast(sb_s[pl.ds(S * b + 128 * sg + 16 * p, 16), :], U32)
                                 for sg in range(2 * j - 6, 2 * j + 2)]
                        plane = 32 * (j // 4) + 4 * p + j % 4
                        win = transposed(jnp.concatenate(parts, axis=0))
                        aw_s[pl.ds(plane * PITCH + 128 * b, 128), :] = win
                        yield 4, win[120:], LAG_T

        def conv_filter_and_first_head():
            dc_s[...] = column(d_ref[...].reshape(1, C))
            lane = lax.broadcasted_iota(I32, (32, 128), 1)
            for r0 in range(0, C, 32):
                rows = slice(r0, r0 + 32)
                for a in range(NB):
                    hf = hk_s[rows, 128 * a:128 * (a + 1)].astype(F32)
                    hs = delayed(hk_s, rows, a, 1)
                    if a == 0:
                        hf = jnp.where(lane == 0, hf + dc_s[rows, :], hf)
                        hs = jnp.where(lane == 1, hs + dc_s[rows, :], hs)
                    wrd = _pack(hf, hs)
                    g_s[a, rows, :] = wrd
                    yield 1, _digest([wrd]), LAG
            for r0 in range(0, 256, 16):
                for o in range(7):
                    yield 1, extract(0, r0, o, None, zero * (o + 1)), LAG

        def c_terms():
            for ck in range(4):
                for half in range(2):
                    for r0 in range(0, 128, 16):
                        for o in range(7):
                            def block(n, m):
                                row = 256 * ck + 128 * (n // 2) + 64 * (m // 2) + 16 * (r0 // 32)
                                col = 4 * (n % 2) + 2 * (m % 2) + half + zero * (o + 1)
                                w = jnp.concatenate([c_w[col, pl.ds(row + e, 8, stride=2), :] for e in range(2)],
                                                    axis=0)
                                return _hi(w) if r0 % 32 else _lo(w)

                            terms = [_join(t) for t in _inner_terms(_LHS, o, block)]
                            for i, t in enumerate(terms):
                                cs_w[ck, 7 * o + i, half, r0 // 2:r0 // 2 + 8, :] = t
                            yield 1, _digest(terms), LAG

        units = [(g, jp) for g in range(3) for jp in (0, 1)] + [(g, jp) for g in range(3) for jp in (2, 3)]
        units += [(g, jp) for g in (3, 4) for jp in range(4)] + [(g, jp) for g in range(5) for jp in range(4, NP)]
        units += [(g, jp) for g in range(5, H) for jp in range(NP)]
        last = 7 * len(units) - 2 - LAG
        streams = [[(v for jp in (2, 3) for v in x_terms(jp)), 14, 7 * U2 + 1, 7 * 6 - 1, 0],
                   [(v for jp in range(4, NP) for v in x_terms(jp)), 28, 7 * UX + 2, 7 * 20 - 1 - LAG, 0],
                   [conv_inputs(), 2 * 14 * NB + 4 * 4 * (NB + 64), 7 * UA + SLACK, 7 * UD + SLACK, 0],
                   [c_terms(), 448, 7 * UB + SLACK, last, 0],
                   [conv_filter_and_first_head(), 14 * NB + 112, 7 * UD + SLACK, last, 0]]
        later = {}

        def pump():
            n = len(toks)
            for st in streams:
                want = min(st[1], max(0, (n - st[2] + 1) * st[1] // (st[3] - st[2])))
                while st[4] < want:
                    cost, v, lag = next(st[0])
                    later.setdefault(n + lag, []).append(v)
                    st[4] += cost
            due.extend(later.pop(n, []))

        starts = {UX: gb, UA: gd, UB: kv_copies(1)}
        waits = {U1: cq[1:3], U2: cx[1:2], UX: cq[3:5] + cx[2:], UA: ga, UB: gb, UD: gd}
        _wait(cx[:1])
        list(x_terms(0))
        list(x_terms(1))
        _wait(cq[:1])
        wts = {}
        for u, (g, jp) in enumerate(units):
            _start(starts.get(u, []))
            _wait(waits.get(u, []))
            for g_ in range(H):
                if g_ not in wts and units.index((g_, 0)) - (4 if g_ >= 5 else 1) <= u:
                    wts[g_] = w_terms(g_ // 2, g_ % 2)

            def prod(i):
                pump()
                m = _dot(_tied(wts[g][i], due, never), xs_s[256 * (NP * i + jp):256 * (NP * i + jp + 1), :])
                toks.append(m[:8])
                return m

            def emit(r, c, val):
                qc_w[2 * (g // 2) + c, 2 * jp + r, 64 * (g % 2):64 * (g % 2 + 1), :] = _join32(val * QSCALE)

            _strassen(prod, emit)
        assert all(st[4] == st[1] for st in streams) and not later

    phase0()
    _start(late_copies)

    def head(h, carry):
        @pl.when(h % 2 == 1)
        def _():
            _wait(kv_copies((h + 1) // 2))
            _start(kv_copies((h + 3) // 2))

        zero = h // H
        toks = []
        due = []
        lane8 = lax.broadcasted_iota(I32, (8, 128), 1)
        sub8 = lax.broadcasted_iota(I32, (8, 128), 0)
        lane16 = lax.broadcasted_iota(I32, (16, 128), 1)
        sub16 = lax.broadcasted_iota(I32, (16, 128), 0)
        tri = (lax.broadcasted_iota(I32, (128, 128), 0) <= lax.broadcasted_iota(I32, (128, 128), 1))
        h_next = h + 1
        never = _never(zero)

        def tied(lhs):
            return _tied(lhs, due, never)

        def chan_mm(c):
            m_b = lane8 < _after(128 - 2 * sub8, toks[-5] if len(toks) >= 5 else None, never)
            gs = [jnp.broadcast_to(g_s[a, pl.ds(c, 1), :], (8, 128)) for a in range(NB)]
            bt = [pltpu.roll(jnp.where(m_b, gs[a], gs[a - 1] if a > 0 else jnp.uint32(0)), 0, 1,
                             stride=2, stride_axis=0) for a in range(NB)]
            b1 = pltpu.bitcast(jnp.concatenate(bt[7::-1], axis=0), BF16)
            b2 = pltpu.bitcast(jnp.concatenate(bt[15:7:-1], axis=0), BF16)
            am = pltpu.bitcast(aw_s[pl.ds(c, 64, stride=PITCH), :], BF16)
            z1 = _dot(tied(am), b1)
            z2 = _dot(am[:64], b2)
            return c, z1[:64], z1[64:] + z2

        def chan_post(c, zlo, zhi):
            acc = car = None
            for p in range(8):
                z = jnp.concatenate([zlo[8 * p:8 * p + 8], zhi[8 * p:8 * p + 8]], axis=0)
                if p == 0:
                    acc = z
                else:
                    z = pltpu.roll(z, 16 * p, 1)
                    cz = jnp.where(lane16 < 16 * p, z, 0.0)
                    acc = acc + z
                    car = cz if car is None else car + cz
            y = (acc - car) + jnp.where(sub16 > 0, pltpu.roll(car, 1, 0), 0.0)
            y_s[pl.ds(c, NB, stride=PITCH), :] = pltpu.bitcast(y, U32)

        def next_weights():
            for r0 in range(0, 256, 16):
                for o in (0, 1, 3, 4, 6, 2, 5):
                    shift = jnp.full((8, 128), (1 - h_next % 2) * 16, I32).astype(U32)
                    yield extract(h_next, r0, o, shift, zero * (o + 1))

        weights, done, clock = next_weights(), [0], [0]

        def tick(cycles):
            while done[0] < min(112, max(0, (clock[0] - 1500) * 112 // 6080)):
                due.append(next(weights))
                done[0] += 1
            clock[0] += cycles

        def kv_chunk(ck):
            def prod(o):
                out = {}
                for r0 in (0, 64):
                    def inner(i):
                        lhs = jnp.concatenate([cs_s[ck, 7 * o + i, k, r0:r0 + 64, :] for k in range(2)], axis=1)
                        m = _dot(tied(lhs), wx_s[7 * o + i])
                        if i == 3 and r0 == 0:
                            toks.append(m[:8])
                        return m

                    _strassen(inner, lambda r, n, val: out.__setitem__((r, n, r0), val))
                return jnp.concatenate([jnp.concatenate([out[r, 0, r0], out[r, 1, r0]], axis=1)
                                        for r in range(2) for r0 in (0, 64)], axis=0)

            def emit(r, n, val):
                jp = 2 * ck + r
                if n == 0:
                    if jp < NP - 1:
                        blocks = [val[:128, :128], val[:128, 128:], val[128:, :128], val[128:, 128:]]
                        for i in _SUMS:
                            kt_w[i, jp] = _join32(_term(_LHS, i, blocks.__getitem__))
                    for k in range(2):
                        k_w[k, 128 * jp:128 * (jp + 1), :] = _join32(val[:, 128 * k:128 * (k + 1)])
                else:
                    blocks = [val[128 * t:128 * (t + 1), 128 * k:128 * (k + 1)].T
                              for k in range(2) for t in range(2)]
                    outs = [v.astype(BF16) for v in blocks]
                    for m, v in enumerate(outs):
                        vt_s[2 * jp + m % 2, 128 * (m // 2):128 * (m // 2 + 1), :] = v
                    if jp < NP - 1:
                        for i in _SUMS:
                            vx_s[i, jp] = _term(_LHS, i, blocks.__getitem__).astype(BF16)

            return _strassen_steps(prod, emit)

        kv = [kv_chunk(ck) for ck in range(4)]
        lse, pr = {}, {}

        def s_at(u, r0):
            first = [v for v in range(u) if (v // 4) % 2 == (u // 4) % 2]
            return (sa_s, sb_s)[(u // 4) % 2], 128 * sum(v + 1 for v in first) + r0

        def qk(jq):
            run = [None, None]

            def put(n, r0, val):
                buf, row = s_at(2 * jq + n, r0)
                buf[row:row + 64, :] = val
                vs = [val[r:r + 8] for r in range(0, 64, 8)]
                m = _fold(jnp.maximum, vs)
                if run[n] is not None:
                    m = jnp.maximum(m, run[n][0])
                l = _fold(jnp.add, [jnp.exp2(v - m) for v in vs])
                if run[n] is not None:
                    l = l + run[n][1] * jnp.exp2(run[n][0] - m)
                run[n] = (m, l)

            if jq > 0:
                qt = _word_terms(_RHS, [qc_w[h, 2 * jq + n % 2, 64 * (n // 2):64 * (n // 2 + 1), :]
                                        for n in range(4)])
            for jp in range(jq):
                for r0 in (0, 64):
                    def prod(i):
                        if i == 2:
                            lhs = k_s[0, 256 * jp + r0:256 * jp + r0 + 64, :]
                        elif i == 3:
                            lhs = k_s[1, 256 * jp + 128 + r0:256 * jp + 128 + r0 + 64, :]
                        else:
                            lhs = kt_s[i, jp, r0:r0 + 64, :]
                        m = _dot(tied(lhs), qt[i])
                        if i == 3 and r0 == 0:
                            toks.append(m[:8])
                        return m

                    _strassen(prod, lambda r, n, val: put(n, 256 * jp + 128 * r + r0, val))
            q0 = 256 * jq
            for n in range(2):
                rows = slice(q0, q0 + 128 * (n + 1))
                sd = _dot(tied(jnp.concatenate([k_s[0, rows, :], k_s[1, rows, :]], axis=1)), qc_s[h, 2 * jq + n])
                last = jnp.where(tri, sd[128 * n:], NEG)
                sd = jnp.concatenate([sd[:128], last], axis=0) if n else last
                for r0 in range(0, 128 * (n + 1), 64):
                    put(n, q0 + r0, sd[r0:r0 + 64])
            toks.append(sd[:8])
            for n in range(2):
                m, l = run[n]
                top = jnp.max(m, axis=0, keepdims=True)
                lse[2 * jq + n] = top + jnp.log2(jnp.sum(l * jnp.exp2(m - top), axis=0, keepdims=True))

        def probs(u, r0):
            buf, row = s_at(u, r0)
            x = jnp.concatenate([buf[pl.ds(row + e + zero, 8, stride=4), :] for e in (0, 2)], axis=0)
            return jnp.exp2(x - lse[u])

        def softmax(jq, jps, deadline):
            starts = [r + e for r in range(0, 256, 32) for e in range(2)]
            for jp in jps:
                if jp == jq:
                    out = [jnp.concatenate([_join(probs(2 * jq + n, 256 * jq + r)) for r in starts[:8 * (n + 1)]],
                                           axis=0) for n in range(2)]
                else:
                    parts = []
                    for r in starts[:8]:
                        blocks = [probs(2 * jq + m % 2, 256 * jp + 128 * (m // 2) + r) for m in range(4)]
                        parts.append([_join(t) for t in _terms(_RHS, blocks)])
                    out = [jnp.concatenate([p[i] for p in parts], axis=0) for i in range(7)]
                pr[jq, jp] = out
                if deadline:
                    due.append(_digest(out[:1]) ^ _digest(out[1:]) if jp == jq else _digest(out))

        def pv(jq):
            softmax(jq, [jp for jp in range(jq + 1) if (jq, jp) not in pr], False)
            diag = pr.pop((jq, jq))
            ps = [pr.pop((jq, jp)) for jp in range(jq)]
            base = []
            for n in range(2):
                tick(64 * (n + 1))
                vt = jnp.concatenate([vt_s[2 * jq + i] for i in range(n + 1)], axis=1)
                base.append(_dot(tied(vt), pltpu.bitcast(diag[n], BF16)))

            def emit(r, n, val):
                val = base[n][128 * r:128 * (r + 1)] if val is None else val + base[n][128 * r:128 * (r + 1)]
                qc_s[h, 2 * jq + n, 128 * r:128 * (r + 1), :] = val.astype(BF16)

            def prod(i):
                tick(32 * jq)
                if i == 2:
                    lhs = [vt_s[2 * jp, 0:128, :] for jp in range(jq)]
                elif i == 3:
                    lhs = [vt_s[2 * jp + 1, 128:256, :] for jp in range(jq)]
                else:
                    lhs = [vx_s[i, jp] for jp in range(jq)]
                rhs = pltpu.bitcast(jnp.concatenate([p[i] for p in ps], axis=0), BF16)
                return _dot(tied(jnp.concatenate(lhs, axis=1)), rhs)

            if jq:
                _strassen(prod, emit)
            else:
                for r in range(2):
                    for n in range(2):
                        emit(r, n, None)

        chans = [h * CPH + i for i in range(CPH)]
        pend = []
        for step in HEAD_STEPS.split():
            kind, arg = step[0], [int(x) for x in step[1:]]
            if kind == 'E':
                softmax(arg[0], arg[1:] or range(arg[0] + 1), True)
                continue
            old, pend = pend, []
            if kind == 'C':
                pend = [chan_mm(chans.pop(0)) for _ in range(arg[0])]
            elif kind == 'M':
                for o in arg[1:]:
                    kv[arg[0]](o)
            else:
                for jq in arg:
                    (qk if kind == 'Q' else pv)(jq)
            for args in old:
                chan_post(*args)
        assert done[0] == 112 and not (chans or pend or due or pr)
        return carry + zero

    zero_end = lax.fori_loop(0, H, head, 0)

    _wait(late_copies + kv_copies(H // 2 + 1))
    HH = H // 2

    def wo_block(rh, kh):
        rows = [(C * (H * b + h) + CH * rh) // 2 for h in range(HH * kh, HH * (kh + 1)) for b in range(2)]
        return jnp.concatenate([xs_w[r:r + CH // 2, :] for r in rows], axis=1)

    wt = _word_terms(_RHS, [wo_block(0, 0), wo_block(1, 0), wo_block(0, 1), wo_block(1, 1)])
    outs = []
    due, late = [], []
    never = _never(zero_end)

    def put(t, b, z, opaque=False):
        z = z.T
        r0 = pl.multiple_of(zero_end * 16 + 128 * t, 16) if opaque else 128 * t
        out_s[pl.ds(r0, 128), 128 * b:128 * (b + 1)] = z.astype(BF16)
        late.append(z[120:])

    for jp in range(NP):
        ct = _word_terms(_LHS, [jnp.concatenate([qc_w[h, 2 * jp + r] for h in range(HH * kh, HH * (kh + 1))], axis=0)
                                for r in range(2) for kh in range(2)])
        za = {}
        dues = {3: list(late)}
        late.clear()
        for r in range(2):
            t = 2 * jp + r
            za[r] = (pltpu.bitcast(y_s[t * PITCH:t * PITCH + C, :], F32)
                     * x_s[:, 128 * t:128 * (t + 1)].astype(F32))
            for b in range(3):
                put(t, b, za[r][128 * b:128 * (b + 1)], opaque=(r == 0 and b == 0 and jp > 0))
        dues[6] = list(late)
        late.clear()
        res = {}
        step = _strassen_steps(lambda i: _dot(_tied(wt[i], due, never), ct[i]),
                               lambda r, c, val: res.__setitem__((r, c), val))
        for n, i in enumerate((1, 4, 3, 6, 0, 2, 5)):
            due.extend(dues.get(n, []))
            step(i)
        for r in range(2):
            z = jnp.concatenate([za[r][384:], res[r, 0], res[r, 1]], axis=0)
            for b in range(4):
                put(2 * jp + r, 3 + b, z[128 * b:128 * (b + 1)])
        rows = pl.ds(256 * jp, 256)
        outs.append(cp(out_s.at[rows], o_hbm.at[rows], 26 + jp))
        outs[-1].start()
    _wait(outs)


def _tiles(w):
    rows = w.shape[0]
    return w.reshape(rows, 2, 8, 2, 128).transpose(0, 1, 3, 2, 4).reshape(rows, 32, 128)


@jax.jit
def pallas_concat_heads__ssm_conv_h3__compressed_kv_cla__prompt_kernel(
    A_q: jax.Array,
    A_k: jax.Array,
    A_v: jax.Array,
    A_shift_k: jax.Array,
    A_ssm_k: jax.Array,
    A_ssm_D: jax.Array,
    B_x: jax.Array,
    B_c_kv: jax.Array,
    B_w_q: jax.Array,
    B_w_uk: jax.Array,
    B_w_uv: jax.Array,
    B_w_o: jax.Array,
):
    hbm = pl.BlockSpec(memory_space=pltpu.HBM)
    out = pl.pallas_call(
        _kernel,
        in_specs=[hbm] * 12,
        out_specs=hbm,
        out_shape=jax.ShapeDtypeStruct((S, 2 * C), BF16),
        scratch_shapes=[
            pltpu.VMEM((8, S // 2, 128), U32),
            pltpu.VMEM((4, 49, 2, 64, 128), U32),
            pltpu.VMEM((2, 4, DC, 128), U32),
            pltpu.VMEM((H, NB, D // 2, 128), U32),
            pltpu.VMEM((64 * PITCH, 128), U32),
            pltpu.VMEM((NB, C, 128), U32),
            pltpu.VMEM((NB * PITCH, 128), U32),
            pltpu.VMEM((CH, S), U32),
            pltpu.VMEM((512, 128), F32),
            pltpu.VMEM((2, S // 2, 128), U32),
            pltpu.VMEM((7, NP, 64, 128), U32),
            pltpu.VMEM((NB, D // 2, 128), U32),
            pltpu.VMEM((7, NP, 64, 128), U32),
            pltpu.VMEM((49, DC // 8, 128), U32),
            pltpu.VMEM((NB * C, 128), F32),
            pltpu.VMEM((84 * 128, 128), F32),
            pltpu.VMEM((CH, S), U32),
            pltpu.VMEM((7 * NP * 128, 128), U32),
            pltpu.VMEM((CH, S), U32),
            pltpu.VMEM((CH, S), U32),
            pltpu.VMEM((2, 8, 128, 128), F32),
            pltpu.VMEM((S, 2 * C), BF16),
            pltpu.VMEM((4, C), BF16),
            pltpu.VMEM((C,), BF16),
            pltpu.SemaphoreType.REGULAR,
            pltpu.SemaphoreType.DMA((36,)),
        ],
        compiler_params=pltpu.CompilerParams(vmem_limit_bytes=127 * 2 ** 20, disable_semaphore_checks=True),
    )(
        A_q[0].T, A_k[0].T, A_v[0].T, A_shift_k.T, A_ssm_k, A_ssm_D, B_x[0].T, B_c_kv[0],
        _tiles(B_w_q), _tiles(B_w_uk), _tiles(B_w_uv),
        jnp.swapaxes(B_w_o, 1, 2).reshape(H * C, D),
    )
    return out.reshape(1, S, 2 * C)
```

```python
import math

import jax
import jax.numpy as jnp
from jax import lax
import jax.experimental.pallas as pl
import jax.experimental.pallas.tpu as pltpu

F32 = jnp.float32
BF16 = jnp.bfloat16
U32 = jnp.uint32
I32 = jnp.int32

S = 2048
C = 448
H = 16
D = 256
DC = 1024
NB = S // 128
NP = NB // 2
CH = C // 2
PITCH = 520
CPH = C // H
LOG2E = math.log2(math.e)
QSCALE = (D ** -0.5) * LOG2E
NEG = -1e9 * LOG2E
HI_MASK = 0xFFFF0000

HEAD_STEPS = ("M001 C2 M034 C2 M06 M101 C2 Q01 M134 C2 M16 M201 C2 Q23 M234 C2 M26 M301 C2 E0 E1 E2 Q45 M334 C2 "
              "M36 E3 M02 C2 Q67 M05 C2 M12 C2 E4 M15 C2 E5012 M22 C2 E5345 M25 C2 M32 E6012 M35 E63456 P01234567")


def _dot(a, b):
    return jnp.dot(a, b, preferred_element_type=F32)


def _lo(x):
    return pltpu.bitcast(x << 16, F32)


def _hi(x):
    return pltpu.bitcast(x & jnp.uint32(HI_MASK), F32)


def _pack(even, odd):
    return pltpu.pack_elementwise([even, odd], packed_dtype=BF16).astype(U32)


def _split(words):
    return jnp.concatenate([_lo(words), _hi(words)], axis=0)


def _join(x):
    n = x.shape[0] // 2
    return _pack(x[:n], x[n:])


def _join32(x):
    return jnp.concatenate([_pack(x[m:m + 16], x[m + 16:m + 32]) for m in range(0, x.shape[0], 32)], axis=0)


_LHS = ((0, 1, 3), (2, 1, 3), (0,), (3,), (0, 1, 1), (2, -1, 0), (1, -1, 3))
_RHS = ((0, 1, 3), (0,), (1, -1, 3), (2, -1, 0), (3,), (0, 1, 1), (2, 1, 3))
_SUMS = (0, 1, 4, 5, 6)


def _term(table, i, block):
    spec = table[i]
    if len(spec) == 1:
        return block(spec[0])
    return block(spec[0]) + block(spec[2]) if spec[1] > 0 else block(spec[0]) - block(spec[2])


def _terms(table, blocks):
    return [_term(table, i, blocks.__getitem__) for i in range(7)]


def _word_terms(table, words):
    full = [_split(w) for w in words]
    return [pltpu.bitcast(words[table[i][0]] if len(table[i]) == 1
                          else _join(_term(table, i, full.__getitem__)), BF16) for i in range(7)]


def _inner_terms(table, o, block):
    return _terms(table, [_term(table, o, lambda n: block(n, m)) for m in range(4)])


def _strassen_steps(prod, emit):
    uses = {(0, 0): {0: 1, 3: 1, 4: -1, 6: 1}, (0, 1): {2: 1, 4: 1},
            (1, 0): {1: 1, 3: 1}, (1, 1): {0: 1, 1: -1, 2: 1, 5: 1}}
    acc = {}
    neg = {}

    def step(i):
        m = prod(i)
        for key, terms in uses.items():
            if i not in terms:
                continue
            sign = terms.pop(i)
            if key not in acc:
                acc[key] = m
                neg[key] = sign < 0
            elif neg[key]:
                assert sign > 0
                acc[key] = m - acc[key]
                neg[key] = False
            else:
                acc[key] = acc[key] + m if sign > 0 else acc[key] - m
            if not terms:
                emit(key[0], key[1], acc.pop(key))

    return step


def _strassen(prod, emit, order=(0, 1, 3, 2, 4, 5, 6)):
    step = _strassen_steps(prod, emit)
    for i in order:
        step(i)


def _never(zero):
    return lax.broadcasted_iota(I32, (8, 128), 1) < zero


def _after(x, tok, never):
    if tok is None:
        return x
    return jnp.where(never, pltpu.bitcast(tok, x.dtype), x)


def _tied(lhs, due, never):
    if not due:
        return lhs
    t = None
    for d in due:
        d = pltpu.bitcast(jnp.broadcast_to(d, (8, 128)), U32)
        t = d if t is None else t ^ d
    due.clear()
    x = pltpu.bitcast(_after(pltpu.bitcast(lhs[:16, :128], U32), t, never), BF16)
    if lhs.shape[1] > 128:
        x = jnp.concatenate([x, lhs[:16, 128:]], axis=1)
    return jnp.concatenate([x, lhs[16:]], axis=0)


def _digest(words):
    acc = None
    for r in range(words[0].shape[0] // 8):
        for w in words:
            w = w[8 * r:8 * (r + 1)]
            acc = w if acc is None else acc ^ w
    return acc


def _fold(op, xs):
    accs = list(xs[:2])
    for k, x in enumerate(xs[2:]):
        accs[k % 2] = op(accs[k % 2], x)
    return op(accs[0], accs[1])


class _Packed:
    def __init__(self, ref):
        self.ref = ref

    def _index(self, idx):
        idx = idx if isinstance(idx, tuple) else (idx,)
        axis = len(self.ref.shape) - 2
        if len(idx) <= axis:
            return idx + (slice(None),) * (axis + 2 - len(idx))
        r = idx[axis]
        r = slice(None if r.start is None else r.start // 2, None if r.stop is None else r.stop // 2)
        return idx[:axis] + (r,) + idx[axis + 1:]

    def __getitem__(self, idx):
        return pltpu.bitcast(self.ref[self._index(idx)], BF16)

    def __setitem__(self, idx, val):
        self.ref[self._index(idx)] = pltpu.bitcast(val, U32)


def _start(copies):
    for c_ in copies:
        c_.start()


def _wait(copies):
    for c_ in copies:
        c_.wait()


def _kernel(qa_hbm, ka_hbm, va_hbm, sk_hbm, hk_hbm, d_hbm, x_hbm, c_hbm, wq_hbm, wk_hbm, wv_hbm, wo_hbm,
            o_hbm,
            c_w, cs_w, wp_s, qc_w, aw_s, g_s, y_s, hk_w, dc_s, k_w, kt_w, vt_w, vx_w, wx_w, sa_s, sb_s,
            x_w, xs_w, ka_w, va_w, wt_s, out_s, sk_ref, d_ref, sems):
    def cp(src, dst, i):
        return pltpu.make_async_copy(src, dst, sems.at[i])

    cs_s, qc_s, k_s, kt_s, vt_s, vx_s, wx_s, xs_s, x_s, ka_s, va_s, hk_s = (
        _Packed(r) for r in (cs_w, qc_w, k_w, kt_w, vt_w, vx_w, wx_w, xs_w, x_w, ka_w, va_w, hk_w))
    qa_hbm, ka_hbm, va_hbm, hk_hbm, x_hbm, c_hbm, wo_hbm, wq_hbm, wk_hbm, wv_hbm = (
        r.bitcast(U32)
        for r in (qa_hbm, ka_hbm, va_hbm, hk_hbm, x_hbm, c_hbm, wo_hbm, wq_hbm, wk_hbm, wv_hbm))

    def word_row(pair, b):
        return 8 * (pair // 4) + 4 * b + pair % 4

    def kv_copies(pair):
        src = min(pair, H // 2 - 1) if isinstance(pair, int) else jnp.minimum(pair, H // 2 - 1)
        return [cp(w.at[:, word_row(src, b), :], wp_s.at[pair % 2, 2 * n + b], 16 + pair % 2)
                for n, w in enumerate((wk_hbm, wv_hbm)) for b in range(2)]

    late_copies = [cp(qa_hbm, x_w, 21)] + [
        cp(wo_hbm.at[:, pl.ds(128 * b, 128)], xs_w.at[pl.ds(H * CH * b, H * CH)], 6 + b) for b in range(2)]

    def extract(h, r0, o, shift, z):
        def block(n, kq, b):
            x = jnp.concatenate([wp_s[(h // 2) % 2 + z, 2 * n + b, pl.ds(256 * kq + r0 + e, 8, stride=2), :]
                                 for e in range(2)], axis=0)
            if isinstance(h, int):
                return _lo(x) if h % 2 == 0 else _hi(x)
            return _hi(x << jnp.concatenate([shift] * 2, axis=0))

        terms = [_join(t) for t in _inner_terms(
            _RHS, o, lambda n, m: block(n % 2, 2 * (n // 2) + m // 2, m % 2))]
        for i, t in enumerate(terms):
            wx_w[7 * o + i, r0 // 2:r0 // 2 + 8, :] = t
        return _digest(terms)

    def phase0():
        U1, U2, UX, UA, UB, UD = 1, 3, 10, 33, 60, 98
        LAG, LAG_U, LAG_T, BACK, BACK_W, SLACK = 12, 8, 4, 8, 6, 12
        cq = [cp(wq_hbm.at[:, word_row(g // 2, g % 2), :], y_s.at[pl.ds(C * g, C)],
                 (0, 35, 35, 19, 19, 1, 1, 1)[g] if g < 8 else 18) for g in range(H)]
        cx = [cp(x_hbm.at[:, pl.ds(512 * i, 512)], x_w.at[:, pl.ds(512 * i, 512)], 22 + i) for i in range(4)]
        ga = cq[5:8] + [cp(sk_hbm, sk_ref, 2), cp(ka_hbm, ka_w, 3), cp(va_hbm, va_w, 4)]
        gb = cq[8:] + [cp(c_hbm.at[:, pl.ds(128 * b, 128)], c_w.at[b], 8 + b) for b in range(8)]
        gd = [cp(d_hbm, d_ref, 20), cp(hk_hbm, hk_w, 5)] + kv_copies(0)
        _start(cx[:1] + cq[:3] + cx[1:2] + cq[3:5] + cx[2:] + ga)
        zero = lax.fori_loop(0, H, lambda i, z: z + i // H, 0)
        never = _never(zero)
        due = []
        toks = []

        def gate(x):
            return _after(x, toks[-BACK], never)

        def w_terms(j, b):
            tok = toks[-BACK_W] if len(toks) >= BACK_W else None
            x = y_s[C * (2 * j + b):C * (2 * j + b + 1), :]
            g16 = jnp.concatenate([_after(jnp.full((8, 128), 16, U32), tok, never)] * (C // 8), axis=0)
            gm = jnp.concatenate([_after(jnp.full((8, 128), HI_MASK, U32), tok, never)] * (C // 8), axis=0)
            lo, hi = pltpu.bitcast(x << g16, F32), pltpu.bitcast(x & gm, F32)
            pad = jnp.zeros((256 - CH, 128), F32)
            blocks = [jnp.concatenate([t, pad], axis=0).T for t in (lo[:CH], hi[:CH], lo[CH:], hi[CH:])]
            for n, t in enumerate(blocks):
                for k in range(2):
                    wt_s[b, 2 * n + k] = t[:, 128 * k:128 * (k + 1)]
            quarter = [[jnp.concatenate([wt_s[b, 2 * n + k, pl.ds(e, 32, stride=4), :] for k in range(2)], axis=1)
                        for n in range(4)] for e in range(4)]
            terms = [_terms(_RHS, q) for q in quarter]
            out = []
            for i in range(7):
                ev, od = _pack(terms[0][i], terms[2][i]), _pack(terms[1][i], terms[3][i])
                rows = [w[8 * m:8 * (m + 1)] for m in range(4) for w in (ev, od)]
                out.append(pltpu.bitcast(jnp.concatenate(rows, axis=0), BF16))
            return out

        def x_terms(jp):
            top = slice(256 * jp, 256 * jp + 128)
            bot = slice(256 * jp + 128, 256 * jp + 256)
            for i in range(7):
                xs_s[256 * (NP * i + jp) + CH:256 * (NP * i + jp + 1), :] = jnp.zeros((256 - CH, 128), BF16)
            for r in range(0, CH // 2, 16):
                lo, hi = slice(r, r + 16), slice(CH // 2 + r, CH // 2 + r + 16)
                blocks = [x_w[lo, top], x_w[hi, top], x_w[lo, bot], x_w[hi, bot]]
                terms = [_join(t) for t in _terms(_LHS, [_split(t) for t in blocks])]
                terms[2], terms[3] = blocks[0], blocks[3]
                for i, t in enumerate(terms):
                    xs_w[128 * (NP * i + jp) + r:128 * (NP * i + jp) + r + 16, :] = t
                yield 1, _digest(terms), LAG

        def column(row):
            row = jnp.concatenate([row.astype(F32), jnp.zeros((1, 512 - C), F32)], axis=1)
            return jnp.broadcast_to(row, (128, 512)).T

        def delayed(ref, rows, sg, n):
            cur = pltpu.bitcast(ref[rows, 128 * sg:128 * (sg + 1)], U32)
            lane = jnp.concatenate([gate(lax.broadcasted_iota(I32, (8, 128), 1))] * (cur.shape[0] // 8), axis=0)
            prev = pltpu.bitcast(ref[rows, 128 * (sg - 1):128 * sg], U32) if sg > 0 else jnp.uint32(0)
            x = pltpu.roll(jnp.where(lane < 128 - n, cur, prev), n, 1)
            return pltpu.bitcast(x, BF16).astype(F32)

        def transposed(x):
            return jnp.concatenate([gate(x[:8]), x[8:]], axis=0).T

        def conv_inputs():
            taps = [column(sk_ref[j:j + 1, :]) for j in range(4)]
            for b in range(4):
                for r0 in range(128 * b, min(C, 128 * (b + 1)), 32):
                    rows = slice(r0, r0 + 32)
                    tp = [t[rows] for t in taps]
                    prev = jnp.zeros((32, 128), F32)
                    for sg in range(NB):
                        cols = slice(128 * sg, 128 * (sg + 1))
                        ksh = ((delayed(ka_s, rows, sg, 3) * tp[3] + delayed(ka_s, rows, sg, 2) * tp[2])
                               + (delayed(ka_s, rows, sg, 1) * tp[1] + ka_s[rows, cols].astype(F32) * tp[0]))
                        kv = ksh * va_s[rows, cols].astype(F32)
                        wrd = _pack(prev, kv)
                        sa_s[C * sg + r0:C * sg + r0 + 32, :] = pltpu.bitcast(wrd, F32)
                        prev = kv
                        yield 2, _digest([wrd]), LAG_U
                for sg in range(NB):
                    r0 = C * sg + 128 * b
                    if b < 3:
                        wrd = sa_s[r0:r0 + 128, :]
                    else:
                        wrd = jnp.concatenate([sa_s[r0:r0 + C - 384, :], jnp.zeros((512 - C, 128), F32)], axis=0)
                    wrd = transposed(pltpu.bitcast(wrd, U32))
                    sb_s[S * b + 128 * sg:S * b + 128 * (sg + 1), :] = pltpu.bitcast(wrd, F32)
                    yield 3, wrd[120:], LAG_T
                for p in range(8):
                    for j in range(8):
                        parts = [jnp.zeros((16, 128), U32) if sg < 0 else
                                 pltpu.bitcast(sb_s[pl.ds(S * b + 128 * sg + 16 * p, 16), :], U32)
                                 for sg in range(2 * j - 6, 2 * j + 2)]
                        plane = 32 * (j // 4) + 4 * p + j % 4
                        win = transposed(jnp.concatenate(parts, axis=0))
                        aw_s[pl.ds(plane * PITCH + 128 * b, 128), :] = win
                        yield 3, win[120:], LAG_T

        def conv_filter_and_first_head():
            dc_s[...] = column(d_ref[...].reshape(1, C))
            lane = lax.broadcasted_iota(I32, (32, 128), 1)
            for r0 in range(0, C, 32):
                rows = slice(r0, r0 + 32)
                for a in range(NB):
                    hf = hk_s[rows, 128 * a:128 * (a + 1)].astype(F32)
                    hs = delayed(hk_s, rows, a, 1)
                    if a == 0:
                        hf = jnp.where(lane == 0, hf + dc_s[rows, :], hf)
                        hs = jnp.where(lane == 1, hs + dc_s[rows, :], hs)
                    wrd = _pack(hf, hs)
                    g_s[a, rows, :] = wrd
                    yield 1, _digest([wrd]), LAG
            for r0 in range(0, 256, 16):
                for o in range(7):
                    yield 1, extract(0, r0, o, None, zero * (o + 1)), LAG

        def c_terms():
            for ck in range(4):
                for half in range(2):
                    for r0 in range(0, 128, 16):
                        for o in range(7):
                            def block(n, m):
                                row = 256 * ck + 128 * (n // 2) + 64 * (m // 2) + 16 * (r0 // 32)
                                col = 4 * (n % 2) + 2 * (m % 2) + half + zero * (o + 1)
                                w = jnp.concatenate([c_w[col, pl.ds(row + e, 8, stride=2), :] for e in range(2)],
                                                    axis=0)
                                return _hi(w) if r0 % 32 else _lo(w)

                            terms = [_join(t) for t in _inner_terms(_LHS, o, block)]
                            for i, t in enumerate(terms):
                                cs_w[ck, 7 * o + i, half, r0 // 2:r0 // 2 + 8, :] = t
                            yield 1, _digest(terms), LAG

        units = [(g, jp) for g in range(3) for jp in (0, 1)] + [(g, jp) for g in range(3) for jp in (2, 3)]
        units += [(g, jp) for g in (3, 4) for jp in range(4)] + [(g, jp) for g in range(5) for jp in range(4, NP)]
        units += [(g, jp) for g in range(5, H) for jp in range(NP)]
        last = 7 * len(units) - 2 - LAG
        streams = [[(v for jp in (2, 3) for v in x_terms(jp)), 14, 7 * U2 + 1, 7 * 6 - 1, 0],
                   [(v for jp in range(4, NP) for v in x_terms(jp)), 28, 7 * UX + 2, 7 * 20 - 1 - LAG, 0],
                   [conv_inputs(), 2 * 14 * NB + 3 * 4 * (NB + 64), 7 * UA + SLACK, 7 * UD + SLACK, 0],
                   [c_terms(), 448, 7 * UB + SLACK, last, 0],
                   [conv_filter_and_first_head(), 14 * NB + 112, 7 * UD + SLACK, last, 0]]
        later = {}

        def pump():
            n = len(toks)
            for st in streams:
                want = min(st[1], max(0, (n - st[2] + 1) * st[1] // (st[3] - st[2])))
                while st[4] < want:
                    cost, v, lag = next(st[0])
                    later.setdefault(n + lag, []).append(v)
                    st[4] += cost
            due.extend(later.pop(n, []))

        starts = {UX: gb, UA: gd, UB: kv_copies(1)}
        waits = {U1: cq[1:3], U2: cx[1:2], UX: cq[3:5] + cx[2:], UA: ga, UB: gb, UD: gd}
        _wait(cx[:1])
        list(x_terms(0))
        list(x_terms(1))
        _wait(cq[:1])
        wts = {}
        for u, (g, jp) in enumerate(units):
            _start(starts.get(u, []))
            _wait(waits.get(u, []))
            for g_ in range(H):
                if g_ not in wts and units.index((g_, 0)) - (4 if g_ >= 5 else 1) <= u:
                    wts[g_] = w_terms(g_ // 2, g_ % 2)

            def prod(i):
                pump()
                m = _dot(_tied(wts[g][i], due, never), xs_s[256 * (NP * i + jp):256 * (NP * i + jp + 1), :])
                toks.append(m[:8])
                return m

            def emit(r, c, val):
                qc_w[2 * (g // 2) + c, 2 * jp + r, 64 * (g % 2):64 * (g % 2 + 1), :] = _join32(val * QSCALE)

            _strassen(prod, emit)
        assert all(st[4] == st[1] for st in streams) and not later

    phase0()
    _start(late_copies)

    def head(h, carry):
        @pl.when(h % 2 == 1)
        def _():
            _wait(kv_copies((h + 1) // 2))
            _start(kv_copies((h + 3) // 2))

        zero = h // H
        toks = []
        due = []
        lane8 = lax.broadcasted_iota(I32, (8, 128), 1)
        sub8 = lax.broadcasted_iota(I32, (8, 128), 0)
        lane16 = lax.broadcasted_iota(I32, (16, 128), 1)
        sub16 = lax.broadcasted_iota(I32, (16, 128), 0)
        tri = (lax.broadcasted_iota(I32, (128, 128), 0) <= lax.broadcasted_iota(I32, (128, 128), 1))
        h_next = h + 1
        never = _never(zero)

        def tied(lhs):
            return _tied(lhs, due, never)

        def chan_mm(c):
            m_b = lane8 < _after(128 - 2 * sub8, toks[-5] if len(toks) >= 5 else None, never)
            gs = [jnp.broadcast_to(g_s[a, pl.ds(c, 1), :], (8, 128)) for a in range(NB)]
            bt = [pltpu.roll(jnp.where(m_b, gs[a], gs[a - 1] if a > 0 else jnp.uint32(0)), 0, 1,
                             stride=2, stride_axis=0) for a in range(NB)]
            b1 = pltpu.bitcast(jnp.concatenate(bt[7::-1], axis=0), BF16)
            b2 = pltpu.bitcast(jnp.concatenate(bt[15:7:-1], axis=0), BF16)
            am = pltpu.bitcast(aw_s[pl.ds(c, 64, stride=PITCH), :], BF16)
            z1 = _dot(tied(am), b1)
            z2 = _dot(am[:64], b2)
            return c, z1[:64], z1[64:] + z2

        def chan_post(c, zlo, zhi):
            acc = car = None
            for p in range(8):
                z = jnp.concatenate([zlo[8 * p:8 * p + 8], zhi[8 * p:8 * p + 8]], axis=0)
                if p == 0:
                    acc = z
                else:
                    z = pltpu.roll(z, 16 * p, 1)
                    cz = jnp.where(lane16 < 16 * p, z, 0.0)
                    acc = acc + z
                    car = cz if car is None else car + cz
            y = (acc - car) + jnp.where(sub16 > 0, pltpu.roll(car, 1, 0), 0.0)
            y_s[pl.ds(c, NB, stride=PITCH), :] = pltpu.bitcast(y, U32)

        def next_weights():
            for r0 in range(0, 256, 16):
                for o in (0, 1, 3, 4, 6, 2, 5):
                    shift = jnp.full((8, 128), (1 - h_next % 2) * 16, I32).astype(U32)
                    yield extract(h_next, r0, o, shift, zero * (o + 1))

        weights, done, clock = next_weights(), [0], [0]

        def tick(cycles):
            while done[0] < min(112, max(0, (clock[0] - 1500) * 112 // 6080)):
                due.append(next(weights))
                done[0] += 1
            clock[0] += cycles

        def kv_chunk(ck):
            def prod(o):
                out = {}
                for r0 in (0, 64):
                    def inner(i):
                        lhs = jnp.concatenate([cs_s[ck, 7 * o + i, k, r0:r0 + 64, :] for k in range(2)], axis=1)
                        m = _dot(tied(lhs), wx_s[7 * o + i])
                        if i == 3 and r0 == 0:
                            toks.append(m[:8])
                        return m

                    _strassen(inner, lambda r, n, val: out.__setitem__((r, n, r0), val))
                return jnp.concatenate([jnp.concatenate([out[r, 0, r0], out[r, 1, r0]], axis=1)
                                        for r in range(2) for r0 in (0, 64)], axis=0)

            def emit(r, n, val):
                jp = 2 * ck + r
                if n == 0:
                    if jp < NP - 1:
                        blocks = [val[:128, :128], val[:128, 128:], val[128:, :128], val[128:, 128:]]
                        for i in _SUMS:
                            kt_w[i, jp] = _join32(_term(_LHS, i, blocks.__getitem__))
                    for k in range(2):
                        k_w[k, 128 * jp:128 * (jp + 1), :] = _join32(val[:, 128 * k:128 * (k + 1)])
                else:
                    blocks = [val[128 * t:128 * (t + 1), 128 * k:128 * (k + 1)].T
                              for k in range(2) for t in range(2)]
                    outs = [v.astype(BF16) for v in blocks]
                    for m, v in enumerate(outs):
                        vt_s[2 * jp + m % 2, 128 * (m // 2):128 * (m // 2 + 1), :] = v
                    if jp < NP - 1:
                        for i in _SUMS:
                            vx_s[i, jp] = _term(_LHS, i, blocks.__getitem__).astype(BF16)

            return _strassen_steps(prod, emit)

        kv = [kv_chunk(ck) for ck in range(4)]
        lse, pr = {}, {}

        def s_at(u, r0):
            first = [v for v in range(u) if (v // 4) % 2 == (u // 4) % 2]
            return (sa_s, sb_s)[(u // 4) % 2], 128 * sum(v + 1 for v in first) + r0

        def qk(jq):
            run = [None, None]

            def put(n, r0, val):
                buf, row = s_at(2 * jq + n, r0)
                buf[row:row + 64, :] = val
                vs = [val[r:r + 8] for r in range(0, 64, 8)]
                m = _fold(jnp.maximum, vs)
                if run[n] is not None:
                    m = jnp.maximum(m, run[n][0])
                l = _fold(jnp.add, [jnp.exp2(v - m) for v in vs])
                if run[n] is not None:
                    l = l + run[n][1] * jnp.exp2(run[n][0] - m)
                run[n] = (m, l)

            if jq > 0:
                qt = _word_terms(_RHS, [qc_w[h, 2 * jq + n % 2, 64 * (n // 2):64 * (n // 2 + 1), :]
                                        for n in range(4)])
            for jp in range(jq):
                for r0 in (0, 64):
                    def prod(i):
                        if i == 2:
                            lhs = k_s[0, 256 * jp + r0:256 * jp + r0 + 64, :]
                        elif i == 3:
                            lhs = k_s[1, 256 * jp + 128 + r0:256 * jp + 128 + r0 + 64, :]
                        else:
                            lhs = kt_s[i, jp, r0:r0 + 64, :]
                        m = _dot(tied(lhs), qt[i])
                        if i == 3 and r0 == 0:
                            toks.append(m[:8])
                        return m

                    _strassen(prod, lambda r, n, val: put(n, 256 * jp + 128 * r + r0, val))
            q0 = 256 * jq
            for n in range(2):
                rows = slice(q0, q0 + 128 * (n + 1))
                sd = _dot(tied(jnp.concatenate([k_s[0, rows, :], k_s[1, rows, :]], axis=1)), qc_s[h, 2 * jq + n])
                last = jnp.where(tri, sd[128 * n:], NEG)
                sd = jnp.concatenate([sd[:128], last], axis=0) if n else last
                for r0 in range(0, 128 * (n + 1), 64):
                    put(n, q0 + r0, sd[r0:r0 + 64])
            toks.append(sd[:8])
            for n in range(2):
                m, l = run[n]
                top = jnp.max(m, axis=0, keepdims=True)
                lse[2 * jq + n] = top + jnp.log2(jnp.sum(l * jnp.exp2(m - top), axis=0, keepdims=True))

        def probs(u, r0):
            buf, row = s_at(u, r0)
            x = jnp.concatenate([buf[pl.ds(row + e + zero, 8, stride=4), :] for e in (0, 2)], axis=0)
            return jnp.exp2(x - lse[u])

        def softmax(jq, jps, deadline):
            starts = [r + e for r in range(0, 256, 32) for e in range(2)]
            for jp in jps:
                if jp == jq:
                    out = [jnp.concatenate([_join(probs(2 * jq + n, 256 * jq + r)) for r in starts[:8 * (n + 1)]],
                                           axis=0) for n in range(2)]
                else:
                    parts = []
                    for r in starts[:8]:
                        blocks = [probs(2 * jq + m % 2, 256 * jp + 128 * (m // 2) + r) for m in range(4)]
                        parts.append([_join(t) for t in _terms(_RHS, blocks)])
                    out = [jnp.concatenate([p[i] for p in parts], axis=0) for i in range(7)]
                pr[jq, jp] = out
                if deadline:
                    due.append(_digest(out[:1]) ^ _digest(out[1:]) if jp == jq else _digest(out))

        def pv(jq):
            softmax(jq, [jp for jp in range(jq + 1) if (jq, jp) not in pr], False)
            diag = pr.pop((jq, jq))
            ps = [pr.pop((jq, jp)) for jp in range(jq)]
            base = []
            for n in range(2):
                tick(64 * (n + 1))
                vt = jnp.concatenate([vt_s[2 * jq + i] for i in range(n + 1)], axis=1)
                base.append(_dot(tied(vt), pltpu.bitcast(diag[n], BF16)))

            def emit(r, n, val):
                val = base[n][128 * r:128 * (r + 1)] if val is None else val + base[n][128 * r:128 * (r + 1)]
                qc_s[h, 2 * jq + n, 128 * r:128 * (r + 1), :] = val.astype(BF16)

            def prod(i):
                tick(32 * jq)
                if i == 2:
                    lhs = [vt_s[2 * jp, 0:128, :] for jp in range(jq)]
                elif i == 3:
                    lhs = [vt_s[2 * jp + 1, 128:256, :] for jp in range(jq)]
                else:
                    lhs = [vx_s[i, jp] for jp in range(jq)]
                rhs = pltpu.bitcast(jnp.concatenate([p[i] for p in ps], axis=0), BF16)
                return _dot(tied(jnp.concatenate(lhs, axis=1)), rhs)

            if jq:
                _strassen(prod, emit)
            else:
                for r in range(2):
                    for n in range(2):
                        emit(r, n, None)

        chans = [h * CPH + i for i in range(CPH)]
        pend = []
        for step in HEAD_STEPS.split():
            kind, arg = step[0], [int(x) for x in step[1:]]
            if kind == 'E':
                softmax(arg[0], arg[1:] or range(arg[0] + 1), True)
                continue
            old, pend = pend, []
            if kind == 'C':
                pend = [chan_mm(chans.pop(0)) for _ in range(arg[0])]
            elif kind == 'M':
                for o in arg[1:]:
                    kv[arg[0]](o)
            else:
                for jq in arg:
                    (qk if kind == 'Q' else pv)(jq)
            for args in old:
                chan_post(*args)
        assert done[0] == 112 and not (chans or pend or due or pr)
        return carry + zero

    zero_end = lax.fori_loop(0, H, head, 0)

    _wait(late_copies + kv_copies(H // 2 + 1))
    HH = H // 2

    def wo_block(rh, kh):
        rows = [(C * (H * b + h) + CH * rh) // 2 for h in range(HH * kh, HH * (kh + 1)) for b in range(2)]
        return jnp.concatenate([xs_w[r:r + CH // 2, :] for r in rows], axis=1)

    wt = _word_terms(_RHS, [wo_block(0, 0), wo_block(1, 0), wo_block(0, 1), wo_block(1, 1)])
    outs = []
    due, late = [], []
    never = _never(zero_end)

    def put(t, b, z, opaque=False):
        z = z.T
        r0 = pl.multiple_of(zero_end * 16 + 128 * t, 16) if opaque else 128 * t
        out_s[pl.ds(r0, 128), 128 * b:128 * (b + 1)] = z.astype(BF16)
        late.append(z[120:])

    for jp in range(NP):
        ct = _word_terms(_LHS, [jnp.concatenate([qc_w[h, 2 * jp + r] for h in range(HH * kh, HH * (kh + 1))], axis=0)
                                for r in range(2) for kh in range(2)])
        za = {}
        dues = {3: list(late)}
        late.clear()
        for r in range(2):
            t = 2 * jp + r
            za[r] = (pltpu.bitcast(y_s[t * PITCH:t * PITCH + C, :], F32)
                     * x_s[:, 128 * t:128 * (t + 1)].astype(F32))
            for b in range(3):
                put(t, b, za[r][128 * b:128 * (b + 1)], opaque=(r == 0 and b == 0 and jp > 0))
        dues[6] = list(late)
        late.clear()
        res = {}
        step = _strassen_steps(lambda i: _dot(_tied(wt[i], due, never), ct[i]),
                               lambda r, c, val: res.__setitem__((r, c), val))
        for n, i in enumerate((1, 4, 3, 6, 0, 2, 5)):
            due.extend(dues.get(n, []))
            step(i)
        for r in range(2):
            z = jnp.concatenate([za[r][384:], res[r, 0], res[r, 1]], axis=0)
            for b in range(4):
                put(2 * jp + r, 3 + b, z[128 * b:128 * (b + 1)])
        rows = pl.ds(256 * jp, 256)
        outs.append(cp(out_s.at[rows], o_hbm.at[rows], 26 + jp))
        outs[-1].start()
    _wait(outs)


def _tiles(w):
    rows = w.shape[0]
    return w.reshape(rows, 2, 8, 2, 128).transpose(0, 1, 3, 2, 4).reshape(rows, 32, 128)


@jax.jit
def pallas_concat_heads__ssm_conv_h3__compressed_kv_cla__prompt_kernel(
    A_q: jax.Array,
    A_k: jax.Array,
    A_v: jax.Array,
    A_shift_k: jax.Array,
    A_ssm_k: jax.Array,
    A_ssm_D: jax.Array,
    B_x: jax.Array,
    B_c_kv: jax.Array,
    B_w_q: jax.Array,
    B_w_uk: jax.Array,
    B_w_uv: jax.Array,
    B_w_o: jax.Array,
):
    hbm = pl.BlockSpec(memory_space=pltpu.HBM)
    out = pl.pallas_call(
        _kernel,
        in_specs=[hbm] * 12,
        out_specs=hbm,
        out_shape=jax.ShapeDtypeStruct((S, 2 * C), BF16),
        scratch_shapes=[
            pltpu.VMEM((8, S // 2, 128), U32),
            pltpu.VMEM((4, 49, 2, 64, 128), U32),
            pltpu.VMEM((2, 4, DC, 128), U32),
            pltpu.VMEM((H, NB, D // 2, 128), U32),
            pltpu.VMEM((64 * PITCH, 128), U32),
            pltpu.VMEM((NB, C, 128), U32),
            pltpu.VMEM((NB * PITCH, 128), U32),
            pltpu.VMEM((CH, S), U32),
            pltpu.VMEM((512, 128), F32),
            pltpu.VMEM((2, S // 2, 128), U32),
            pltpu.VMEM((7, NP, 64, 128), U32),
            pltpu.VMEM((NB, D // 2, 128), U32),
            pltpu.VMEM((7, NP, 64, 128), U32),
            pltpu.VMEM((49, DC // 8, 128), U32),
            pltpu.VMEM((NB * C, 128), F32),
            pltpu.VMEM((84 * 128, 128), F32),
            pltpu.VMEM((CH, S), U32),
            pltpu.VMEM((7 * NP * 128, 128), U32),
            pltpu.VMEM((CH, S), U32),
            pltpu.VMEM((CH, S), U32),
            pltpu.VMEM((2, 8, 128, 128), F32),
            pltpu.VMEM((S, 2 * C), BF16),
            pltpu.VMEM((4, C), BF16),
            pltpu.VMEM((C,), BF16),
            pltpu.SemaphoreType.DMA((36,)),
        ],
        compiler_params=pltpu.CompilerParams(vmem_limit_bytes=127 * 2 ** 20, disable_semaphore_checks=True),
    )(
        A_q[0].T, A_k[0].T, A_v[0].T, A_shift_k.T, A_ssm_k, A_ssm_D, B_x[0].T, B_c_kv[0],
        _tiles(B_w_q), _tiles(B_w_uk), _tiles(B_w_uv),
        jnp.swapaxes(B_w_o, 1, 2).reshape(H * C, D),
    )
    return out.reshape(1, S, 2 * C)
```
